```python
import jax
import jax.numpy as jnp

def _softmax(x, axis=-1):
    return jax.nn.softmax(x, axis=axis)

def _gelu(x):
    return jax.nn.gelu(x, approximate=True)

def _silu(x):
    return jax.nn.silu(x)

def _sigmoid(x):
    return jax.nn.sigmoid(x)

def _layernorm(x, axis=-1, eps=1e-05):
    m = jnp.mean(x, axis=axis, keepdims=True)
    v = jnp.var(x, axis=axis, keepdims=True)
    return (x - m) / jnp.sqrt(v + eps)

def _scatter_add(tgt, idx, src, axis=0):
    return tgt.at[idx].add(src)

def _segment_sum(src, seg, n):
    return jax.ops.segment_sum(src, seg, n)

class _Rng:

    def __init__(self, key):
        self._k = key

    def _next(self):
        self._k, sub = jax.random.split(self._k)
        return sub

    def normal(self, shape):
        return jax.random.normal(self._next(), shape, dtype=jnp.bfloat16)

    def randint(self, lo, hi, shape):
        return jax.random.randint(self._next(), shape, lo, hi, dtype=jnp.int32)

    def uniform(self, shape, lo=0.0, hi=1.0):
        return jax.random.uniform(self._next(), shape, jnp.bfloat16, lo, hi)

    def permutation(self, n):
        return jax.random.permutation(self._next(), n)
kernel_name = 'recurrent_scan__memory_aug_recurrent_mem_tr__mixer_s_mlp__prompt'

def setup_inputs():
    _rng = _Rng(jax.random.key(int.from_bytes(__import__("os").urandom(4), "little")))
    _w = lambda a: (lambda t: t.astype(jnp.bfloat16) if jnp.issubdtype(t.dtype, jnp.floating) else t)(jnp.asarray(a))

    def _A_setup():
        B, S, Dm = (1, 2048, 1024)
        H, Dh = (32, 128)
        M, seg = (8, 32)
        seg = min(seg, S)
        S = S // seg * seg
        return {'x': _w((lambda *s: _rng.normal(s) * 0.05)(B, S, Dm)), 'mem0': _w((lambda *s: _rng.normal(s) * 0.05)(B, M, Dm)), 'Wq': _w((lambda *s: _rng.normal(s) * 0.05)(Dm, H, Dh) * Dm ** (-0.5)), 'Wk': _w((lambda *s: _rng.normal(s) * 0.05)(Dm, H, Dh) * Dm ** (-0.5)), 'Wv': _w((lambda *s: _rng.normal(s) * 0.05)(Dm, H, Dh) * Dm ** (-0.5)), 'Wo': _w((lambda *s: _rng.normal(s) * 0.05)(H, Dh, Dm) * (H * Dh) ** (-0.5)), 'seg_len': seg}
    _A_in = _A_setup()

    def _B_setup():
        B, S, D, F = (1, 2048, 1024, 3584)
        return {'x': _w((lambda *s: _rng.normal(s) * 0.05)(B, S, D)), 'w1': _w((lambda *s: _rng.normal(s) * 0.05)(D, D) * D ** (-0.5)), 'w2': _w((lambda *s: _rng.normal(s) * 0.05)(D, D) * D ** (-0.5)), 'w3': _w((lambda *s: _rng.normal(s) * 0.05)(D, F) * D ** (-0.5)), 'w4': _w((lambda *s: _rng.normal(s) * 0.05)(F, D) * F ** (-0.5))}
    _B_in = _B_setup()
    return {'A_x': _A_in['x'], 'A_mem0': _A_in['mem0'], 'A_Wq': _A_in['Wq'], 'A_Wk': _A_in['Wk'], 'A_Wv': _A_in['Wv'], 'A_Wo': _A_in['Wo'], 'A_seg_len': _A_in['seg_len'], 'B_x': _B_in['x'], 'B_w1': _B_in['w1'], 'B_w2': _B_in['w2'], 'B_w3': _B_in['w3'], 'B_w4': _B_in['w4']}

def reference(A_x, A_mem0, A_Wq, A_Wk, A_Wv, A_Wo, A_seg_len, B_x, B_w1, B_w2, B_w3, B_w4):

    def _A_ref(x, mem0, Wq, Wk, Wv, Wo, seg_len):
        B, S, Dm = x.shape
        H, Dh = (Wq.shape[1], Wq.shape[2])
        M = mem0.shape[1]
        scale = Dh ** (-0.5)
        n_seg = S // seg_len
        L = M + seg_len
        idx = jnp.arange(L)
        mask = (idx[:, None] < M) | (idx[:, None] >= idx[None, :])
        mem = mem0
        outs = []
        for s in range(n_seg):
            xs = x[:, s * seg_len:(s + 1) * seg_len, :].copy()
            h = jnp.concatenate([mem, xs], axis=1)
            q = jnp.einsum('btd,dhe->bhte', h, Wq)
            k = jnp.einsum('btd,dhe->bhte', h, Wk)
            v = jnp.einsum('btd,dhe->bhte', h, Wv)
            scores = jnp.einsum('bhqe,bhke->bhqk', q, k) * scale
            scores = jnp.where(mask[None, None], scores, -1000000000.0)
            p = _softmax(scores, axis=-1)
            o = jnp.einsum('bhqk,bhke->bhqe', p, v)
            o = jnp.einsum('bhte,hed->btd', o, Wo)
            mem = o[:, :M, :].copy()
            outs.append(o[:, M:, :])
        return jnp.concatenate(outs, axis=1)

    def _B_ref(x, w1, w2, w3, w4):
        B, S, D = x.shape
        h = _gelu(_layernorm(x, axis=-1) @ w1)
        c = D // 4
        g0 = jnp.pad(h[:, :, 0 * c:1 * c], ((0, 0), (1, 0), (0, 0)))[:, :S, :]
        g1 = jnp.pad(h[:, :, 1 * c:2 * c], ((0, 0), (0, 1), (0, 0)))[:, 1:, :]
        g2 = jnp.pad(h[:, :, 2 * c:3 * c], ((0, 0), (2, 0), (0, 0)))[:, :S, :]
        g3 = jnp.pad(h[:, :, 3 * c:], ((0, 0), (0, 2), (0, 0)))[:, 2:, :]
        hs = jnp.concatenate([g0, g1, g2, g3], axis=-1) @ w2
        x1 = x + hs
        h2 = _gelu(_layernorm(x1, axis=-1) @ w3) @ w4
        return x1 + h2
    x = A_x
    xn = _layernorm(x, axis=-1)
    s = _A_ref(xn, A_mem0, A_Wq, A_Wk, A_Wv, A_Wo, A_seg_len)
    g = _silu(_B_ref(xn, B_w1, B_w2, B_w3, B_w4))
    return x + s * g
```

```python
import functools

import jax
import jax.numpy as jnp
from jax import lax
import jax.experimental.pallas as pl
import jax.experimental.pallas.tpu as pltpu

F32 = jnp.float32
BF16 = jnp.bfloat16
U32 = jnp.uint32

S = 2048
D = 1024
H = 32
E = 128
M = 8
SEG = 32
L = M + SEG
FF = 3584
NCB = D // 128
NFB = FF // 128
NIT = S // (2 * SEG)
HB = 2 * L
PRE = 512
BR = (S - PRE) // NIT
HS = D // 2
EPS = 1e-5
SCALE = float(E) ** -0.5
RB = 256


def _dot(a, b):
    return jnp.dot(a, b, preferred_element_type=F32)


def _ln(x):
    m = jnp.mean(x, axis=-1, keepdims=True)
    xc = x - m
    v = jnp.mean(xc * xc, axis=-1, keepdims=True)
    return xc * lax.rsqrt(v + EPS)


def _gelu(x):
    c = 0.7978845608028654
    return 0.5 * x * (1.0 + jnp.tanh(c * (x + 0.044715 * (x * x * x))))


def _silu(x):
    return x * (1.0 / (1.0 + jnp.exp(-x)))


def _kernel(x_hbm, mem0_ref, wq_hbm, wk_hbm, wv_hbm, wo_hbm, w1_hbm, w2_hbm, w3_hbm, w4_hbm,
            out_hbm,
            xbuf, hbuf, hf, x1buf, x1nbuf, h3buf, stg, wqkv, wo, w1, w2, w3, w4, fillbuf,
            sem, osem):
    def colblock_copies(src, dst, nblk, s):
        return [pltpu.make_async_copy(src.at[:, pl.ds(c * 128, 128)], dst.at[c], sem.at[s])
                for c in range(nblk)]

    cp_w1 = [pltpu.make_async_copy(w1_hbm, w1, sem.at[0])]
    cp_x = [pltpu.make_async_copy(x_hbm, xbuf, sem.at[1])]
    cp_w2 = [pltpu.make_async_copy(w2_hbm, w2, sem.at[2])]
    cp_w3 = colblock_copies(w3_hbm, w3, NFB, 3)
    cp_w4 = colblock_copies(w4_hbm, w4, NCB, 4)
    cp_qkv = [[pltpu.make_async_copy(w, stg.at[i], sem.at[5 + i])]
              for i, w in enumerate((wq_hbm, wk_hbm, wv_hbm))]
    cp_wo = colblock_copies(wo_hbm, wo, NCB, 8)
    for grp in (cp_w1, cp_x, cp_w2, cp_w3, cp_w4, *cp_qkv, cp_wo):
        for c in grp:
            c.start()

    def wait(grp):
        for c in grp:
            c.wait()

    r = lax.broadcasted_iota(jnp.int32, (HB, HB), 0)
    c = lax.broadcasted_iota(jnp.int32, (HB, HB), 1)
    rr = jnp.where(r >= L, r - L, r)
    cc = jnp.where(c >= L, c - L, c)
    same = (r >= L) == (c >= L)
    allowed = (rr < M) | (rr >= cc)
    fillbuf[...] = jnp.where(same, jnp.where(allowed, 1.0, -1e9), -jnp.inf).astype(F32)

    hf[:, 0:8, :] = jnp.zeros((NCB, 8, 128), F32)
    hf[:, S + 8:S + 16, :] = jnp.zeros((NCB, 8, 128), F32)
    hbuf[0:M, :] = mem0_ref[...]

    wait(cp_w1)
    wait(cp_x)

    def stage1(i, carry):
        r0 = pl.multiple_of(i * RB, RB)
        xn = _ln(xbuf[pl.ds(r0, RB), :].astype(F32)).astype(BF16)
        for u in range(RB // 64):
            b0 = pl.multiple_of((i * (RB // 64) + u) * HB, 16)
            hbuf[pl.ds(b0 + 8, 40), :] = xn[u * 64:u * 64 + 40]
            hbuf[pl.ds(b0 + 56, 24), :] = xn[u * 64 + 40:u * 64 + 64]
        x1buf[pl.ds(r0, RB), :] = xn
        xnn = _ln(xn.astype(F32)).astype(BF16)
        h = _gelu(_dot(xnn, w1[...]).astype(BF16).astype(F32)).astype(BF16).astype(F32)
        for cb in range(NCB):
            hf[cb, pl.ds(r0 + 8, RB), :] = h[:, cb * 128:(cb + 1) * 128]
        return carry

    lax.fori_loop(0, S // RB, stage1, 0)

    wait(cp_w2)
    shifts = (7, 7, 9, 9, 6, 6, 10, 10)

    def stage2(i, carry):
        r0 = pl.multiple_of(i * RB, RB)
        hs = jnp.concatenate(
            [hf[cb, pl.ds(r0 + shifts[cb], RB), :] for cb in range(NCB)], axis=1).astype(BF16)
        y = _dot(hs, w2[...]).astype(BF16).astype(F32)
        x1 = (x1buf[pl.ds(r0, RB), :].astype(F32) + y).astype(BF16)
        x1buf[pl.ds(r0, RB), :] = x1
        x1nbuf[pl.ds(r0, RB), :] = _ln(x1.astype(F32)).astype(BF16)
        return carry

    lax.fori_loop(0, S // RB, stage2, 0)

    wait(cp_w3)
    wait(cp_w4)

    def w3_part(lhs, blocks, rows):
        for f in blocks:
            h3 = _gelu(_dot(lhs, w3[f]).astype(BF16).astype(F32))
            h3buf[f, 0:rows, :] = h3.astype(BF16)

    def w4_part(r0, rows, blocks):
        lhs = jnp.concatenate([h3buf[f, 0:rows, :] for f in range(NFB)], axis=1)
        for cb in blocks:
            h2 = _dot(lhs, w4[cb]).astype(BF16).astype(F32)
            sl = (pl.ds(r0, rows), slice(cb * 128, (cb + 1) * 128))
            y = (x1buf[sl].astype(F32) + h2).astype(BF16).astype(F32)
            x1buf[sl] = _silu(y).astype(BF16)

    SB = 128

    def stage3(i, carry):
        r0 = pl.multiple_of(i * SB, SB)
        w3_part(x1nbuf[pl.ds(r0, SB), :], range(NFB), SB)
        w4_part(r0, SB, range(NCB))
        return carry

    lax.fori_loop(0, PRE // SB, stage3, 0)
    w3_part(x1nbuf[PRE:PRE + BR, :], range(NFB), BR)

    for m_ in range(3):
        wait(cp_qkv[m_])

        def relayout(p8, carry, m_=m_):
            r0 = pl.multiple_of(p8 * 512, 512)
            xx = pltpu.bitcast(stg[m_, pl.ds(r0, 512), :], U32).reshape(8, 2, 16, 128)
            a = xx[:, 0]
            b = xx[:, 1]
            lo = (a & U32(0xFFFF)) | (b << 16)
            hi = (a >> 16) | (b & U32(0xFFFF0000))
            lo = jnp.swapaxes(lo, 0, 1)
            hi = jnp.swapaxes(hi, 0, 1)
            p0 = pl.multiple_of(p8 * 8, 8)
            for j in range(16):
                wqkv[(2 * j) * 3 + m_, pl.ds(p0, 8), :] = lo[j]
                wqkv[(2 * j + 1) * 3 + m_, pl.ds(p0, 8), :] = hi[j]
            return carry

        lax.fori_loop(0, D // 16, relayout, 0)
    wait(cp_wo)

    def qkv_pair(lhs, j):
        return [_dot(lhs, pltpu.bitcast(wqkv[6 * j + i], BF16)) for i in range(6)]

    def scores(q, k):
        return lax.dot_general(q, k, (((1,), (1,)), ((), ())), preferred_element_type=F32)

    def softmax(s):
        fill = fillbuf[...]
        s = jnp.where(fill > 0.0, s * SCALE, fill)
        mx = jnp.max(s, axis=1, keepdims=True)
        e = jnp.exp(s - mx)
        l = jnp.sum(e, axis=1, keepdims=True)
        rc = pl.reciprocal(l, approx=True)
        rc = rc * (2.0 - l * rc)
        return (e * rc).astype(BF16)

    def attn_step(lhs, select, filler1):
        NP = H // 2
        qkv = [None] * NP
        sc = [None] * NP
        o = [None] * NP

        def do_qkv(j):
            rs = qkv_pair(lhs, j)
            rs = [select(j, i, v) for i, v in enumerate(rs)]
            qkv[j] = [jnp.concatenate([rs[i], rs[3 + i]], axis=0).astype(BF16) for i in range(3)]

        def do_s(j):
            sc[j] = softmax(scores(qkv[j][0], qkv[j][1]))

        def do_pv(j):
            o[j] = _dot(sc[j], qkv[j][2])

        for j in range(NP + 2):
            if j < NP:
                do_qkv(j)
            else:
                filler1(j - NP)
            if 0 <= j - 1 < NP:
                do_s(j - 1)
            if 0 <= j - 2 < NP:
                do_pv(j - 2)
        oh = []
        for j in range(NP):
            oh += [o[j][0:L], o[j][L:2 * L]]
        return oh

    def body(t, carry):
        base = pl.multiple_of(t * HB, 16)
        R0 = pl.multiple_of(t * 64, 64)
        B0 = pl.multiple_of(PRE + t * BR, 16)
        B1 = pl.multiple_of(jnp.minimum(B0 + BR, S - BR), 16)

        keep = {}

        def sel_a(j, i, v):
            keep[(j, i)] = v[L:L + 8]
            return v[0:L]

        lhs_a = hbuf[pl.ds(base, 48), :]
        oa = attn_step(lhs_a, sel_a, lambda n: w4_part(B0, BR, range(2 * n, 2 * n + 2)))
        w4_part(B0, BR, range(4, 6))
        lo_a = jnp.concatenate([v[0:32] for v in oa], axis=1).astype(BF16)
        ra = [_dot(lo_a, wo[cb]) for cb in range(NCB)]
        for cb in range(NCB):
            hbuf[pl.ds(base + 48, 8), cb * 128:(cb + 1) * 128] = ra[cb][0:8].astype(BF16)
        w4_part(B0, BR, range(6, 8))

        def sel_b(j, i, v):
            return jnp.concatenate([v[0:8], keep[(j, i)], v[8:32]], axis=0)

        lhs3 = x1nbuf[pl.ds(B1, BR), :]
        lhs_b = hbuf[pl.ds(base + 48, 32), :]
        ob = attn_step(lhs_b, sel_b, lambda n: w3_part(lhs3, range(7 * n, 7 * n + 7), BR))
        w3_part(lhs3, range(14, 21), BR)
        lo_b = jnp.concatenate(
            [jnp.concatenate([va[32:40], vb], axis=0) for va, vb in zip(oa, ob)],
            axis=1).astype(BF16)
        for cb in range(NCB):
            rb = _dot(lo_b, wo[cb])
            cs = slice(cb * 128, (cb + 1) * 128)
            hbuf[pl.ds(base + HB, 8), cs] = rb[8:16].astype(BF16)
            s_ = jnp.concatenate([ra[cb][8:32], rb[0:8], rb[16:48]], axis=0)
            s_ = s_.astype(BF16).astype(F32)
            sl = (pl.ds(R0, 64), cs)
            xbuf[sl] = (xbuf[sl].astype(F32) + s_ * x1buf[sl].astype(F32)).astype(BF16)
        w3_part(lhs3, range(21, 28), BR)

        pltpu.make_async_copy(xbuf.at[pl.ds(R0, 64), :], out_hbm.at[pl.ds(R0, 64), :], osem).start()
        return carry

    lax.fori_loop(0, NIT, body, 0)
    pltpu.make_async_copy(xbuf, out_hbm, osem).wait()


@functools.partial(jax.jit, static_argnames=("A_seg_len",))
def pallas_recurrent_scan__memory_aug_recurrent_mem_tr__mixer_s_mlp__prompt_kernel(
    A_x: jax.Array,
    A_mem0: jax.Array,
    A_Wq: jax.Array,
    A_Wk: jax.Array,
    A_Wv: jax.Array,
    A_Wo: jax.Array,
    A_seg_len,
    B_x: jax.Array,
    B_w1: jax.Array,
    B_w2: jax.Array,
    B_w3: jax.Array,
    B_w4: jax.Array,
):
    assert A_seg_len == SEG
    assert A_x.shape == (1, S, D) and A_mem0.shape == (1, M, D)
    assert A_Wq.shape == (D, H, E) and A_Wo.shape == (H, E, D)
    assert B_w3.shape == (D, FF)
    del B_x

    any_spec = pl.BlockSpec(memory_space=pl.ANY)
    out = pl.pallas_call(
        _kernel,
        out_shape=jax.ShapeDtypeStruct((S, D), BF16),
        in_specs=[any_spec, pl.BlockSpec(memory_space=pltpu.VMEM)] + [any_spec] * 8,
        out_specs=any_spec,
        scratch_shapes=[
            pltpu.VMEM((S, D), BF16),
            pltpu.VMEM((NIT * HB + 16, D), BF16),
            pltpu.VMEM((NCB, S + 16, 128), F32),
            pltpu.VMEM((S, D), BF16),
            pltpu.VMEM((S, D), BF16),
            pltpu.VMEM((NFB, 128, 128), BF16),
            pltpu.VMEM((3, D * H, E), BF16),
            pltpu.VMEM((3 * H, HS, 128), U32),
            pltpu.VMEM((NCB, H * E, 128), BF16),
            pltpu.VMEM((D, D), BF16),
            pltpu.VMEM((D, D), BF16),
            pltpu.VMEM((NFB, D, 128), BF16),
            pltpu.VMEM((NCB, FF, 128), BF16),
            pltpu.VMEM((HB, HB), F32),
            pltpu.SemaphoreType.DMA((9,)),
            pltpu.SemaphoreType.DMA(()),
        ],
        compiler_params=pltpu.CompilerParams(vmem_limit_bytes=120 * 1024 * 1024),
    )(
        A_x.reshape(S, D), A_mem0.reshape(M, D),
        A_Wq.reshape(D * H, E), A_Wk.reshape(D * H, E), A_Wv.reshape(D * H, E),
        A_Wo.reshape(H * E, D), B_w1, B_w2, B_w3, B_w4,
    )
    return out.reshape(1, S, D)
```

```python
import functools

import jax
import jax.numpy as jnp
from jax import lax
import jax.experimental.pallas as pl
import jax.experimental.pallas.tpu as pltpu

F32 = jnp.float32
BF16 = jnp.bfloat16
U32 = jnp.uint32

S = 2048
D = 1024
H = 32
E = 128
M = 8
SEG = 32
L = M + SEG
FF = 3584
NCB = D // 128
NFB = FF // 128
NIT = S // (2 * SEG)
HB = 2 * L
PRE = 512
BR = (S - PRE) // NIT
HS = D // 2 + 8
EPS = 1e-5
SCALE = float(E) ** -0.5
RB = 256
CFG = {}


def _dot(a, b):
    return jnp.dot(a, b, preferred_element_type=F32)


def _ln(x):
    m = jnp.mean(x, axis=-1, keepdims=True)
    xc = x - m
    v = jnp.mean(xc * xc, axis=-1, keepdims=True)
    return xc * lax.rsqrt(v + EPS)


def _gelu(x):
    c = 0.7978845608028654
    return 0.5 * x * (1.0 + jnp.tanh(c * (x + 0.044715 * (x * x * x))))


def _silu(x):
    return x * (1.0 / (1.0 + jnp.exp(-x)))


def _kernel(x_hbm, mem0_ref, wq_hbm, wk_hbm, wv_hbm, wo_hbm, w1_hbm, w2_hbm, w3_hbm, w4_hbm,
            out_hbm,
            xbuf, hbuf, hf, x1buf, x1nbuf, h3buf, stg, wqkv, wo, w1, w2, w3, w4, fillbuf,
            sem, qsem, osem):
    def colblock_copies(src, dst, nblk, s):
        return [pltpu.make_async_copy(src.at[:, pl.ds(c * 128, 128)], dst.at[c], sem.at[s])
                for c in range(nblk)]

    NXB = S // RB
    cp_x = [pltpu.make_async_copy(x_hbm.at[pl.ds(i * RB, RB), :], xbuf.at[pl.ds(i * RB, RB), :],
                                  sem.at[min(i, 3)]) for i in range(NXB)]
    cp_w1 = colblock_copies(w1_hbm, w1, NCB, 4)
    cp_w2 = colblock_copies(w2_hbm, w2, NCB, 5)
    cp_w3 = colblock_copies(w3_hbm, w3, NFB, 6)
    cp_w4 = colblock_copies(w4_hbm, w4, NCB, 7)
    cp_wo = colblock_copies(wo_hbm, wo, NCB, 8)
    CH = 512
    PR = 16 * CH
    cp_qkv = [pltpu.make_async_copy(src.at[pl.ds(k * PR, PR), :], stg.at[k, pl.ds(m_ * PR, PR), :],
                                    qsem.at[k])
              for k in range(4) for m_, src in enumerate((wq_hbm, wk_hbm, wv_hbm))]
    for grp in (cp_x[:1], cp_w1, cp_x[1:], cp_w2, cp_w3, cp_w4, cp_qkv, cp_wo):
        for c in grp:
            c.start()

    def wait(grp):
        for c in grp:
            c.wait()

    r = lax.broadcasted_iota(jnp.int32, (HB, HB), 0)
    c = lax.broadcasted_iota(jnp.int32, (HB, HB), 1)
    rr = jnp.where(r >= L, r - L, r)
    cc = jnp.where(c >= L, c - L, c)
    same = (r >= L) == (c >= L)
    allowed = (rr < M) | (rr >= cc)
    fillbuf[...] = jnp.where(same, jnp.where(allowed, 1.0, -1e9), -jnp.inf).astype(F32)

    hf[:, 0:8, :] = jnp.zeros((NCB, 8, 128), F32)
    hf[:, S + 8:S + 16, :] = jnp.zeros((NCB, 8, 128), F32)
    hbuf[0:M, :] = mem0_ref[...]

    SB = 128

    def zero_of(trig):
        return (pltpu.bitcast(trig, U32) >> 16) >> 16

    def ln_chunk(xsrc, hdst, x1dst, x1ndst, u, trig):
        xb = xsrc[16 * u:16 * u + 16, :]
        if trig is not None:
            z = zero_of(trig)
            xb = pltpu.bitcast(pltpu.bitcast(xb, U32) | jnp.concatenate([z] * NCB, axis=1), BF16)
        xn = _ln(xb.astype(F32)).astype(BF16)
        for hh in range(2):
            q, rr_ = divmod(16 * u + 8 * hh, 64)
            o = q * HB + rr_ + (8 if rr_ < 40 else 16)
            hdst[o:o + 8, :] = xn[8 * hh:8 * hh + 8]
        x1dst[16 * u:16 * u + 16, :] = xn
        x1ndst[16 * u:16 * u + 16, :] = _ln(xn.astype(F32)).astype(BF16)

    def w1_sub(xnn, hfdst, r0, hook):
        for cb in range(NCB):
            pre = _dot(xnn, w1[cb])
            h = _gelu(pre.astype(BF16).astype(F32)).astype(BF16).astype(F32)
            hfdst[cb, r0 + 8:r0 + 8 + SB, :] = h
            hook(cb, pre)

    shifts = (7, 7, 9, 9, 6, 6, 10, 10)

    def w2_sub(hfsrc, x1v, x1nv, r0, hook):
        hs = jnp.concatenate(
            [hfsrc[cb, r0 + shifts[cb]:r0 + shifts[cb] + SB, :] for cb in range(NCB)],
            axis=1).astype(BF16)
        cols = []
        for cb in range(NCB):
            pre = _dot(hs, w2[cb])
            y = pre.astype(BF16).astype(F32)
            cs = slice(cb * 128, (cb + 1) * 128)
            x1 = (x1v[r0:r0 + SB, cs].astype(F32) + y).astype(BF16)
            x1v[r0:r0 + SB, cs] = x1
            cols.append(x1.astype(F32))
            hook(cb, pre)
        x1nv[r0:r0 + SB, :] = _ln(jnp.concatenate(cols, axis=1)).astype(BF16)

    def w3_part(lhs, blocks, rows):
        for f in blocks:
            pre = _dot(lhs, w3[f])
            h3 = _gelu(pre.astype(BF16).astype(F32))
            h3buf[f, 0:rows, :] = h3.astype(BF16)
        return pre

    def w4_part(r0, rows, blocks):
        lhs = jnp.concatenate([h3buf[f, 0:rows, :] for f in range(NFB)], axis=1)
        for cb in blocks:
            pre = _dot(lhs, w4[cb])
            h2 = pre.astype(BF16).astype(F32)
            sl = (pl.ds(r0, rows), slice(cb * 128, (cb + 1) * 128))
            y = (x1buf[sl].astype(F32) + h2).astype(BF16).astype(F32)
            x1buf[sl] = _silu(y).astype(BF16)
        return pre

    def relayout(src, dst, u, trig):
        m_, c_ = divmod(u, 16)
        d0 = m_ * (H * HS) + c_ * 8
        for pp in range(8):
            r0 = u * CH + pp * 64
            t = trig[pp * 16:pp * 16 + 8, :]
            z = zero_of(t)
            two = lambda v: jnp.concatenate([v, v], axis=0)
            mlo, mhi, sh = two(z | U32(0xFFFF)), two(z | U32(0xFFFF0000)), two(z | U32(16))
            a = pltpu.bitcast(src[r0:r0 + 32, :], U32)
            b = pltpu.bitcast(src[r0 + 32:r0 + 64, :], U32)
            lo = (a & mlo) | (b << sh)
            hi = (a >> sh) | (b & mhi)
            dst[pl.ds(d0 + pp, 16, stride=HS), :] = lo
            dst[pl.ds(d0 + 16 * HS + pp, 16, stride=HS), :] = hi

    cp_x[0].wait()
    for u in range(16):
        ln_chunk(xbuf, hbuf, x1buf, x1nbuf, u, None)
    wait(cp_w1)
    HBB = (RB // 64) * HB

    def views(i, lag):
        r0 = pl.multiple_of((i - lag) * RB, RB)
        n = (lag + 2) * RB
        xsrc = xbuf.at[pl.ds(pl.multiple_of(jnp.minimum(i + 1, NXB - 1) * RB, RB), RB), :]
        hdst = hbuf.at[pl.ds(pl.multiple_of((i + 1) * HBB, 16), HBB), :]
        x1v = x1buf.at[pl.ds(r0, n), :]
        x1nv = x1nbuf.at[pl.ds(r0, n), :]
        hfv = hf.at[:, pl.ds(r0, (lag + 1) * RB + 16), :]
        nxt = (lag + 1) * RB
        ln = lambda u, trig: ln_chunk(xsrc, hdst, x1v.at[nxt:nxt + RB, :], x1nv.at[nxt:nxt + RB, :],
                                      u, trig)
        return x1v, x1nv, hfv, ln

    def loop_a1(i, carry):
        pltpu.make_async_copy(xbuf.at[pl.ds(0, RB), :], xbuf.at[pl.ds(0, RB), :], sem.at[i + 1]).wait()
        x1v, x1nv, hfv, ln = views(i, 0)
        for sb in range(2):
            def hook(cb, pre, sb=sb):
                u = sb * 8 + cb
                if u == 14:
                    ln(14, pre[64:72])
                    ln(15, pre[120:128])
                elif u < 14:
                    ln(u, pre[120:128])
            w1_sub(x1nv[sb * SB:(sb + 1) * SB, :], hfv, sb * SB, hook)
        return carry

    lax.fori_loop(0, 2, loop_a1, 0)
    wait(cp_x[3:])
    wait(cp_w2)

    def loop_a2(i, carry):
        x1v, x1nv, hfv, ln = views(i, 2)
        plan = {(0, 0): 0, (0, 1): 1, (0, 2): 2, (0, 3): 3, (0, 4): 4, (0, 5): 5, (0, 6): 6,
                (1, 2): 7, (1, 3): 8, (1, 4): 9, (1, 5): 10, (1, 6): 11,
                (2, 3): 12, (2, 5): 13, (2, 7): 14, (3, 2): 15}

        def mk(ph):
            def hook(cb, pre):
                if (ph, cb) in plan:
                    ln(plan[(ph, cb)], pre[120:128])
            return hook
        for sb in range(2):
            w2_sub(hfv, x1v, x1nv, sb * SB, mk(sb))
        for sb in range(2):
            r0 = 2 * RB + sb * SB
            w1_sub(x1nv[r0:r0 + SB, :], hfv, r0, mk(2 + sb))
        return carry

    lax.fori_loop(2, NXB, loop_a2, 0)
    wait(cp_w3)
    wait(cp_w4)

    def loop_s3(k, carry):
        pltpu.make_async_copy(stg.at[k], stg.at[k], qsem.at[k]).wait()
        r0 = pl.multiple_of(k * SB, SB)
        src = stg.at[k]
        dst = wqkv.at[pl.ds(pl.multiple_of(k * 128, 128), 3 * H * HS - 384), :]
        n = S - PRE + SB
        x1v = x1buf.at[pl.ds(r0, n), :]
        x1nv = x1nbuf.at[pl.ds(r0, n), :]
        hfv = hf.at[:, pl.ds(r0, n + 16), :]
        lhs = x1nv[0:SB, :]
        for f in range(NFB):
            pre = w3_part(lhs, [f], SB)
            relayout(src, dst, f, pre)
        w2_sub(hfv, x1v, x1nv, S - PRE,
               lambda cb, pre: relayout(src, dst, NFB + cb, pre) if cb < 6 else None)
        lhs4 = jnp.concatenate([h3buf[f, 0:SB, :] for f in range(NFB)], axis=1)
        for cb in range(NCB):
            hk = FF // 2
            p0 = _dot(lhs4[:, :hk], w4[cb, 0:hk, :])
            pre = p0 + _dot(lhs4[:, hk:], w4[cb, hk:FF, :])
            if cb < 7:
                relayout(src, dst, NFB + 6 + 2 * cb, p0)
                relayout(src, dst, NFB + 7 + 2 * cb, pre)
            cs = slice(cb * 128, (cb + 1) * 128)
            y = (x1v[0:SB, cs].astype(F32) + pre.astype(BF16).astype(F32)).astype(BF16).astype(F32)
            x1v[0:SB, cs] = _silu(y).astype(BF16)
        return carry

    lax.fori_loop(0, PRE // SB, loop_s3, 0)
    w3_part(x1nbuf[PRE:PRE + BR, :], range(NFB), BR)
    wait(cp_wo)

    def qkv_pair(lhs, j):
        def blk(m_, h):
            r0 = (m_ * H + (h % 2) * 16 + h // 2) * HS
            return pltpu.bitcast(wqkv[r0:r0 + D // 2, :], BF16)
        return [_dot(lhs, blk(i % 3, 2 * j + i // 3)) for i in range(6)]

    def scores(q, k):
        return lax.dot_general(q, k, (((1,), (1,)), ((), ())), preferred_element_type=F32)

    def softmax(s):
        fill = fillbuf[...]
        s = jnp.where(fill > 0.0, s * SCALE, fill)
        mx = jnp.max(s, axis=1, keepdims=True)
        e = jnp.exp(s - mx)
        l = jnp.sum(e, axis=1, keepdims=True)
        rc = pl.reciprocal(l, approx=True)
        rc = rc * (2.0 - l * rc)
        return (e * rc).astype(BF16)

    def attn_step(lhs, select, filler1):
        NP = H // 2
        qkv = [None] * NP
        sc = [None] * NP
        o = [None] * NP

        def do_qkv(j):
            rs = qkv_pair(lhs, j)
            rs = [select(j, i, v) for i, v in enumerate(rs)]
            qkv[j] = [jnp.concatenate([rs[i], rs[3 + i]], axis=0).astype(BF16) for i in range(3)]

        def do_s(j):
            sc[j] = softmax(scores(qkv[j][0], qkv[j][1]))

        def do_pv(j):
            o[j] = _dot(sc[j], qkv[j][2])

        for j in range(NP + 2):
            if j < NP:
                do_qkv(j)
            else:
                filler1(j - NP)
            if 0 <= j - 1 < NP:
                do_s(j - 1)
            if 0 <= j - 2 < NP:
                do_pv(j - 2)
        oh = []
        for j in range(NP):
            oh += [o[j][0:L], o[j][L:2 * L]]
        return oh

    def body(t, carry):
        base = pl.multiple_of(t * HB, 16)
        R0 = pl.multiple_of(t * 64, 64)
        B0 = pl.multiple_of(PRE + t * BR, 16)
        B1 = pl.multiple_of(jnp.minimum(B0 + BR, S - BR), 16)

        keep = {}

        def sel_a(j, i, v):
            keep[(j, i)] = v[L:L + 8]
            return v[0:L]

        lhs_a = hbuf[pl.ds(base, 48), :]
        oa = attn_step(lhs_a, sel_a, lambda n: w4_part(B0, BR, range(2 * n, 2 * n + 2)))
        w4_part(B0, BR, range(4, 6))
        lo_a = jnp.concatenate([v[0:32] for v in oa], axis=1).astype(BF16)
        ra = [_dot(lo_a, wo[cb]) for cb in range(NCB)]
        for cb in range(NCB):
            hbuf[pl.ds(base + 48, 8), cb * 128:(cb + 1) * 128] = ra[cb][0:8].astype(BF16)
        w4_part(B0, BR, range(6, 8))

        def sel_b(j, i, v):
            return jnp.concatenate([v[0:8], keep[(j, i)], v[8:32]], axis=0)

        lhs3 = x1nbuf[pl.ds(B1, BR), :]
        lhs_b = hbuf[pl.ds(base + 48, 32), :]
        ob = attn_step(lhs_b, sel_b, lambda n: w3_part(lhs3, range(7 * n, 7 * n + 7), BR))
        w3_part(lhs3, range(14, 21), BR)
        lo_b = jnp.concatenate(
            [jnp.concatenate([va[32:40], vb], axis=0) for va, vb in zip(oa, ob)],
            axis=1).astype(BF16)
        for cb in range(NCB):
            rb = _dot(lo_b, wo[cb])
            cs = slice(cb * 128, (cb + 1) * 128)
            hbuf[pl.ds(base + HB, 8), cs] = rb[8:16].astype(BF16)
            s_ = jnp.concatenate([ra[cb][8:32], rb[0:8], rb[16:48]], axis=0)
            s_ = s_.astype(BF16).astype(F32)
            sl = (pl.ds(R0, 64), cs)
            xbuf[sl] = (xbuf[sl].astype(F32) + s_ * x1buf[sl].astype(F32)).astype(BF16)
        w3_part(lhs3, range(21, 28), BR)

        pltpu.make_async_copy(xbuf.at[pl.ds(R0, 64), :], out_hbm.at[pl.ds(R0, 64), :], osem).start()
        return carry

    nit = CFG.get("nit", NIT)
    lax.fori_loop(0, nit, body, 0)
    pltpu.make_async_copy(xbuf.at[pl.ds(0, nit * 64), :], out_hbm.at[pl.ds(0, nit * 64), :], osem).wait()


@functools.partial(jax.jit, static_argnames=("A_seg_len",))
def pallas_recurrent_scan__memory_aug_recurrent_mem_tr__mixer_s_mlp__prompt_kernel(
    A_x: jax.Array,
    A_mem0: jax.Array,
    A_Wq: jax.Array,
    A_Wk: jax.Array,
    A_Wv: jax.Array,
    A_Wo: jax.Array,
    A_seg_len,
    B_x: jax.Array,
    B_w1: jax.Array,
    B_w2: jax.Array,
    B_w3: jax.Array,
    B_w4: jax.Array,
):
    assert A_seg_len == SEG
    assert A_x.shape == (1, S, D) and A_mem0.shape == (1, M, D)
    assert A_Wq.shape == (D, H, E) and A_Wo.shape == (H, E, D)
    assert B_w3.shape == (D, FF)
    del B_x

    any_spec = pl.BlockSpec(memory_space=pl.ANY)
    out = pl.pallas_call(
        _kernel,
        out_shape=jax.ShapeDtypeStruct((S, D), BF16),
        in_specs=[any_spec, pl.BlockSpec(memory_space=pltpu.VMEM)] + [any_spec] * 8,
        out_specs=any_spec,
        scratch_shapes=[
            pltpu.VMEM((S, D), BF16),
            pltpu.VMEM(((NIT + 4) * HB, D), BF16),
            pltpu.VMEM((NCB, S + 16, 128), F32),
            pltpu.VMEM((S + RB, D), BF16),
            pltpu.VMEM((S + RB, D), BF16),
            pltpu.VMEM((NFB, 128, 128), BF16),
            pltpu.VMEM((4, 3 * D * H // 4, E), BF16),
            pltpu.VMEM((3 * H * HS, 128), U32),
            pltpu.VMEM((NCB, H * E, 128), BF16),
            pltpu.VMEM((NCB, D, 128), BF16),
            pltpu.VMEM((NCB, D, 128), BF16),
            pltpu.VMEM((NFB, D, 128), BF16),
            pltpu.VMEM((NCB, FF, 128), BF16),
            pltpu.VMEM((HB, HB), F32),
            pltpu.SemaphoreType.DMA((9,)),
            pltpu.SemaphoreType.DMA((4,)),
            pltpu.SemaphoreType.DMA(()),
        ],
        compiler_params=pltpu.CompilerParams(vmem_limit_bytes=120 * 1024 * 1024),
    )(
        A_x.reshape(S, D), A_mem0.reshape(M, D),
        A_Wq.reshape(D * H, E), A_Wk.reshape(D * H, E), A_Wv.reshape(D * H, E),
        A_Wo.reshape(H * E, D), B_w1, B_w2, B_w3, B_w4,
    )
    return out.reshape(1, S, D)
```

```python
import functools

import jax
import jax.numpy as jnp
from jax import lax
import jax.experimental.pallas as pl
import jax.experimental.pallas.tpu as pltpu

F32 = jnp.float32
BF16 = jnp.bfloat16
U32 = jnp.uint32

S = 2048
D = 1024
H = 32
E = 128
M = 8
SEG = 32
L = M + SEG
FF = 3584
NCB = D // 128
NFB = FF // 128
NIT = S // (2 * SEG)
HB = 2 * L
PRE = 512
BR = (S - PRE) // NIT
HS = D // 2 + 8
EPS = 1e-5
SCALE = float(E) ** -0.5
RB = 256
CFG = {}


def _dot(a, b):
    return jnp.dot(a, b, preferred_element_type=F32)


def _ln(x):
    m = jnp.mean(x, axis=-1, keepdims=True)
    xc = x - m
    v = jnp.mean(xc * xc, axis=-1, keepdims=True)
    return xc * lax.rsqrt(v + EPS)


def _gelu(x):
    c = 0.7978845608028654
    return 0.5 * x * (1.0 + jnp.tanh(c * (x + 0.044715 * (x * x * x))))


def _silu(x):
    return x * (1.0 / (1.0 + jnp.exp(-x)))


def _kernel(x_hbm, mem0_ref, wq_hbm, wk_hbm, wv_hbm, wo_hbm, w1_hbm, w2_hbm, w3_hbm, w4_hbm,
            out_hbm,
            xbuf, hbuf, hf, x1buf, x1nbuf, h3buf, stg, wqkv, wo, w1, w2, w3, w4, fillbuf,
            sem, qsem, osem):
    def colblock_copies(src, dst, nblk, s):
        return [pltpu.make_async_copy(src.at[:, pl.ds(c * 128, 128)], dst.at[c], sem.at[s])
                for c in range(nblk)]

    NXB = S // RB
    cp_x = [pltpu.make_async_copy(x_hbm.at[pl.ds(i * RB, RB), :], xbuf.at[pl.ds(i * RB, RB), :],
                                  sem.at[min(i, 3)]) for i in range(NXB)]
    cp_w1 = colblock_copies(w1_hbm, w1, NCB, 4)
    cp_w2 = colblock_copies(w2_hbm, w2, NCB, 5)
    cp_w3 = colblock_copies(w3_hbm, w3, NFB, 6)
    cp_w4 = colblock_copies(w4_hbm, w4, NCB, 7)
    cp_wo = colblock_copies(wo_hbm, wo, NCB, 8)
    CH = 512
    PR = 16 * CH
    cp_qkv = [pltpu.make_async_copy(src.at[pl.ds(k * PR, PR), :], stg.at[k, pl.ds(m_ * PR, PR), :],
                                    qsem.at[k])
              for k in range(4) for m_, src in enumerate((wq_hbm, wk_hbm, wv_hbm))]
    for grp in (cp_x[:1], cp_w1, cp_x[1:], cp_w2, cp_w3, cp_w4, cp_qkv, cp_wo):
        for c in grp:
            c.start()

    def wait(grp):
        for c in grp:
            c.wait()

    r = lax.broadcasted_iota(jnp.int32, (HB, HB), 0)
    c = lax.broadcasted_iota(jnp.int32, (HB, HB), 1)
    rr = jnp.where(r >= L, r - L, r)
    cc = jnp.where(c >= L, c - L, c)
    same = (r >= L) == (c >= L)
    allowed = (rr < M) | (rr >= cc)
    fillbuf[...] = jnp.where(same, jnp.where(allowed, 1.0, -1e9), -jnp.inf).astype(F32)

    hf[:, 0:8, :] = jnp.zeros((NCB, 8, 128), F32)
    hf[:, S + 8:S + 16, :] = jnp.zeros((NCB, 8, 128), F32)
    hbuf[0:M, :] = mem0_ref[...]

    SB = 128

    def zero_of(trig):
        return (pltpu.bitcast(trig, U32) >> 16) >> 16

    def ln_chunk(xsrc, hdst, x1dst, x1ndst, u, trig):
        xb = xsrc[16 * u:16 * u + 16, :]
        if trig is not None:
            z = zero_of(trig)
            xb = pltpu.bitcast(pltpu.bitcast(xb, U32) | jnp.concatenate([z] * NCB, axis=1), BF16)
        xn = _ln(xb.astype(F32)).astype(BF16)
        for hh in range(2):
            q, rr_ = divmod(16 * u + 8 * hh, 64)
            o = q * HB + rr_ + (8 if rr_ < 40 else 16)
            hdst[o:o + 8, :] = xn[8 * hh:8 * hh + 8]
        x1dst[16 * u:16 * u + 16, :] = xn
        x1ndst[16 * u:16 * u + 16, :] = _ln(xn.astype(F32)).astype(BF16)

    def w1_sub(xnn, hfdst, r0, hook):
        for cb in range(NCB):
            pre = _dot(xnn, w1[cb])
            h = _gelu(pre.astype(BF16).astype(F32)).astype(BF16).astype(F32)
            hfdst[cb, r0 + 8:r0 + 8 + SB, :] = h
            hook(cb, pre)

    shifts = (7, 7, 9, 9, 6, 6, 10, 10)

    def w2_sub(hfsrc, x1v, x1nv, r0, hook):
        hs = jnp.concatenate(
            [hfsrc[cb, r0 + shifts[cb]:r0 + shifts[cb] + SB, :] for cb in range(NCB)],
            axis=1).astype(BF16)
        cols = []
        for cb in range(NCB):
            pre = _dot(hs, w2[cb])
            y = pre.astype(BF16).astype(F32)
            cs = slice(cb * 128, (cb + 1) * 128)
            x1 = (x1v[r0:r0 + SB, cs].astype(F32) + y).astype(BF16)
            x1v[r0:r0 + SB, cs] = x1
            cols.append(x1.astype(F32))
            hook(cb, pre)
        x1nv[r0:r0 + SB, :] = _ln(jnp.concatenate(cols, axis=1)).astype(BF16)

    def w3_part(lhs, blocks, rows):
        for f in blocks:
            pre = _dot(lhs, w3[f])
            h3 = _gelu(pre.astype(BF16).astype(F32))
            h3buf[f, 0:rows, :] = h3.astype(BF16)
        return pre

    def w4_part(r0, rows, blocks):
        lhs = jnp.concatenate([h3buf[f, 0:rows, :] for f in range(NFB)], axis=1)
        for cb in blocks:
            pre = _dot(lhs, w4[cb])
            h2 = pre.astype(BF16).astype(F32)
            sl = (pl.ds(r0, rows), slice(cb * 128, (cb + 1) * 128))
            y = (x1buf[sl].astype(F32) + h2).astype(BF16).astype(F32)
            x1buf[sl] = _silu(y).astype(BF16)
        return pre

    def relayout(src, dst, u, trig):
        m_, c_ = divmod(u, 16)
        d0 = m_ * (H * HS) + c_ * 8
        for pp in range(8):
            r0 = u * CH + pp * 64
            t = trig[pp * 16:pp * 16 + 8, :]
            z = zero_of(t)
            two = lambda v: jnp.concatenate([v, v], axis=0)
            mlo, mhi, sh = two(z | U32(0xFFFF)), two(z | U32(0xFFFF0000)), two(z | U32(16))
            a = pltpu.bitcast(src[r0:r0 + 32, :], U32)
            b = pltpu.bitcast(src[r0 + 32:r0 + 64, :], U32)
            lo = (a & mlo) | (b << sh)
            hi = (a >> sh) | (b & mhi)
            dst[pl.ds(d0 + pp, 16, stride=HS), :] = lo
            dst[pl.ds(d0 + 16 * HS + pp, 16, stride=HS), :] = hi

    with jax.named_scope("wait_x0"):
        cp_x[0].wait()
    with jax.named_scope("ln0"):
        for u in range(16):
            ln_chunk(xbuf, hbuf, x1buf, x1nbuf, u, None)
    with jax.named_scope("wait_w1"):
        wait(cp_w1)
    HBB = (RB // 64) * HB

    def views(i, lag):
        r0 = pl.multiple_of((i - lag) * RB, RB)
        n = (lag + 2) * RB
        xsrc = xbuf.at[pl.ds(pl.multiple_of(jnp.minimum(i + 1, NXB - 1) * RB, RB), RB), :]
        hdst = hbuf.at[pl.ds(pl.multiple_of((i + 1) * HBB, 16), HBB), :]
        x1v = x1buf.at[pl.ds(r0, n), :]
        x1nv = x1nbuf.at[pl.ds(r0, n), :]
        hfv = hf.at[:, pl.ds(r0, (lag + 1) * RB + 16), :]
        nxt = (lag + 1) * RB
        ln = lambda u, trig: ln_chunk(xsrc, hdst, x1v.at[nxt:nxt + RB, :], x1nv.at[nxt:nxt + RB, :],
                                      u, trig)
        return x1v, x1nv, hfv, ln

    def loop_a1(i, carry):
        pltpu.make_async_copy(xbuf.at[pl.ds(0, RB), :], xbuf.at[pl.ds(0, RB), :], sem.at[i + 1]).wait()
        x1v, x1nv, hfv, ln = views(i, 0)
        for sb in range(2):
            def hook(cb, pre, sb=sb):
                u = sb * 8 + cb
                if u == 14:
                    ln(14, pre[64:72])
                    ln(15, pre[120:128])
                elif u < 14:
                    ln(u, pre[120:128])
            w1_sub(x1nv[sb * SB:(sb + 1) * SB, :], hfv, sb * SB, hook)
        return carry

    with jax.named_scope("a1"):
        lax.fori_loop(0, 2, loop_a1, 0)
    with jax.named_scope("wait_w2"):
        wait(cp_x[3:])
        wait(cp_w2)

    def loop_a2(i, carry):
        x1v, x1nv, hfv, ln = views(i, 2)
        plan = {(0, 0): 0, (0, 1): 1, (0, 2): 2, (0, 3): 3, (0, 4): 4, (0, 5): 5, (0, 6): 6,
                (1, 2): 7, (1, 3): 8, (1, 4): 9, (1, 5): 10, (1, 6): 11,
                (2, 3): 12, (2, 5): 13, (2, 7): 14, (3, 2): 15}

        def mk(ph):
            def hook(cb, pre):
                if (ph, cb) in plan:
                    ln(plan[(ph, cb)], pre[120:128])
            return hook
        for sb in range(2):
            w2_sub(hfv, x1v, x1nv, sb * SB, mk(sb))
        for sb in range(2):
            r0 = 2 * RB + sb * SB
            w1_sub(x1nv[r0:r0 + SB, :], hfv, r0, mk(2 + sb))
        return carry

    with jax.named_scope("a2"):
        lax.fori_loop(2, NXB, loop_a2, 0)
    with jax.named_scope("wait_w34"):
        wait(cp_w3)
        wait(cp_w4)

    def loop_s3(k, carry):
        pltpu.make_async_copy(stg.at[k], stg.at[k], qsem.at[k]).wait()
        r0 = pl.multiple_of(k * SB, SB)
        src = stg.at[k]
        dst = wqkv.at[pl.ds(pl.multiple_of(k * 128, 128), 3 * H * HS - 384), :]
        n = S - PRE + SB
        x1v = x1buf.at[pl.ds(r0, n), :]
        x1nv = x1nbuf.at[pl.ds(r0, n), :]
        hfv = hf.at[:, pl.ds(r0, n + 16), :]
        lhs = x1nv[0:SB, :]
        for f in range(NFB):
            pre = w3_part(lhs, [f], SB)
            relayout(src, dst, f, pre)
        w2_sub(hfv, x1v, x1nv, S - PRE,
               lambda cb, pre: relayout(src, dst, NFB + cb, pre) if cb < 6 else None)
        lhs4 = jnp.concatenate([h3buf[f, 0:SB, :] for f in range(NFB)], axis=1)
        for cb in range(NCB):
            hk = FF // 2
            p0 = _dot(lhs4[:, :hk], w4[cb, 0:hk, :])
            pre = _dot(lhs4[:, hk:], w4[cb, hk:FF, :]) + p0
            if cb < 7:
                relayout(src, dst, NFB + 6 + 2 * cb, p0)
                relayout(src, dst, NFB + 7 + 2 * cb, pre)
            cs = slice(cb * 128, (cb + 1) * 128)
            y = (x1v[0:SB, cs].astype(F32) + pre.astype(BF16).astype(F32)).astype(BF16).astype(F32)
            x1v[0:SB, cs] = _silu(y).astype(BF16)
        return carry

    with jax.named_scope("s3"):
        lax.fori_loop(0, PRE // SB, loop_s3, 0)
    with jax.named_scope("w3pre"):
        w3_part(x1nbuf[PRE:PRE + BR, :], range(NFB), BR)
    with jax.named_scope("wait_wo"):
        wait(cp_wo)

    def qkv_pair(lhs, j):
        def blk(m_, h):
            r0 = (m_ * H + (h % 2) * 16 + h // 2) * HS
            return pltpu.bitcast(wqkv[r0:r0 + D // 2, :], BF16)
        return [_dot(lhs, blk(i % 3, 2 * j + i // 3)) for i in range(6)]

    def scores(q, k):
        return lax.dot_general(q, k, (((1,), (1,)), ((), ())), preferred_element_type=F32)

    def softmax(s):
        fill = fillbuf[...]
        s = jnp.where(fill > 0.0, s * SCALE, fill)
        mx = jnp.max(s, axis=1, keepdims=True)
        e = jnp.exp(s - mx)
        l = jnp.sum(e, axis=1, keepdims=True)
        rc = pl.reciprocal(l, approx=True)
        rc = rc * (2.0 - l * rc)
        return (e * rc).astype(BF16)

    NP = H // 2

    def attn_step(lhs, select, wo_rows, fill, wsplit):
        qkv = [None] * NP
        sc = [None] * NP
        oh = [None] * H
        acc = [None] * NCB

        def do_qkv(j):
            rs = qkv_pair(lhs, j)
            rs = [select(j, i, v) for i, v in enumerate(rs)]
            qkv[j] = [jnp.concatenate([rs[i], rs[3 + i]], axis=0).astype(BF16) for i in range(3)]

        def do_s(j):
            sc[j] = softmax(scores(qkv[j][0], qkv[j][1]))

        def do_pv(j):
            o = _dot(sc[j], qkv[j][2])
            oh[2 * j] = wo_rows(2 * j, o[0:L]).astype(BF16)
            oh[2 * j + 1] = wo_rows(2 * j + 1, o[L:2 * L]).astype(BF16)

        def do_wo(n):
            h0, h1 = wsplit[n], wsplit[n + 1]
            if h1 == h0:
                return
            lo = jnp.concatenate(oh[h0:h1], axis=1)
            for cb in range(NCB):
                part = _dot(lo, wo[cb, h0 * E:h1 * E, :])
                acc[cb] = part if acc[cb] is None else part + acc[cb]
                fill(NP + n * NCB + cb)

        for j in range(NP + 2):
            if j < NP:
                do_qkv(j)
                fill(j)
            else:
                do_wo(j - NP)
            if 0 <= j - 1 < NP:
                do_s(j - 1)
            if 0 <= j - 2 < NP:
                do_pv(j - 2)
        do_wo(2)
        do_wo(3)
        return acc

    def body(t, carry):
        base = pl.multiple_of(t * HB, 16)
        R0 = pl.multiple_of(t * 64, 64)
        B0 = pl.multiple_of(PRE + t * BR, 16)
        B1 = pl.multiple_of(jnp.minimum(B0 + BR, S - BR), 16)

        nslot = NP + 4 * NCB + 1
        fa = dict(CFG.get("fa", [[17, 1], [21, 1], [26, 1], [30, 1], [34, 1], [38, 1], [48, 2]]))
        fb = dict(CFG.get("fb", [[j, 1 + (j % 3 == 0)] for j in range(16)] + [[48, 6]]))
        fa = [fa.get(n, 0) for n in range(nslot)]
        fb = [fb.get(n, 0) for n in range(nslot)]
        assert sum(fa) == NCB and sum(fb) == NFB
        wsa = CFG.get("wsa", [0, 8, 20, 28, 32])
        wsb = CFG.get("wsb", [0, 8, 20, 28, 32])

        def fill_a(n):
            if fa[n]:
                w4_part(B0, BR, range(sum(fa[:n]), sum(fa[:n + 1])))

        def fill_b(n):
            if fb[n]:
                w3_part(lhs3, range(sum(fb[:n]), sum(fb[:n + 1])), BR)

        keep = {}
        keep_o = {}

        def sel_a(j, i, v):
            keep[(j, i)] = v[L:L + 8]
            return v[0:L]

        def wo_a(h, o):
            keep_o[h] = o[32:40]
            return o[0:32]

        lhs_a = hbuf[pl.ds(base, 48), :]
        ra = attn_step(lhs_a, sel_a, wo_a, fill_a, wsa)
        for cb in range(NCB):
            hbuf[pl.ds(base + 48, 8), cb * 128:(cb + 1) * 128] = ra[cb][0:8].astype(BF16)
        fill_a(nslot - 1)

        def sel_b(j, i, v):
            return jnp.concatenate([v[0:8], keep[(j, i)], v[8:32]], axis=0)

        def wo_b(h, o):
            return jnp.concatenate([keep_o[h], o], axis=0)

        lhs3 = x1nbuf[pl.ds(B1, BR), :]
        lhs_b = hbuf[pl.ds(base + 48, 32), :]
        rb = attn_step(lhs_b, sel_b, wo_b, fill_b, wsb)
        for cb in range(NCB):
            cs = slice(cb * 128, (cb + 1) * 128)
            hbuf[pl.ds(base + HB, 8), cs] = rb[cb][8:16].astype(BF16)
            s_ = jnp.concatenate([ra[cb][8:32], rb[cb][0:8], rb[cb][16:48]], axis=0)
            s_ = s_.astype(BF16).astype(F32)
            sl = (pl.ds(R0, 64), cs)
            xbuf[sl] = (xbuf[sl].astype(F32) + s_ * x1buf[sl].astype(F32)).astype(BF16)
        fill_b(nslot - 1)

        pltpu.make_async_copy(xbuf.at[pl.ds(R0, 64), :], out_hbm.at[pl.ds(R0, 64), :], osem).start()
        return carry

    nit = CFG.get("nit", NIT)
    with jax.named_scope("main"):
        lax.fori_loop(0, nit, body, 0)
    with jax.named_scope("wait_out"):
        pltpu.make_async_copy(xbuf.at[pl.ds(0, nit * 64), :], out_hbm.at[pl.ds(0, nit * 64), :], osem).wait()


@functools.partial(jax.jit, static_argnames=("A_seg_len",))
def pallas_recurrent_scan__memory_aug_recurrent_mem_tr__mixer_s_mlp__prompt_kernel(
    A_x: jax.Array,
    A_mem0: jax.Array,
    A_Wq: jax.Array,
    A_Wk: jax.Array,
    A_Wv: jax.Array,
    A_Wo: jax.Array,
    A_seg_len,
    B_x: jax.Array,
    B_w1: jax.Array,
    B_w2: jax.Array,
    B_w3: jax.Array,
    B_w4: jax.Array,
):
    assert A_seg_len == SEG
    assert A_x.shape == (1, S, D) and A_mem0.shape == (1, M, D)
    assert A_Wq.shape == (D, H, E) and A_Wo.shape == (H, E, D)
    assert B_w3.shape == (D, FF)
    del B_x

    any_spec = pl.BlockSpec(memory_space=pl.ANY)
    out = pl.pallas_call(
        _kernel,
        out_shape=jax.ShapeDtypeStruct((S, D), BF16),
        in_specs=[any_spec, pl.BlockSpec(memory_space=pltpu.VMEM)] + [any_spec] * 8,
        out_specs=any_spec,
        scratch_shapes=[
            pltpu.VMEM((S, D), BF16),
            pltpu.VMEM(((NIT + 4) * HB, D), BF16),
            pltpu.VMEM((NCB, S + 16, 128), F32),
            pltpu.VMEM((S + RB, D), BF16),
            pltpu.VMEM((S + RB, D), BF16),
            pltpu.VMEM((NFB, 128, 128), BF16),
            pltpu.VMEM((4, 3 * D * H // 4, E), BF16),
            pltpu.VMEM((3 * H * HS, 128), U32),
            pltpu.VMEM((NCB, H * E, 128), BF16),
            pltpu.VMEM((NCB, D, 128), BF16),
            pltpu.VMEM((NCB, D, 128), BF16),
            pltpu.VMEM((NFB, D, 128), BF16),
            pltpu.VMEM((NCB, FF, 128), BF16),
            pltpu.VMEM((HB, HB), F32),
            pltpu.SemaphoreType.DMA((9,)),
            pltpu.SemaphoreType.DMA((4,)),
            pltpu.SemaphoreType.DMA(()),
        ],
        compiler_params=pltpu.CompilerParams(vmem_limit_bytes=120 * 1024 * 1024),
    )(
        A_x.reshape(S, D), A_mem0.reshape(M, D),
        A_Wq.reshape(D * H, E), A_Wk.reshape(D * H, E), A_Wv.reshape(D * H, E),
        A_Wo.reshape(H * E, D), B_w1, B_w2, B_w3, B_w4,
    )
    return out.reshape(1, S, D)
```

```python
import functools

import jax
import jax.numpy as jnp
from jax import lax
import jax.experimental.pallas as pl
import jax.experimental.pallas.tpu as pltpu

F32 = jnp.float32
BF16 = jnp.bfloat16
U32 = jnp.uint32

S = 2048
D = 1024
H = 32
E = 128
M = 8
SEG = 32
L = M + SEG
FF = 3584
NCB = D // 128
NFB = FF // 128
NIT = S // (2 * SEG)
HB = 2 * L
PRE = 512
BR = (S - PRE) // NIT
HS = D // 2 + 8
EPS = 1e-5
SCALE = float(E) ** -0.5
RB = 256
CFG = {}


def _dot(a, b):
    return jnp.dot(a, b, preferred_element_type=F32)


def _ln(x):
    m = jnp.mean(x, axis=-1, keepdims=True)
    xc = x - m
    v = jnp.mean(xc * xc, axis=-1, keepdims=True)
    return xc * lax.rsqrt(v + EPS)


def _ln2(x):
    m = jnp.mean(x, axis=-1, keepdims=True)
    xc = x - m
    v = jnp.mean(xc * xc, axis=-1, keepdims=True)
    r1 = lax.rsqrt(v + EPS)
    r2 = lax.rsqrt(v * r1 * r1 + EPS)
    return xc * r1, xc * (r1 * r2)


def _gelu(x):
    c = 0.7978845608028654
    hx = 0.5 * x
    return hx * jnp.tanh(x * (c + (c * 0.044715) * (x * x))) + hx


def _silu(x):
    hx = 0.5 * x
    return hx * jnp.tanh(hx) + hx


def _kernel(x_hbm, mem0_hbm, wq_hbm, wk_hbm, wv_hbm, wo_hbm, w1_hbm, w2_hbm, w3_hbm, w4_hbm,
            out_hbm,
            xbuf, hbuf, hf, x1buf, h3buf, stg, wqkv, wo, w1, w2, w3, w4, fillbuf,
            sem, osem):
    def colblock_copies(src, dst, s):
        n, _, cw = dst.shape
        return [pltpu.make_async_copy(src.at[:, pl.ds(c * cw, cw)], dst.at[c], sem.at[s(c)])
                for c in range(n)]

    def col(w, cb, k0=0, k1=None):
        _, kk, cw = w.shape
        q, r_ = divmod(cb * 128, cw)
        return w[q, k0:(kk if k1 is None else k1), r_:r_ + 128]

    SB = 128
    NXB = S // RB
    XS, QS = 7, 12
    xch = [(0, SB), (SB, SB), (RB, RB), (2 * RB, RB), (3 * RB, S - 3 * RB)]
    cp_x = [pltpu.make_async_copy(x_hbm.at[pl.ds(r, n), :], xbuf.at[pl.ds(r, n), :], sem.at[XS + i])
            for i, (r, n) in enumerate(xch)]
    cp_w1 = colblock_copies(w1_hbm, w1, lambda c: 2 * c // w1.shape[0])
    cp_w1a, cp_w1b = cp_w1[:len(cp_w1) // 2], cp_w1[len(cp_w1) // 2:]
    cp_mem = [pltpu.make_async_copy(mem0_hbm, hbuf.at[0:M, :], sem.at[2])]
    cp_w2 = colblock_copies(w2_hbm, w2, lambda c: 3)
    cp_w3 = colblock_copies(w3_hbm, w3, lambda c: 4)
    cp_w4 = colblock_copies(w4_hbm, w4, lambda c: 5)
    cp_wo = colblock_copies(wo_hbm, wo, lambda c: 6)
    CH = 512
    PR = 16 * CH
    cp_qkv = [pltpu.make_async_copy(src.at[pl.ds(k * PR, PR), :], stg.at[k, pl.ds(m_ * PR, PR), :],
                                    sem.at[QS + k])
              for k in range(4) for m_, src in enumerate((wq_hbm, wk_hbm, wv_hbm))]
    def start(*grps, priority=0):
        for grp in grps:
            for c in grp:
                c.start(priority=priority)

    mode = CFG.get("dma", 0)
    if mode == 0:
        start(cp_x[:1], cp_w1a, cp_x[1:2], cp_w1b, cp_x[2:3], cp_w2, cp_x[3:], cp_mem, cp_w3, cp_w4, cp_qkv, cp_wo)
    elif mode == 1:
        start(cp_x[:1], cp_w1a, cp_x[1:2], cp_w1b, cp_x[2:3])
        start(cp_w2, cp_x[3:], cp_mem, cp_w3, cp_w4, cp_qkv, cp_wo, priority=1)
    elif mode == 2:
        start(cp_x[:1], cp_w1a, cp_x[1:2], cp_w1b, cp_x[2:3])

    def wait(grp):
        for c in grp:
            c.wait()

    r = lax.broadcasted_iota(jnp.int32, (HB, HB), 0)
    c = lax.broadcasted_iota(jnp.int32, (HB, HB), 1)
    rr = jnp.where(r >= L, r - L, r)
    cc = jnp.where(c >= L, c - L, c)
    same = (r >= L) == (c >= L)
    allowed = (rr < M) | (rr >= cc)
    fillbuf[...] = jnp.where(same, jnp.where(allowed, 1.0, -1e9), -jnp.inf).astype(F32)

    hf[:, 0:8, :] = jnp.zeros((NCB, 8, 128), F32)
    hf[:, S + 8:S + 16, :] = jnp.zeros((NCB, 8, 128), F32)

    HSB = (SB // 64) * HB

    def zero_of(trig):
        return (pltpu.bitcast(trig, U32) >> 16) >> 16

    def hrow(r):
        q, rr_ = divmod(r, 64)
        return q * HB + rr_ + (8 if rr_ < 40 else 16)

    def ln_sub(xv, hv, sb):
        out = []
        for u in range(SB // 16):
            r = sb * SB + 16 * u
            xn, xnn = _ln2(xv[r:r + 16, :].astype(F32))
            xn = xn.astype(BF16)
            for hh in range(2):
                o = hrow(r + 8 * hh)
                hv[o:o + 8, :] = xn[8 * hh:8 * hh + 8]
            out.append(xnn.astype(BF16))
        return out

    def after(w, vals):
        if not vals:
            return w
        z = None
        for v in vals:
            zv = zero_of(v[0:16, D - 128:D])
            z = zv if z is None else z | zv
        head = pltpu.bitcast(pltpu.bitcast(w[0:16, :], U32) | z, BF16)
        return jnp.concatenate([head, w[16:, :]], axis=0)

    def w1_sub(xnn, hfv, sb, cbs=range(NCB), deps={}):
        xnn = jnp.concatenate(xnn, axis=0)
        for cb in cbs:
            w = after(col(w1, cb), deps.get(cb, []))
            hfv[cb, sb * SB + 8:sb * SB + 8 + SB, :] = _gelu(_dot(xnn, w))

    shifts = (7, 7, 9, 9, 6, 6, 10, 10)

    def w2_lhs(hfv, sb):
        r0 = sb * SB
        return jnp.concatenate(
            [hfv[cb, r0 + shifts[cb]:r0 + shifts[cb] + SB, :] for cb in range(NCB)],
            axis=1).astype(BF16)

    def w2_sub(hs, hv, x1v, sb, cbs=range(NCB), hook=None, deps={}):
        r0 = sb * SB
        for cb in cbs:
            pre = _dot(hs, after(col(w2, cb), deps.get(cb, [])))
            cs = slice(cb * 128, (cb + 1) * 128)
            xn = jnp.concatenate(
                [hv[hrow(r0 + a_):hrow(r0 + a_) + n_, cs].astype(F32)
                 for a_, n_ in ((0, 40), (40, 24), (64, 40), (104, 24))], axis=0)
            x1v[r0:r0 + SB, cs] = (xn + pre).astype(BF16)
            if hook is not None:
                hook(cb, pre)

    def w3_lhs(src, r0, rows):
        return [_ln(src[pl.ds(r0 + 16 * u, 16), :].astype(F32)).astype(BF16)
                for u in range(rows // 16)]

    def w3_part(lhs, blocks, rows):
        for f in blocks:
            pre = _dot(lhs, col(w3, f))
            h3buf[f, 0:rows, :] = _gelu(pre).astype(BF16)
        return pre

    def w4_part(r0, rows, blocks):
        lhs = jnp.concatenate([h3buf[f, 0:rows, :] for f in range(NFB)], axis=1)
        for cb in blocks:
            pre = _dot(lhs, col(w4, cb))
            sl = (pl.ds(r0, rows), slice(cb * 128, (cb + 1) * 128))
            x1buf[sl] = _silu(x1buf[sl].astype(F32) + pre).astype(BF16)

    def relayout(src, dst, u, trig):
        m_, c_ = divmod(u, 16)
        d0 = m_ * (H * HS) + c_ * 8
        for pp in range(8):
            r0 = u * CH + pp * 64
            t = trig[pp * 16:pp * 16 + 8, :]
            z = zero_of(t)
            two = lambda v: jnp.concatenate([v, v], axis=0)
            mlo, mhi, sh = two(z | U32(0xFFFF)), two(z | U32(0xFFFF0000)), two(z | U32(16))
            a = pltpu.bitcast(src[r0:r0 + 32, :], U32)
            b = pltpu.bitcast(src[r0 + 32:r0 + 64, :], U32)
            lo = (a & mlo) | (b << sh)
            hi = (a >> sh) | (b & mhi)
            dst[pl.ds(d0 + pp, 16, stride=HS), :] = lo
            dst[pl.ds(d0 + 16 * HS + pp, 16, stride=HS), :] = hi

    spread4 = lambda c, o: {o + 2: c[0:3], o + 3: c[3:6]}
    spread8 = lambda c: {2: c[0:1], 3: c[1:2], 4: c[2:4], 5: c[4:5], 6: c[5:7], 7: c[7:8]}
    with jax.named_scope("wx0"):
        cp_x[0].wait()
    with jax.named_scope("ln0"):
        xnn0 = ln_sub(xbuf, hbuf, 0)
    with jax.named_scope("ww1a"):
        wait(cp_w1a)
    with jax.named_scope("wx1"):
        cp_x[1].wait()
        if mode == 2:
            start(cp_w2, cp_x[3:], cp_mem, cp_w3, cp_w4, cp_qkv, cp_wo)
    with jax.named_scope("a00"):
        xnn1 = ln_sub(xbuf, hbuf, 1)
        w1_sub(xnn0, hf, 0, range(0, 4), spread4(xnn1, 0))
        w1_sub(xnn1, hf, 1, range(0, 4))
    with jax.named_scope("ww1b"):
        wait(cp_w1b)
    with jax.named_scope("a01"):
        w1_sub(xnn0, hf, 0, range(4, 8))
    with jax.named_scope("wx2"):
        cp_x[2].wait()
    with jax.named_scope("a1"):
        xnn2 = ln_sub(xbuf, hbuf, 2)
        xnn3 = ln_sub(xbuf, hbuf, 3)
        w1_sub(xnn1, hf, 1, range(4, 8), spread4(xnn2, 4))
        w1_sub(xnn2, hf, 2, deps=spread8(xnn3))
        w1_sub(xnn3, hf, 3)
    with jax.named_scope("wait_w2"):
        wait(cp_w2)
        cp_x[3].wait()

    def loop_a2(i, carry):
        @pl.when(i == 3)
        def _():
            cp_x[4].wait()

        r0 = pl.multiple_of((i - 2) * RB, RB)
        xv = xbuf.at[pl.ds(r0, 3 * RB), :]
        hv = hbuf.at[pl.ds(pl.multiple_of((i - 2) * 2 * HSB, 16), 6 * HSB), :]
        x1v = x1buf.at[pl.ds(r0, RB), :]
        hfv = hf.at[:, pl.ds(r0, 3 * RB + 16), :]
        for sb in range(2):
            xnn = ln_sub(xv, hv, 4 + sb)
            w2_sub(w2_lhs(hfv, sb), hv, x1v, sb, deps=spread8(xnn))
            w1_sub(xnn, hfv, 4 + sb)
        return carry

    with jax.named_scope("a2"):
        lax.fori_loop(2, NXB, loop_a2, 0)
    with jax.named_scope("wait_w34"):
        wait(cp_w3)
        wait(cp_w4)

    def loop_s3(k, carry):
        pltpu.make_async_copy(stg.at[k], stg.at[k], sem.at[QS + k]).wait()
        r0 = pl.multiple_of(k * SB, SB)
        src = stg.at[k]
        dst = wqkv.at[pl.ds(pl.multiple_of(k * 128, 128), 3 * H * HS - 384), :]
        sb2 = (S - PRE) // SB
        x1v = x1buf.at[pl.ds(r0, (sb2 + 1) * SB), :]
        hv = hbuf.at[pl.ds(pl.multiple_of(k * HSB, 16), (sb2 + 1) * HSB), :]
        hfv = hf.at[:, pl.ds(r0, (sb2 + 1) * SB + 16), :]
        hook = lambda cb, pre: relayout(src, dst, cb, pre) if cb < 6 else None
        hs = w2_lhs(hfv, sb2)
        lhs = w3_lhs(x1v, 0, SB)
        w2_sub(hs, hv, x1v, sb2, range(0, 6), hook, {2: lhs[0:1], 3: lhs[1:3], 4: lhs[3:5], 5: lhs[5:7]})
        lhs = jnp.concatenate(lhs, axis=0)
        for f in range(NFB):
            pre = w3_part(lhs, [f], SB)
            relayout(src, dst, 6 + f, pre)
        w2_sub(hs, hv, x1v, sb2, range(6, 8), hook)
        lhs4 = jnp.concatenate([h3buf[f, 0:SB, :] for f in range(NFB)], axis=1)
        for cb in range(NCB):
            hk = 12 * 128
            p0 = _dot(lhs4[:, :hk], col(w4, cb, 0, hk))
            pre = _dot(lhs4[:, hk:], col(w4, cb, hk, FF)) + p0
            if cb < 7:
                relayout(src, dst, NFB + 6 + 2 * cb, p0)
                relayout(src, dst, NFB + 7 + 2 * cb, pre)
            cs = slice(cb * 128, (cb + 1) * 128)
            x1v[0:SB, cs] = _silu(x1v[0:SB, cs].astype(F32) + pre).astype(BF16)
        return carry

    with jax.named_scope("s3"):
        lax.fori_loop(0, PRE // SB, loop_s3, 0)
    with jax.named_scope("w3pre"):
        w3_part(jnp.concatenate(w3_lhs(x1buf, PRE, BR), axis=0), range(NFB), BR)
    with jax.named_scope("wait_wo"):
        wait(cp_wo)
        wait(cp_mem)

    def qkv_pair(lhs, j):
        def blk(m_, h):
            r0 = (m_ * H + (h % 2) * 16 + h // 2) * HS
            return pltpu.bitcast(wqkv[r0:r0 + D // 2, :], BF16)
        return [_dot(lhs, blk(i % 3, 2 * j + i // 3)) for i in range(6)]

    def scores(q, k):
        return lax.dot_general(q, k, (((1,), (1,)), ((), ())), preferred_element_type=F32)

    def softmax(s):
        fill = fillbuf[...]
        s = jnp.where(fill > 0.0, s * SCALE, fill)
        mx = jnp.max(s, axis=1, keepdims=True)
        e = jnp.exp(s - mx)
        l = jnp.sum(e, axis=1, keepdims=True)
        rc = pl.reciprocal(l, approx=True)
        rc = rc * (2.0 - l * rc)
        return (e * rc).astype(BF16)

    NP = H // 2

    def attn_step(lhs, select, wo_rows, fill, wsplit):
        qkv = [None] * NP
        sc = [None] * NP
        oh = [None] * H
        acc = [None] * NCB

        def do_qkv(j):
            rs = qkv_pair(lhs, j)
            rs = [select(j, i, v) for i, v in enumerate(rs)]
            qkv[j] = [jnp.concatenate([rs[i], rs[3 + i]], axis=0).astype(BF16) for i in range(3)]

        def do_s(j):
            sc[j] = softmax(scores(qkv[j][0], qkv[j][1]))

        def do_pv(j):
            o = _dot(sc[j], qkv[j][2])
            oh[2 * j] = wo_rows(2 * j, o[0:L]).astype(BF16)
            oh[2 * j + 1] = wo_rows(2 * j + 1, o[L:2 * L]).astype(BF16)

        def do_wo(n):
            h0, h1 = wsplit[n], wsplit[n + 1]
            if h1 == h0:
                return
            lo = jnp.concatenate(oh[h0:h1], axis=1)
            for cb in range(NCB):
                part = _dot(lo, col(wo, cb, h0 * E, h1 * E))
                acc[cb] = part if acc[cb] is None else part + acc[cb]
                fill(NP + n * NCB + cb)

        for j in range(NP + 2):
            if j < NP:
                do_qkv(j)
                fill(j)
            else:
                do_wo(j - NP)
            if 0 <= j - 1 < NP:
                do_s(j - 1)
            if 0 <= j - 2 < NP:
                do_pv(j - 2)
        do_wo(2)
        do_wo(3)
        return acc

    def body(t, carry):
        base = pl.multiple_of(t * HB, 16)
        R0 = pl.multiple_of(t * 64, 64)
        B0 = pl.multiple_of(PRE + t * BR, 16)
        B1 = pl.multiple_of(jnp.minimum(B0 + BR, S - BR), 16)

        nslot = NP + 4 * NCB + 1
        fa = dict(CFG.get("fa", [[17, 1], [21, 1], [26, 1], [30, 1], [34, 1], [38, 1], [48, 2]]))
        fb = dict(CFG.get("fb", [[j, 1 + (j % 3 == 0)] for j in range(16)] + [[48, 6]]))
        fa = [fa.get(n, 0) for n in range(nslot)]
        fb = [fb.get(n, 0) for n in range(nslot)]
        assert sum(fa) == NCB and sum(fb) == NFB
        wsa = CFG.get("wsa", [0, 8, 20, 28, 32])
        wsb = CFG.get("wsb", [0, 8, 20, 28, 32])

        def fill_a(n):
            if fa[n]:
                w4_part(B0, BR, range(sum(fa[:n]), sum(fa[:n + 1])))

        def fill_b(n):
            if fb[n]:
                w3_part(lhs3, range(sum(fb[:n]), sum(fb[:n + 1])), BR)

        lhs3 = jnp.concatenate(w3_lhs(x1buf, B1, BR), axis=0)

        keep = {}
        keep_o = {}

        def sel_a(j, i, v):
            keep[(j, i)] = v[L:L + 8]
            return v[0:L]

        def wo_a(h, o):
            keep_o[h] = o[32:40]
            return o[0:32]

        lhs_a = hbuf[pl.ds(base, 48), :]
        ra = attn_step(lhs_a, sel_a, wo_a, fill_a, wsa)
        for cb in range(NCB):
            hbuf[pl.ds(base + 48, 8), cb * 128:(cb + 1) * 128] = ra[cb][0:8].astype(BF16)
        fill_a(nslot - 1)

        def sel_b(j, i, v):
            return jnp.concatenate([v[0:8], keep[(j, i)], v[8:32]], axis=0)

        def wo_b(h, o):
            return jnp.concatenate([keep_o[h], o], axis=0)

        lhs_b = hbuf[pl.ds(base + 48, 32), :]
        rb = attn_step(lhs_b, sel_b, wo_b, fill_b, wsb)
        for cb in range(NCB):
            cs = slice(cb * 128, (cb + 1) * 128)
            hbuf[pl.ds(base + HB, 8), cs] = rb[cb][8:16].astype(BF16)
            s_ = jnp.concatenate([ra[cb][8:32], rb[cb][0:8], rb[cb][16:48]], axis=0)
            sl = (pl.ds(R0, 64), cs)
            xbuf[sl] = (xbuf[sl].astype(F32) + s_ * x1buf[sl].astype(F32)).astype(BF16)
        fill_b(nslot - 1)

        pltpu.make_async_copy(xbuf.at[pl.ds(R0, 64), :], out_hbm.at[pl.ds(R0, 64), :], osem).start()
        return carry

    nit = CFG.get("nit", NIT)
    with jax.named_scope("main"):
        un = CFG.get("unroll", 1)

        def body_u(t, carry):
            for u in range(un):
                body(t * un + u, carry)
            return carry

        lax.fori_loop(0, nit // un, body_u, 0)
    with jax.named_scope("wait_out"):
        pltpu.make_async_copy(xbuf.at[pl.ds(0, nit * 64), :], out_hbm.at[pl.ds(0, nit * 64), :], osem).wait()


@functools.partial(jax.jit, static_argnames=("A_seg_len",))
def pallas_recurrent_scan__memory_aug_recurrent_mem_tr__mixer_s_mlp__prompt_kernel(
    A_x: jax.Array,
    A_mem0: jax.Array,
    A_Wq: jax.Array,
    A_Wk: jax.Array,
    A_Wv: jax.Array,
    A_Wo: jax.Array,
    A_seg_len,
    B_x: jax.Array,
    B_w1: jax.Array,
    B_w2: jax.Array,
    B_w3: jax.Array,
    B_w4: jax.Array,
):
    assert A_seg_len == SEG
    assert A_x.shape == (1, S, D) and A_mem0.shape == (1, M, D)
    assert A_Wq.shape == (D, H, E) and A_Wo.shape == (H, E, D)
    assert B_w3.shape == (D, FF)
    del B_x

    cw1, cw2, cw3, cwo = CFG.get('cw1', 512), 512, 512, 512
    any_spec = pl.BlockSpec(memory_space=pl.ANY)
    out = pl.pallas_call(
        _kernel,
        out_shape=jax.ShapeDtypeStruct((S, D), BF16),
        in_specs=[any_spec] * 10,
        out_specs=any_spec,
        scratch_shapes=[
            pltpu.VMEM((S, D), BF16),
            pltpu.VMEM((NIT * HB + 16, D), BF16),
            pltpu.VMEM((NCB, S + 16, 128), F32),
            pltpu.VMEM((S, D), BF16),
            pltpu.VMEM((NFB, 128, 128), BF16),
            pltpu.VMEM((4, 3 * D * H // 4, E), BF16),
            pltpu.VMEM((3 * H * HS, 128), U32),
            pltpu.VMEM((D // cwo, H * E, cwo), BF16),
            pltpu.VMEM((D // cw1, D, cw1), BF16),
            pltpu.VMEM((D // cw2, D, cw2), BF16),
            pltpu.VMEM((FF // cw3, D, cw3), BF16),
            pltpu.VMEM((D // cw3, FF, cw3), BF16),
            pltpu.VMEM((HB, HB), F32),
            pltpu.SemaphoreType.DMA((16,)),
            pltpu.SemaphoreType.DMA(()),
        ],
        compiler_params=pltpu.CompilerParams(vmem_limit_bytes=120 * 1024 * 1024),
    )(
        A_x.reshape(S, D), A_mem0.reshape(M, D),
        A_Wq.reshape(D * H, E), A_Wk.reshape(D * H, E), A_Wv.reshape(D * H, E),
        A_Wo.reshape(H * E, D), B_w1, B_w2, B_w3, B_w4,
    )
    return out.reshape(1, S, D)
```

```python
import functools

import jax
import jax.numpy as jnp
from jax import lax
import jax.experimental.pallas as pl
import jax.experimental.pallas.tpu as pltpu

F32 = jnp.float32
BF16 = jnp.bfloat16
U32 = jnp.uint32

S = 2048
D = 1024
H = 32
E = 128
M = 8
SEG = 32
L = M + SEG
FF = 3584
NCB = D // 128
NFB = FF // 128
NIT = S // (2 * SEG)
HB = 2 * L
PRE = 512
LAG = 64
BR = (S - PRE) // NIT
HS = D // 2 + 8
EPS = 1e-5
SCALE = float(E) ** -0.5
RB = 256
CFG = {}


def _dot(a, b):
    return jnp.dot(a, b, preferred_element_type=F32)


def _ln(x):
    m = jnp.mean(x, axis=-1, keepdims=True)
    xc = x - m
    v = jnp.mean(xc * xc, axis=-1, keepdims=True)
    return xc * lax.rsqrt(v + EPS)


def _ln2(x):
    m = jnp.mean(x, axis=-1, keepdims=True)
    xc = x - m
    v = jnp.mean(xc * xc, axis=-1, keepdims=True)
    r1 = lax.rsqrt(v + EPS)
    r2 = lax.rsqrt(v * r1 * r1 + EPS)
    return xc * r1, xc * (r1 * r2)


def _gelu(x):
    c = 0.7978845608028654
    hx = 0.5 * x
    return hx * jnp.tanh(x * (c + (c * 0.044715) * (x * x))) + hx


def _silu(x):
    hx = 0.5 * x
    return hx * jnp.tanh(hx) + hx


def _kernel(x_hbm, mem0_hbm, wq_hbm, wk_hbm, wv_hbm, wo_hbm, w1_hbm, w2_hbm, w3_hbm, w4_hbm,
            out_hbm,
            xbuf, hbuf_all, hf, x1buf, h3buf, sbuf, stg, wqkv, wo, w1, w2, w3, w4, fillbuf,
            sem, osem):
    hbuf = hbuf_all.at[HB:, :]

    def colblock_copies(src, dst, s):
        n, _, cw = dst.shape
        return [pltpu.make_async_copy(src.at[:, pl.ds(c * cw, cw)], dst.at[c], sem.at[s(c)])
                for c in range(n)]

    def col(w, cb, k0=0, k1=None):
        _, kk, cw = w.shape
        q, r_ = divmod(cb * 128, cw)
        return w[q, k0:(kk if k1 is None else k1), r_:r_ + 128]

    SB = 128
    NXB = S // RB
    XS, QS = 7, 12
    xch = [(0, SB), (SB, SB), (RB, RB), (2 * RB, RB), (3 * RB, S - 3 * RB)]
    cp_x = [pltpu.make_async_copy(x_hbm.at[pl.ds(r, n), :], xbuf.at[pl.ds(r, n), :], sem.at[XS + i])
            for i, (r, n) in enumerate(xch)]
    cp_w1 = colblock_copies(w1_hbm, w1, lambda c: 2 * c // w1.shape[0])
    cp_w1a, cp_w1b = cp_w1[:len(cp_w1) // 2], cp_w1[len(cp_w1) // 2:]
    cp_mem = [pltpu.make_async_copy(mem0_hbm, hbuf.at[0:M, :], sem.at[2])]
    cp_w2 = colblock_copies(w2_hbm, w2, lambda c: 3)
    cp_w3 = colblock_copies(w3_hbm, w3, lambda c: 4)
    cp_w4 = colblock_copies(w4_hbm, w4, lambda c: 5)
    cp_wo = colblock_copies(wo_hbm, wo, lambda c: 6)
    CH = 512
    PR = 16 * CH
    cp_qkv = [pltpu.make_async_copy(src.at[pl.ds(k * PR, PR), :], stg.at[k, pl.ds(m_ * PR, PR), :],
                                    sem.at[QS + k])
              for k in range(4) for m_, src in enumerate((wq_hbm, wk_hbm, wv_hbm))]
    def start(*grps, priority=0):
        for grp in grps:
            for c in grp:
                c.start(priority=priority)

    mode = CFG.get("dma", 2)
    if mode == 0:
        start(cp_x[:1], cp_w1a, cp_x[1:2], cp_w1b, cp_x[2:3], cp_w2, cp_x[3:], cp_mem, cp_w3, cp_w4, cp_qkv, cp_wo)
    elif mode == 1:
        start(cp_x[:1], cp_w1a, cp_x[1:2], cp_w1b, cp_x[2:3])
        start(cp_w2, cp_x[3:], cp_mem, cp_w3, cp_w4, cp_qkv, cp_wo, priority=1)
    elif mode == 2:
        start(cp_x[:1], cp_w1a, cp_x[1:2], cp_w1b, cp_x[2:3])

    def wait(grp):
        for c in grp:
            c.wait()

    r = lax.broadcasted_iota(jnp.int32, (HB, HB), 0)
    c = lax.broadcasted_iota(jnp.int32, (HB, HB), 1)
    rr = jnp.where(r >= L, r - L, r)
    cc = jnp.where(c >= L, c - L, c)
    same = (r >= L) == (c >= L)
    allowed = (rr < M) | (rr >= cc)
    fillbuf[...] = jnp.where(same, jnp.where(allowed, 1.0, -1e9), -jnp.inf).astype(F32)

    hf[:, 0:8, :] = jnp.zeros((NCB, 8, 128), F32)
    hf[:, S + 8:S + 16, :] = jnp.zeros((NCB, 8, 128), F32)
    sbuf[...] = jnp.zeros(sbuf.shape, sbuf.dtype)

    HSB = (SB // 64) * HB

    def zero_of(trig):
        return (pltpu.bitcast(trig, U32) >> 16) >> 16

    def hrow(r):
        q, rr_ = divmod(r, 64)
        return q * HB + rr_ + (8 if rr_ < 40 else 16)

    def ln_sub(xv, hv, sb):
        out = []
        for u in range(SB // 16):
            r = sb * SB + 16 * u
            xn, xnn = _ln2(xv[r:r + 16, :].astype(F32))
            xn = xn.astype(BF16)
            for hh in range(2):
                o = hrow(r + 8 * hh)
                hv[o:o + 8, :] = xn[8 * hh:8 * hh + 8]
            out.append(xnn.astype(BF16))
        return out

    def after(w, vals):
        if not vals:
            return w
        z = None
        for v in vals:
            zv = zero_of(v[0:16, D - 128:D])
            z = zv if z is None else z | zv
        head = pltpu.bitcast(pltpu.bitcast(w[0:16, :], U32) | z, BF16)
        return jnp.concatenate([head, w[16:, :]], axis=0)

    def w1_sub(xnn, hfv, sb, cbs=range(NCB), deps={}):
        xnn = jnp.concatenate(xnn, axis=0)
        for cb in cbs:
            w = after(col(w1, cb), deps.get(cb, []))
            hfv[cb, sb * SB + 8:sb * SB + 8 + SB, :] = _gelu(_dot(xnn, w))

    shifts = (7, 7, 9, 9, 6, 6, 10, 10)

    def w2_lhs(hfv, sb):
        r0 = sb * SB
        return jnp.concatenate(
            [hfv[cb, r0 + shifts[cb]:r0 + shifts[cb] + SB, :] for cb in range(NCB)],
            axis=1).astype(BF16)

    def w2_sub(hs, hv, x1v, sb, cbs=range(NCB), hook=None, deps={}):
        r0 = sb * SB
        for cb in cbs:
            pre = _dot(hs, after(col(w2, cb), deps.get(cb, [])))
            cs = slice(cb * 128, (cb + 1) * 128)
            xn = jnp.concatenate(
                [hv[hrow(r0 + a_):hrow(r0 + a_) + n_, cs].astype(F32)
                 for a_, n_ in ((0, 40), (40, 24), (64, 40), (104, 24))], axis=0)
            x1v[r0:r0 + SB, cs] = (xn + pre).astype(BF16)
            if hook is not None:
                hook(cb, pre)

    def w3_lhs(src, r0, rows):
        return [_ln(src[pl.ds(r0 + 16 * u, 16), :].astype(F32)).astype(BF16)
                for u in range(rows // 16)]

    def w3_part(lhs, h3v, r0, rows, blocks):
        for f in blocks:
            pre = _dot(lhs, col(w3, f))
            h3v[r0:r0 + rows, f * 128:(f + 1) * 128] = _gelu(pre).astype(BF16)
        return pre

    def w4_lhs(h3v, rows):
        return h3v[0:rows, :]

    def w4_part(lhs, x1v, rows, blocks):
        for cb in blocks:
            pre = _dot(lhs, col(w4, cb))
            cs = slice(cb * 128, (cb + 1) * 128)
            x1v[0:rows, cs] = _silu(x1v[0:rows, cs].astype(F32) + pre).astype(BF16)

    def relayout(src, dst, u, trig):
        m_, c_ = divmod(u, 16)
        d0 = m_ * (H * HS) + c_ * 8
        for pp in range(8):
            r0 = u * CH + pp * 64
            tr = (pp * trig.shape[0] // 64) * 8
            t = trig[tr:tr + 8, :]
            z = zero_of(t)
            two = lambda v: jnp.concatenate([v, v], axis=0)
            mlo, mhi, sh = two(z | U32(0xFFFF)), two(z | U32(0xFFFF0000)), two(z | U32(16))
            a = pltpu.bitcast(src[r0:r0 + 32, :], U32)
            b = pltpu.bitcast(src[r0 + 32:r0 + 64, :], U32)
            lo = (a & mlo) | (b << sh)
            hi = (a >> sh) | (b & mhi)
            dst[pl.ds(d0 + pp, 16, stride=HS), :] = lo
            dst[pl.ds(d0 + 16 * HS + pp, 16, stride=HS), :] = hi

    spread4 = lambda c, o: {o + 2: c[0:3], o + 3: c[3:6]}
    spread8 = lambda c: {2: c[0:1], 3: c[1:2], 4: c[2:4], 5: c[4:5], 6: c[5:7], 7: c[7:8]}
    with jax.named_scope("wx0"):
        cp_x[0].wait()
    with jax.named_scope("ln0"):
        xnn0 = ln_sub(xbuf, hbuf, 0)
    with jax.named_scope("ww1a"):
        wait(cp_w1a)
    with jax.named_scope("wx1"):
        cp_x[1].wait()
        if mode == 2:
            start(cp_w2, cp_x[3:], cp_mem, cp_w3, cp_w4, cp_qkv, cp_wo)
    with jax.named_scope("a00"):
        xnn1 = ln_sub(xbuf, hbuf, 1)
        w1_sub(xnn0, hf, 0, range(0, 4), spread4(xnn1, 0))
        w1_sub(xnn1, hf, 1, range(0, 4))
    with jax.named_scope("ww1b"):
        wait(cp_w1b)
    with jax.named_scope("a01"):
        w1_sub(xnn0, hf, 0, range(4, 8))
    with jax.named_scope("wx2"):
        cp_x[2].wait()
    with jax.named_scope("a1"):
        xnn2 = ln_sub(xbuf, hbuf, 2)
        xnn3 = ln_sub(xbuf, hbuf, 3)
        w1_sub(xnn1, hf, 1, range(4, 8), spread4(xnn2, 4))
        w1_sub(xnn2, hf, 2, deps=spread8(xnn3))
        w1_sub(xnn3, hf, 3)
    with jax.named_scope("wait_w2"):
        wait(cp_w2)
        cp_x[3].wait()

    def loop_a2(i, carry):
        @pl.when(i == 3)
        def _():
            cp_x[4].wait()

        r0 = pl.multiple_of((i - 2) * RB, RB)
        xv = xbuf.at[pl.ds(r0, 3 * RB), :]
        hv = hbuf.at[pl.ds(pl.multiple_of((i - 2) * 2 * HSB, 16), 6 * HSB), :]
        x1v = x1buf.at[pl.ds(r0, RB), :]
        hfv = hf.at[:, pl.ds(r0, 3 * RB + 16), :]
        for sb in range(2):
            xnn = ln_sub(xv, hv, 4 + sb)
            w2_sub(w2_lhs(hfv, sb), hv, x1v, sb, deps=spread8(xnn))
            w1_sub(xnn, hfv, 4 + sb)
        return carry

    with jax.named_scope("a2"):
        lax.fori_loop(2, NXB, loop_a2, 0)
    with jax.named_scope("wait_w34"):
        wait(cp_w3)
        wait(cp_w4)

    def loop_s3(k, carry):
        pltpu.make_async_copy(stg.at[k], stg.at[k], sem.at[QS + k]).wait()
        r0 = pl.multiple_of(k * SB, SB)
        src = stg.at[k]
        dst = wqkv.at[pl.ds(pl.multiple_of(k * 128, 128), 3 * H * HS - 384), :]
        sb2 = (S - PRE) // SB
        x1v = x1buf.at[pl.ds(r0, (sb2 + 1) * SB), :]
        hv = hbuf.at[pl.ds(pl.multiple_of(k * HSB, 16), (sb2 + 1) * HSB), :]
        hfv = hf.at[:, pl.ds(r0, (sb2 + 1) * SB + 16), :]
        hook = lambda cb, pre: relayout(src, dst, cb, pre) if cb < 6 else None
        hs = w2_lhs(hfv, sb2)
        lhs = w3_lhs(x1v, 0, SB)
        w2_sub(hs, hv, x1v, sb2, range(0, 6), hook, {2: lhs[0:1], 3: lhs[1:3], 4: lhs[3:5], 5: lhs[5:7]})
        lhs = jnp.concatenate(lhs, axis=0)
        h3v = h3buf.at[pl.ds(r0, SB), :]
        for f in range(NFB):
            pre = w3_part(lhs, h3v, 0, SB, [f])
            relayout(src, dst, 6 + f, pre)
        w2_sub(hs, hv, x1v, sb2, range(6, 8), hook)
        R4 = (PRE - LAG) // 4
        r4 = pl.multiple_of(k * R4, 16)
        lhs4 = w4_lhs(h3buf.at[pl.ds(r4, R4), :], R4)
        x4v = x1buf.at[pl.ds(r4, R4), :]
        for cb in range(NCB):
            hk = 12 * 128
            p0 = _dot(lhs4[:, :hk], col(w4, cb, 0, hk))
            pre = _dot(lhs4[:, hk:], col(w4, cb, hk, FF)) + p0
            if cb < 7:
                relayout(src, dst, NFB + 6 + 2 * cb, p0)
                relayout(src, dst, NFB + 7 + 2 * cb, pre)
            cs = slice(cb * 128, (cb + 1) * 128)
            x4v[:, cs] = _silu(x4v[:, cs].astype(F32) + pre).astype(BF16)
        return carry

    with jax.named_scope("s3"):
        lax.fori_loop(0, PRE // SB, loop_s3, 0)
    with jax.named_scope("wait_wo"):
        wait(cp_wo)
        wait(cp_mem)

    def qkv_pair(lhs, j):
        def blk(m_, h):
            r0 = (m_ * H + (h % 2) * 16 + h // 2) * HS
            return pltpu.bitcast(wqkv[r0:r0 + D // 2, :], BF16)
        return [_dot(lhs, blk(i % 3, 2 * j + i // 3)) for i in range(6)]

    def scores(q, k):
        return lax.dot_general(q, k, (((1,), (1,)), ((), ())), preferred_element_type=F32)

    def softmax(s):
        fill = fillbuf[...]
        s = jnp.where(fill > 0.0, s * SCALE, fill)
        mx = jnp.max(s, axis=1, keepdims=True)
        e = jnp.exp(s - mx)
        l = jnp.sum(e, axis=1, keepdims=True)
        rc = pl.reciprocal(l, approx=True)
        rc = rc * (2.0 - l * rc)
        return (e * rc).astype(BF16)

    NP = H // 2

    def attn_step(lhs, select, wo_rows, fill, wsplit):
        qkv = [None] * NP
        sc = [None] * NP
        oh = [None] * H
        acc = [None] * NCB

        def do_qkv(j):
            rs = qkv_pair(lhs, j)
            rs = [select(j, i, v) for i, v in enumerate(rs)]
            qkv[j] = [jnp.concatenate([rs[i], rs[3 + i]], axis=0).astype(BF16) for i in range(3)]

        def do_s(j):
            sc[j] = softmax(scores(qkv[j][0], qkv[j][1]))

        def do_pv(j):
            o = _dot(sc[j], qkv[j][2])
            oh[2 * j] = wo_rows(2 * j, o[0:L]).astype(BF16)
            oh[2 * j + 1] = wo_rows(2 * j + 1, o[L:2 * L]).astype(BF16)

        def do_wo(n):
            h0, h1 = wsplit[n], wsplit[n + 1]
            if h1 == h0:
                return
            lo = jnp.concatenate(oh[h0:h1], axis=1)
            for cb in range(NCB):
                part = _dot(lo, col(wo, cb, h0 * E, h1 * E))
                acc[cb] = part if acc[cb] is None else part + acc[cb]
                fill(NP + n * NCB + cb)

        for j in range(NP + 2):
            if j < NP:
                do_qkv(j)
                fill(j)
            else:
                do_wo(j - NP)
            if 0 <= j - 1 < NP:
                do_s(j - 1)
            if 0 <= j - 2 < NP:
                do_pv(j - 2)
        do_wo(2)
        do_wo(3)
        return acc

    def combine(r0, dst, cbs):
        for cb in cbs:
            cs = slice(cb * 128, (cb + 1) * 128)
            sl = (pl.ds(r0, 64), cs)
            dst[0:64, cs] = (xbuf[sl].astype(F32) + sbuf[cb] * x1buf[sl].astype(F32)).astype(BF16)

    def out_copy(t):
        return pltpu.make_async_copy(hbuf.at[pl.ds(pl.multiple_of(t * HB, 16), 64), :],
                                     out_hbm.at[pl.ds(pl.multiple_of(t * 64, 64), 64), :], osem)

    def body(t, carry):
        hv = hbuf_all.at[pl.ds(pl.multiple_of(t * HB, 16), 2 * HB + 16), :]
        Rp = pl.multiple_of(jnp.maximum(t - 1, 0) * 64, 64)
        B4 = pl.multiple_of(PRE - LAG + t * BR, 16)
        x1v = x1buf.at[pl.ds(B4, LAG + BR), :]
        h3v = h3buf.at[pl.ds(B4, LAG + BR), :]

        nslot = NP + 4 * NCB + 1
        fa = dict(CFG.get("fa", [[17, 1], [21, 1], [26, 1], [30, 1], [34, 1], [38, 1], [48, 2]]))
        fb = dict(CFG.get("fb", [[j, 1 + (j % 3 == 0)] for j in range(16)] + [[48, 6]]))
        fa = [fa.get(n, 0) for n in range(nslot)]
        fb = [fb.get(n, 0) for n in range(nslot)]
        assert sum(fa) == NCB and sum(fb) == NFB
        wsa = CFG.get("wsa", [0, 8, 20, 28, 32])
        wsb = CFG.get("wsb", [0, 8, 20, 28, 32])

        def fill_a(n):
            if fa[n]:
                w4_part(lhs4, x1v, BR, range(sum(fa[:n]), sum(fa[:n + 1])))

        def fill_b(n):
            if fb[n]:
                w3_part(lhs3, h3v, LAG, BR, range(sum(fb[:n]), sum(fb[:n + 1])))
            if n < NCB:
                combine(Rp, hv, [n])

        lhs3 = jnp.concatenate(w3_lhs(x1v, LAG, BR), axis=0)
        lhs4 = w4_lhs(h3v, BR)

        keep = {}
        keep_o = {}

        def sel_a(j, i, v):
            keep[(j, i)] = v[L:L + 8]
            return v[0:L]

        def wo_a(h, o):
            keep_o[h] = o[32:40]
            return o[0:32]

        lhs_a = hv[HB:HB + 48, :]
        ra = attn_step(lhs_a, sel_a, wo_a, fill_a, wsa)
        for cb in range(NCB):
            hv[HB + 48:HB + 56, cb * 128:(cb + 1) * 128] = ra[cb][0:8].astype(BF16)
        fill_a(nslot - 1)

        def sel_b(j, i, v):
            return jnp.concatenate([v[0:8], keep[(j, i)], v[8:32]], axis=0)

        def wo_b(h, o):
            return jnp.concatenate([keep_o[h], o], axis=0)

        lhs_b = hv[HB + 48:2 * HB, :]
        rb = attn_step(lhs_b, sel_b, wo_b, fill_b, wsb)
        for cb in range(NCB):
            cs = slice(cb * 128, (cb + 1) * 128)
            hv[2 * HB:2 * HB + 8, cs] = rb[cb][8:16].astype(BF16)
            sbuf[cb] = jnp.concatenate([ra[cb][8:32], rb[cb][0:8], rb[cb][16:48]], axis=0)
        fill_b(nslot - 1)

        if CFG.get("outdma", 1) == 1:
            @pl.when(t > 0)
            def _():
                out_copy(t - 1).start()

        return carry

    nit = CFG.get("nit", NIT)
    with jax.named_scope("main"):
        lax.fori_loop(0, nit, body, 0)
    with jax.named_scope("epilogue"):
        last = hbuf.at[(nit - 1) * HB:nit * HB, :]
        lhs4 = w4_lhs(h3buf.at[S - LAG:S, :], LAG)
        for cb in range(NCB):
            w4_part(lhs4, x1buf.at[S - LAG:S, :], LAG, [cb])
            combine((nit - 1) * 64, last, [cb])
        out_copy(nit - 1).start()
        if CFG.get("outdma", 1) == 0:
            for t in range(nit - 1):
                out_copy(t).start()
    with jax.named_scope("wait_out"):
        pltpu.make_async_copy(xbuf.at[pl.ds(0, nit * 64), :], out_hbm.at[pl.ds(0, nit * 64), :], osem).wait()


@functools.partial(jax.jit, static_argnames=("A_seg_len",))
def pallas_recurrent_scan__memory_aug_recurrent_mem_tr__mixer_s_mlp__prompt_kernel(
    A_x: jax.Array,
    A_mem0: jax.Array,
    A_Wq: jax.Array,
    A_Wk: jax.Array,
    A_Wv: jax.Array,
    A_Wo: jax.Array,
    A_seg_len,
    B_x: jax.Array,
    B_w1: jax.Array,
    B_w2: jax.Array,
    B_w3: jax.Array,
    B_w4: jax.Array,
):
    assert A_seg_len == SEG
    assert A_x.shape == (1, S, D) and A_mem0.shape == (1, M, D)
    assert A_Wq.shape == (D, H, E) and A_Wo.shape == (H, E, D)
    assert B_w3.shape == (D, FF)
    del B_x

    cw1, cw2, cw3, cwo = CFG.get('cw1', 512), 512, 512, 512
    any_spec = pl.BlockSpec(memory_space=pl.ANY)
    out = pl.pallas_call(
        _kernel,
        out_shape=jax.ShapeDtypeStruct((S, D), BF16),
        in_specs=[any_spec] * 10,
        out_specs=any_spec,
        scratch_shapes=[
            pltpu.VMEM((S, D), BF16),
            pltpu.VMEM(((NIT + 1) * HB + 16, D), BF16),
            pltpu.VMEM((NCB, S + 16, 128), F32),
            pltpu.VMEM((S, D), BF16),
            pltpu.VMEM((S, FF), BF16),
            pltpu.VMEM((NCB, 64, 128), F32),
            pltpu.VMEM((4, 3 * D * H // 4, E), BF16),
            pltpu.VMEM((3 * H * HS, 128), U32),
            pltpu.VMEM((D // cwo, H * E, cwo), BF16),
            pltpu.VMEM((D // cw1, D, cw1), BF16),
            pltpu.VMEM((D // cw2, D, cw2), BF16),
            pltpu.VMEM((FF // cw3, D, cw3), BF16),
            pltpu.VMEM((D // cw3, FF, cw3), BF16),
            pltpu.VMEM((HB, HB), F32),
            pltpu.SemaphoreType.DMA((16,)),
            pltpu.SemaphoreType.DMA(()),
        ],
        compiler_params=pltpu.CompilerParams(vmem_limit_bytes=120 * 1024 * 1024,
                                             disable_bounds_checks=True),
    )(
        A_x.reshape(S, D), A_mem0.reshape(M, D),
        A_Wq.reshape(D * H, E), A_Wk.reshape(D * H, E), A_Wv.reshape(D * H, E),
        A_Wo.reshape(H * E, D), B_w1, B_w2, B_w3, B_w4,
    )
    return out.reshape(1, S, D)
```

```python
import functools

import jax
import jax.numpy as jnp
from jax import lax
import jax.experimental.pallas as pl
import jax.experimental.pallas.tpu as pltpu

F32 = jnp.float32
BF16 = jnp.bfloat16
U32 = jnp.uint32

S = 2048
D = 1024
H = 32
E = 128
M = 8
SEG = 32
L = M + SEG
FF = 3584
NCB = D // 128
NFB = FF // 128
NIT = S // (2 * SEG)
HB = 2 * L
PRE = 512
LAG = 64
BR = (S - PRE) // NIT
HS = D // 2 + 8
EPS = 1e-5
SCALE = float(E) ** -0.5
RB = 256
CFG = {}


def _dot(a, b):
    return jnp.dot(a, b, preferred_element_type=F32)


def _ln(x):
    m = jnp.mean(x, axis=-1, keepdims=True)
    xc = x - m
    v = jnp.mean(xc * xc, axis=-1, keepdims=True)
    return xc * lax.rsqrt(v + EPS)


def _ln2(x):
    m = jnp.mean(x, axis=-1, keepdims=True)
    xc = x - m
    v = jnp.mean(xc * xc, axis=-1, keepdims=True)
    r1 = lax.rsqrt(v + EPS)
    r2 = lax.rsqrt(v * r1 * r1 + EPS)
    return xc * r1, xc * (r1 * r2)


def _gelu(x):
    c = 0.7978845608028654
    hx = 0.5 * x
    return hx * jnp.tanh(x * (c + (c * 0.044715) * (x * x))) + hx


def _silu(x):
    hx = 0.5 * x
    return hx * jnp.tanh(hx) + hx


def _kernel(x_hbm, mem0_hbm, wq_hbm, wk_hbm, wv_hbm, wo_hbm, w1_hbm, w2_hbm, w3_hbm, w4_hbm,
            out_hbm,
            xbuf, hbuf_all, hf, x1buf, h3buf, sbuf, stg, wqkv, wo, w1, w2, w3, w4, fillbuf,
            sem, osem):
    hbuf = hbuf_all.at[HB:, :]

    def colblock_copies(src, dst, s):
        n, _, cw = dst.shape
        return [pltpu.make_async_copy(src.at[:, pl.ds(c * cw, cw)], dst.at[c], sem.at[s(c)])
                for c in range(n)]

    def col(w, cb, k0=0, k1=None):
        _, kk, cw = w.shape
        q, r_ = divmod(cb * 128, cw)
        return w[q, k0:(kk if k1 is None else k1), r_:r_ + 128]

    SB = 128
    NXB = S // RB
    XS, QS = 7, 12
    xch = [(0, SB), (SB, SB), (RB, RB), (2 * RB, RB), (3 * RB, S - 3 * RB)]
    cp_x = [pltpu.make_async_copy(x_hbm.at[pl.ds(r, n), :], xbuf.at[pl.ds(r, n), :], sem.at[XS + i])
            for i, (r, n) in enumerate(xch)]
    cp_w1 = colblock_copies(w1_hbm, w1, lambda c: (0, 1, 16, 16)[c])
    cp_mem = [pltpu.make_async_copy(mem0_hbm, hbuf.at[0:M, :], sem.at[2])]
    cp_w2 = colblock_copies(w2_hbm, w2, lambda c: 3)
    cp_w3 = colblock_copies(w3_hbm, w3, lambda c: 4)
    cp_w4 = colblock_copies(w4_hbm, w4, lambda c: 5)
    cp_wo = colblock_copies(wo_hbm, wo, lambda c: 6)
    CH = 512
    PR = 16 * CH
    cp_qkv = [pltpu.make_async_copy(src.at[pl.ds(k * PR, PR), :], stg.at[k, pl.ds(m_ * PR, PR), :],
                                    sem.at[QS + k])
              for k in range(4) for m_, src in enumerate((wq_hbm, wk_hbm, wv_hbm))]
    def start(*grps, priority=0):
        for grp in grps:
            for c in grp:
                c.start(priority=priority)

    mode = CFG.get("dma", 1)
    start(cp_x[:2], cp_w1[:2], cp_x[2:3], cp_w1[2:])
    if mode == 1:
        start(cp_w2, cp_x[3:4])
        start(cp_x[4:], cp_mem, cp_w3, cp_w4, cp_qkv, cp_wo, priority=1)

    def wait(grp):
        for c in grp:
            c.wait()

    r = lax.broadcasted_iota(jnp.int32, (HB, HB), 0)
    c = lax.broadcasted_iota(jnp.int32, (HB, HB), 1)
    rr = jnp.where(r >= L, r - L, r)
    cc = jnp.where(c >= L, c - L, c)
    same = (r >= L) == (c >= L)
    allowed = (rr < M) | (rr >= cc)
    fillbuf[...] = jnp.where(same, jnp.where(allowed, 1.0, -1e9), -jnp.inf).astype(F32)

    hf[:, 0:8, :] = jnp.zeros((NCB, 8, 128), F32)
    hf[:, S + 8:S + 16, :] = jnp.zeros((NCB, 8, 128), F32)
    sbuf[...] = jnp.zeros(sbuf.shape, sbuf.dtype)

    HSB = (SB // 64) * HB

    def zero_of(trig):
        return (pltpu.bitcast(trig, U32) >> 16) >> 16

    def hrow(r):
        q, rr_ = divmod(r, 64)
        return q * HB + rr_ + (8 if rr_ < 40 else 16)

    def ln_sub(xv, hv, sb):
        out = []
        for u in range(SB // 16):
            r = sb * SB + 16 * u
            xn, xnn = _ln2(xv[r:r + 16, :].astype(F32))
            xn = xn.astype(BF16)
            for hh in range(2):
                o = hrow(r + 8 * hh)
                hv[o:o + 8, :] = xn[8 * hh:8 * hh + 8]
            out.append(xnn.astype(BF16))
        return out

    def after(w, vals):
        if not vals:
            return w
        z = None
        for v in vals:
            zv = zero_of(v[0:16, D - 128:D])
            z = zv if z is None else z | zv
        head = pltpu.bitcast(pltpu.bitcast(w[0:16, :], U32) | z, BF16)
        return jnp.concatenate([head, w[16:, :]], axis=0)

    def w1_sub(xnn, hfv, sb, cbs=range(NCB), deps={}):
        xnn = jnp.concatenate(xnn, axis=0)
        for cb in cbs:
            w = after(col(w1, cb), deps.get(cb, []))
            hfv[cb, sb * SB + 8:sb * SB + 8 + SB, :] = _gelu(_dot(xnn, w))

    shifts = (7, 7, 9, 9, 6, 6, 10, 10)

    def w2_lhs(hfv, sb):
        r0 = sb * SB
        return jnp.concatenate(
            [hfv[cb, r0 + shifts[cb]:r0 + shifts[cb] + SB, :] for cb in range(NCB)],
            axis=1).astype(BF16)

    def w2_sub(hs, hv, x1v, sb, cbs=range(NCB), hook=None, deps={}):
        r0 = sb * SB
        for cb in cbs:
            pre = _dot(hs, after(col(w2, cb), deps.get(cb, [])))
            cs = slice(cb * 128, (cb + 1) * 128)
            xn = jnp.concatenate(
                [hv[hrow(r0 + a_):hrow(r0 + a_) + n_, cs].astype(F32)
                 for a_, n_ in ((0, 40), (40, 24), (64, 40), (104, 24))], axis=0)
            x1v[r0:r0 + SB, cs] = (xn + pre).astype(BF16)
            if hook is not None:
                hook(cb, pre)

    def w3_lhs(src, r0, rows):
        return [_ln(src[pl.ds(r0 + 16 * u, 16), :].astype(F32)).astype(BF16)
                for u in range(rows // 16)]

    def w3_part(lhs, h3v, r0, rows, blocks):
        for f in blocks:
            pre = _dot(lhs, col(w3, f))
            h3v[r0:r0 + rows, f * 128:(f + 1) * 128] = _gelu(pre).astype(BF16)
        return pre

    def w4_lhs(h3v, rows):
        return h3v[0:rows, :]

    def w4_part(lhs, x1v, rows, blocks):
        for cb in blocks:
            pre = _dot(lhs, col(w4, cb))
            cs = slice(cb * 128, (cb + 1) * 128)
            x1v[0:rows, cs] = _silu(x1v[0:rows, cs].astype(F32) + pre).astype(BF16)

    def relayout(src, dst, u, trig):
        m_, c_ = divmod(u, 16)
        d0 = m_ * (H * HS) + c_ * 8
        for pp in range(8):
            r0 = u * CH + pp * 64
            tr = (pp * trig.shape[0] // 64) * 8
            t = trig[tr:tr + 8, :]
            z = zero_of(t)
            two = lambda v: jnp.concatenate([v, v], axis=0)
            mlo, mhi, sh = two(z | U32(0xFFFF)), two(z | U32(0xFFFF0000)), two(z | U32(16))
            a = pltpu.bitcast(src[r0:r0 + 32, :], U32)
            b = pltpu.bitcast(src[r0 + 32:r0 + 64, :], U32)
            lo = (a & mlo) | (b << sh)
            hi = (a >> sh) | (b & mhi)
            dst[pl.ds(d0 + pp, 16, stride=HS), :] = lo
            dst[pl.ds(d0 + 16 * HS + pp, 16, stride=HS), :] = hi

    spread8 = lambda c: {2: c[0:1], 3: c[1:2], 4: c[2:4], 5: c[4:5], 6: c[5:7], 7: c[7:8]}
    with jax.named_scope("ln01"):
        cp_x[0].wait()
        xnn0 = ln_sub(xbuf, hbuf, 0)
        cp_x[1].wait()
        xnn1 = ln_sub(xbuf, hbuf, 1)
    with jax.named_scope("wp0"):
        cp_w1[0].wait()
        if mode == 2:
            start(cp_w2, cp_x[3:4])
            start(cp_x[4:], cp_mem, cp_w3, cp_w4, cp_qkv, cp_wo, priority=1)
        if mode == 3:
            start(cp_w2, cp_x[3:4])
    with jax.named_scope("a00"):
        w1_sub(xnn0, hf, 0, range(0, 2))
        w1_sub(xnn1, hf, 1, range(0, 2))
    with jax.named_scope("wp1"):
        cp_w1[1].wait()
    with jax.named_scope("a01"):
        w1_sub(xnn0, hf, 0, range(2, 4))
    with jax.named_scope("wx2"):
        cp_x[2].wait()
    with jax.named_scope("a02"):
        xnn2 = ln_sub(xbuf, hbuf, 2)
        xnn3 = ln_sub(xbuf, hbuf, 3)
        w1_sub(xnn1, hf, 1, range(2, 4))
        w1_sub(xnn2, hf, 2, range(0, 4), {1: xnn3[0:2], 2: xnn3[2:4], 3: xnn3[4:6]})
        w1_sub(xnn3, hf, 3, range(0, 4))
    with jax.named_scope("wp23"):
        wait(cp_w1[2:])
        if mode == 3:
            start(cp_x[4:], cp_mem, cp_w3, cp_w4, cp_qkv, cp_wo, priority=1)
    with jax.named_scope("a1"):
        for sb, xnn in enumerate((xnn0, xnn1, xnn2, xnn3)):
            w1_sub(xnn, hf, sb, range(4, 8))
    with jax.named_scope("wait_w2"):
        wait(cp_w2)
        cp_x[3].wait()

    def loop_a2(i, carry):
        @pl.when(i == 3)
        def _():
            cp_x[4].wait()

        r0 = pl.multiple_of((i - 2) * RB, RB)
        xv = xbuf.at[pl.ds(r0, 3 * RB), :]
        hv = hbuf.at[pl.ds(pl.multiple_of((i - 2) * 2 * HSB, 16), 6 * HSB), :]
        x1v = x1buf.at[pl.ds(r0, RB), :]
        hfv = hf.at[:, pl.ds(r0, 3 * RB + 16), :]
        for sb in range(2):
            xnn = ln_sub(xv, hv, 4 + sb)
            w2_sub(w2_lhs(hfv, sb), hv, x1v, sb, deps=spread8(xnn))
            w1_sub(xnn, hfv, 4 + sb)
        return carry

    with jax.named_scope("a2"):
        lax.fori_loop(2, NXB, loop_a2, 0)
    with jax.named_scope("wait_w34"):
        wait(cp_w3)
        wait(cp_w4)

    def loop_s3(k, carry):
        pltpu.make_async_copy(stg.at[k], stg.at[k], sem.at[QS + k]).wait()
        r0 = pl.multiple_of(k * SB, SB)
        src = stg.at[k]
        dst = wqkv.at[pl.ds(pl.multiple_of(k * 128, 128), 3 * H * HS - 384), :]
        sb2 = (S - PRE) // SB
        x1v = x1buf.at[pl.ds(r0, (sb2 + 1) * SB), :]
        hv = hbuf.at[pl.ds(pl.multiple_of(k * HSB, 16), (sb2 + 1) * HSB), :]
        hfv = hf.at[:, pl.ds(r0, (sb2 + 1) * SB + 16), :]
        hook = lambda cb, pre: relayout(src, dst, cb, pre) if cb < 6 else None
        hs = w2_lhs(hfv, sb2)
        lhs = w3_lhs(x1v, 0, SB)
        w2_sub(hs, hv, x1v, sb2, range(0, 6), hook, {2: lhs[0:1], 3: lhs[1:3], 4: lhs[3:5], 5: lhs[5:7]})
        lhs = jnp.concatenate(lhs, axis=0)
        h3v = h3buf.at[pl.ds(r0, SB), :]
        for f in range(NFB):
            pre = w3_part(lhs, h3v, 0, SB, [f])
            relayout(src, dst, 6 + f, pre)
        w2_sub(hs, hv, x1v, sb2, range(6, 8), hook)
        R4 = (PRE - LAG) // 4
        r4 = pl.multiple_of(k * R4, 16)
        lhs4 = w4_lhs(h3buf.at[pl.ds(r4, R4), :], R4)
        x4v = x1buf.at[pl.ds(r4, R4), :]
        for cb in range(NCB):
            hk = 12 * 128
            p0 = _dot(lhs4[:, :hk], col(w4, cb, 0, hk))
            pre = _dot(lhs4[:, hk:], col(w4, cb, hk, FF)) + p0
            if cb < 7:
                relayout(src, dst, NFB + 6 + 2 * cb, p0)
                relayout(src, dst, NFB + 7 + 2 * cb, pre)
            cs = slice(cb * 128, (cb + 1) * 128)
            x4v[:, cs] = _silu(x4v[:, cs].astype(F32) + pre).astype(BF16)
        return carry

    with jax.named_scope("s3"):
        lax.fori_loop(0, PRE // SB, loop_s3, 0)
    with jax.named_scope("wait_wo"):
        wait(cp_wo)
        wait(cp_mem)

    def qkv_pair(lhs, j, fill):
        def blk(m_, h):
            r0 = (m_ * H + (h % 2) * 16 + h // 2) * HS
            return pltpu.bitcast(wqkv[r0:r0 + D // 2, :], BF16)
        out = []
        for i in range(6):
            out.append(_dot(lhs, blk(i % 3, 2 * j + i // 3)))
            fill(100 + 6 * j + i, out[-1])
        return out

    def scores(q, k):
        return lax.dot_general(q, k, (((1,), (1,)), ((), ())), preferred_element_type=F32)

    def softmax(s):
        fill = fillbuf[...]
        s = jnp.where(fill > 0.0, s * SCALE, fill)
        mx = jnp.max(s, axis=1, keepdims=True)
        e = jnp.exp(s - mx)
        l = jnp.sum(e, axis=1, keepdims=True)
        rc = pl.reciprocal(l, approx=True)
        rc = rc * (2.0 - l * rc)
        return (e * rc).astype(BF16)

    NP = H // 2

    def attn_step(lhs, select, wo_rows, fill, wsplit):
        qkv = [None] * NP
        sc = [None] * NP
        oh = [None] * H
        acc = [None] * NCB

        def do_qkv(j):
            rs = qkv_pair(lhs, j, fill)
            rs = [select(j, i, v) for i, v in enumerate(rs)]
            qkv[j] = [jnp.concatenate([rs[i], rs[3 + i]], axis=0).astype(BF16) for i in range(3)]

        def do_s(j):
            sc[j] = softmax(scores(qkv[j][0], qkv[j][1]))

        def do_pv(j):
            o = _dot(sc[j], qkv[j][2])
            oh[2 * j] = wo_rows(2 * j, o[0:L]).astype(BF16)
            oh[2 * j + 1] = wo_rows(2 * j + 1, o[L:2 * L]).astype(BF16)

        def do_wo(n):
            h0, h1 = wsplit[n], wsplit[n + 1]
            if h1 == h0:
                return
            lo = jnp.concatenate(oh[h0:h1], axis=1)
            for cb in range(NCB):
                part = _dot(lo, col(wo, cb, h0 * E, h1 * E))
                acc[cb] = part if acc[cb] is None else part + acc[cb]
                fill(NP + n * NCB + cb, part)

        for j in range(NP + 2):
            if j < NP:
                do_qkv(j)
                fill(j)
            else:
                do_wo(j - NP)
            if 0 <= j - 1 < NP:
                do_s(j - 1)
            if 0 <= j - 2 < NP:
                do_pv(j - 2)
        do_wo(2)
        do_wo(3)
        return acc

    def combine(r0, dst, cbs, trig=None):
        for cb in cbs:
            cs = slice(cb * 128, (cb + 1) * 128)
            sl = (pl.ds(r0, 64), cs)
            xx, gg = xbuf[sl], x1buf[sl]
            if trig is not None:
                z = jnp.concatenate([zero_of(trig[0:8, :])] * 4, axis=0)
                xx = pltpu.bitcast(pltpu.bitcast(xx, U32) | z, BF16)
                gg = pltpu.bitcast(pltpu.bitcast(gg, U32) | z, BF16)
            dst[0:64, cs] = (xx.astype(F32) + sbuf[cb] * gg.astype(F32)).astype(BF16)

    def out_copy(t):
        return pltpu.make_async_copy(hbuf.at[pl.ds(pl.multiple_of(t * HB, 16), 64), :],
                                     out_hbm.at[pl.ds(pl.multiple_of(t * 64, 64), 64), :], osem)

    def body(t, carry):
        hv = hbuf_all.at[pl.ds(pl.multiple_of(t * HB, 16), 2 * HB + 16), :]
        Rp = pl.multiple_of(jnp.maximum(t - 1, 0) * 64, 64)
        B4 = pl.multiple_of(PRE - LAG + t * BR, 16)
        x1v = x1buf.at[pl.ds(B4, LAG + BR), :]
        h3v = h3buf.at[pl.ds(B4, LAG + BR), :]

        nslot = NP + 4 * NCB + 1
        fa = dict(CFG.get("fa", [[17, "4"], [21, "4"], [26, "4"], [30, "4"], [34, "4"], [38, "4"],
                                 [48, "44"]]))
        fb = {100 + (i * 96) // 27: "3" for i in range(27)}
        fb.update({24 + 2 * i: "c" for i in range(NCB)})
        fb[48] = "3"
        fb = dict(CFG.get("fb", fb))
        wsa = CFG.get("wsa", [0, 8, 20, 28, 32])
        wsb = CFG.get("wsb", [0, 8, 20, 28, 32])
        done = {"3": 0, "4": 0, "c": 0}

        def fill(plan, n, last=None):
            for ch in plan.get(n, ""):
                i = done[ch]
                done[ch] += 1
                if ch == "3":
                    w3_part(lhs3, h3v, LAG, BR, [i])
                elif ch == "4":
                    w4_part(lhs4, x1v, BR, [i])
                else:
                    assert done["4"] == NCB
                    combine(Rp, hv, [i], last)

        fill_a = functools.partial(fill, fa)
        fill_b = functools.partial(fill, fb)

        lhs3 = jnp.concatenate(w3_lhs(x1v, LAG, BR), axis=0)
        lhs4 = w4_lhs(h3v, BR)

        keep = {}
        keep_o = {}

        def sel_a(j, i, v):
            keep[(j, i)] = v[L:L + 8]
            return v[0:L]

        def wo_a(h, o):
            keep_o[h] = o[32:40]
            return o[0:32]

        lhs_a = hv[HB:HB + 48, :]
        ra = attn_step(lhs_a, sel_a, wo_a, fill_a, wsa)
        for cb in range(NCB):
            hv[HB + 48:HB + 56, cb * 128:(cb + 1) * 128] = ra[cb][0:8].astype(BF16)
        fill_a(nslot - 1)

        def sel_b(j, i, v):
            return jnp.concatenate([v[0:8], keep[(j, i)], v[8:32]], axis=0)

        def wo_b(h, o):
            return jnp.concatenate([keep_o[h], o], axis=0)

        lhs_b = hv[HB + 48:2 * HB, :]
        rb = attn_step(lhs_b, sel_b, wo_b, fill_b, wsb)
        for cb in range(NCB):
            cs = slice(cb * 128, (cb + 1) * 128)
            hv[2 * HB:2 * HB + 8, cs] = rb[cb][8:16].astype(BF16)
            sbuf[cb] = jnp.concatenate([ra[cb][8:32], rb[cb][0:8], rb[cb][16:48]], axis=0)
        fill_b(nslot - 1)
        assert done == {"3": NFB, "4": NCB, "c": NCB}

        if CFG.get("outdma", 1) == 1:
            @pl.when(t > 0)
            def _():
                out_copy(t - 1).start()

        return carry

    nit = CFG.get("nit", NIT)
    with jax.named_scope("main"):
        lax.fori_loop(0, nit, body, 0)
    with jax.named_scope("epilogue"):
        last = hbuf.at[(nit - 1) * HB:nit * HB, :]
        lhs4 = w4_lhs(h3buf.at[S - LAG:S, :], LAG)
        for cb in range(NCB):
            w4_part(lhs4, x1buf.at[S - LAG:S, :], LAG, [cb])
            combine((nit - 1) * 64, last, [cb])
        out_copy(nit - 1).start()
        if CFG.get("outdma", 1) == 0:
            for t in range(nit - 1):
                out_copy(t).start()
    with jax.named_scope("wait_out"):
        pltpu.make_async_copy(xbuf.at[pl.ds(0, nit * 64), :], out_hbm.at[pl.ds(0, nit * 64), :], osem).wait()


@functools.partial(jax.jit, static_argnames=("A_seg_len",))
def pallas_recurrent_scan__memory_aug_recurrent_mem_tr__mixer_s_mlp__prompt_kernel(
    A_x: jax.Array,
    A_mem0: jax.Array,
    A_Wq: jax.Array,
    A_Wk: jax.Array,
    A_Wv: jax.Array,
    A_Wo: jax.Array,
    A_seg_len,
    B_x: jax.Array,
    B_w1: jax.Array,
    B_w2: jax.Array,
    B_w3: jax.Array,
    B_w4: jax.Array,
):
    assert A_seg_len == SEG
    assert A_x.shape == (1, S, D) and A_mem0.shape == (1, M, D)
    assert A_Wq.shape == (D, H, E) and A_Wo.shape == (H, E, D)
    assert B_w3.shape == (D, FF)
    del B_x

    cw1, cw2, cw3, cwo = 256, 512, 512, 512
    any_spec = pl.BlockSpec(memory_space=pl.ANY)
    out = pl.pallas_call(
        _kernel,
        out_shape=jax.ShapeDtypeStruct((S, D), BF16),
        in_specs=[any_spec] * 10,
        out_specs=any_spec,
        scratch_shapes=[
            pltpu.VMEM((S, D), BF16),
            pltpu.VMEM(((NIT + 1) * HB + 16, D), BF16),
            pltpu.VMEM((NCB, S + 16, 128), F32),
            pltpu.VMEM((S, D), BF16),
            pltpu.VMEM((S, FF), BF16),
            pltpu.VMEM((NCB, 64, 128), F32),
            pltpu.VMEM((4, 3 * D * H // 4, E), BF16),
            pltpu.VMEM((3 * H * HS, 128), U32),
            pltpu.VMEM((D // cwo, H * E, cwo), BF16),
            pltpu.VMEM((D // cw1, D, cw1), BF16),
            pltpu.VMEM((D // cw2, D, cw2), BF16),
            pltpu.VMEM((FF // cw3, D, cw3), BF16),
            pltpu.VMEM((D // cw3, FF, cw3), BF16),
            pltpu.VMEM((HB, HB), F32),
            pltpu.SemaphoreType.DMA((17,)),
            pltpu.SemaphoreType.DMA(()),
        ],
        compiler_params=pltpu.CompilerParams(vmem_limit_bytes=120 * 1024 * 1024,
                                             disable_bounds_checks=True),
    )(
        A_x.reshape(S, D), A_mem0.reshape(M, D),
        A_Wq.reshape(D * H, E), A_Wk.reshape(D * H, E), A_Wv.reshape(D * H, E),
        A_Wo.reshape(H * E, D), B_w1, B_w2, B_w3, B_w4,
    )
    return out.reshape(1, S, D)
```

```python
import functools

import jax
import jax.numpy as jnp
from jax import lax
import jax.experimental.pallas as pl
import jax.experimental.pallas.tpu as pltpu

F32 = jnp.float32
BF16 = jnp.bfloat16
U32 = jnp.uint32

S = 2048
D = 1024
H = 32
E = 128
M = 8
SEG = 32
L = M + SEG
FF = 3584
NCB = D // 128
NFB = FF // 128
NIT = S // (2 * SEG)
HB = 2 * L
PRE = 512
LAG = 64
BR = (S - PRE) // NIT
HS = D // 2 + 8
EPS = 1e-5
SCALE = float(E) ** -0.5
RB = 256
CFG = {}


def _dot(a, b):
    return jnp.dot(a, b, preferred_element_type=F32)


def _ln(x):
    m = jnp.mean(x, axis=-1, keepdims=True)
    xc = x - m
    v = jnp.mean(xc * xc, axis=-1, keepdims=True)
    return xc * lax.rsqrt(v + EPS)


def _ln2(x):
    m = jnp.mean(x, axis=-1, keepdims=True)
    xc = x - m
    v = jnp.mean(xc * xc, axis=-1, keepdims=True)
    r1 = lax.rsqrt(v + EPS)
    r2 = lax.rsqrt(v * r1 * r1 + EPS)
    return xc * r1, xc * (r1 * r2)


def _gelu(x):
    c = 0.7978845608028654
    hx = 0.5 * x
    return hx * jnp.tanh(x * (c + (c * 0.044715) * (x * x))) + hx


def _silu(x):
    hx = 0.5 * x
    return hx * jnp.tanh(hx) + hx


def _kernel(x_hbm, mem0_hbm, wq_hbm, wk_hbm, wv_hbm, wo_hbm, w1_hbm, w2_hbm, w3_hbm, w4_hbm,
            out_hbm,
            xbuf, hbuf_all, hf, x1buf, h3buf, sbuf, stg, wqkv, wo, w1, w2, w3, w4, fillbuf,
            sem, osem):
    hbuf = hbuf_all.at[HB:, :]

    def colblock_copies(src, dst, s):
        n, _, cw = dst.shape
        return [pltpu.make_async_copy(src.at[:, pl.ds(c * cw, cw)], dst.at[c], sem.at[s(c)])
                for c in range(n)]

    def col(w, cb, k0=0, k1=None):
        _, kk, cw = w.shape
        q, r_ = divmod(cb * 128, cw)
        return w[q, k0:(kk if k1 is None else k1), r_:r_ + 128]

    SB = 128
    NXB = S // RB
    XS, QS = 7, 12
    xch = [(0, SB), (SB, SB), (RB, RB), (2 * RB, RB), (3 * RB, S - 3 * RB)]
    cp_x = [pltpu.make_async_copy(x_hbm.at[pl.ds(r, n), :], xbuf.at[pl.ds(r, n), :], sem.at[XS + i])
            for i, (r, n) in enumerate(xch)]
    cp_w1 = colblock_copies(w1_hbm, w1, lambda c: (0, 1, 16, 16)[c])
    cp_mem = [pltpu.make_async_copy(mem0_hbm, hbuf.at[0:M, :], sem.at[2])]
    cp_w2 = colblock_copies(w2_hbm, w2, lambda c: 3)
    cp_w3 = colblock_copies(w3_hbm, w3, lambda c: 4)
    cp_w4 = colblock_copies(w4_hbm, w4, lambda c: 5)
    cp_wo = colblock_copies(wo_hbm, wo, lambda c: 6)
    CH = 512
    PR = 16 * CH
    cp_qkv = [pltpu.make_async_copy(src.at[pl.ds(k * PR, PR), :], stg.at[k, pl.ds(m_ * PR, PR), :],
                                    sem.at[QS + k])
              for k in range(4) for m_, src in enumerate((wq_hbm, wk_hbm, wv_hbm))]
    def start(*grps, priority=0):
        for grp in grps:
            for c in grp:
                c.start(priority=priority)

    start(cp_x[:2], cp_w1[:2], cp_x[2:3], cp_w1[2:], cp_w2, cp_x[3:4])
    start(cp_x[4:], cp_mem, cp_w3, cp_w4, cp_qkv, cp_wo, priority=1)

    def wait(grp):
        for c in grp:
            c.wait()

    r = lax.broadcasted_iota(jnp.int32, (HB, HB), 0)
    c = lax.broadcasted_iota(jnp.int32, (HB, HB), 1)
    rr = jnp.where(r >= L, r - L, r)
    cc = jnp.where(c >= L, c - L, c)
    same = (r >= L) == (c >= L)
    allowed = (rr < M) | (rr >= cc)
    fillbuf[...] = jnp.where(same, jnp.where(allowed, 1.0, -1e9), -jnp.inf).astype(F32)

    hf[:, 0:8, :] = jnp.zeros((NCB, 8, 128), F32)
    hf[:, S + 8:S + 16, :] = jnp.zeros((NCB, 8, 128), F32)
    sbuf[...] = jnp.zeros(sbuf.shape, sbuf.dtype)

    HSB = (SB // 64) * HB

    def zero_of(trig):
        return (pltpu.bitcast(trig, U32) >> 16) >> 16

    def hrow(r):
        q, rr_ = divmod(r, 64)
        return q * HB + rr_ + (8 if rr_ < 40 else 16)

    def ln_sub(xv, hv, sb):
        out = []
        for u in range(SB // 16):
            r = sb * SB + 16 * u
            xn, xnn = _ln2(xv[r:r + 16, :].astype(F32))
            xn = xn.astype(BF16)
            for hh in range(2):
                o = hrow(r + 8 * hh)
                hv[o:o + 8, :] = xn[8 * hh:8 * hh + 8]
            out.append(xnn.astype(BF16))
        return out

    def after(w, vals):
        if not vals:
            return w
        z = None
        for v in vals:
            zv = zero_of(v[0:16, D - 128:D])
            z = zv if z is None else z | zv
        head = pltpu.bitcast(pltpu.bitcast(w[0:16, :], U32) | z, BF16)
        return jnp.concatenate([head, w[16:, :]], axis=0)

    def w1_sub(xnn, hfv, sb, cbs=range(NCB), deps={}):
        xnn = jnp.concatenate(xnn, axis=0)
        for cb in cbs:
            w = after(col(w1, cb), deps.get(cb, []))
            hfv[cb, sb * SB + 8:sb * SB + 8 + SB, :] = _gelu(_dot(xnn, w))

    shifts = (7, 7, 9, 9, 6, 6, 10, 10)

    def w2_lhs(hfv, sb):
        r0 = sb * SB
        return jnp.concatenate(
            [hfv[cb, r0 + shifts[cb]:r0 + shifts[cb] + SB, :] for cb in range(NCB)],
            axis=1).astype(BF16)

    def w2_sub(hs, hv, x1v, sb, cbs=range(NCB), hook=None, deps={}):
        r0 = sb * SB
        for cb in cbs:
            pre = _dot(hs, after(col(w2, cb), deps.get(cb, [])))
            cs = slice(cb * 128, (cb + 1) * 128)
            xn = jnp.concatenate(
                [hv[hrow(r0 + a_):hrow(r0 + a_) + n_, cs].astype(F32)
                 for a_, n_ in ((0, 40), (40, 24), (64, 40), (104, 24))], axis=0)
            x1v[r0:r0 + SB, cs] = (xn + pre).astype(BF16)
            if hook is not None:
                hook(cb, pre)

    def w3_lhs(src, r0, rows):
        return [_ln(src[pl.ds(r0 + 16 * u, 16), :].astype(F32)).astype(BF16)
                for u in range(rows // 16)]

    def w3_part(lhs, h3v, r0, rows, blocks):
        for f in blocks:
            pre = _dot(lhs, col(w3, f))
            h3v[r0:r0 + rows, f * 128:(f + 1) * 128] = _gelu(pre).astype(BF16)
        return pre

    def w4_lhs(h3v, rows):
        return h3v[0:rows, :]

    def w4_part(lhs, x1v, rows, blocks):
        for cb in blocks:
            pre = _dot(lhs, col(w4, cb))
            cs = slice(cb * 128, (cb + 1) * 128)
            x1v[0:rows, cs] = _silu(x1v[0:rows, cs].astype(F32) + pre).astype(BF16)

    def relayout(src, dst, u, trig):
        m_, c_ = divmod(u, 16)
        d0 = m_ * (H * HS) + c_ * 8
        for pp in range(8):
            r0 = u * CH + pp * 64
            tr = (pp * trig.shape[0] // 64) * 8
            t = trig[tr:tr + 8, :]
            z = zero_of(t)
            two = lambda v: jnp.concatenate([v, v], axis=0)
            mlo, mhi, sh = two(z | U32(0xFFFF)), two(z | U32(0xFFFF0000)), two(z | U32(16))
            a = pltpu.bitcast(src[r0:r0 + 32, :], U32)
            b = pltpu.bitcast(src[r0 + 32:r0 + 64, :], U32)
            lo = (a & mlo) | (b << sh)
            hi = (a >> sh) | (b & mhi)
            dst[pl.ds(d0 + pp, 16, stride=HS), :] = lo
            dst[pl.ds(d0 + 16 * HS + pp, 16, stride=HS), :] = hi

    spread8 = lambda c: {2: c[0:1], 3: c[1:2], 4: c[2:4], 5: c[4:5], 6: c[5:7], 7: c[7:8]}
    with jax.named_scope("ln01"):
        cp_x[0].wait()
        xnn0 = ln_sub(xbuf, hbuf, 0)
        cp_x[1].wait()
        xnn1 = ln_sub(xbuf, hbuf, 1)
    with jax.named_scope("wp0"):
        cp_w1[0].wait()
    with jax.named_scope("a00"):
        w1_sub(xnn0, hf, 0, range(0, 2))
        w1_sub(xnn1, hf, 1, range(0, 2))
    with jax.named_scope("wp1"):
        cp_w1[1].wait()
    with jax.named_scope("a01"):
        w1_sub(xnn0, hf, 0, range(2, 4))
    with jax.named_scope("wx2"):
        cp_x[2].wait()
    with jax.named_scope("a02"):
        xnn2 = ln_sub(xbuf, hbuf, 2)
        w1_sub(xnn1, hf, 1, range(2, 4))
        w1_sub(xnn2, hf, 2, range(0, 4))
    with jax.named_scope("wp23"):
        wait(cp_w1[2:])
    with jax.named_scope("a1"):
        xnn3 = ln_sub(xbuf, hbuf, 3)
        w1_sub(xnn0, hf, 0, range(4, 8), {6: xnn3[0:1], 7: xnn3[1:2]})
        w1_sub(xnn1, hf, 1, range(4, 8), {4 + i: xnn3[2 + i:3 + i] for i in range(4)})
        w1_sub(xnn2, hf, 2, range(4, 8), {4: xnn3[6:7], 5: xnn3[7:8]})
        w1_sub(xnn3, hf, 3)
    with jax.named_scope("wait_w2"):
        wait(cp_w2)
        cp_x[3].wait()

    def loop_a2(i, carry):
        @pl.when(i == 3)
        def _():
            cp_x[4].wait()

        r0 = pl.multiple_of((i - 2) * RB, RB)
        xv = xbuf.at[pl.ds(r0, 3 * RB), :]
        hv = hbuf.at[pl.ds(pl.multiple_of((i - 2) * 2 * HSB, 16), 6 * HSB), :]
        x1v = x1buf.at[pl.ds(r0, RB), :]
        hfv = hf.at[:, pl.ds(r0, 3 * RB + 16), :]
        for sb in range(2):
            xnn = ln_sub(xv, hv, 4 + sb)
            w2_sub(w2_lhs(hfv, sb), hv, x1v, sb, deps=spread8(xnn))
            w1_sub(xnn, hfv, 4 + sb)
        return carry

    with jax.named_scope("a2"):
        lax.fori_loop(2, NXB, loop_a2, 0)
    with jax.named_scope("wait_w34"):
        wait(cp_w3)
        wait(cp_w4)

    def loop_s3(k, carry):
        pltpu.make_async_copy(stg.at[k], stg.at[k], sem.at[QS + k]).wait()
        r0 = pl.multiple_of(k * SB, SB)
        src = stg.at[k]
        dst = wqkv.at[pl.ds(pl.multiple_of(k * 128, 128), 3 * H * HS - 384), :]
        sb2 = (S - PRE) // SB
        x1v = x1buf.at[pl.ds(r0, (sb2 + 1) * SB), :]
        hv = hbuf.at[pl.ds(pl.multiple_of(k * HSB, 16), (sb2 + 1) * HSB), :]
        hfv = hf.at[:, pl.ds(r0, (sb2 + 1) * SB + 16), :]
        todo = list(range(48))
        rl = lambda trig: relayout(src, dst, todo.pop(0), trig) if todo else None
        hs = w2_lhs(hfv, sb2)
        lhs = w3_lhs(x1v, 0, SB)
        n2 = CFG.get("s3_n2", 6)
        deps = {int(k_): lhs[v[0]:v[1]] for k_, v in
                CFG.get("s3_deps", {3: (0, 2), 4: (2, 4), 5: (4, 6)}).items()}
        w2_sub(hs, hv, x1v, sb2, range(0, n2), None, deps)
        lhs = jnp.concatenate(lhs, axis=0)
        h3v = h3buf.at[pl.ds(r0, SB), :]
        for f in range(NFB):
            rl(w3_part(lhs, h3v, 0, SB, [f]))
        w2_sub(hs, hv, x1v, sb2, range(n2, 8), lambda cb, pre: rl(pre))
        R4 = (PRE - LAG) // 4
        r4 = pl.multiple_of(k * R4, 16)
        lhs4 = w4_lhs(h3buf.at[pl.ds(r4, R4), :], R4)
        x4v = x1buf.at[pl.ds(r4, R4), :]
        ks = [128 * v for v in CFG.get("s3_ks", (0, 8, 16, 28))]
        for cb in range(NCB):
            pre = None
            for k0, k1 in zip(ks[:-1], ks[1:]):
                part = _dot(lhs4[:, k0:k1], col(w4, cb, k0, k1))
                pre = part if pre is None else part + pre
                rl(pre)
            cs = slice(cb * 128, (cb + 1) * 128)
            x4v[:, cs] = _silu(x4v[:, cs].astype(F32) + pre).astype(BF16)
        assert not todo
        return carry

    with jax.named_scope("s3"):
        lax.fori_loop(0, PRE // SB, loop_s3, 0)
    with jax.named_scope("wait_wo"):
        wait(cp_wo)
        wait(cp_mem)

    def qkv_pair(lhs, j, fill):
        def blk(m_, h):
            r0 = (m_ * H + (h % 2) * 16 + h // 2) * HS
            return pltpu.bitcast(wqkv[r0:r0 + D // 2, :], BF16)
        out = []
        for i in range(6):
            out.append(_dot(lhs, blk(i % 3, 2 * j + i // 3)))
            fill(100 + 6 * j + i, out[-1])
        return out

    def scores(q, k):
        return lax.dot_general(q, k, (((1,), (1,)), ((), ())), preferred_element_type=F32)

    def softmax(s):
        fill = fillbuf[...]
        s = jnp.where(fill > 0.0, s * SCALE, fill)
        mx = jnp.max(s, axis=1, keepdims=True)
        e = jnp.exp(s - mx)
        l = jnp.sum(e, axis=1, keepdims=True)
        rc = pl.reciprocal(l, approx=True)
        rc = rc * (2.0 - l * rc)
        return (e * rc).astype(BF16)

    NP = H // 2

    def attn_step(lhs, select, wo_rows, fill, wsplit):
        qkv = [None] * NP
        sc = [None] * NP
        oh = [None] * H
        acc = [None] * NCB

        def do_qkv(j):
            rs = qkv_pair(lhs, j, fill)
            rs = [select(j, i, v) for i, v in enumerate(rs)]
            qkv[j] = [jnp.concatenate([rs[i], rs[3 + i]], axis=0).astype(BF16) for i in range(3)]

        def do_s(j):
            sc[j] = softmax(scores(qkv[j][0], qkv[j][1]))

        def do_pv(j):
            o = _dot(sc[j], qkv[j][2])
            oh[2 * j] = wo_rows(2 * j, o[0:L]).astype(BF16)
            oh[2 * j + 1] = wo_rows(2 * j + 1, o[L:2 * L]).astype(BF16)

        def do_wo(n):
            h0, h1 = wsplit[n], wsplit[n + 1]
            if h1 == h0:
                return
            lo = jnp.concatenate(oh[h0:h1], axis=1)
            for cb in range(NCB):
                part = _dot(lo, col(wo, cb, h0 * E, h1 * E))
                acc[cb] = part if acc[cb] is None else part + acc[cb]
                fill(NP + n * NCB + cb, part)

        for j in range(NP + 2):
            if j < NP:
                do_qkv(j)
                fill(j)
            else:
                do_wo(j - NP)
            if 0 <= j - 1 < NP:
                do_s(j - 1)
            if 0 <= j - 2 < NP:
                do_pv(j - 2)
        do_wo(2)
        do_wo(3)
        return acc

    def combine(r0, dst, cbs, trig=None):
        for cb in cbs:
            cs = slice(cb * 128, (cb + 1) * 128)
            sl = (pl.ds(r0, 64), cs)
            xx, gg = xbuf[sl], x1buf[sl]
            if trig is not None:
                z = jnp.concatenate([zero_of(trig[0:8, :])] * 4, axis=0)
                xx = pltpu.bitcast(pltpu.bitcast(xx, U32) | z, BF16)
                gg = pltpu.bitcast(pltpu.bitcast(gg, U32) | z, BF16)
            dst[0:64, cs] = (xx.astype(F32) + sbuf[cb] * gg.astype(F32)).astype(BF16)

    def out_copy(t):
        return pltpu.make_async_copy(hbuf.at[pl.ds(pl.multiple_of(t * HB, 16), 64), :],
                                     out_hbm.at[pl.ds(pl.multiple_of(t * 64, 64), 64), :], osem)

    def body(t, carry):
        hv = hbuf_all.at[pl.ds(pl.multiple_of(t * HB, 16), 2 * HB + 16), :]
        Rp = pl.multiple_of(jnp.maximum(t - 1, 0) * 64, 64)
        B4 = pl.multiple_of(PRE - LAG + t * BR, 16)
        x1v = x1buf.at[pl.ds(B4, LAG + BR), :]
        h3v = h3buf.at[pl.ds(B4, LAG + BR), :]

        nslot = NP + 4 * NCB + 1
        fa = dict(CFG.get("fa", [[17, "4"], [21, "4"], [26, "4"], [30, "4"], [34, "4"], [38, "4"],
                                 [48, "44"]]))
        fb = {100 + (i * 96) // 27: "3" for i in range(27)}
        fb.update({24 + 2 * i: "c" for i in range(NCB)})
        fb[48] = "3"
        fb = dict(CFG.get("fb", fb))
        wsa = CFG.get("wsa", [0, 8, 20, 28, 32])
        wsb = CFG.get("wsb", [0, 8, 20, 28, 32])
        done = {"3": 0, "4": 0, "c": 0}

        def fill(plan, n, last=None):
            for ch in plan.get(n, ""):
                i = done[ch]
                done[ch] += 1
                if ch == "3":
                    w3_part(lhs3, h3v, LAG, BR, [i])
                elif ch == "4":
                    w4_part(lhs4, x1v, BR, [i])
                else:
                    assert done["4"] == NCB
                    combine(Rp, hv, [i], last)

        fill_a = functools.partial(fill, fa)
        fill_b = functools.partial(fill, fb)

        lhs3 = jnp.concatenate(w3_lhs(x1v, LAG, BR), axis=0)
        lhs4 = w4_lhs(h3v, BR)

        keep = {}
        keep_o = {}

        def sel_a(j, i, v):
            keep[(j, i)] = v[L:L + 8]
            return v[0:L]

        def wo_a(h, o):
            keep_o[h] = o[32:40]
            return o[0:32]

        lhs_a = hv[HB:HB + 48, :]
        ra = attn_step(lhs_a, sel_a, wo_a, fill_a, wsa)
        for cb in range(NCB):
            hv[HB + 48:HB + 56, cb * 128:(cb + 1) * 128] = ra[cb][0:8].astype(BF16)
        fill_a(nslot - 1)

        def sel_b(j, i, v):
            return jnp.concatenate([v[0:8], keep[(j, i)], v[8:32]], axis=0)

        def wo_b(h, o):
            return jnp.concatenate([keep_o[h], o], axis=0)

        lhs_b = hv[HB + 48:2 * HB, :]
        rb = attn_step(lhs_b, sel_b, wo_b, fill_b, wsb)
        for cb in range(NCB):
            cs = slice(cb * 128, (cb + 1) * 128)
            hv[2 * HB:2 * HB + 8, cs] = rb[cb][8:16].astype(BF16)
            sbuf[cb] = jnp.concatenate([ra[cb][8:32], rb[cb][0:8], rb[cb][16:48]], axis=0)
        fill_b(nslot - 1)
        assert done == {"3": NFB, "4": NCB, "c": NCB}

        if CFG.get("outdma", 1) == 1:
            @pl.when(t > 0)
            def _():
                out_copy(t - 1).start()

        return carry

    nit = CFG.get("nit", NIT)
    with jax.named_scope("main"):
        lax.fori_loop(0, nit, body, 0)
    with jax.named_scope("epilogue"):
        last = hbuf.at[(nit - 1) * HB:nit * HB, :]
        lhs4 = w4_lhs(h3buf.at[S - LAG:S, :], LAG)
        for cb in range(NCB):
            w4_part(lhs4, x1buf.at[S - LAG:S, :], LAG, [cb])
            combine((nit - 1) * 64, last, [cb])
        out_copy(nit - 1).start()
        if CFG.get("outdma", 1) == 0:
            for t in range(nit - 1):
                out_copy(t).start()
    with jax.named_scope("wait_out"):
        pltpu.make_async_copy(xbuf.at[pl.ds(0, nit * 64), :], out_hbm.at[pl.ds(0, nit * 64), :], osem).wait()


@functools.partial(jax.jit, static_argnames=("A_seg_len",))
def pallas_recurrent_scan__memory_aug_recurrent_mem_tr__mixer_s_mlp__prompt_kernel(
    A_x: jax.Array,
    A_mem0: jax.Array,
    A_Wq: jax.Array,
    A_Wk: jax.Array,
    A_Wv: jax.Array,
    A_Wo: jax.Array,
    A_seg_len,
    B_x: jax.Array,
    B_w1: jax.Array,
    B_w2: jax.Array,
    B_w3: jax.Array,
    B_w4: jax.Array,
):
    assert A_seg_len == SEG
    assert A_x.shape == (1, S, D) and A_mem0.shape == (1, M, D)
    assert A_Wq.shape == (D, H, E) and A_Wo.shape == (H, E, D)
    assert B_w3.shape == (D, FF)
    del B_x

    cw1, cw2, cw3, cwo = 256, 512, 512, 512
    any_spec = pl.BlockSpec(memory_space=pl.ANY)
    out = pl.pallas_call(
        _kernel,
        out_shape=jax.ShapeDtypeStruct((S, D), BF16),
        in_specs=[any_spec] * 10,
        out_specs=any_spec,
        scratch_shapes=[
            pltpu.VMEM((S, D), BF16),
            pltpu.VMEM(((NIT + 1) * HB + 16, D), BF16),
            pltpu.VMEM((NCB, S + 16, 128), F32),
            pltpu.VMEM((S, D), BF16),
            pltpu.VMEM((S, FF), BF16),
            pltpu.VMEM((NCB, 64, 128), F32),
            pltpu.VMEM((4, 3 * D * H // 4, E), BF16),
            pltpu.VMEM((3 * H * HS, 128), U32),
            pltpu.VMEM((D // cwo, H * E, cwo), BF16),
            pltpu.VMEM((D // cw1, D, cw1), BF16),
            pltpu.VMEM((D // cw2, D, cw2), BF16),
            pltpu.VMEM((FF // cw3, D, cw3), BF16),
            pltpu.VMEM((D // cw3, FF, cw3), BF16),
            pltpu.VMEM((HB, HB), F32),
            pltpu.SemaphoreType.DMA((17,)),
            pltpu.SemaphoreType.DMA(()),
        ],
        compiler_params=pltpu.CompilerParams(vmem_limit_bytes=120 * 1024 * 1024,
                                             disable_bounds_checks=True),
    )(
        A_x.reshape(S, D), A_mem0.reshape(M, D),
        A_Wq.reshape(D * H, E), A_Wk.reshape(D * H, E), A_Wv.reshape(D * H, E),
        A_Wo.reshape(H * E, D), B_w1, B_w2, B_w3, B_w4,
    )
    return out.reshape(1, S, D)
```

```python
import functools

import jax
import jax.numpy as jnp
from jax import lax
import jax.experimental.pallas as pl
import jax.experimental.pallas.tpu as pltpu

F32 = jnp.float32
BF16 = jnp.bfloat16
U32 = jnp.uint32

S = 2048
D = 1024
H = 32
E = 128
M = 8
SEG = 32
L = M + SEG
FF = 3584
NCB = D // 128
NFB = FF // 128
NP = H // 2
NIT = S // (2 * SEG)
HB = 2 * L
PRE = 512
LAG = 64
BR = (S - PRE) // NIT
HS = D // 2 + 8
RB = 256
SB = 128
HSB = (SB // 64) * HB
CH = 512
PR = 16 * CH
EPS = 1e-5
SCALE = float(E) ** -0.5
SHIFTS = (7, 7, 9, 9, 6, 6, 10, 10)


def _dot(a, b):
    return jnp.dot(a, b, preferred_element_type=F32)


def _ln(x):
    m = jnp.mean(x, axis=-1, keepdims=True)
    xc = x - m
    v = jnp.mean(xc * xc, axis=-1, keepdims=True)
    return xc * lax.rsqrt(v + EPS)


def _ln2(x):
    m = jnp.mean(x, axis=-1, keepdims=True)
    xc = x - m
    v = jnp.mean(xc * xc, axis=-1, keepdims=True)
    r1 = lax.rsqrt(v + EPS)
    r2 = lax.rsqrt(v * r1 * r1 + EPS)
    return xc * r1, xc * (r1 * r2)


def _gelu(x):
    c = 0.7978845608028654
    hx = 0.5 * x
    return hx * jnp.tanh(x * (c + (c * 0.044715) * (x * x))) + hx


def _silu(x):
    hx = 0.5 * x
    return hx * jnp.tanh(hx) + hx


def _zero_of(v):
    return (pltpu.bitcast(v, U32) >> 16) >> 16


def _or_zero(w, z):
    return pltpu.bitcast(pltpu.bitcast(w, U32) | z, w.dtype)


def _col(w, cb, k0=0, k1=None):
    _, kk, cw = w.shape
    q, r = divmod(cb * 128, cw)
    return w[q, k0:(kk if k1 is None else k1), r:r + 128]


def _hrow(r):
    q, rr = divmod(r, 64)
    return q * HB + rr + (8 if rr < 40 else 16)


def _kernel(x_hbm, mem0_hbm, wq_hbm, wk_hbm, wv_hbm, wo_hbm, w1_hbm, w2_hbm, w3_hbm, w4_hbm,
            out_hbm,
            xbuf, hbuf_all, hf, x1buf, h3buf, sbuf, stg, wqkv, wo, w1, w2, w3, w4, fillbuf,
            sem, osem):
    hbuf = hbuf_all.at[HB:, :]

    def colblock_copies(src, dst, s):
        n, _, cw = dst.shape
        return [pltpu.make_async_copy(src.at[:, pl.ds(c * cw, cw)], dst.at[c], sem.at[s(c)])
                for c in range(n)]

    xs, qs = 7, 12
    xch = [(0, SB), (SB, SB), (RB, RB), (2 * RB, RB), (3 * RB, S - 3 * RB)]
    cp_x = [pltpu.make_async_copy(x_hbm.at[pl.ds(r, n), :], xbuf.at[pl.ds(r, n), :], sem.at[xs + i])
            for i, (r, n) in enumerate(xch)]
    cp_w1 = colblock_copies(w1_hbm, w1, lambda c: (0, 1, 16, 16)[c])
    cp_mem = [pltpu.make_async_copy(mem0_hbm, hbuf.at[0:M, :], sem.at[2])]
    cp_w2 = colblock_copies(w2_hbm, w2, lambda c: 3)
    cp_w3 = colblock_copies(w3_hbm, w3, lambda c: 4)
    cp_w4 = colblock_copies(w4_hbm, w4, lambda c: 5)
    cp_wo = colblock_copies(wo_hbm, wo, lambda c: 6)
    cp_qkv = [pltpu.make_async_copy(src.at[pl.ds(k * PR, PR), :], stg.at[k, pl.ds(m * PR, PR), :],
                                    sem.at[qs + k])
              for k in range(4) for m, src in enumerate((wq_hbm, wk_hbm, wv_hbm))]

    for c in cp_x[:2] + cp_w1[:2] + cp_x[2:3] + cp_w1[2:] + cp_w2 + cp_x[3:4]:
        c.start()
    for c in cp_x[4:] + cp_mem + cp_w3 + cp_w4 + cp_qkv + cp_wo:
        c.start(priority=1)

    def wait(grp):
        for c in grp:
            c.wait()

    r = lax.broadcasted_iota(jnp.int32, (HB, HB), 0)
    c = lax.broadcasted_iota(jnp.int32, (HB, HB), 1)
    rr = jnp.where(r >= L, r - L, r)
    cc = jnp.where(c >= L, c - L, c)
    same = (r >= L) == (c >= L)
    allowed = (rr < M) | (rr >= cc)
    fillbuf[...] = jnp.where(same, jnp.where(allowed, 1.0, -1e9), -jnp.inf).astype(F32)

    hf[:, 0:8, :] = jnp.zeros((NCB, 8, 128), F32)
    hf[:, S + 8:S + 16, :] = jnp.zeros((NCB, 8, 128), F32)
    sbuf[...] = jnp.zeros(sbuf.shape, sbuf.dtype)

    def ln_sub(xv, hv, sb):
        out = []
        for u in range(SB // 16):
            r0 = sb * SB + 16 * u
            xn, xnn = _ln2(xv[r0:r0 + 16, :].astype(F32))
            xn = xn.astype(BF16)
            for hh in range(2):
                o = _hrow(r0 + 8 * hh)
                hv[o:o + 8, :] = xn[8 * hh:8 * hh + 8]
            out.append(xnn.astype(BF16))
        return out

    def after(w, vals):
        if not vals:
            return w
        z = functools.reduce(lambda a, b: a | b, [_zero_of(v[0:16, D - 128:D]) for v in vals])
        return jnp.concatenate([_or_zero(w[0:16, :], z), w[16:, :]], axis=0)

    def w1_sub(xnn, hfv, sb, cbs, deps):
        xnn = jnp.concatenate(xnn, axis=0)
        for cb in cbs:
            w = after(_col(w1, cb), deps.get(cb, []))
            hfv[cb, sb * SB + 8:sb * SB + 8 + SB, :] = _gelu(_dot(xnn, w))

    def w2_lhs(hfv, sb):
        r0 = sb * SB
        return jnp.concatenate(
            [hfv[cb, r0 + SHIFTS[cb]:r0 + SHIFTS[cb] + SB, :] for cb in range(NCB)],
            axis=1).astype(BF16)

    def w2_sub(hs, hv, x1v, sb, cbs, deps, hook=None):
        r0 = sb * SB
        for cb in cbs:
            pre = _dot(hs, after(_col(w2, cb), deps.get(cb, [])))
            cs = slice(cb * 128, (cb + 1) * 128)
            xn = jnp.concatenate(
                [hv[_hrow(r0 + a):_hrow(r0 + a) + n, cs].astype(F32)
                 for a, n in ((0, 40), (40, 24), (64, 40), (104, 24))], axis=0)
            x1v[r0:r0 + SB, cs] = (xn + pre).astype(BF16)
            if hook is not None:
                hook(pre)

    def w3_lhs(x1v, r0, rows):
        return [_ln(x1v[r0 + 16 * u:r0 + 16 * u + 16, :].astype(F32)).astype(BF16)
                for u in range(rows // 16)]

    def w3_block(lhs, h3v, r0, f):
        pre = _dot(lhs, _col(w3, f))
        h3v[r0:r0 + lhs.shape[0], f * 128:(f + 1) * 128] = _gelu(pre).astype(BF16)
        return pre

    def w4_block(lhs, x1v, cb, ks=(0, FF), hook=None):
        pre = None
        for k0, k1 in zip(ks[:-1], ks[1:]):
            part = _dot(lhs[:, k0:k1], _col(w4, cb, k0, k1))
            pre = part if pre is None else part + pre
            if hook is not None:
                hook(pre)
        sl = (slice(0, lhs.shape[0]), slice(cb * 128, (cb + 1) * 128))
        x1v[sl] = _silu(x1v[sl].astype(F32) + pre).astype(BF16)

    def relayout(src, dst, u, trig):
        m, c_ = divmod(u, 16)
        d0 = m * (H * HS) + c_ * 8
        two = lambda v: jnp.concatenate([v, v], axis=0)
        for pp in range(8):
            r0 = u * CH + pp * 64
            tr = (pp * trig.shape[0] // 64) * 8
            z = _zero_of(trig[tr:tr + 8, :])
            mlo, mhi, sh = two(z | U32(0xFFFF)), two(z | U32(0xFFFF0000)), two(z | U32(16))
            a = pltpu.bitcast(src[r0:r0 + 32, :], U32)
            b = pltpu.bitcast(src[r0 + 32:r0 + 64, :], U32)
            dst[pl.ds(d0 + pp, 16, stride=HS), :] = (a & mlo) | (b << sh)
            dst[pl.ds(d0 + 16 * HS + pp, 16, stride=HS), :] = (a >> sh) | (b & mhi)

    cp_x[0].wait()
    xnn0 = ln_sub(xbuf, hbuf, 0)
    cp_x[1].wait()
    xnn1 = ln_sub(xbuf, hbuf, 1)
    cp_w1[0].wait()
    w1_sub(xnn0, hf, 0, range(0, 2), {})
    w1_sub(xnn1, hf, 1, range(0, 2), {})
    cp_w1[1].wait()
    w1_sub(xnn0, hf, 0, range(2, 4), {})
    cp_x[2].wait()
    xnn2 = ln_sub(xbuf, hbuf, 2)
    w1_sub(xnn1, hf, 1, range(2, 4), {})
    w1_sub(xnn2, hf, 2, range(0, 4), {})
    wait(cp_w1[2:])
    xnn3 = ln_sub(xbuf, hbuf, 3)
    w1_sub(xnn0, hf, 0, range(4, 8), {6: xnn3[0:1], 7: xnn3[1:2]})
    w1_sub(xnn1, hf, 1, range(4, 8), {4 + i: xnn3[2 + i:3 + i] for i in range(4)})
    w1_sub(xnn2, hf, 2, range(4, 8), {4: xnn3[6:7], 5: xnn3[7:8]})
    w1_sub(xnn3, hf, 3, range(NCB), {})
    wait(cp_w2)
    cp_x[3].wait()

    def loop_w12(i, carry):
        @pl.when(i == 3)
        def _():
            cp_x[4].wait()

        r0 = pl.multiple_of((i - 2) * RB, RB)
        xv = xbuf.at[pl.ds(r0, 3 * RB), :]
        hv = hbuf.at[pl.ds(pl.multiple_of((i - 2) * 2 * HSB, 16), 6 * HSB), :]
        x1v = x1buf.at[pl.ds(r0, RB), :]
        hfv = hf.at[:, pl.ds(r0, 3 * RB + 16), :]
        for sb in range(2):
            c = ln_sub(xv, hv, 4 + sb)
            deps = {2: c[0:1], 3: c[1:2], 4: c[2:4], 5: c[4:5], 6: c[5:7], 7: c[7:8]}
            w2_sub(w2_lhs(hfv, sb), hv, x1v, sb, range(NCB), deps)
            w1_sub(c, hfv, 4 + sb, range(NCB), {})
        return carry

    lax.fori_loop(2, S // RB, loop_w12, 0)
    wait(cp_w3)
    wait(cp_w4)

    def loop_w34(k, carry):
        pltpu.make_async_copy(stg.at[k], stg.at[k], sem.at[qs + k]).wait()
        r0 = pl.multiple_of(k * SB, SB)
        src = stg.at[k]
        dst = wqkv.at[pl.ds(pl.multiple_of(k * 128, 128), (3 * H + 1) * HS - 384), :]
        sb2 = (S - PRE) // SB
        x1v = x1buf.at[pl.ds(r0, (sb2 + 1) * SB), :]
        hv = hbuf.at[pl.ds(pl.multiple_of(k * HSB, 16), (sb2 + 1) * HSB), :]
        hfv = hf.at[:, pl.ds(r0, (sb2 + 1) * SB + 16), :]
        todo = list(range(3 * PR // CH))

        def rl(trig):
            if todo:
                relayout(src, dst, todo.pop(0), trig)

        hs = w2_lhs(hfv, sb2)
        c = w3_lhs(x1v, 0, SB)
        w2_sub(hs, hv, x1v, sb2, range(0, 6), {3: c[0:2], 4: c[2:4], 5: c[4:6]})
        lhs3 = jnp.concatenate(c, axis=0)
        h3v = h3buf.at[pl.ds(r0, SB), :]
        for f in range(NFB):
            rl(w3_block(lhs3, h3v, 0, f))
        w2_sub(hs, hv, x1v, sb2, range(6, 8), {}, rl)
        n4 = (PRE - LAG) // 4
        r4 = pl.multiple_of(k * n4, 16)
        lhs4 = h3buf[pl.ds(r4, n4), :]
        for cb in range(NCB):
            w4_block(lhs4, x1buf.at[pl.ds(r4, n4), :], cb, (0, 1024, 2048, FF), rl)
        assert not todo
        return carry

    lax.fori_loop(0, PRE // SB, loop_w34, 0)
    wait(cp_wo)
    wait(cp_mem)

    def softmax(s):
        fill = fillbuf[...]
        s = jnp.where(fill > 0.0, s * SCALE, fill)
        mx = jnp.max(s, axis=1, keepdims=True)
        e = jnp.exp(s - mx)
        l = jnp.sum(e, axis=1, keepdims=True)
        rc = pl.reciprocal(l, approx=True)
        rc = rc * (2.0 - l * rc)
        return (e * rc).astype(BF16)

    def attn_step(lhs, select, wo_rows, fill):
        qkv = [None] * NP
        p = [None] * NP
        oh = [None] * H
        acc = [None] * NCB
        wsplit = (0, 8, 20, 28, 32)

        def do_qkv(j):
            rs = []
            for i in range(6):
                h = 2 * j + i // 3
                r0 = ((i % 3) * H + (h % 2) * 16 + h // 2) * HS
                v = _dot(lhs, pltpu.bitcast(wqkv[r0:r0 + D // 2, :], BF16))
                fill(("qkv", 6 * j + i), v)
                rs.append(select(j, i, v))
            qkv[j] = [jnp.concatenate([rs[i], rs[3 + i]], axis=0).astype(BF16) for i in range(3)]

        def do_s(j):
            p[j] = softmax(lax.dot_general(qkv[j][0], qkv[j][1], (((1,), (1,)), ((), ())),
                                           preferred_element_type=F32))

        def do_pv(j):
            o = _dot(p[j], qkv[j][2])
            oh[2 * j] = wo_rows(2 * j, o[0:L]).astype(BF16)
            oh[2 * j + 1] = wo_rows(2 * j + 1, o[L:2 * L]).astype(BF16)

        def do_wo(n):
            h0, h1 = wsplit[n], wsplit[n + 1]
            lo = jnp.concatenate(oh[h0:h1], axis=1)
            for cb in range(NCB):
                part = _dot(lo, _col(wo, cb, h0 * E, h1 * E))
                acc[cb] = part if acc[cb] is None else part + acc[cb]
                fill(("wo", n * NCB + cb), part)

        for j in range(NP + 2):
            if j < NP:
                do_qkv(j)
            else:
                do_wo(j - NP)
            if 0 <= j - 1 < NP:
                do_s(j - 1)
            if 0 <= j - 2 < NP:
                do_pv(j - 2)
        do_wo(2)
        do_wo(3)
        return acc

    def combine(r0, dst, cb, trig=None):
        cs = slice(cb * 128, (cb + 1) * 128)
        xx, gg = xbuf[pl.ds(r0, 64), cs], x1buf[pl.ds(r0, 64), cs]
        if trig is not None:
            z = jnp.concatenate([_zero_of(trig[0:8, :])] * 4, axis=0)
            xx, gg = _or_zero(xx, z), _or_zero(gg, z)
        dst[0:64, cs] = (xx.astype(F32) + sbuf[cb] * gg.astype(F32)).astype(BF16)

    def out_copy(t, aligned):
        return pltpu.make_async_copy(hbuf.at[pl.ds(aligned(t * HB, 16), 64), :],
                                     out_hbm.at[pl.ds(aligned(t * 64, 64), 64), :], osem)

    def body(t, carry):
        hv = hbuf_all.at[pl.ds(pl.multiple_of(t * HB, 16), 2 * HB + 16), :]
        prev = pl.multiple_of(jnp.maximum(t - 1, 0) * 64, 64)
        b4 = pl.multiple_of(PRE - LAG + t * BR, 16)
        x1v = x1buf.at[pl.ds(b4, LAG + BR), :]
        h3v = h3buf.at[pl.ds(b4, LAG + BR), :]
        lhs3 = jnp.concatenate(w3_lhs(x1v, LAG, BR), axis=0)
        lhs4 = h3v[0:BR, :]
        todo3, todo4, todoc = list(range(NFB)), list(range(NCB)), list(range(NCB))

        keep = {}

        def sel_a(j, i, v):
            keep[(j, i)] = v[L:L + 8]
            return v[0:L]

        def wo_a(h, o):
            keep[h] = o[32:40]
            return o[0:32]

        def fill_a(slot, v):
            if slot[0] == "wo" and slot[1] in (1, 5, 10, 14, 18, 22):
                w4_block(lhs4, x1v, todo4.pop(0))

        ra = attn_step(hv[HB:HB + 48, :], sel_a, wo_a, fill_a)
        for cb in range(NCB):
            hv[HB + 48:HB + 56, cb * 128:(cb + 1) * 128] = ra[cb][0:8].astype(BF16)
        while todo4:
            w4_block(lhs4, x1v, todo4.pop(0))

        def sel_b(j, i, v):
            return jnp.concatenate([v[0:8], keep[(j, i)], v[8:32]], axis=0)

        def wo_b(h, o):
            return jnp.concatenate([keep[h], o], axis=0)

        w3_slots = [(i * 6 * NP) // (NFB - 1) for i in range(NFB - 1)]

        def fill_b(slot, v):
            if slot[0] == "qkv" and slot[1] in w3_slots:
                w3_block(lhs3, h3v, LAG, todo3.pop(0))
            if slot[0] == "wo" and slot[1] in range(8, 24, 2):
                combine(prev, hv, todoc.pop(0), v)

        rb = attn_step(hv[HB + 48:2 * HB, :], sel_b, wo_b, fill_b)
        for cb in range(NCB):
            hv[2 * HB:2 * HB + 8, cb * 128:(cb + 1) * 128] = rb[cb][8:16].astype(BF16)
            sbuf[cb] = jnp.concatenate([ra[cb][8:32], rb[cb][0:8], rb[cb][16:48]], axis=0)
        w3_block(lhs3, h3v, LAG, todo3.pop(0))
        assert not (todo3 or todo4 or todoc)

        @pl.when(t > 0)
        def _():
            out_copy(t - 1, pl.multiple_of).start()

        return carry

    lax.fori_loop(0, NIT, body, 0)

    lhs4 = h3buf[S - LAG:S, :]
    for cb in range(NCB):
        w4_block(lhs4, x1buf.at[S - LAG:S, :], cb)
        combine(S - 64, hbuf.at[(NIT - 1) * HB:NIT * HB, :], cb)
    out_copy(NIT - 1, lambda v, n: v).start()
    pltpu.make_async_copy(xbuf, out_hbm, osem).wait()


@jax.jit
def pallas_recurrent_scan__memory_aug_recurrent_mem_tr__mixer_s_mlp__prompt_kernel(
    A_x: jax.Array,
    A_mem0: jax.Array,
    A_Wq: jax.Array,
    A_Wk: jax.Array,
    A_Wv: jax.Array,
    A_Wo: jax.Array,
    A_seg_len: jax.Array,
    B_x: jax.Array,
    B_w1: jax.Array,
    B_w2: jax.Array,
    B_w3: jax.Array,
    B_w4: jax.Array,
):
    del A_seg_len, B_x
    assert A_x.shape == (1, S, D) and A_mem0.shape == (1, M, D)
    assert A_Wq.shape == (D, H, E) and A_Wo.shape == (H, E, D)
    assert B_w3.shape == (D, FF) and B_w4.shape == (FF, D)

    any_spec = pl.BlockSpec(memory_space=pl.ANY)
    out = pl.pallas_call(
        _kernel,
        out_shape=jax.ShapeDtypeStruct((S, D), BF16),
        in_specs=[any_spec] * 10,
        out_specs=any_spec,
        scratch_shapes=[
            pltpu.VMEM((S, D), BF16),
            pltpu.VMEM(((NIT + 1) * HB + 16, D), BF16),
            pltpu.VMEM((NCB, S + 16, 128), F32),
            pltpu.VMEM((S, D), BF16),
            pltpu.VMEM((S, FF), BF16),
            pltpu.VMEM((NCB, 64, 128), F32),
            pltpu.VMEM((4, 3 * PR, E), BF16),
            pltpu.VMEM(((3 * H + 1) * HS, 128), U32),
            pltpu.VMEM((D // 512, H * E, 512), BF16),
            pltpu.VMEM((D // 256, D, 256), BF16),
            pltpu.VMEM((D // 512, D, 512), BF16),
            pltpu.VMEM((FF // 512, D, 512), BF16),
            pltpu.VMEM((D // 512, FF, 512), BF16),
            pltpu.VMEM((HB, HB), F32),
            pltpu.SemaphoreType.DMA((17,)),
            pltpu.SemaphoreType.DMA(()),
        ],
        compiler_params=pltpu.CompilerParams(vmem_limit_bytes=120 * 1024 * 1024),
    )(
        A_x.reshape(S, D), A_mem0.reshape(M, D),
        A_Wq.reshape(D * H, E), A_Wk.reshape(D * H, E), A_Wv.reshape(D * H, E),
        A_Wo.reshape(H * E, D), B_w1, B_w2, B_w3, B_w4,
    )
    return out.reshape(1, S, D)
```

```python
import functools

import jax
import jax.numpy as jnp
from jax import lax
import jax.experimental.pallas as pl
import jax.experimental.pallas.tpu as pltpu

F32 = jnp.float32
BF16 = jnp.bfloat16
U32 = jnp.uint32

S = 2048
D = 1024
H = 32
E = 128
M = 8
SEG = 32
L = M + SEG
FF = 3584
NCB = D // 128
NFB = FF // 128
NP = H // 2
NIT = S // (2 * SEG)
HB = 2 * L
PRE = 512
LAG = 64
BR = (S - PRE) // NIT
HS = D // 2 + 8
RB = 256
SB = 128
HSB = (SB // 64) * HB
CH = 512
PR = 16 * CH
EPS = 1e-5
SCALE = float(E) ** -0.5
SHIFTS = (7, 7, 9, 9, 6, 6, 10, 10)


def _dot(a, b):
    return jnp.dot(a, b, preferred_element_type=F32)


def _ln(x):
    m = jnp.mean(x, axis=-1, keepdims=True)
    xc = x - m
    v = jnp.mean(xc * xc, axis=-1, keepdims=True)
    return xc * lax.rsqrt(v + EPS)


def _ln2(x):
    m = jnp.mean(x, axis=-1, keepdims=True)
    xc = x - m
    v = jnp.mean(xc * xc, axis=-1, keepdims=True)
    r1 = lax.rsqrt(v + EPS)
    r2 = lax.rsqrt(v * r1 * r1 + EPS)
    return xc * r1, xc * (r1 * r2)


def _gelu(x):
    c = 0.7978845608028654
    hx = 0.5 * x
    return hx * jnp.tanh(x * (c + (c * 0.044715) * (x * x))) + hx


def _silu(x):
    hx = 0.5 * x
    return hx * jnp.tanh(hx) + hx


def _zero_of(v):
    return (pltpu.bitcast(v, U32) >> 16) >> 16


def _or_zero(w, z):
    return pltpu.bitcast(pltpu.bitcast(w, U32) | z, w.dtype)


def _col(w, cb, k0=0, k1=None):
    _, kk, cw = w.shape
    q, r = divmod(cb * 128, cw)
    return w[q, k0:(kk if k1 is None else k1), r:r + 128]


def _hrow(r):
    q, rr = divmod(r, 64)
    return q * HB + rr + (8 if rr < 40 else 16)


def _kernel(x_hbm, mem0_hbm, wq_hbm, wk_hbm, wv_hbm, wo_hbm, w1_hbm, w2_hbm, w3_hbm, w4_hbm,
            out_hbm,
            xbuf, hbuf_all, hf, x1buf, h3buf, sbuf, stg, wqkv, wo, w1, w2, w3, w4, fillbuf,
            sem, osem):
    hbuf = hbuf_all.at[HB:, :]

    def colblock_copies(src, dst, s):
        n, _, cw = dst.shape
        return [pltpu.make_async_copy(src.at[:, pl.ds(c * cw, cw)], dst.at[c], sem.at[s(c)])
                for c in range(n)]

    xs, qs = 7, 12
    xch = [(0, SB), (SB, SB), (RB, RB), (2 * RB, RB), (3 * RB, S - 3 * RB)]
    cp_x = [pltpu.make_async_copy(x_hbm.at[pl.ds(r, n), :], xbuf.at[pl.ds(r, n), :], sem.at[xs + i])
            for i, (r, n) in enumerate(xch)]
    cp_w1 = colblock_copies(w1_hbm, w1, lambda c: (0, 1, 16, 16)[c])
    cp_mem = [pltpu.make_async_copy(mem0_hbm, hbuf.at[0:M, :], sem.at[2])]
    cp_w2 = colblock_copies(w2_hbm, w2, lambda c: 3)
    cp_w3 = colblock_copies(w3_hbm, w3, lambda c: 4)
    cp_w4 = colblock_copies(w4_hbm, w4, lambda c: 5)
    cp_wo = colblock_copies(wo_hbm, wo, lambda c: 6)
    cp_qkv = [pltpu.make_async_copy(src.at[pl.ds(k * PR, PR), :], stg.at[k, pl.ds(m * PR, PR), :],
                                    sem.at[qs + k])
              for k in range(4) for m, src in enumerate((wq_hbm, wk_hbm, wv_hbm))]

    for c in cp_x[:2] + cp_w1[:2] + cp_x[2:3] + cp_w1[2:] + cp_w2 + cp_x[3:4]:
        c.start()
    for c in cp_x[4:] + cp_mem + cp_w3 + cp_w4 + cp_qkv + cp_wo:
        c.start(priority=1)

    def wait(grp):
        for c in grp:
            c.wait()

    r = lax.broadcasted_iota(jnp.int32, (HB, HB), 0)
    c = lax.broadcasted_iota(jnp.int32, (HB, HB), 1)
    rr = jnp.where(r >= L, r - L, r)
    cc = jnp.where(c >= L, c - L, c)
    same = (r >= L) == (c >= L)
    allowed = (rr < M) | (rr >= cc)
    fillbuf[...] = jnp.where(same, jnp.where(allowed, 1.0, -1e9), -jnp.inf).astype(F32)

    hf[:, 0:8, :] = jnp.zeros((NCB, 8, 128), F32)
    hf[:, S + 8:S + 16, :] = jnp.zeros((NCB, 8, 128), F32)
    sbuf[...] = jnp.zeros(sbuf.shape, sbuf.dtype)

    def ln_sub(xv, hv, sb):
        out = []
        for u in range(SB // 16):
            r0 = sb * SB + 16 * u
            xn, xnn = _ln2(xv[r0:r0 + 16, :].astype(F32))
            xn = xn.astype(BF16)
            for hh in range(2):
                o = _hrow(r0 + 8 * hh)
                hv[o:o + 8, :] = xn[8 * hh:8 * hh + 8]
            out.append(xnn.astype(BF16))
        return out

    def after(w, vals):
        if not vals:
            return w
        z = functools.reduce(lambda a, b: a | b, [_zero_of(v[0:16, D - 128:D]) for v in vals])
        return jnp.concatenate([_or_zero(w[0:16, :], z), w[16:, :]], axis=0)

    def w1_sub(xnn, hfv, sb, cbs, deps):
        xnn = jnp.concatenate(xnn, axis=0)
        for cb in cbs:
            w = after(_col(w1, cb), deps.get(cb, []))
            hfv[cb, sb * SB + 8:sb * SB + 8 + SB, :] = _gelu(_dot(xnn, w))

    def w2_lhs(hfv, sb):
        r0 = sb * SB
        return jnp.concatenate(
            [hfv[cb, r0 + SHIFTS[cb]:r0 + SHIFTS[cb] + SB, :] for cb in range(NCB)],
            axis=1).astype(BF16)

    def w2_sub(hs, hv, x1v, sb, cbs, deps, hook=None):
        r0 = sb * SB
        for cb in cbs:
            pre = _dot(hs, after(_col(w2, cb), deps.get(cb, [])))
            cs = slice(cb * 128, (cb + 1) * 128)
            xn = jnp.concatenate(
                [hv[_hrow(r0 + a):_hrow(r0 + a) + n, cs].astype(F32)
                 for a, n in ((0, 40), (40, 24), (64, 40), (104, 24))], axis=0)
            x1v[r0:r0 + SB, cs] = (xn + pre).astype(BF16)
            if hook is not None:
                hook(pre)

    def w3_lhs(x1v, r0, rows):
        return [_ln(x1v[r0 + 16 * u:r0 + 16 * u + 16, :].astype(F32)).astype(BF16)
                for u in range(rows // 16)]

    def w3_block(lhs, h3v, r0, f):
        pre = _dot(lhs, _col(w3, f))
        h3v[r0:r0 + lhs.shape[0], f * 128:(f + 1) * 128] = _gelu(pre).astype(BF16)
        return pre

    def w4_block(lhs, x1v, cb, ks=(0, FF), hook=None):
        pre = None
        for k0, k1 in zip(ks[:-1], ks[1:]):
            part = _dot(lhs[:, k0:k1], _col(w4, cb, k0, k1))
            pre = part if pre is None else part + pre
            if hook is not None:
                hook(pre)
        sl = (slice(0, lhs.shape[0]), slice(cb * 128, (cb + 1) * 128))
        x1v[sl] = _silu(x1v[sl].astype(F32) + pre).astype(BF16)

    def relayout(src, dst, u, trig):
        m, c_ = divmod(u, 16)
        d0 = m * (H * HS) + c_ * 8
        two = lambda v: jnp.concatenate([v, v], axis=0)
        for pp in range(8):
            r0 = u * CH + pp * 64
            tr = (pp * trig.shape[0] // 64) * 8
            z = _zero_of(trig[tr:tr + 8, :])
            mlo, mhi, sh = two(z | U32(0xFFFF)), two(z | U32(0xFFFF0000)), two(z | U32(16))
            a = pltpu.bitcast(src[r0:r0 + 32, :], U32)
            b = pltpu.bitcast(src[r0 + 32:r0 + 64, :], U32)
            dst[pl.ds(d0 + pp, 16, stride=HS), :] = (a & mlo) | (b << sh)
            dst[pl.ds(d0 + 16 * HS + pp, 16, stride=HS), :] = (a >> sh) | (b & mhi)

    cp_x[0].wait()
    xnn0 = ln_sub(xbuf, hbuf, 0)
    cp_x[1].wait()
    xnn1 = ln_sub(xbuf, hbuf, 1)
    cp_w1[0].wait()
    w1_sub(xnn0, hf, 0, range(0, 2), {})
    w1_sub(xnn1, hf, 1, range(0, 2), {})
    cp_w1[1].wait()
    w1_sub(xnn0, hf, 0, range(2, 4), {})
    cp_x[2].wait()
    xnn2 = ln_sub(xbuf, hbuf, 2)
    w1_sub(xnn1, hf, 1, range(2, 4), {})
    w1_sub(xnn2, hf, 2, range(0, 4), {})
    wait(cp_w1[2:])
    xnn3 = ln_sub(xbuf, hbuf, 3)
    w1_sub(xnn0, hf, 0, range(4, 8), {6: xnn3[0:1], 7: xnn3[1:2]})
    w1_sub(xnn1, hf, 1, range(4, 8), {4 + i: xnn3[2 + i:3 + i] for i in range(4)})
    w1_sub(xnn2, hf, 2, range(4, 8), {4: xnn3[6:7], 5: xnn3[7:8]})
    w1_sub(xnn3, hf, 3, range(NCB), {})
    wait(cp_w2)
    cp_x[3].wait()

    def loop_w12(i, carry):
        @pl.when(i == 3)
        def _():
            cp_x[4].wait()

        r0 = pl.multiple_of((i - 2) * RB, RB)
        xv = xbuf.at[pl.ds(r0, 3 * RB), :]
        hv = hbuf.at[pl.ds(pl.multiple_of((i - 2) * 2 * HSB, 16), 6 * HSB), :]
        x1v = x1buf.at[pl.ds(r0, RB), :]
        hfv = hf.at[:, pl.ds(r0, 3 * RB + 16), :]
        for sb in range(2):
            c = ln_sub(xv, hv, 4 + sb)
            deps = {2: c[0:1], 3: c[1:2], 4: c[2:4], 5: c[4:5], 6: c[5:7], 7: c[7:8]}
            w2_sub(w2_lhs(hfv, sb), hv, x1v, sb, range(NCB), deps)
            w1_sub(c, hfv, 4 + sb, range(NCB), {})
        return carry

    lax.fori_loop(2, S // RB, loop_w12, 0)
    wait(cp_w3)
    wait(cp_w4)

    def loop_w34(k, carry):
        pltpu.make_async_copy(stg.at[k], stg.at[k], sem.at[qs + k]).wait()
        r0 = pl.multiple_of(k * SB, SB)
        src = stg.at[k]
        dst = wqkv.at[pl.ds(pl.multiple_of(k * 128, 128), (3 * H + 1) * HS - 384), :]
        sb2 = (S - PRE) // SB
        x1v = x1buf.at[pl.ds(r0, (sb2 + 1) * SB), :]
        hv = hbuf.at[pl.ds(pl.multiple_of(k * HSB, 16), (sb2 + 1) * HSB), :]
        hfv = hf.at[:, pl.ds(r0, (sb2 + 1) * SB + 16), :]
        todo = list(range(3 * PR // CH))

        def rl(trig):
            if todo:
                relayout(src, dst, todo.pop(0), trig)

        hs = w2_lhs(hfv, sb2)
        c = w3_lhs(x1v, 0, SB)
        w2_sub(hs, hv, x1v, sb2, range(0, 6), {3: c[0:2], 4: c[2:4], 5: c[4:6]})
        lhs3 = jnp.concatenate(c, axis=0)
        h3v = h3buf.at[pl.ds(r0, SB), :]
        for f in range(NFB):
            rl(w3_block(lhs3, h3v, 0, f))
        w2_sub(hs, hv, x1v, sb2, range(6, 8), {}, rl)
        n4 = (PRE - LAG) // 4
        r4 = pl.multiple_of(k * n4, 16)
        lhs4 = h3buf[pl.ds(r4, n4), :]
        for cb in range(NCB):
            w4_block(lhs4, x1buf.at[pl.ds(r4, n4), :], cb, (0, 1024, 2048, FF), rl)
        assert not todo
        return carry

    lax.fori_loop(0, PRE // SB, loop_w34, 0)
    wait(cp_wo)
    wait(cp_mem)

    def softmax(s):
        fill = fillbuf[...]
        s = jnp.where(fill > 0.0, s * SCALE, fill)
        mx = jnp.max(s, axis=1, keepdims=True)
        e = jnp.exp(s - mx)
        l = jnp.sum(e, axis=1, keepdims=True)
        rc = pl.reciprocal(l, approx=True)
        rc = rc * (2.0 - l * rc)
        return (e * rc).astype(BF16)

    def attn_step(lhs, select, wo_rows, fill):
        qkv = [None] * NP
        p = [None] * NP
        oh = [None] * H
        acc = [None] * NCB
        wsplit = (0, 8, 20, 28, 32)

        def do_qkv(j):
            rs = []
            for i in range(6):
                h = 2 * j + i // 3
                r0 = ((i % 3) * H + (h % 2) * 16 + h // 2) * HS
                v = _dot(lhs, pltpu.bitcast(wqkv[r0:r0 + D // 2, :], BF16))
                fill(("qkv", 6 * j + i), v)
                rs.append(select(j, i, v))
            qkv[j] = [jnp.concatenate([rs[i], rs[3 + i]], axis=0).astype(BF16) for i in range(3)]

        def do_s(j):
            p[j] = softmax(lax.dot_general(qkv[j][0], qkv[j][1], (((1,), (1,)), ((), ())),
                                           preferred_element_type=F32))

        def do_pv(j):
            o = _dot(p[j], qkv[j][2])
            oh[2 * j] = wo_rows(2 * j, o[0:L]).astype(BF16)
            oh[2 * j + 1] = wo_rows(2 * j + 1, o[L:2 * L]).astype(BF16)

        def do_wo(n):
            h0, h1 = wsplit[n], wsplit[n + 1]
            lo = jnp.concatenate(oh[h0:h1], axis=1)
            for cb in range(NCB):
                part = _dot(lo, _col(wo, cb, h0 * E, h1 * E))
                acc[cb] = part if acc[cb] is None else part + acc[cb]
                fill(("wo", n * NCB + cb), part)

        for j in range(NP + 2):
            if j < NP:
                do_qkv(j)
            else:
                do_wo(j - NP)
            if 0 <= j - 1 < NP:
                do_s(j - 1)
            if 0 <= j - 2 < NP:
                do_pv(j - 2)
        do_wo(2)
        do_wo(3)
        return acc

    def combine(r0, dst, cb, trig=None):
        cs = slice(cb * 128, (cb + 1) * 128)
        xx, gg = xbuf[pl.ds(r0, 64), cs], x1buf[pl.ds(r0, 64), cs]
        if trig is not None:
            z = jnp.concatenate([_zero_of(trig[0:8, :])] * 4, axis=0)
            xx, gg = _or_zero(xx, z), _or_zero(gg, z)
        dst[0:64, cs] = (xx.astype(F32) + sbuf[cb] * gg.astype(F32)).astype(BF16)

    def body(t, carry):
        hv = hbuf_all.at[pl.ds(pl.multiple_of(t * HB, 16), 2 * HB + 16), :]
        prev = pl.multiple_of(jnp.maximum(t - 1, 0) * 64, 64)
        b4 = pl.multiple_of(PRE - LAG + t * BR, 16)
        x1v = x1buf.at[pl.ds(b4, LAG + BR), :]
        h3v = h3buf.at[pl.ds(b4, LAG + BR), :]
        lhs3 = jnp.concatenate(w3_lhs(x1v, LAG, BR), axis=0)
        lhs4 = h3v[0:BR, :]
        todo3, todo4, todoc = list(range(NFB)), list(range(NCB)), list(range(NCB))

        keep = {}

        def sel_a(j, i, v):
            keep[(j, i)] = v[L:L + 8]
            return v[0:L]

        def wo_a(h, o):
            keep[h] = o[32:40]
            return o[0:32]

        def fill_a(slot, v):
            if slot[0] == "wo" and slot[1] in (1, 5, 10, 14, 18, 22):
                w4_block(lhs4, x1v, todo4.pop(0))

        ra = attn_step(hv[HB:HB + 48, :], sel_a, wo_a, fill_a)
        for cb in range(NCB):
            hv[HB + 48:HB + 56, cb * 128:(cb + 1) * 128] = ra[cb][0:8].astype(BF16)
        while todo4:
            w4_block(lhs4, x1v, todo4.pop(0))

        def sel_b(j, i, v):
            return jnp.concatenate([v[0:8], keep[(j, i)], v[8:32]], axis=0)

        def wo_b(h, o):
            return jnp.concatenate([keep[h], o], axis=0)

        w3_slots = [(i * 6 * NP) // NFB for i in range(NFB)]

        def fill_b(slot, v):
            if slot[0] == "qkv" and slot[1] in w3_slots:
                w3_block(lhs3, h3v, LAG, todo3.pop(0))
            if slot[0] == "wo" and slot[1] in range(0, 16, 2):
                combine(prev, hv, todoc.pop(0), v)

        rb = attn_step(hv[HB + 48:2 * HB, :], sel_b, wo_b, fill_b)
        for cb in range(NCB):
            hv[2 * HB:2 * HB + 8, cb * 128:(cb + 1) * 128] = rb[cb][8:16].astype(BF16)
            sbuf[cb] = jnp.concatenate([ra[cb][8:32], rb[cb][0:8], rb[cb][16:48]], axis=0)
        assert not (todo3 or todo4 or todoc)

        @pl.when(t > 0)
        def _():
            pltpu.make_async_copy(hv.at[0:64, :], out_hbm.at[pl.ds(prev, 64), :], osem).start()

        return carry

    lax.fori_loop(0, NIT, body, 0)

    lhs4 = h3buf[S - LAG:S, :]
    last = hbuf.at[(NIT - 1) * HB:NIT * HB, :]
    c0 = 0
    for cb in range(NCB):
        w4_block(lhs4, x1buf.at[S - LAG:S, :], cb)
        combine(S - 64, last, cb)
        if cb in (3, 6, 7):
            cs = pl.ds(c0, (cb + 1) * 128 - c0)
            pltpu.make_async_copy(last.at[0:64, cs], out_hbm.at[S - 64:S, cs], osem).start()
            c0 = (cb + 1) * 128
    pltpu.make_async_copy(xbuf, out_hbm, osem).wait()


@jax.jit
def pallas_recurrent_scan__memory_aug_recurrent_mem_tr__mixer_s_mlp__prompt_kernel(
    A_x: jax.Array,
    A_mem0: jax.Array,
    A_Wq: jax.Array,
    A_Wk: jax.Array,
    A_Wv: jax.Array,
    A_Wo: jax.Array,
    A_seg_len: jax.Array,
    B_x: jax.Array,
    B_w1: jax.Array,
    B_w2: jax.Array,
    B_w3: jax.Array,
    B_w4: jax.Array,
):
    del A_seg_len, B_x
    assert A_x.shape == (1, S, D) and A_mem0.shape == (1, M, D)
    assert A_Wq.shape == (D, H, E) and A_Wo.shape == (H, E, D)
    assert B_w3.shape == (D, FF) and B_w4.shape == (FF, D)

    any_spec = pl.BlockSpec(memory_space=pl.ANY)
    out = pl.pallas_call(
        _kernel,
        out_shape=jax.ShapeDtypeStruct((S, D), BF16),
        in_specs=[any_spec] * 10,
        out_specs=any_spec,
        scratch_shapes=[
            pltpu.VMEM((S, D), BF16),
            pltpu.VMEM(((NIT + 1) * HB + 16, D), BF16),
            pltpu.VMEM((NCB, S + 16, 128), F32),
            pltpu.VMEM((S, D), BF16),
            pltpu.VMEM((S, FF), BF16),
            pltpu.VMEM((NCB, 64, 128), F32),
            pltpu.VMEM((4, 3 * PR, E), BF16),
            pltpu.VMEM(((3 * H + 1) * HS, 128), U32),
            pltpu.VMEM((D // 512, H * E, 512), BF16),
            pltpu.VMEM((D // 256, D, 256), BF16),
            pltpu.VMEM((D // 512, D, 512), BF16),
            pltpu.VMEM((FF // 512, D, 512), BF16),
            pltpu.VMEM((D // 512, FF, 512), BF16),
            pltpu.VMEM((HB, HB), F32),
            pltpu.SemaphoreType.DMA((17,)),
            pltpu.SemaphoreType.DMA(()),
        ],
        compiler_params=pltpu.CompilerParams(vmem_limit_bytes=120 * 1024 * 1024),
    )(
        A_x.reshape(S, D), A_mem0.reshape(M, D),
        A_Wq.reshape(D * H, E), A_Wk.reshape(D * H, E), A_Wv.reshape(D * H, E),
        A_Wo.reshape(H * E, D), B_w1, B_w2, B_w3, B_w4,
    )
    return out.reshape(1, S, D)
```

```python
import functools

import jax
import jax.numpy as jnp
from jax import lax
import jax.experimental.pallas as pl
import jax.experimental.pallas.tpu as pltpu

F32 = jnp.float32
BF16 = jnp.bfloat16
U32 = jnp.uint32

S = 2048
D = 1024
H = 32
E = 128
M = 8
SEG = 32
L = M + SEG
FF = 3584
NCB = D // 128
NFB = FF // 128
NP = H // 2
NIT = S // (2 * SEG)
HB = 2 * L
PRE = 512
LAG = 64
BR = (S - PRE) // NIT
HS = D // 2 + 8
RB = 256
SB = 128
HSB = (SB // 64) * HB
CH = 512
PR = 16 * CH
EPS = 1e-5
SCALE = float(E) ** -0.5
SHIFTS = (7, 7, 9, 9, 6, 6, 10, 10)


def _dot(a, b):
    return jnp.dot(a, b, preferred_element_type=F32)


def _ln(x):
    m = jnp.mean(x, axis=-1, keepdims=True)
    xc = x - m
    v = jnp.mean(xc * xc, axis=-1, keepdims=True)
    return xc * lax.rsqrt(v + EPS)


def _ln2(x):
    m = jnp.mean(x, axis=-1, keepdims=True)
    xc = x - m
    v = jnp.mean(xc * xc, axis=-1, keepdims=True)
    r1 = lax.rsqrt(v + EPS)
    r2 = lax.rsqrt(v * r1 * r1 + EPS)
    return xc * r1, xc * (r1 * r2)


def _gelu(x):
    c = 0.7978845608028654
    hx = 0.5 * x
    return hx * jnp.tanh(x * (c + (c * 0.044715) * (x * x))) + hx


def _silu(x):
    hx = 0.5 * x
    return hx * jnp.tanh(hx) + hx


def _zero_of(v):
    return (pltpu.bitcast(v, U32) >> 16) >> 16


def _or_zero(w, z):
    return pltpu.bitcast(pltpu.bitcast(w, U32) | z, w.dtype)


def _col(w, cb, k0=0, k1=None):
    _, kk, cw = w.shape
    q, r = divmod(cb * 128, cw)
    return w[q, k0:(kk if k1 is None else k1), r:r + 128]


def _hrow(r):
    q, rr = divmod(r, 64)
    return q * HB + rr + (8 if rr < 40 else 16)


def _kernel(x_hbm, mem0_hbm, wq_hbm, wk_hbm, wv_hbm, wo_hbm, w1_hbm, w2_hbm, w3_hbm, w4_hbm,
            out_hbm,
            xbuf, hbuf_all, hf, x1buf, h3buf, sbuf, stg, wqkv, wo, w1, w2, w3, w4, fillbuf,
            sem, osem):
    hbuf = hbuf_all.at[HB:, :]

    def colblock_copies(src, dst, s):
        n, _, cw = dst.shape
        return [pltpu.make_async_copy(src.at[:, pl.ds(c * cw, cw)], dst.at[c], sem.at[s(c)])
                for c in range(n)]

    xs, qs = 7, 12
    xch = [(0, SB), (SB, SB), (RB, RB), (2 * RB, RB), (3 * RB, S - 3 * RB)]
    cp_x = [pltpu.make_async_copy(x_hbm.at[pl.ds(r, n), :], xbuf.at[pl.ds(r, n), :], sem.at[xs + i])
            for i, (r, n) in enumerate(xch)]
    cp_w1 = colblock_copies(w1_hbm, w1, lambda c: (0, 1, 16, 16)[c])
    cp_mem = [pltpu.make_async_copy(mem0_hbm, hbuf.at[0:M, :], sem.at[2])]
    cp_w2 = colblock_copies(w2_hbm, w2, lambda c: 3)
    cp_w3 = colblock_copies(w3_hbm, w3, lambda c: 4)
    cp_w4 = colblock_copies(w4_hbm, w4, lambda c: 5)
    cp_wo = colblock_copies(wo_hbm, wo, lambda c: 6)
    cp_qkv = [pltpu.make_async_copy(src.at[pl.ds(k * PR, PR), :], stg.at[k, pl.ds(m * PR, PR), :],
                                    sem.at[qs + k])
              for k in range(4) for m, src in enumerate((wq_hbm, wk_hbm, wv_hbm))]

    for c in cp_x[:2] + cp_w1[:2] + cp_x[2:3] + cp_w1[2:] + cp_w2 + cp_x[3:4]:
        c.start()
    for c in cp_x[4:] + cp_mem + cp_w3 + cp_w4 + cp_qkv + cp_wo:
        c.start(priority=1)

    def wait(grp):
        for c in grp:
            c.wait()

    r = lax.broadcasted_iota(jnp.int32, (HB, HB), 0)
    c = lax.broadcasted_iota(jnp.int32, (HB, HB), 1)
    rr = jnp.where(r >= L, r - L, r)
    cc = jnp.where(c >= L, c - L, c)
    same = (r >= L) == (c >= L)
    allowed = (rr < M) | (rr >= cc)
    fillbuf[...] = jnp.where(same, jnp.where(allowed, 1.0, -1e9), -jnp.inf).astype(F32)

    hf[:, 0:8, :] = jnp.zeros((NCB, 8, 128), F32)
    hf[:, S + 8:S + 16, :] = jnp.zeros((NCB, 8, 128), F32)
    sbuf[...] = jnp.zeros(sbuf.shape, sbuf.dtype)

    def ln_sub(xv, hv, sb):
        out = []
        for u in range(SB // 16):
            r0 = sb * SB + 16 * u
            xn, xnn = _ln2(xv[r0:r0 + 16, :].astype(F32))
            xn = xn.astype(BF16)
            for hh in range(2):
                o = _hrow(r0 + 8 * hh)
                hv[o:o + 8, :] = xn[8 * hh:8 * hh + 8]
            out.append(xnn.astype(BF16))
        return out

    def after(w, vals):
        if not vals:
            return w
        z = functools.reduce(lambda a, b: a | b, [_zero_of(v[0:16, D - 128:D]) for v in vals])
        return jnp.concatenate([_or_zero(w[0:16, :], z), w[16:, :]], axis=0)

    def w1_sub(xnn, hfv, sb, cbs, deps):
        xnn = jnp.concatenate(xnn, axis=0)
        for cb in cbs:
            w = after(_col(w1, cb), deps.get(cb, []))
            hfv[cb, sb * SB + 8:sb * SB + 8 + SB, :] = _gelu(_dot(xnn, w))

    def w2_lhs(hfv, sb):
        r0 = sb * SB
        return jnp.concatenate(
            [hfv[cb, r0 + SHIFTS[cb]:r0 + SHIFTS[cb] + SB, :] for cb in range(NCB)],
            axis=1).astype(BF16)

    def w2_sub(hs, hv, x1v, sb, cbs, deps, hook=None):
        r0 = sb * SB
        for cb in cbs:
            pre = _dot(hs, after(_col(w2, cb), deps.get(cb, [])))
            cs = slice(cb * 128, (cb + 1) * 128)
            xn = jnp.concatenate(
                [hv[_hrow(r0 + a):_hrow(r0 + a) + n, cs].astype(F32)
                 for a, n in ((0, 40), (40, 24), (64, 40), (104, 24))], axis=0)
            x1v[r0:r0 + SB, cs] = (xn + pre).astype(BF16)
            if hook is not None:
                hook(pre)

    def w3_lhs(x1v, r0, rows):
        return [_ln(x1v[r0 + 16 * u:r0 + 16 * u + 16, :].astype(F32)).astype(BF16)
                for u in range(rows // 16)]

    def w3_block(lhs, h3v, r0, f):
        pre = _dot(lhs, _col(w3, f))
        h3v[r0:r0 + lhs.shape[0], f * 128:(f + 1) * 128] = _gelu(pre).astype(BF16)
        return pre

    def w4_block(lhs, x1v, cb, ks=(0, FF), hook=None):
        pre = None
        for k0, k1 in zip(ks[:-1], ks[1:]):
            part = _dot(lhs[:, k0:k1], _col(w4, cb, k0, k1))
            pre = part if pre is None else part + pre
            if hook is not None:
                hook(pre)
        sl = (slice(0, lhs.shape[0]), slice(cb * 128, (cb + 1) * 128))
        x1v[sl] = _silu(x1v[sl].astype(F32) + pre).astype(BF16)

    def relayout(src, dst, u, trig):
        m, c_ = divmod(u, 16)
        d0 = m * (H * HS) + c_ * 8
        two = lambda v: jnp.concatenate([v, v], axis=0)
        for pp in range(8):
            r0 = u * CH + pp * 64
            tr = (pp * trig.shape[0] // 64) * 8
            z = _zero_of(trig[tr:tr + 8, :])
            mlo, mhi, sh = two(z | U32(0xFFFF)), two(z | U32(0xFFFF0000)), two(z | U32(16))
            a = pltpu.bitcast(src[r0:r0 + 32, :], U32)
            b = pltpu.bitcast(src[r0 + 32:r0 + 64, :], U32)
            dst[pl.ds(d0 + pp, 16, stride=HS), :] = (a & mlo) | (b << sh)
            dst[pl.ds(d0 + 16 * HS + pp, 16, stride=HS), :] = (a >> sh) | (b & mhi)

    cp_x[0].wait()
    xnn0 = ln_sub(xbuf, hbuf, 0)
    cp_x[1].wait()
    xnn1 = ln_sub(xbuf, hbuf, 1)
    cp_w1[0].wait()
    w1_sub(xnn0, hf, 0, range(0, 2), {})
    w1_sub(xnn1, hf, 1, range(0, 2), {})
    cp_w1[1].wait()
    w1_sub(xnn0, hf, 0, range(2, 4), {})
    cp_x[2].wait()
    xnn2 = ln_sub(xbuf, hbuf, 2)
    w1_sub(xnn1, hf, 1, range(2, 4), {})
    w1_sub(xnn2, hf, 2, range(0, 4), {})
    wait(cp_w1[2:])
    xnn3 = ln_sub(xbuf, hbuf, 3)
    w1_sub(xnn0, hf, 0, range(4, 8), {6: xnn3[0:1], 7: xnn3[1:2]})
    w1_sub(xnn1, hf, 1, range(4, 8), {4 + i: xnn3[2 + i:3 + i] for i in range(4)})
    w1_sub(xnn2, hf, 2, range(4, 8), {4: xnn3[6:7], 5: xnn3[7:8]})
    w1_sub(xnn3, hf, 3, range(NCB), {})
    wait(cp_w2)
    cp_x[3].wait()

    def loop_w12(i, carry):
        @pl.when(i == 3)
        def _():
            cp_x[4].wait()

        r0 = pl.multiple_of((i - 2) * RB, RB)
        xv = xbuf.at[pl.ds(r0, 3 * RB), :]
        hv = hbuf.at[pl.ds(pl.multiple_of((i - 2) * 2 * HSB, 16), 6 * HSB), :]
        x1v = x1buf.at[pl.ds(r0, RB), :]
        hfv = hf.at[:, pl.ds(r0, 3 * RB + 16), :]
        for sb in range(2):
            c = ln_sub(xv, hv, 4 + sb)
            deps = {2: c[0:1], 3: c[1:2], 4: c[2:4], 5: c[4:5], 6: c[5:7], 7: c[7:8]}
            w2_sub(w2_lhs(hfv, sb), hv, x1v, sb, range(NCB), deps)
            w1_sub(c, hfv, 4 + sb, range(NCB), {})
        return carry

    lax.fori_loop(2, S // RB, loop_w12, 0)
    wait(cp_w3)
    wait(cp_w4)

    def loop_w34(k, carry):
        pltpu.make_async_copy(stg.at[k], stg.at[k], sem.at[qs + k]).wait()
        r0 = pl.multiple_of(k * SB, SB)
        src = stg.at[k]
        dst = wqkv.at[pl.ds(pl.multiple_of(k * 128, 128), (3 * H + 1) * HS - 384), :]
        sb2 = (S - PRE) // SB
        x1v = x1buf.at[pl.ds(r0, (sb2 + 1) * SB), :]
        hv = hbuf.at[pl.ds(pl.multiple_of(k * HSB, 16), (sb2 + 1) * HSB), :]
        hfv = hf.at[:, pl.ds(r0, (sb2 + 1) * SB + 16), :]
        todo = list(range(3 * PR // CH))

        def rl(trig):
            if todo:
                relayout(src, dst, todo.pop(0), trig)

        hs = w2_lhs(hfv, sb2)
        c = w3_lhs(x1v, 0, SB)
        w2_sub(hs, hv, x1v, sb2, range(0, 6), {3: c[0:2], 4: c[2:4], 5: c[4:6]})
        lhs3 = jnp.concatenate(c, axis=0)
        h3v = h3buf.at[pl.ds(r0, SB), :]
        for f in range(NFB):
            rl(w3_block(lhs3, h3v, 0, f))
        w2_sub(hs, hv, x1v, sb2, range(6, 8), {}, rl)
        n4 = (PRE - LAG) // 4
        r4 = pl.multiple_of(k * n4, 16)
        lhs4 = h3buf[pl.ds(r4, n4), :]
        for cb in range(NCB):
            w4_block(lhs4, x1buf.at[pl.ds(r4, n4), :], cb, (0, 1024, 2048, FF), rl)
        assert not todo
        return carry

    lax.fori_loop(0, PRE // SB, loop_w34, 0)
    wait(cp_wo)
    wait(cp_mem)

    def softmax(s):
        fill = fillbuf[...]
        s = jnp.where(fill > 0.0, s * SCALE, fill)
        mx = jnp.max(s, axis=1, keepdims=True)
        e = jnp.exp(s - mx)
        l = jnp.sum(e, axis=1, keepdims=True)
        rc = pl.reciprocal(l, approx=True)
        rc = rc * (2.0 - l * rc)
        return (e * rc).astype(BF16)

    def attn_step(lhs, select, wo_rows, fill):
        qkv = [None] * NP
        p = [None] * NP
        oh = [None] * H
        acc = [None] * NCB
        wsplit = (0, 8, 20, 28, 32)

        def do_qkv(j):
            rs = []
            for i in range(6):
                h = 2 * j + i // 3
                r0 = ((i % 3) * H + (h % 2) * 16 + h // 2) * HS
                v = _dot(lhs, pltpu.bitcast(wqkv[r0:r0 + D // 2, :], BF16))
                fill(("qkv", 6 * j + i), v)
                rs.append(select(j, i, v))
            qkv[j] = [jnp.concatenate([rs[i], rs[3 + i]], axis=0).astype(BF16) for i in range(3)]

        def do_s(j):
            p[j] = softmax(lax.dot_general(qkv[j][0], qkv[j][1], (((1,), (1,)), ((), ())),
                                           preferred_element_type=F32))

        def do_pv(j):
            o = _dot(p[j], qkv[j][2])
            oh[2 * j] = wo_rows(2 * j, o[0:L]).astype(BF16)
            oh[2 * j + 1] = wo_rows(2 * j + 1, o[L:2 * L]).astype(BF16)

        def do_wo(n):
            h0, h1 = wsplit[n], wsplit[n + 1]
            lo = jnp.concatenate(oh[h0:h1], axis=1)
            for cb in range(NCB):
                part = _dot(lo, _col(wo, cb, h0 * E, h1 * E))
                acc[cb] = part if acc[cb] is None else part + acc[cb]
                fill(("wo", n * NCB + cb), part)

        for j in range(NP + 2):
            if j < NP:
                do_qkv(j)
            else:
                do_wo(j - NP)
            if 0 <= j - 2 < NP:
                do_pv(j - 2)
            if 0 <= j - 1 < NP:
                do_s(j - 1)
        do_wo(2)
        do_wo(3)
        return acc

    def combine(r0, dst, cb, trig=None):
        cs = slice(cb * 128, (cb + 1) * 128)
        xx, gg = xbuf[pl.ds(r0, 64), cs], x1buf[pl.ds(r0, 64), cs]
        if trig is not None:
            z = jnp.concatenate([_zero_of(trig[0:8, :])] * 4, axis=0)
            xx, gg = _or_zero(xx, z), _or_zero(gg, z)
        dst[0:64, cs] = (xx.astype(F32) + sbuf[cb] * gg.astype(F32)).astype(BF16)

    def body(t, carry):
        hv = hbuf_all.at[pl.ds(pl.multiple_of(t * HB, 16), 2 * HB + 16), :]
        prev = pl.multiple_of(jnp.maximum(t - 1, 0) * 64, 64)
        b4 = pl.multiple_of(PRE - LAG + t * BR, 16)
        x1v = x1buf.at[pl.ds(b4, LAG + BR), :]
        h3v = h3buf.at[pl.ds(b4, LAG + BR), :]
        lhs3 = jnp.concatenate(w3_lhs(x1v, LAG, BR), axis=0)
        lhs4 = h3v[0:BR, :]
        todo3, todo4, todoc = list(range(NFB)), list(range(NCB)), list(range(NCB))

        keep = {}

        def sel_a(j, i, v):
            keep[(j, i)] = v[L:L + 8]
            return v[0:L]

        def wo_a(h, o):
            keep[h] = o[32:40]
            return o[0:32]

        def fill_a(slot, v):
            if slot[0] == "wo" and slot[1] in (1, 5, 10, 14, 18, 22):
                w4_block(lhs4, x1v, todo4.pop(0))

        ra = attn_step(hv[HB:HB + 48, :], sel_a, wo_a, fill_a)
        for cb in range(NCB):
            hv[HB + 48:HB + 56, cb * 128:(cb + 1) * 128] = ra[cb][0:8].astype(BF16)
        while todo4:
            w4_block(lhs4, x1v, todo4.pop(0))

        def sel_b(j, i, v):
            return jnp.concatenate([v[0:8], keep[(j, i)], v[8:32]], axis=0)

        def wo_b(h, o):
            return jnp.concatenate([keep[h], o], axis=0)

        w3_slots = [(i * 96) // NFB + 2 for i in range(NFB)]

        def fill_b(slot, v):
            if slot[0] == "qkv" and slot[1] in w3_slots:
                w3_block(lhs3, h3v, LAG, todo3.pop(0))
            if slot[0] == "wo" and slot[1] in range(0, 8):
                combine(prev, hv, todoc.pop(0), v)
                if not todoc:
                    @pl.when(t > 0)
                    def _():
                        pltpu.make_async_copy(hv.at[0:64, :], out_hbm.at[pl.ds(prev, 64), :],
                                              osem).start()

        rb = attn_step(hv[HB + 48:2 * HB, :], sel_b, wo_b, fill_b)
        for cb in range(NCB):
            hv[2 * HB:2 * HB + 8, cb * 128:(cb + 1) * 128] = rb[cb][8:16].astype(BF16)
            sbuf[cb] = jnp.concatenate([ra[cb][8:32], rb[cb][0:8], rb[cb][16:48]], axis=0)
        assert not (todo3 or todo4 or todoc)
        return carry

    lax.fori_loop(0, NIT, body, 0)

    lhs4 = h3buf[S - LAG:S, :]
    last = hbuf.at[(NIT - 1) * HB:NIT * HB, :]
    c0 = 0
    for cb in range(NCB):
        w4_block(lhs4, x1buf.at[S - LAG:S, :], cb)
        combine(S - 64, last, cb)
        if cb in (3, 6, 7):
            cs = pl.ds(c0, (cb + 1) * 128 - c0)
            pltpu.make_async_copy(last.at[0:64, cs], out_hbm.at[S - 64:S, cs], osem).start()
            c0 = (cb + 1) * 128
    pltpu.make_async_copy(xbuf, out_hbm, osem).wait()


@jax.jit
def pallas_recurrent_scan__memory_aug_recurrent_mem_tr__mixer_s_mlp__prompt_kernel(
    A_x: jax.Array,
    A_mem0: jax.Array,
    A_Wq: jax.Array,
    A_Wk: jax.Array,
    A_Wv: jax.Array,
    A_Wo: jax.Array,
    A_seg_len: jax.Array,
    B_x: jax.Array,
    B_w1: jax.Array,
    B_w2: jax.Array,
    B_w3: jax.Array,
    B_w4: jax.Array,
):
    del A_seg_len, B_x
    assert A_x.shape == (1, S, D) and A_mem0.shape == (1, M, D)
    assert A_Wq.shape == (D, H, E) and A_Wo.shape == (H, E, D)
    assert B_w3.shape == (D, FF) and B_w4.shape == (FF, D)

    any_spec = pl.BlockSpec(memory_space=pl.ANY)
    out = pl.pallas_call(
        _kernel,
        out_shape=jax.ShapeDtypeStruct((S, D), BF16),
        in_specs=[any_spec] * 10,
        out_specs=any_spec,
        scratch_shapes=[
            pltpu.VMEM((S, D), BF16),
            pltpu.VMEM(((NIT + 1) * HB + 16, D), BF16),
            pltpu.VMEM((NCB, S + 16, 128), F32),
            pltpu.VMEM((S, D), BF16),
            pltpu.VMEM((S, FF), BF16),
            pltpu.VMEM((NCB, 64, 128), F32),
            pltpu.VMEM((4, 3 * PR, E), BF16),
            pltpu.VMEM(((3 * H + 1) * HS, 128), U32),
            pltpu.VMEM((D // 512, H * E, 512), BF16),
            pltpu.VMEM((D // 256, D, 256), BF16),
            pltpu.VMEM((D // 512, D, 512), BF16),
            pltpu.VMEM((FF // 512, D, 512), BF16),
            pltpu.VMEM((D // 512, FF, 512), BF16),
            pltpu.VMEM((HB, HB), F32),
            pltpu.SemaphoreType.DMA((17,)),
            pltpu.SemaphoreType.DMA(()),
        ],
        compiler_params=pltpu.CompilerParams(vmem_limit_bytes=120 * 1024 * 1024),
    )(
        A_x.reshape(S, D), A_mem0.reshape(M, D),
        A_Wq.reshape(D * H, E), A_Wk.reshape(D * H, E), A_Wv.reshape(D * H, E),
        A_Wo.reshape(H * E, D), B_w1, B_w2, B_w3, B_w4,
    )
    return out.reshape(1, S, D)
```

```python
import functools

import jax
import jax.numpy as jnp
from jax import lax
import jax.experimental.pallas as pl
import jax.experimental.pallas.tpu as pltpu

F32 = jnp.float32
BF16 = jnp.bfloat16
U32 = jnp.uint32

S = 2048
D = 1024
H = 32
E = 128
M = 8
SEG = 32
L = M + SEG
FF = 3584
NCB = D // 128
NFB = FF // 128
NP = H // 2
NIT = S // (2 * SEG)
HB = 2 * L
PRE = 512
LAG = 64
BR = (S - PRE) // NIT
HS = D // 2 + 8
RB = 256
SB = 128
HSB = (SB // 64) * HB
CH = 512
PR = 16 * CH
EPS = 1e-5
SCALE = float(E) ** -0.5
SHIFTS = (7, 7, 9, 9, 6, 6, 10, 10)


def _dot(a, b):
    return jnp.dot(a, b, preferred_element_type=F32)


def _ln(x):
    m = jnp.mean(x, axis=-1, keepdims=True)
    xc = x - m
    v = jnp.mean(xc * xc, axis=-1, keepdims=True)
    return xc * lax.rsqrt(v + EPS)


def _ln2(x):
    m = jnp.mean(x, axis=-1, keepdims=True)
    xc = x - m
    v = jnp.mean(xc * xc, axis=-1, keepdims=True)
    r1 = lax.rsqrt(v + EPS)
    r2 = lax.rsqrt(v * r1 * r1 + EPS)
    return xc * r1, xc * (r1 * r2)


def _gelu(x):
    c = 0.7978845608028654
    hx = 0.5 * x
    return hx * jnp.tanh(x * (c + (c * 0.044715) * (x * x))) + hx


def _silu(x):
    hx = 0.5 * x
    return hx * jnp.tanh(hx) + hx


def _zero_of(v):
    return (pltpu.bitcast(v, U32) >> 16) >> 16


def _or_zero(w, z):
    return pltpu.bitcast(pltpu.bitcast(w, U32) | z, w.dtype)


def _col(w, cb, k0=0, k1=None):
    _, kk, cw = w.shape
    q, r = divmod(cb * 128, cw)
    return w[q, k0:(kk if k1 is None else k1), r:r + 128]


def _hrow(r):
    q, rr = divmod(r, 64)
    return q * HB + rr + (8 if rr < 40 else 16)


def _kernel(x_hbm, mem0_hbm, wq_hbm, wk_hbm, wv_hbm, wo_hbm, w1_hbm, w2_hbm, w3_hbm, w4_hbm,
            out_hbm,
            xbuf, hbuf_all, hf, x1buf, h3buf, sbuf, stg, wqkv, wo, w1, w2, w3, w4, fillbuf,
            sem, osem):
    hbuf = hbuf_all.at[HB:, :]

    def colblock_copies(src, dst, s):
        n, _, cw = dst.shape
        return [pltpu.make_async_copy(src.at[:, pl.ds(c * cw, cw)], dst.at[c], sem.at[s(c)])
                for c in range(n)]

    xs, qs = 7, 12
    xch = [(0, SB), (SB, SB), (RB, RB), (2 * RB, RB), (3 * RB, S - 3 * RB)]
    cp_x = [pltpu.make_async_copy(x_hbm.at[pl.ds(r, n), :], xbuf.at[pl.ds(r, n), :], sem.at[xs + i])
            for i, (r, n) in enumerate(xch)]
    cp_w1 = colblock_copies(w1_hbm, w1, lambda c: (0, 1, 16, 16)[c])
    cp_mem = [pltpu.make_async_copy(mem0_hbm, hbuf.at[0:M, :], sem.at[2])]
    cp_w2 = colblock_copies(w2_hbm, w2, lambda c: 3)
    cp_w3 = colblock_copies(w3_hbm, w3, lambda c: 4)
    cp_w4 = colblock_copies(w4_hbm, w4, lambda c: 5)
    cp_wo = colblock_copies(wo_hbm, wo, lambda c: 6)
    cp_qkv = [pltpu.make_async_copy(src.at[pl.ds(k * PR, PR), :], stg.at[k, pl.ds(m * PR, PR), :],
                                    sem.at[qs + k])
              for k in range(4) for m, src in enumerate((wq_hbm, wk_hbm, wv_hbm))]

    for c in cp_x[:2] + cp_w1[:2] + cp_x[2:3] + cp_w1[2:] + cp_w2 + cp_x[3:4]:
        c.start()
    for c in cp_x[4:] + cp_mem + cp_w3 + cp_w4 + cp_qkv + cp_wo:
        c.start(priority=1)

    def wait(grp):
        for c in grp:
            c.wait()

    r = lax.broadcasted_iota(jnp.int32, (HB, HB), 0)
    c = lax.broadcasted_iota(jnp.int32, (HB, HB), 1)
    rr = jnp.where(r >= L, r - L, r)
    cc = jnp.where(c >= L, c - L, c)
    same = (r >= L) == (c >= L)
    allowed = (rr < M) | (rr >= cc)
    fillbuf[...] = jnp.where(same, jnp.where(allowed, 1.0, -1e9), -jnp.inf).astype(F32)

    hf[:, 0:8, :] = jnp.zeros((NCB, 8, 128), F32)
    hf[:, S + 8:S + 16, :] = jnp.zeros((NCB, 8, 128), F32)
    sbuf[...] = jnp.zeros(sbuf.shape, sbuf.dtype)

    def ln_sub(xv, hv, sb):
        out = []
        for u in range(SB // 16):
            r0 = sb * SB + 16 * u
            xn, xnn = _ln2(xv[r0:r0 + 16, :].astype(F32))
            xn = xn.astype(BF16)
            for hh in range(2):
                o = _hrow(r0 + 8 * hh)
                hv[o:o + 8, :] = xn[8 * hh:8 * hh + 8]
            out.append(xnn.astype(BF16))
        return out

    def after(w, vals):
        if not vals:
            return w
        z = functools.reduce(lambda a, b: a | b, [_zero_of(v[0:16, D - 128:D]) for v in vals])
        return jnp.concatenate([_or_zero(w[0:16, :], z), w[16:, :]], axis=0)

    def w1_sub(xnn, hfv, sb, cbs, deps):
        xnn = jnp.concatenate(xnn, axis=0)
        for cb in cbs:
            w = after(_col(w1, cb), deps.get(cb, []))
            hfv[cb, sb * SB + 8:sb * SB + 8 + SB, :] = _gelu(_dot(xnn, w))

    def w2_lhs(hfv, sb):
        r0 = sb * SB
        return jnp.concatenate(
            [hfv[cb, r0 + SHIFTS[cb]:r0 + SHIFTS[cb] + SB, :] for cb in range(NCB)],
            axis=1).astype(BF16)

    def w2_sub(hs, hv, x1v, sb, cbs, deps, hook=None):
        r0 = sb * SB
        for cb in cbs:
            pre = _dot(hs, after(_col(w2, cb), deps.get(cb, [])))
            cs = slice(cb * 128, (cb + 1) * 128)
            xn = jnp.concatenate(
                [hv[_hrow(r0 + a):_hrow(r0 + a) + n, cs].astype(F32)
                 for a, n in ((0, 40), (40, 24), (64, 40), (104, 24))], axis=0)
            x1v[r0:r0 + SB, cs] = (xn + pre).astype(BF16)
            if hook is not None:
                hook(pre)

    def w3_lhs(x1v, r0, rows):
        return [_ln(x1v[r0 + 16 * u:r0 + 16 * u + 16, :].astype(F32)).astype(BF16)
                for u in range(rows // 16)]

    def w3_block(lhs, h3v, r0, f):
        pre = _dot(lhs, _col(w3, f))
        h3v[r0:r0 + lhs.shape[0], f * 128:(f + 1) * 128] = _gelu(pre).astype(BF16)
        return pre

    def w4_block(lhs, x1v, cb, ks=(0, FF), hook=None):
        pre = None
        for k0, k1 in zip(ks[:-1], ks[1:]):
            part = _dot(lhs[:, k0:k1], _col(w4, cb, k0, k1))
            pre = part if pre is None else part + pre
            if hook is not None:
                hook(pre)
        sl = (slice(0, lhs.shape[0]), slice(cb * 128, (cb + 1) * 128))
        x1v[sl] = _silu(x1v[sl].astype(F32) + pre).astype(BF16)

    def relayout(src, dst, u, trig):
        m, c_ = divmod(u, 16)
        d0 = m * (H * HS) + c_ * 8
        two = lambda v: jnp.concatenate([v, v], axis=0)
        for pp in range(8):
            r0 = u * CH + pp * 64
            tr = (pp * trig.shape[0] // 64) * 8
            z = _zero_of(trig[tr:tr + 8, :])
            mlo, mhi, sh = two(z | U32(0xFFFF)), two(z | U32(0xFFFF0000)), two(z | U32(16))
            a = pltpu.bitcast(src[r0:r0 + 32, :], U32)
            b = pltpu.bitcast(src[r0 + 32:r0 + 64, :], U32)
            dst[pl.ds(d0 + pp, 16, stride=HS), :] = (a & mlo) | (b << sh)
            dst[pl.ds(d0 + 16 * HS + pp, 16, stride=HS), :] = (a >> sh) | (b & mhi)

    cp_x[0].wait()
    xnn0 = ln_sub(xbuf, hbuf, 0)
    cp_x[1].wait()
    xnn1 = ln_sub(xbuf, hbuf, 1)
    cp_w1[0].wait()
    w1_sub(xnn0, hf, 0, range(0, 2), {})
    w1_sub(xnn1, hf, 1, range(0, 2), {})
    cp_w1[1].wait()
    w1_sub(xnn0, hf, 0, range(2, 4), {})
    cp_x[2].wait()
    xnn2 = ln_sub(xbuf, hbuf, 2)
    w1_sub(xnn1, hf, 1, range(2, 4), {})
    w1_sub(xnn2, hf, 2, range(0, 4), {})
    wait(cp_w1[2:])
    xnn3 = ln_sub(xbuf, hbuf, 3)
    w1_sub(xnn0, hf, 0, range(4, 8), {6: xnn3[0:1], 7: xnn3[1:2]})
    w1_sub(xnn1, hf, 1, range(4, 8), {4 + i: xnn3[2 + i:3 + i] for i in range(4)})
    w1_sub(xnn2, hf, 2, range(4, 8), {4: xnn3[6:7], 5: xnn3[7:8]})
    w1_sub(xnn3, hf, 3, range(NCB), {})
    wait(cp_w2)
    cp_x[3].wait()

    def loop_w12(i, carry):
        @pl.when(i == 3)
        def _():
            cp_x[4].wait()

        r0 = pl.multiple_of((i - 2) * RB, RB)
        xv = xbuf.at[pl.ds(r0, 3 * RB), :]
        hv = hbuf.at[pl.ds(pl.multiple_of((i - 2) * 2 * HSB, 16), 6 * HSB), :]
        x1v = x1buf.at[pl.ds(r0, RB), :]
        hfv = hf.at[:, pl.ds(r0, 3 * RB + 16), :]
        spread = lambda c: {2: c[0:1], 3: c[1:2], 4: c[2:4], 5: c[4:5], 6: c[5:7], 7: c[7:8]}
        ca, cb_ = ln_sub(xv, hv, 4), ln_sub(xv, hv, 5)
        w2_sub(w2_lhs(hfv, 0), hv, x1v, 0, range(NCB), spread(ca))
        w1_sub(ca, hfv, 4, range(NCB), spread(cb_))
        w1_sub(cb_, hfv, 5, range(NCB), {})
        w2_sub(w2_lhs(hfv, 1), hv, x1v, 1, range(NCB), {})
        return carry

    lax.fori_loop(2, S // RB, loop_w12, 0)
    wait(cp_w3)
    wait(cp_w4)

    def loop_w34(k, carry):
        pltpu.make_async_copy(stg.at[k], stg.at[k], sem.at[qs + k]).wait()
        r0 = pl.multiple_of(k * SB, SB)
        src = stg.at[k]
        dst = wqkv.at[pl.ds(pl.multiple_of(k * 128, 128), (3 * H + 1) * HS - 384), :]
        sb2 = (S - PRE) // SB
        x1v = x1buf.at[pl.ds(r0, (sb2 + 1) * SB), :]
        hv = hbuf.at[pl.ds(pl.multiple_of(k * HSB, 16), (sb2 + 1) * HSB), :]
        hfv = hf.at[:, pl.ds(r0, (sb2 + 1) * SB + 16), :]
        todo = list(range(3 * PR // CH))

        def rl(trig):
            if todo:
                relayout(src, dst, todo.pop(0), trig)

        hs = w2_lhs(hfv, sb2)
        c = w3_lhs(x1v, 0, SB)
        w2_sub(hs, hv, x1v, sb2, range(0, 6), {3: c[0:2], 4: c[2:4], 5: c[4:6]})
        lhs3 = jnp.concatenate(c, axis=0)
        h3v = h3buf.at[pl.ds(r0, SB), :]
        for f in range(NFB):
            rl(w3_block(lhs3, h3v, 0, f))
        w2_sub(hs, hv, x1v, sb2, range(6, 7), {}, rl)
        n4 = (PRE - LAG) // 4
        r4 = pl.multiple_of(k * n4, 16)
        lhs4 = h3buf[pl.ds(r4, n4), :]
        for cb in range(NCB):
            w4_block(lhs4, x1buf.at[pl.ds(r4, n4), :], cb, (0, 1024, 2048, FF), rl)
        w2_sub(hs, hv, x1v, sb2, range(7, 8), {})
        assert not todo
        return carry

    lax.fori_loop(0, PRE // SB, loop_w34, 0)
    wait(cp_wo)
    wait(cp_mem)

    def softmax(s):
        fill = fillbuf[...]
        s = jnp.where(fill > 0.0, s * SCALE, fill)
        mx = jnp.max(s, axis=1, keepdims=True)
        e = jnp.exp(s - mx)
        l = jnp.sum(e, axis=1, keepdims=True)
        rc = pl.reciprocal(l, approx=True)
        rc = rc * (2.0 - l * rc)
        return (e * rc).astype(BF16)

    def attn_step(lhs, select, wo_rows, fill):
        qkv = [None] * NP
        p = [None] * NP
        oh = [None] * H
        acc = [None] * NCB
        wsplit = (0, 8, 20, 28, 32)

        def do_qkv(j):
            rs = []
            for i in range(6):
                h = 2 * j + i // 3
                r0 = ((i % 3) * H + (h % 2) * 16 + h // 2) * HS
                v = _dot(lhs, pltpu.bitcast(wqkv[r0:r0 + D // 2, :], BF16))
                fill(("qkv", 6 * j + i), v)
                rs.append(select(j, i, v))
            qkv[j] = [jnp.concatenate([rs[i], rs[3 + i]], axis=0).astype(BF16) for i in range(3)]

        def do_s(j):
            p[j] = softmax(lax.dot_general(qkv[j][0], qkv[j][1], (((1,), (1,)), ((), ())),
                                           preferred_element_type=F32))

        def do_pv(j):
            o = _dot(p[j], qkv[j][2])
            oh[2 * j] = wo_rows(2 * j, o[0:L]).astype(BF16)
            oh[2 * j + 1] = wo_rows(2 * j + 1, o[L:2 * L]).astype(BF16)

        def do_wo(n):
            h0, h1 = wsplit[n], wsplit[n + 1]
            lo = jnp.concatenate(oh[h0:h1], axis=1)
            for cb in range(NCB):
                part = _dot(lo, _col(wo, cb, h0 * E, h1 * E))
                acc[cb] = part if acc[cb] is None else part + acc[cb]
                fill(("wo", n * NCB + cb), part)

        for j in range(NP + 2):
            if j < NP:
                do_qkv(j)
            else:
                do_wo(j - NP)
            if 0 <= j - 2 < NP:
                do_pv(j - 2)
            if 0 <= j - 1 < NP:
                do_s(j - 1)
        do_wo(2)
        do_wo(3)
        return acc

    def combine(r0, dst, cb, trig=None):
        cs = slice(cb * 128, (cb + 1) * 128)
        xx, gg = xbuf[pl.ds(r0, 64), cs], x1buf[pl.ds(r0, 64), cs]
        if trig is not None:
            z = jnp.concatenate([_zero_of(trig[0:8, :])] * 4, axis=0)
            xx, gg = _or_zero(xx, z), _or_zero(gg, z)
        dst[0:64, cs] = (xx.astype(F32) + sbuf[cb] * gg.astype(F32)).astype(BF16)

    def body(t, carry):
        hv = hbuf_all.at[pl.ds(pl.multiple_of(t * HB, 16), 2 * HB + 16), :]
        prev = pl.multiple_of(jnp.maximum(t - 1, 0) * 64, 64)
        b4 = pl.multiple_of(PRE - LAG + t * BR, 16)
        x1v = x1buf.at[pl.ds(b4, LAG + BR), :]
        h3v = h3buf.at[pl.ds(b4, LAG + BR), :]
        lhs3 = jnp.concatenate(w3_lhs(x1v, LAG, BR), axis=0)
        lhs4 = h3v[0:BR, :]
        todo3, todo4, todoc = list(range(NFB)), list(range(NCB)), list(range(NCB))

        keep = {}

        def sel_a(j, i, v):
            keep[(j, i)] = v[L:L + 8]
            return v[0:L]

        def wo_a(h, o):
            keep[h] = o[32:40]
            return o[0:32]

        def fill_a(slot, v):
            if slot[0] == "wo" and slot[1] in (1, 5, 10, 14, 18, 22):
                w4_block(lhs4, x1v, todo4.pop(0))

        ra = attn_step(hv[HB:HB + 48, :], sel_a, wo_a, fill_a)
        for cb in range(NCB):
            hv[HB + 48:HB + 56, cb * 128:(cb + 1) * 128] = ra[cb][0:8].astype(BF16)
        while todo4:
            w4_block(lhs4, x1v, todo4.pop(0))

        def sel_b(j, i, v):
            return jnp.concatenate([v[0:8], keep[(j, i)], v[8:32]], axis=0)

        def wo_b(h, o):
            return jnp.concatenate([keep[h], o], axis=0)

        w3_slots = [(i * 96) // NFB + 2 for i in range(NFB)]

        def fill_b(slot, v):
            if slot[0] == "qkv" and slot[1] in w3_slots:
                w3_block(lhs3, h3v, LAG, todo3.pop(0))
            if slot[0] == "wo" and slot[1] in range(0, 8):
                combine(prev, hv, todoc.pop(0), v)
                if not todoc:
                    @pl.when(t > 0)
                    def _():
                        pltpu.make_async_copy(hv.at[0:64, :], out_hbm.at[pl.ds(prev, 64), :],
                                              osem).start()

        rb = attn_step(hv[HB + 48:2 * HB, :], sel_b, wo_b, fill_b)
        for cb in range(NCB):
            hv[2 * HB:2 * HB + 8, cb * 128:(cb + 1) * 128] = rb[cb][8:16].astype(BF16)
            sbuf[cb] = jnp.concatenate([ra[cb][8:32], rb[cb][0:8], rb[cb][16:48]], axis=0)
        assert not (todo3 or todo4 or todoc)
        return carry

    lax.fori_loop(0, NIT, body, 0)

    lhs4 = h3buf[S - LAG:S, :]
    last = hbuf.at[(NIT - 1) * HB:NIT * HB, :]
    c0 = 0
    for cb in range(NCB):
        w4_block(lhs4, x1buf.at[S - LAG:S, :], cb)
        combine(S - 64, last, cb)
        if cb in (3, 6, 7):
            cs = pl.ds(c0, (cb + 1) * 128 - c0)
            pltpu.make_async_copy(last.at[0:64, cs], out_hbm.at[S - 64:S, cs], osem).start()
            c0 = (cb + 1) * 128
    pltpu.make_async_copy(xbuf, out_hbm, osem).wait()


@jax.jit
def pallas_recurrent_scan__memory_aug_recurrent_mem_tr__mixer_s_mlp__prompt_kernel(
    A_x: jax.Array,
    A_mem0: jax.Array,
    A_Wq: jax.Array,
    A_Wk: jax.Array,
    A_Wv: jax.Array,
    A_Wo: jax.Array,
    A_seg_len: jax.Array,
    B_x: jax.Array,
    B_w1: jax.Array,
    B_w2: jax.Array,
    B_w3: jax.Array,
    B_w4: jax.Array,
):
    del A_seg_len, B_x
    assert A_x.shape == (1, S, D) and A_mem0.shape == (1, M, D)
    assert A_Wq.shape == (D, H, E) and A_Wo.shape == (H, E, D)
    assert B_w3.shape == (D, FF) and B_w4.shape == (FF, D)

    any_spec = pl.BlockSpec(memory_space=pl.ANY)
    out = pl.pallas_call(
        _kernel,
        out_shape=jax.ShapeDtypeStruct((S, D), BF16),
        in_specs=[any_spec] * 10,
        out_specs=any_spec,
        scratch_shapes=[
            pltpu.VMEM((S, D), BF16),
            pltpu.VMEM(((NIT + 1) * HB + 16, D), BF16),
            pltpu.VMEM((NCB, S + 16, 128), F32),
            pltpu.VMEM((S, D), BF16),
            pltpu.VMEM((S, FF), BF16),
            pltpu.VMEM((NCB, 64, 128), F32),
            pltpu.VMEM((4, 3 * PR, E), BF16),
            pltpu.VMEM(((3 * H + 1) * HS, 128), U32),
            pltpu.VMEM((D // 512, H * E, 512), BF16),
            pltpu.VMEM((D // 256, D, 256), BF16),
            pltpu.VMEM((D // 512, D, 512), BF16),
            pltpu.VMEM((FF // 512, D, 512), BF16),
            pltpu.VMEM((D // 512, FF, 512), BF16),
            pltpu.VMEM((HB, HB), F32),
            pltpu.SemaphoreType.DMA((17,)),
            pltpu.SemaphoreType.DMA(()),
        ],
        compiler_params=pltpu.CompilerParams(vmem_limit_bytes=120 * 1024 * 1024),
    )(
        A_x.reshape(S, D), A_mem0.reshape(M, D),
        A_Wq.reshape(D * H, E), A_Wk.reshape(D * H, E), A_Wv.reshape(D * H, E),
        A_Wo.reshape(H * E, D), B_w1, B_w2, B_w3, B_w4,
    )
    return out.reshape(1, S, D)
```

```python
import functools

import jax
import jax.numpy as jnp
from jax import lax
import jax.experimental.pallas as pl
import jax.experimental.pallas.tpu as pltpu

F32 = jnp.float32
BF16 = jnp.bfloat16
U32 = jnp.uint32

S = 2048
D = 1024
H = 32
E = 128
M = 8
SEG = 32
L = M + SEG
FF = 3584
NCB = D // 128
NFB = FF // 128
NP = H // 2
NIT = S // (2 * SEG)
HB = 2 * L
PRE = 512
LAG = 128
BR = (S - PRE) // NIT
CLAG = 4
NSB = 8
H3R = PRE - 2 * 2 * BR
HS = D // 2 + 8
RB = 256
SB = 128
HSB = (SB // 64) * HB
CH = 512
PR = 16 * CH
EPS = 1e-5
DEP4 = (8, 4)
CSLOTS = range(10, 42, 4)
W4SLOTS = (1, 3, 5, 7, 9, 11, 13, 15, 18, 21)
W3OFF = 0
DEP3 = (70, 8)
SCALE = float(E) ** -0.5
SHIFTS = (7, 7, 9, 9, 6, 6, 10, 10)


def _dot(a, b):
    return jnp.dot(a, b, preferred_element_type=F32)


def _ln(x):
    m = jnp.mean(x, axis=-1, keepdims=True)
    xc = x - m
    v = jnp.mean(xc * xc, axis=-1, keepdims=True)
    return xc * lax.rsqrt(v + EPS)


def _ln2(x):
    m = jnp.mean(x, axis=-1, keepdims=True)
    xc = x - m
    v = jnp.mean(xc * xc, axis=-1, keepdims=True)
    r1 = lax.rsqrt(v + EPS)
    r2 = lax.rsqrt(v * r1 * r1 + EPS)
    return xc * r1, xc * (r1 * r2)


def _gelu(x):
    c = 0.7978845608028654
    hx = 0.5 * x
    return hx * jnp.tanh(x * (c + (c * 0.044715) * (x * x))) + hx


def _silu(x):
    hx = 0.5 * x
    return hx * jnp.tanh(hx) + hx


def _zero_of(v):
    return (pltpu.bitcast(v, U32) >> 16) >> 16


def _or_zero(w, z):
    return pltpu.bitcast(pltpu.bitcast(w, U32) | z, w.dtype)


def _col(w, cb, k0=0, k1=None):
    _, kk, cw = w.shape
    q, r = divmod(cb * 128, cw)
    return w[q, k0:(kk if k1 is None else k1), r:r + 128]


def _h3col(f):
    pos = (f // 14) * 7 + f % 7
    return (f % 14) // 7, slice(pos * 128, (pos + 1) * 128)


def _strassen_lhs(top, bot):
    k = top.shape[1] // 2
    a11, a12, a21, a22 = top[:, :k], top[:, k:], bot[:, :k], bot[:, k:]
    return [v.astype(BF16) for v in
            (a11 + a22, a21 + a22, a11, a21 - a11, a22, a11 + a12, a12 - a22)]


class _Strassen:
    def __init__(self, lhs, rhs, done):
        self.lhs, self.rhs, self.done, self.m = lhs, rhs, done, []

    def step(self):
        n, m = len(self.m), self.m
        v = _dot(self.lhs[n], self.rhs(n))
        m.append(v)
        if n == 3:
            self.done(1, 1, v + (m[0] - m[1] + m[2]))
        elif n == 4:
            self.done(1, 0, v + m[1])
        elif n == 5:
            self.done(0, 1, v + m[2])
        elif n == 6:
            self.done(0, 0, v + (m[0] + m[4] - m[5]))


def _hrow(r):
    q, rr = divmod(r, 64)
    return q * HB + rr + (8 if rr < 40 else 16)


def _kernel(x_hbm, mem0_hbm, wq_hbm, wk_hbm, wv_hbm, wo_hbm, w1_hbm, w2_hbm, w3_hbm, w4_hbm,
            out_hbm,
            xbuf, hbuf_all, hf, x1buf, h3buf, sbuf, stg, wqkv, wo, w1, w2, w3, w4, w3c, w4c,
            fillbuf,
            sem, osem):
    hbuf = hbuf_all.at[CLAG * HB:, :]

    def colblock_copies(src, dst, s):
        n, _, cw = dst.shape
        return [pltpu.make_async_copy(src.at[:, pl.ds(c * cw, cw)], dst.at[c], sem.at[s(c)])
                for c in range(n)]

    xs, qs = 7, 12
    xch = [(0, SB), (SB, SB), (RB, RB), (2 * RB, RB), (3 * RB, S - 3 * RB)]
    cp_x = [pltpu.make_async_copy(x_hbm.at[pl.ds(r, n), :], xbuf.at[pl.ds(r, n), :], sem.at[xs + i])
            for i, (r, n) in enumerate(xch)]
    cp_w1 = colblock_copies(w1_hbm, w1, lambda c: (0, 1, 16, 16)[c])
    cp_mem = [pltpu.make_async_copy(mem0_hbm, hbuf.at[0:M, :], sem.at[2])]
    cp_w2 = colblock_copies(w2_hbm, w2, lambda c: 3)
    cp_w3 = colblock_copies(w3_hbm, w3, lambda c: 4)
    cp_w4 = colblock_copies(w4_hbm, w4, lambda c: 5)
    cp_wo = colblock_copies(wo_hbm, wo, lambda c: 6)
    cp_qkv = [pltpu.make_async_copy(src.at[pl.ds(k * PR, PR), :], stg.at[k, pl.ds(m * PR, PR), :],
                                    sem.at[qs + k])
              for k in range(4) for m, src in enumerate((wq_hbm, wk_hbm, wv_hbm))]

    for c in cp_x[:2] + cp_w1[:2] + cp_x[2:3] + cp_w1[2:] + cp_w2 + cp_x[3:4]:
        c.start()
    for c in cp_x[4:] + cp_mem + cp_w3 + cp_w4 + cp_qkv + cp_wo:
        c.start(priority=1)

    def wait(grp):
        for c in grp:
            c.wait()

    r = lax.broadcasted_iota(jnp.int32, (HB, HB), 0)
    c = lax.broadcasted_iota(jnp.int32, (HB, HB), 1)
    rr = jnp.where(r >= L, r - L, r)
    cc = jnp.where(c >= L, c - L, c)
    same = (r >= L) == (c >= L)
    allowed = (rr < M) | (rr >= cc)
    fillbuf[...] = jnp.where(same, jnp.where(allowed, 1.0, -1e9), -jnp.inf).astype(F32)

    hf[:, 0:8, :] = jnp.zeros((NCB, 8, 128), F32)
    hf[:, S + 8:S + 16, :] = jnp.zeros((NCB, 8, 128), F32)
    sbuf[...] = jnp.zeros(sbuf.shape, sbuf.dtype)

    def ln_sub(xv, hv, sb):
        out = []
        for u in range(SB // 16):
            r0 = sb * SB + 16 * u
            xn, xnn = _ln2(xv[r0:r0 + 16, :].astype(F32))
            xn = xn.astype(BF16)
            for hh in range(2):
                o = _hrow(r0 + 8 * hh)
                hv[o:o + 8, :] = xn[8 * hh:8 * hh + 8]
            out.append(xnn.astype(BF16))
        return out

    def after(w, vals):
        if not vals:
            return w
        z = functools.reduce(lambda a, b: a | b, [_zero_of(v[-16:, -128:]) for v in vals])
        return jnp.concatenate([_or_zero(w[0:16, :], z), w[16:, :]], axis=0)

    def w1_sub(xnn, hfv, sb, cbs, deps):
        xnn = jnp.concatenate(xnn, axis=0)
        for cb in cbs:
            w = after(_col(w1, cb), deps.get(cb, []))
            hfv[cb, sb * SB + 8:sb * SB + 8 + SB, :] = _gelu(_dot(xnn, w))

    def w2_lhs(hfv, sb):
        r0 = sb * SB
        return jnp.concatenate(
            [hfv[cb, r0 + SHIFTS[cb]:r0 + SHIFTS[cb] + SB, :] for cb in range(NCB)],
            axis=1).astype(BF16)

    def w2_sub(hs, hv, x1v, sb, cbs, deps, hook=None):
        r0 = sb * SB
        for cb in cbs:
            pre = _dot(hs, after(_col(w2, cb), deps.get(cb, [])))
            cs = slice(cb * 128, (cb + 1) * 128)
            xn = jnp.concatenate(
                [hv[_hrow(r0 + a):_hrow(r0 + a) + n, cs].astype(F32)
                 for a, n in ((0, 40), (40, 24), (64, 40), (104, 24))], axis=0)
            x1v[r0:r0 + SB, cs] = (xn + pre).astype(BF16)
            if hook is not None:
                hook(pre)

    def w3_lhs(x1v, r0, rows):
        return [_ln(x1v[r0 + 16 * u:r0 + 16 * u + 16, :].astype(F32)) for u in range(rows // 16)]

    def h3_rows(r0, rows):
        p0, p1 = h3buf[0, pl.ds(r0, rows), :], h3buf[1, pl.ds(r0, rows), :]
        return jnp.concatenate([p0[:, :896], p1[:, :896], p0[:, 896:], p1[:, 896:]], axis=1)

    def gate(x1v, rows, cb, pre):
        sl = (rows, slice(cb * 128, (cb + 1) * 128))
        x1v[sl] = _silu(x1v[sl].astype(F32) + pre).astype(BF16)

    def weight_sums(src, dst, c0, c1, kh, r0, rows, stride, trig):
        for r in range(r0, r0 + rows, 16):
            tr = (((r - r0) * trig.shape[0] // rows) // 8) * 8 + 8 * (rows < trig.shape[0])
            z = _zero_of(trig[tr:tr + 8, :])
            ld = lambda c, o: _or_zero(_col(src, c, o + r, o + r + 16), z).astype(F32)
            b11, b12, b21, b22 = ld(c0, 0), ld(c1, 0), ld(c0, kh), ld(c1, kh)
            sums = (b11 + b22, b12 - b22, b11 + b12, b21 - b11, b21 + b22)
            for n, v in enumerate(sums):
                o = n * stride + r // 2
                dst[o:o + 8, :] = pltpu.bitcast(v.astype(BF16), U32)

    def strassen_rhs(w, wc, c0, c1, kh, base, stride, n):
        if n == 1:
            return _col(w, c0, 0, kh)
        if n == 5:
            return _col(w, c1, kh, 2 * kh)
        o = base + {0: 0, 2: 1, 3: 2, 4: 3, 6: 4}[n] * stride
        return pltpu.bitcast(wc[o:o + kh // 2, :], BF16)

    def relayout(src, dst, u, trig):
        m, c_ = divmod(u, 16)
        d0 = m * (H * HS) + c_ * 8
        two = lambda v: jnp.concatenate([v, v], axis=0)
        for pp in range(8):
            r0 = u * CH + pp * 64
            tr = (pp * trig.shape[0] // 64) * 8
            z = _zero_of(trig[tr:tr + 8, :])
            mlo, mhi, sh = two(z | U32(0xFFFF)), two(z | U32(0xFFFF0000)), two(z | U32(16))
            a = pltpu.bitcast(src[r0:r0 + 32, :], U32)
            b = pltpu.bitcast(src[r0 + 32:r0 + 64, :], U32)
            dst[pl.ds(d0 + pp, 16, stride=HS), :] = (a & mlo) | (b << sh)
            dst[pl.ds(d0 + 16 * HS + pp, 16, stride=HS), :] = (a >> sh) | (b & mhi)

    cp_x[0].wait()
    xnn0 = ln_sub(xbuf, hbuf, 0)
    cp_x[1].wait()
    xnn1 = ln_sub(xbuf, hbuf, 1)
    cp_w1[0].wait()
    w1_sub(xnn0, hf, 0, range(0, 2), {})
    w1_sub(xnn1, hf, 1, range(0, 2), {})
    cp_w1[1].wait()
    w1_sub(xnn0, hf, 0, range(2, 4), {})
    cp_x[2].wait()
    xnn2 = ln_sub(xbuf, hbuf, 2)
    w1_sub(xnn1, hf, 1, range(2, 4), {})
    w1_sub(xnn2, hf, 2, range(0, 4), {})
    wait(cp_w1[2:])
    xnn3 = ln_sub(xbuf, hbuf, 3)
    w1_sub(xnn0, hf, 0, range(4, 8), {6: xnn3[0:1], 7: xnn3[1:2]})
    w1_sub(xnn1, hf, 1, range(4, 8), {4 + i: xnn3[2 + i:3 + i] for i in range(4)})
    w1_sub(xnn2, hf, 2, range(4, 8), {4: xnn3[6:7], 5: xnn3[7:8]})
    w1_sub(xnn3, hf, 3, range(NCB), {})
    wait(cp_w2)
    cp_x[3].wait()

    def loop_w12(i, carry):
        @pl.when(i == 3)
        def _():
            cp_x[4].wait()

        r0 = pl.multiple_of((i - 2) * RB, RB)
        xv = xbuf.at[pl.ds(r0, 3 * RB), :]
        hv = hbuf.at[pl.ds(pl.multiple_of((i - 2) * 2 * HSB, 16), 6 * HSB), :]
        x1v = x1buf.at[pl.ds(r0, RB), :]
        hfv = hf.at[:, pl.ds(r0, 3 * RB + 16), :]
        spread = lambda c: {2: c[0:1], 3: c[1:2], 4: c[2:4], 5: c[4:5], 6: c[5:7], 7: c[7:8]}
        ca, cb_ = ln_sub(xv, hv, 4), ln_sub(xv, hv, 5)
        w2_sub(w2_lhs(hfv, 0), hv, x1v, 0, range(NCB), spread(ca))
        w1_sub(ca, hfv, 4, range(NCB), spread(cb_))
        w1_sub(cb_, hfv, 5, range(NCB), {})
        w2_sub(w2_lhs(hfv, 1), hv, x1v, 1, range(NCB), {})
        return carry

    lax.fori_loop(2, S // RB, loop_w12, 0)
    wait(cp_w3)
    wait(cp_w4)

    def loop_w34(k, carry):
        pltpu.make_async_copy(stg.at[k], stg.at[k], sem.at[qs + k]).wait()
        r0 = pl.multiple_of(k * SB, SB)
        src = stg.at[k]
        dst = wqkv.at[pl.ds(pl.multiple_of(k * 128, 128), (3 * H + 1) * HS - 384), :]
        sb2 = (S - PRE) // SB
        x1v = x1buf.at[pl.ds(r0, (sb2 + 1) * SB), :]
        hv = hbuf.at[pl.ds(pl.multiple_of(k * HSB, 16), (sb2 + 1) * HSB), :]
        hfv = hf.at[:, pl.ds(r0, (sb2 + 1) * SB + 16), :]
        w3v = w3.at[:, pl.ds(r0, D - 384), :]
        w3cv = w3c.at[:, pl.ds(pl.multiple_of(k * 64, 64), 35 * 256 - 192), :]
        w4v = w4.at[:, pl.ds(pl.multiple_of(k * 448, 64), FF - 3 * 448), :]
        w4cv = w4c.at[:, pl.ds(pl.multiple_of(k * 224, 32), 10 * 896 - 3 * 224), :]
        todo = list(range(3 * PR // CH))
        todo3 = [(f, u) for f in range(14) for u in range(2)]
        todo4 = [(c, u) for c in range(4) for u in range(7)]

        def rl(trig):
            if todo:
                relayout(src, dst, todo.pop(0), trig)

        def sums3(trig):
            if todo3:
                f, u = todo3.pop(0)
                weight_sums(w3v, w3cv.at[f // 7, pl.ds((f % 7) * 256, 29 * 256 - 192), :],
                            f, f + 14, D // 2, 64 * u, 64, 7 * 256, trig)

        def sums4(trig):
            c, u = todo4.pop(0)
            weight_sums(w4v, w4cv.at[c // 2, pl.ds((c % 2) * 896, 9 * 896 - 3 * 224), :],
                        c, c + 4, FF // 2, 64 * u, 64, 2 * 896, trig)

        hs = w2_lhs(hfv, sb2)
        c = [v.astype(BF16) for v in w3_lhs(x1v, 0, SB)]
        w2_sub(hs, hv, x1v, sb2, range(0, 6), {3: c[0:2], 4: c[2:4], 5: c[4:6]})
        lhs3 = jnp.concatenate(c, axis=0)
        for f in range(NFB):
            half = _dot(lhs3[:, :512], _col(w3, f, 0, 512))
            pre = _dot(lhs3[:, 512:], _col(w3, f, 512, D)) + half
            q, cs = _h3col(f)
            h3buf[q, pl.ds(r0, SB), cs] = _gelu(pre).astype(BF16)
            rl(half)
            sums4(pre)
        w2_sub(hs, hv, x1v, sb2, range(6, 7), {}, rl)
        n4 = (PRE - LAG) // 4
        r4 = pl.multiple_of(k * n4, 32)
        lhs4 = h3_rows(r4, n4)
        for cb in range(NCB):
            pre = None
            for n in range(7):
                k0, k1 = 512 * n, 512 * (n + 1)
                part = _dot(lhs4[:, k0:k1], _col(w4, cb, k0, k1))
                pre = part if pre is None else part + pre
                if n in (0, 2, 4):
                    rl(pre)
                if n in (1, 3, 5, 6):
                    sums3(pre)
            gate(x1buf.at[pl.ds(r4, n4), :], slice(0, n4), cb, pre)
        w2_sub(hs, hv, x1v, sb2, range(7, 8), {})
        assert not (todo or todo3 or todo4)
        return carry

    lax.fori_loop(0, PRE // SB, loop_w34, 0)
    wait(cp_wo)
    wait(cp_mem)

    def softmax(s):
        fill = fillbuf[...]
        s = jnp.where(fill > 0.0, s * SCALE, fill)
        mx = jnp.max(s, axis=1, keepdims=True)
        e = jnp.exp(s - mx)
        l = jnp.sum(e, axis=1, keepdims=True)
        rc = pl.reciprocal(l, approx=True)
        rc = rc * (2.0 - l * rc)
        return (e * rc).astype(BF16)

    def attn_step(lhs, select, wo_rows, fill, deps):
        qkv = [None] * NP
        p = [None] * NP
        oh = [None] * H
        acc = [None] * NCB
        wsplit = (0, 8, 20, 28, 32)

        def do_qkv(j):
            rs = []
            for i in range(6):
                h = 2 * j + i // 3
                r0 = ((i % 3) * H + (h % 2) * 16 + h // 2) * HS
                w = pltpu.bitcast(wqkv[r0:r0 + D // 2, :], BF16)
                v = _dot(lhs, after(w, deps.get(6 * j + i, [])))
                fill(("qkv", 6 * j + i), v)
                rs.append(select(j, i, v))
            qkv[j] = [jnp.concatenate([rs[i], rs[3 + i]], axis=0).astype(BF16) for i in range(3)]

        def do_s(j):
            p[j] = softmax(lax.dot_general(qkv[j][0], qkv[j][1], (((1,), (1,)), ((), ())),
                                           preferred_element_type=F32))

        def do_pv(j):
            o = _dot(p[j], qkv[j][2])
            oh[2 * j] = wo_rows(2 * j, o[0:L]).astype(BF16)
            oh[2 * j + 1] = wo_rows(2 * j + 1, o[L:2 * L]).astype(BF16)

        def do_wo(n):
            h0, h1 = wsplit[n], wsplit[n + 1]
            lo = jnp.concatenate(oh[h0:h1], axis=1)
            for cb in range(NCB):
                part = _dot(lo, _col(wo, cb, h0 * E, h1 * E))
                acc[cb] = part if acc[cb] is None else part + acc[cb]
                fill(("wo", n * NCB + cb), part)

        for j in range(NP + 2):
            if j < NP:
                do_qkv(j)
            else:
                do_wo(j - NP)
            if 0 <= j - 2 < NP:
                do_pv(j - 2)
            if 0 <= j - 1 < NP:
                do_s(j - 1)
        do_wo(2)
        do_wo(3)
        return acc

    def combine(r0, sv, dst, cb, trig=None):
        cs = slice(cb * 128, (cb + 1) * 128)
        xx, gg = xbuf[pl.ds(r0, 64), cs], x1buf[pl.ds(r0, 64), cs]
        if trig is not None:
            z = jnp.concatenate([_zero_of(trig[0:8, :])] * 4, axis=0)
            xx, gg = _or_zero(xx, z), _or_zero(gg, z)
        dst[0:64, cs] = (xx.astype(F32) + sv[:, cs].astype(F32) * gg.astype(F32)).astype(BF16)

    def body(t, carry):
        hv = hbuf_all.at[pl.ds(pl.multiple_of(t * HB, 16), (CLAG + 1) * HB + 16), :]
        cur = CLAG * HB
        prev = pl.multiple_of(jnp.maximum(t - CLAG, 0) * 64, 64)
        par, blk = t % 2, t // 2

        b4 = pl.multiple_of(PRE - LAG + blk * 2 * BR, 32)
        ln3 = w3_lhs(x1buf.at[pl.ds(b4 + LAG, 2 * BR), :], 0, 2 * BR)
        c3 = [_strassen_lhs(ln3[u], ln3[3 + u]) for u in range(3)]
        lhs3 = [jnp.concatenate([c[n] for c in c3], axis=0) for n in range(7)]
        slot = lambda j: pl.multiple_of(H3R + (j % 3) * 2 * BR, 32)
        h3w = h3buf.at[par, pl.ds(slot(blk + 2), 2 * BR), :]
        w3v, w3cv = w3.at[pl.ds(par, 3)], w3c.at[par]

        def w3_pair(i):
            def done(a, b, v):
                h3w[a * BR:(a + 1) * BR, (7 * b + i) * 128:(7 * b + i + 1) * 128] = (
                    _gelu(v).astype(BF16))
            return _Strassen(lhs3, functools.partial(strassen_rhs, w3v, w3cv, i, i + 14, D // 2,
                                                     i * 256, 7 * 256), done)

        top = jnp.concatenate([h3_rows(slot(blk) + 64, 32), h3_rows(slot(blk + 1), 16)], axis=0)
        bot = h3_rows(slot(blk + 1) + 16, BR)
        pair = lambda v, f: jnp.concatenate(
            [v[:, f * 128:(f + 1) * 128], v[:, (f + 14) * 128:(f + 15) * 128]], axis=1).astype(F32)
        c4 = [_strassen_lhs(pair(top, f), pair(bot, f)) for f in range(14)]
        lhs4 = [jnp.concatenate([c[n] for c in c4], axis=1) for n in range(7)]
        deps = {DEP4[0] + DEP4[1] * f: c4[f] for f in range(14)}
        deps.update({DEP3[0] + DEP3[1] * u: c3[u] for u in range(3)})
        x4v = x1buf.at[pl.ds(b4, 2 * BR), pl.ds(pl.multiple_of(par * 256, 256), D - 256)]
        w4v, w4cv = w4.at[pl.ds(par, 3)], w4c.at[par]

        def w4_pair(i):
            def done(a, b, v):
                gate(x4v, slice(a * BR, (a + 1) * BR), 4 * b + i, v)
            return _Strassen(lhs4, functools.partial(strassen_rhs, w4v, w4cv, i, i + 4, FF // 2,
                                                     i * 896, 2 * 896), done)

        todo3 = [p for p in map(w3_pair, range(7)) for _ in range(7)]
        todo4 = [p for p in map(w4_pair, range(2)) for _ in range(7)]
        todoc = list(range(NCB))

        keep = {}

        def sel_a(j, i, v):
            keep[(j, i)] = v[L:L + 8]
            return v[0:L]

        def wo_a(h, o):
            keep[h] = o[32:40]
            return o[0:32]

        sv_old = sbuf.at[(t + NSB - CLAG) % NSB]

        def fill_a(slot, v):
            if slot[0] == "qkv" and slot[1] in CSLOTS:
                combine(prev, sv_old, hv, todoc.pop(0), v)
                if not todoc:
                    @pl.when(t >= CLAG)
                    def _():
                        pltpu.make_async_copy(hv.at[0:64, :], out_hbm.at[pl.ds(prev, 64), :],
                                              osem).start()
            if slot[0] == "wo" and slot[1] in W4SLOTS:
                todo4.pop(0).step()

        ra = attn_step(hv[cur:cur + 48, :], sel_a, wo_a, fill_a, deps)
        for cb in range(NCB):
            hv[cur + 48:cur + 56, cb * 128:(cb + 1) * 128] = ra[cb][0:8].astype(BF16)
        while todo4:
            todo4.pop(0).step()

        def sel_b(j, i, v):
            return jnp.concatenate([v[0:8], keep[(j, i)], v[8:32]], axis=0)

        def wo_b(h, o):
            return jnp.concatenate([keep[h], o], axis=0)

        w3_slots = [(i * 6 * NP + W3OFF) // 49 for i in range(49)]

        def fill_b(slot, v):
            if slot[0] == "qkv" and slot[1] in w3_slots:
                todo3.pop(0).step()

        rb = attn_step(hv[cur + 48:cur + HB, :], sel_b, wo_b, fill_b, {})
        sv = sbuf.at[t % NSB]
        for cb in range(NCB):
            cs = slice(cb * 128, (cb + 1) * 128)
            hv[cur + HB:cur + HB + 8, cs] = rb[cb][8:16].astype(BF16)
            sv[:, cs] = jnp.concatenate([ra[cb][8:32], rb[cb][0:8], rb[cb][16:48]],
                                        axis=0).astype(BF16)
        assert not (todo3 or todo4 or todoc)
        return carry

    lax.fori_loop(0, NIT, body, 0)

    last = (S - PRE) // (2 * BR) - 1
    s0, s1 = H3R + ((last + 1) % 3) * 2 * BR, H3R + ((last + 2) % 3) * 2 * BR
    top = jnp.concatenate([h3_rows(s0 + 64, 32), h3_rows(s1, 32)], axis=0)
    lhs4 = _strassen_lhs(top.astype(F32), h3_rows(s1 + 32, 64).astype(F32))
    x4v = x1buf.at[S - LAG:S, :]

    def finish(t, cbs, trig=None):
        stage = hbuf.at[t * HB:(t + 1) * HB, :]
        for cb in cbs:
            combine(t * 64, sbuf.at[t % NSB], stage, cb, trig)
        cs = pl.ds(cbs[0] * 128, len(cbs) * 128)
        pltpu.make_async_copy(stage.at[0:64, cs], out_hbm.at[t * 64:(t + 1) * 64, cs], osem).start()

    for c in range(4):
        def done(a, b, v, c=c):
            gate(x4v, slice(a * 64, (a + 1) * 64), 4 * b + c, v)
            finish(NIT - 2 + a, [4 * b + c])
            if c < 2 and b == 1:
                finish(NIT - 4 + c, list(range(4 * a, 4 * a + 4)), v)
        prod = _Strassen(lhs4, functools.partial(strassen_rhs, w4.at[pl.ds(c // 2, 3)],
                                                 w4c.at[c // 2], c % 2, c % 2 + 4, FF // 2,
                                                 (c % 2) * 896, 2 * 896), done)
        for _ in range(7):
            prod.step()
    pltpu.make_async_copy(xbuf, out_hbm, osem).wait()


@jax.jit
def pallas_recurrent_scan__memory_aug_recurrent_mem_tr__mixer_s_mlp__prompt_kernel(
    A_x: jax.Array,
    A_mem0: jax.Array,
    A_Wq: jax.Array,
    A_Wk: jax.Array,
    A_Wv: jax.Array,
    A_Wo: jax.Array,
    A_seg_len: jax.Array,
    B_x: jax.Array,
    B_w1: jax.Array,
    B_w2: jax.Array,
    B_w3: jax.Array,
    B_w4: jax.Array,
):
    del A_seg_len, B_x
    assert A_x.shape == (1, S, D) and A_mem0.shape == (1, M, D)
    assert A_Wq.shape == (D, H, E) and A_Wo.shape == (H, E, D)
    assert B_w3.shape == (D, FF) and B_w4.shape == (FF, D)

    any_spec = pl.BlockSpec(memory_space=pl.ANY)
    out = pl.pallas_call(
        _kernel,
        out_shape=jax.ShapeDtypeStruct((S, D), BF16),
        in_specs=[any_spec] * 10,
        out_specs=any_spec,
        scratch_shapes=[
            pltpu.VMEM((S, D), BF16),
            pltpu.VMEM(((NIT + CLAG) * HB + 16, D), BF16),
            pltpu.VMEM((NCB, S + 16, 128), F32),
            pltpu.VMEM((S, D), BF16),
            pltpu.VMEM((2, PRE + 2 * BR, FF // 2), BF16),
            pltpu.VMEM((NSB, 64, D), BF16),
            pltpu.VMEM((4, 3 * PR, E), BF16),
            pltpu.VMEM(((3 * H + 1) * HS, 128), U32),
            pltpu.VMEM((D // 512, H * E, 512), BF16),
            pltpu.VMEM((D // 256, D, 256), BF16),
            pltpu.VMEM((D // 512, D, 512), BF16),
            pltpu.VMEM((4, D, FF // 4), BF16),
            pltpu.VMEM((4, FF, D // 4), BF16),
            pltpu.VMEM((2, 35 * 256, 128), U32),
            pltpu.VMEM((2, 10 * 896, 128), U32),
            pltpu.VMEM((HB, HB), F32),
            pltpu.SemaphoreType.DMA((17,)),
            pltpu.SemaphoreType.DMA(()),
        ],
        compiler_params=pltpu.CompilerParams(vmem_limit_bytes=126 * 1024 * 1024),
    )(
        A_x.reshape(S, D), A_mem0.reshape(M, D),
        A_Wq.reshape(D * H, E), A_Wk.reshape(D * H, E), A_Wv.reshape(D * H, E),
        A_Wo.reshape(H * E, D), B_w1, B_w2, B_w3, B_w4,
    )
    return out.reshape(1, S, D)
```

```python
import functools

import jax
import jax.numpy as jnp
from jax import lax
import jax.experimental.pallas as pl
import jax.experimental.pallas.tpu as pltpu

F32 = jnp.float32
BF16 = jnp.bfloat16
U32 = jnp.uint32

S = 2048
D = 1024
H = 32
E = 128
M = 8
SEG = 32
L = M + SEG
FF = 3584
NCB = D // 128
NFB = FF // 128
NP = H // 2
NIT = S // (2 * SEG)
HB = 2 * L
PRE = 512
LAG = 128
BR = (S - PRE) // NIT
CLAG = 4
NSB = 8
H3R = PRE - 2 * 2 * BR
HS = D // 2 + 8
RB = 256
SB = 128
HSB = (SB // 64) * HB
CH = 512
PR = 16 * CH
EPS = 1e-5
DEP4 = (8, 4)
CSLOTS = range(10, 42, 4)
W4SLOTS = (1, 3, 5, 7, 9, 11, 13, 15, 18, 21)
W3OFF = 0
DEP3 = (70, 8)
SCALE = float(E) ** -0.5
SHIFTS = (7, 7, 9, 9, 6, 6, 10, 10)


def _dot(a, b):
    return jnp.dot(a, b, preferred_element_type=F32)


def _ln(x):
    m = jnp.mean(x, axis=-1, keepdims=True)
    xc = x - m
    v = jnp.mean(xc * xc, axis=-1, keepdims=True)
    return xc * lax.rsqrt(v + EPS)


def _ln2(x):
    m = jnp.mean(x, axis=-1, keepdims=True)
    xc = x - m
    v = jnp.mean(xc * xc, axis=-1, keepdims=True)
    r1 = lax.rsqrt(v + EPS)
    r2 = lax.rsqrt(v * r1 * r1 + EPS)
    return xc * r1, xc * (r1 * r2)


def _gelu(x):
    c = 0.7978845608028654
    hx = 0.5 * x
    return hx * jnp.tanh(x * (c + (c * 0.044715) * (x * x))) + hx


def _silu(x):
    hx = 0.5 * x
    return hx * jnp.tanh(hx) + hx


def _zero_of(v):
    return (pltpu.bitcast(v, U32) >> 16) >> 16


def _or_zero(w, z):
    return pltpu.bitcast(pltpu.bitcast(w, U32) | z, w.dtype)


def _col(w, cb, k0=0, k1=None):
    _, kk, cw = w.shape
    q, r = divmod(cb * 128, cw)
    return w[q, k0:(kk if k1 is None else k1), r:r + 128]


def _h3col(f):
    pos = (f // 14) * 7 + f % 7
    return (f % 14) // 7, slice(pos * 128, (pos + 1) * 128)


def _strassen_lhs(top, bot):
    k = top.shape[1] // 2
    a11, a12, a21, a22 = top[:, :k], top[:, k:], bot[:, :k], bot[:, k:]
    return [v.astype(BF16) for v in
            (a11 + a22, a21 + a22, a11, a21 - a11, a22, a11 + a12, a12 - a22)]


class _Strassen:
    def __init__(self, lhs, rhs, done):
        self.lhs, self.rhs, self.done, self.m = lhs, rhs, done, []

    def step(self):
        n, m = len(self.m), self.m
        v = _dot(self.lhs[n], self.rhs(n))
        m.append(v)
        if n == 3:
            self.done(1, 1, v + (m[0] - m[1] + m[2]))
        elif n == 4:
            self.done(1, 0, v + m[1])
        elif n == 5:
            self.done(0, 1, v + m[2])
        elif n == 6:
            self.done(0, 0, v + (m[0] + m[4] - m[5]))


def _hrow(r):
    q, rr = divmod(r, 64)
    return q * HB + rr + (8 if rr < 40 else 16)


def _kernel(x_hbm, mem0_hbm, wq_hbm, wk_hbm, wv_hbm, wo_hbm, w1_hbm, w2_hbm, w3_hbm, w4_hbm,
            out_hbm,
            xbuf, hbuf_all, hf, x1buf, h3buf, sbuf, stg, wqkv, wo, w1, w2, w3, w4, w3c, w4c,
            fillbuf,
            sem, osem):
    hbuf = hbuf_all.at[CLAG * HB:, :]

    def colblock_copies(src, dst, s):
        n, _, cw = dst.shape
        return [pltpu.make_async_copy(src.at[:, pl.ds(c * cw, cw)], dst.at[c], sem.at[s(c)])
                for c in range(n)]

    xs, qs = 7, 12
    xch = [(0, SB), (SB, SB), (RB, RB), (2 * RB, RB), (3 * RB, S - 3 * RB)]
    cp_x = [pltpu.make_async_copy(x_hbm.at[pl.ds(r, n), :], xbuf.at[pl.ds(r, n), :], sem.at[xs + i])
            for i, (r, n) in enumerate(xch)]
    cp_w1 = colblock_copies(w1_hbm, w1, lambda c: (0, 1, 16, 16)[c])
    cp_mem = [pltpu.make_async_copy(mem0_hbm, hbuf.at[0:M, :], sem.at[2])]
    cp_w2 = colblock_copies(w2_hbm, w2, lambda c: 3)
    cp_w3 = colblock_copies(w3_hbm, w3, lambda c: 4)
    cp_w4 = colblock_copies(w4_hbm, w4, lambda c: 5)
    cp_wo = colblock_copies(wo_hbm, wo, lambda c: 6)
    cp_qkv = [pltpu.make_async_copy(src.at[pl.ds(k * PR, PR), :], stg.at[k, pl.ds(m * PR, PR), :],
                                    sem.at[qs + k])
              for k in range(4) for m, src in enumerate((wq_hbm, wk_hbm, wv_hbm))]

    for c in cp_x[:2] + cp_w1[:2] + cp_x[2:3] + cp_w1[2:] + cp_w2 + cp_x[3:4]:
        c.start()
    for c in cp_x[4:] + cp_mem + cp_w3 + cp_w4 + cp_qkv + cp_wo:
        c.start(priority=1)

    def wait(grp):
        for c in grp:
            c.wait()

    r = lax.broadcasted_iota(jnp.int32, (HB, HB), 0)
    c = lax.broadcasted_iota(jnp.int32, (HB, HB), 1)
    rr = jnp.where(r >= L, r - L, r)
    cc = jnp.where(c >= L, c - L, c)
    same = (r >= L) == (c >= L)
    allowed = (rr < M) | (rr >= cc)
    fillbuf[...] = jnp.where(same, jnp.where(allowed, 1.0, -1e9), -jnp.inf).astype(F32)

    hf[:, 0:8, :] = jnp.zeros((NCB, 8, 128), F32)
    hf[:, S + 8:S + 16, :] = jnp.zeros((NCB, 8, 128), F32)
    sbuf[...] = jnp.zeros(sbuf.shape, sbuf.dtype)

    def ln_sub(xv, hv, sb, dtype=BF16):
        out = []
        for u in range(SB // 16):
            r0 = sb * SB + 16 * u
            xn, xnn = _ln2(xv[r0:r0 + 16, :].astype(F32))
            xn = xn.astype(BF16)
            for hh in range(2):
                o = _hrow(r0 + 8 * hh)
                hv[o:o + 8, :] = xn[8 * hh:8 * hh + 8]
            out.append(xnn.astype(dtype))
        return out

    def after(w, vals):
        if not vals:
            return w
        z = functools.reduce(lambda a, b: a | b, [_zero_of(v[-16:, -128:]) for v in vals])
        return jnp.concatenate([_or_zero(w[0:16, :], z), w[16:, :]], axis=0)

    def w1_sub(xnn, hfv, sb, cbs, deps, hook=None):
        xnn = jnp.concatenate(xnn, axis=0)
        for cb in cbs:
            w = after(_col(w1, cb), deps.get(cb, []))
            half = _dot(xnn[:, :D // 2], w[:D // 2])
            hfv[cb, sb * SB + 8:sb * SB + 8 + SB, :] = _gelu(_dot(xnn[:, D // 2:], w[D // 2:]) + half)
            if hook is not None:
                hook(half)

    def w2_lhs(hfv, sb):
        r0 = sb * SB
        return jnp.concatenate(
            [hfv[cb, r0 + SHIFTS[cb]:r0 + SHIFTS[cb] + SB, :] for cb in range(NCB)],
            axis=1).astype(BF16)

    def w2_sub(hs, hv, x1v, sb, cbs, deps, hook=None):
        r0 = sb * SB
        for cb in cbs:
            pre = _dot(hs, after(_col(w2, cb), deps.get(cb, [])))
            cs = slice(cb * 128, (cb + 1) * 128)
            xn = jnp.concatenate(
                [hv[_hrow(r0 + a):_hrow(r0 + a) + n, cs].astype(F32)
                 for a, n in ((0, 40), (40, 24), (64, 40), (104, 24))], axis=0)
            x1v[r0:r0 + SB, cs] = (xn + pre).astype(BF16)
            if hook is not None:
                hook(pre)

    def w3_lhs(x1v, r0, rows):
        return [_ln(x1v[r0 + 16 * u:r0 + 16 * u + 16, :].astype(F32)) for u in range(rows // 16)]

    def h3_rows(r0, rows):
        p0, p1 = h3buf[0, pl.ds(r0, rows), :], h3buf[1, pl.ds(r0, rows), :]
        return jnp.concatenate([p0[:, :896], p1[:, :896], p0[:, 896:], p1[:, 896:]], axis=1)

    def gate(x1v, rows, cb, pre):
        sl = (rows, slice(cb * 128, (cb + 1) * 128))
        x1v[sl] = _silu(x1v[sl].astype(F32) + pre).astype(BF16)

    def weight_sums(src, dst, c0, c1, kh, r0, rows, stride, trig):
        for r in range(r0, r0 + rows, 16):
            tr = (((r - r0) * trig.shape[0] // rows) // 8) * 8 + 8 * (rows < trig.shape[0])
            z = _zero_of(trig[tr:tr + 8, :])
            ld = lambda c, o: _or_zero(_col(src, c, o + r, o + r + 16), z).astype(F32)
            b11, b12, b21, b22 = ld(c0, 0), ld(c1, 0), ld(c0, kh), ld(c1, kh)
            sums = (b11 + b22, b12 - b22, b11 + b12, b21 - b11, b21 + b22)
            for n, v in enumerate(sums):
                o = n * stride + r // 2
                dst[o:o + 8, :] = pltpu.bitcast(v.astype(BF16), U32)

    def strassen_rhs(w, wc, c0, c1, kh, base, stride, n):
        if n == 1:
            return _col(w, c0, 0, kh)
        if n == 5:
            return _col(w, c1, kh, 2 * kh)
        o = base + {0: 0, 2: 1, 3: 2, 4: 3, 6: 4}[n] * stride
        return pltpu.bitcast(wc[o:o + kh // 2, :], BF16)

    def relayout(src, dst, u, trig):
        m, c_ = divmod(u, 16)
        d0 = m * (H * HS) + c_ * 8
        two = lambda v: jnp.concatenate([v, v], axis=0)
        for pp in range(8):
            r0 = u * CH + pp * 64
            tr = (pp * trig.shape[0] // 64) * 8
            z = _zero_of(trig[tr:tr + 8, :])
            mlo, mhi, sh = two(z | U32(0xFFFF)), two(z | U32(0xFFFF0000)), two(z | U32(16))
            a = pltpu.bitcast(src[r0:r0 + 32, :], U32)
            b = pltpu.bitcast(src[r0 + 32:r0 + 64, :], U32)
            dst[pl.ds(d0 + pp, 16, stride=HS), :] = (a & mlo) | (b << sh)
            dst[pl.ds(d0 + 16 * HS + pp, 16, stride=HS), :] = (a >> sh) | (b & mhi)

    cp_x[0].wait()
    xnn0 = ln_sub(xbuf, hbuf, 0)
    cp_x[1].wait()
    xnn1 = ln_sub(xbuf, hbuf, 1)
    cp_w1[0].wait()
    w1_sub(xnn0, hf, 0, range(0, 2), {})
    w1_sub(xnn1, hf, 1, range(0, 2), {})
    cp_w1[1].wait()
    w1_sub(xnn0, hf, 0, range(2, 4), {})
    cp_x[2].wait()
    xnn2 = ln_sub(xbuf, hbuf, 2)
    w1_sub(xnn1, hf, 1, range(2, 4), {})
    w1_sub(xnn2, hf, 2, range(0, 4), {})
    wait(cp_w1[2:])
    xnn3 = ln_sub(xbuf, hbuf, 3)
    w1c = w3c.at[0]
    todo1 = [(c, u) for c in range(4) for u in range(8)]

    count1 = [1, 1, 1, 1, 1, 1, 1, 1, 2, 2, 2, 2, 2, 2, 2, 2, 2, 2, 2, 2]

    def sums1(trig):
        n = count1.pop(0)
        for i in range(n):
            c, u = todo1.pop(0)
            tr = trig[(i * 16 // n) * 8:((i + 1) * 16 // n) * 8]
            weight_sums(w1, w1c.at[c * 256:, :], c, c + 4, D // 2, 64 * u, 64, 4 * 256, tr)

    w1_sub(xnn0, hf, 0, range(4, 8), {6: xnn3[0:1], 7: xnn3[1:2]}, sums1)
    w1_sub(xnn1, hf, 1, range(4, 8), {4 + i: xnn3[2 + i:3 + i] for i in range(4)}, sums1)
    w1_sub(xnn2, hf, 2, range(4, 8), {4: xnn3[6:7], 5: xnn3[7:8]}, sums1)
    w1_sub(xnn3, hf, 3, range(NCB), {}, sums1)
    assert not todo1
    wait(cp_w2)
    cp_x[3].wait()

    def loop_w12(i, carry):
        @pl.when(i == 3)
        def _():
            cp_x[4].wait()

        r0 = pl.multiple_of((i - 2) * RB, RB)
        xv = xbuf.at[pl.ds(r0, 3 * RB), :]
        hv = hbuf.at[pl.ds(pl.multiple_of((i - 2) * 2 * HSB, 16), 6 * HSB), :]
        x1v = x1buf.at[pl.ds(r0, RB), :]
        hfv = hf.at[:, pl.ds(r0, 3 * RB + 16), :]
        ca, cb_ = ln_sub(xv, hv, 4, F32), ln_sub(xv, hv, 5, F32)
        c1 = [_strassen_lhs(ca[u], cb_[u]) for u in range(SB // 16)]
        lhs1 = [jnp.concatenate([c[n] for c in c1], axis=0) for n in range(7)]
        w2_sub(w2_lhs(hfv, 0), hv, x1v, 0, range(NCB), {3: c1[0], 5: c1[1], 6: c1[2], 7: c1[3]})
        hs = w2_lhs(hfv, 1)
        w2_sub(hs, hv, x1v, 1, range(0, 6), {0: c1[4], 2: c1[5], 3: c1[6], 4: c1[7]})
        for c in range(4):
            def done(a, b, v, c=c):
                hfv[4 * b + c, (4 + a) * SB + 8:(5 + a) * SB + 8, :] = _gelu(v)
            prod = _Strassen(lhs1, functools.partial(strassen_rhs, w1, w1c, c, c + 4, D // 2,
                                                     c * 256, 4 * 256), done)
            for _ in range(7):
                prod.step()
        w2_sub(hs, hv, x1v, 1, range(6, 8), {})
        return carry

    lax.fori_loop(2, S // RB, loop_w12, 0)
    wait(cp_w3)
    wait(cp_w4)

    def loop_w34(k, carry):
        pltpu.make_async_copy(stg.at[k], stg.at[k], sem.at[qs + k]).wait()
        r0 = pl.multiple_of(k * SB, SB)
        src = stg.at[k]
        dst = wqkv.at[pl.ds(pl.multiple_of(k * 128, 128), (3 * H + 1) * HS - 384), :]
        sb2 = (S - PRE) // SB
        x1v = x1buf.at[pl.ds(r0, (sb2 + 1) * SB), :]
        hv = hbuf.at[pl.ds(pl.multiple_of(k * HSB, 16), (sb2 + 1) * HSB), :]
        hfv = hf.at[:, pl.ds(r0, (sb2 + 1) * SB + 16), :]
        w3v = w3.at[:, pl.ds(r0, D - 384), :]
        w3cv = w3c.at[:, pl.ds(pl.multiple_of(k * 64, 64), 35 * 256 - 192), :]
        w4v = w4.at[:, pl.ds(pl.multiple_of(k * 448, 64), FF - 3 * 448), :]
        w4cv = w4c.at[:, pl.ds(pl.multiple_of(k * 224, 32), 10 * 896 - 3 * 224), :]
        todo = list(range(3 * PR // CH))
        todo3 = [(f, u) for f in range(14) for u in range(2)]
        todo4 = [(c, u) for c in range(4) for u in range(7)]

        def rl(trig):
            if todo:
                relayout(src, dst, todo.pop(0), trig)

        def sums3(trig):
            if todo3:
                f, u = todo3.pop(0)
                weight_sums(w3v, w3cv.at[f // 7, pl.ds((f % 7) * 256, 29 * 256 - 192), :],
                            f, f + 14, D // 2, 64 * u, 64, 7 * 256, trig)

        def sums4(trig):
            c, u = todo4.pop(0)
            weight_sums(w4v, w4cv.at[c // 2, pl.ds((c % 2) * 896, 9 * 896 - 3 * 224), :],
                        c, c + 4, FF // 2, 64 * u, 64, 2 * 896, trig)

        hs = w2_lhs(hfv, sb2)
        c = [v.astype(BF16) for v in w3_lhs(x1v, 0, SB)]
        w2_sub(hs, hv, x1v, sb2, range(0, 6), {3: c[0:2], 4: c[2:4], 5: c[4:6]})
        lhs3 = jnp.concatenate(c, axis=0)
        for f in range(NFB):
            half = _dot(lhs3[:, :512], _col(w3, f, 0, 512))
            pre = _dot(lhs3[:, 512:], _col(w3, f, 512, D)) + half
            q, cs = _h3col(f)
            h3buf[q, pl.ds(r0, SB), cs] = _gelu(pre).astype(BF16)
            rl(half)
            sums4(pre)
        w2_sub(hs, hv, x1v, sb2, range(6, 7), {}, rl)
        n4 = (PRE - LAG) // 4
        r4 = pl.multiple_of(k * n4, 32)
        lhs4 = h3_rows(r4, n4)
        for cb in range(NCB):
            pre = None
            for n in range(7):
                k0, k1 = 512 * n, 512 * (n + 1)
                part = _dot(lhs4[:, k0:k1], _col(w4, cb, k0, k1))
                pre = part if pre is None else part + pre
                if n in (0, 2, 4):
                    rl(pre)
                if n in (1, 3, 5, 6):
                    sums3(pre)
            gate(x1buf.at[pl.ds(r4, n4), :], slice(0, n4), cb, pre)
        w2_sub(hs, hv, x1v, sb2, range(7, 8), {})
        assert not (todo or todo3 or todo4)
        return carry

    lax.fori_loop(0, PRE // SB, loop_w34, 0)
    wait(cp_wo)
    wait(cp_mem)

    def softmax(s):
        fill = fillbuf[...]
        s = jnp.where(fill > 0.0, s * SCALE, fill)
        mx = jnp.max(s, axis=1, keepdims=True)
        e = jnp.exp(s - mx)
        l = jnp.sum(e, axis=1, keepdims=True)
        rc = pl.reciprocal(l, approx=True)
        rc = rc * (2.0 - l * rc)
        return (e * rc).astype(BF16)

    def attn_step(lhs, select, wo_rows, fill, deps):
        qkv = [None] * NP
        p = [None] * NP
        oh = [None] * H
        acc = [None] * NCB
        wsplit = (0, 8, 20, 28, 32)

        def do_qkv(j):
            rs = []
            for i in range(6):
                h = 2 * j + i // 3
                r0 = ((i % 3) * H + (h % 2) * 16 + h // 2) * HS
                w = pltpu.bitcast(wqkv[r0:r0 + D // 2, :], BF16)
                v = _dot(lhs, after(w, deps.get(6 * j + i, [])))
                fill(("qkv", 6 * j + i), v)
                rs.append(select(j, i, v))
            qkv[j] = [jnp.concatenate([rs[i], rs[3 + i]], axis=0).astype(BF16) for i in range(3)]

        def do_s(j):
            p[j] = softmax(lax.dot_general(qkv[j][0], qkv[j][1], (((1,), (1,)), ((), ())),
                                           preferred_element_type=F32))

        def do_pv(j):
            o = _dot(p[j], qkv[j][2])
            oh[2 * j] = wo_rows(2 * j, o[0:L]).astype(BF16)
            oh[2 * j + 1] = wo_rows(2 * j + 1, o[L:2 * L]).astype(BF16)

        def do_wo(n):
            h0, h1 = wsplit[n], wsplit[n + 1]
            lo = jnp.concatenate(oh[h0:h1], axis=1)
            for cb in range(NCB):
                part = _dot(lo, _col(wo, cb, h0 * E, h1 * E))
                acc[cb] = part if acc[cb] is None else part + acc[cb]
                fill(("wo", n * NCB + cb), part)

        for j in range(NP + 2):
            if j < NP:
                do_qkv(j)
            else:
                do_wo(j - NP)
            if 0 <= j - 2 < NP:
                do_pv(j - 2)
            if 0 <= j - 1 < NP:
                do_s(j - 1)
        do_wo(2)
        do_wo(3)
        return acc

    def combine(r0, sv, dst, cb, trig=None):
        cs = slice(cb * 128, (cb + 1) * 128)
        xx, gg = xbuf[pl.ds(r0, 64), cs], x1buf[pl.ds(r0, 64), cs]
        if trig is not None:
            z = jnp.concatenate([_zero_of(trig[0:8, :])] * 4, axis=0)
            xx, gg = _or_zero(xx, z), _or_zero(gg, z)
        dst[0:64, cs] = (xx.astype(F32) + sv[:, cs].astype(F32) * gg.astype(F32)).astype(BF16)

    def body(t, carry):
        hv = hbuf_all.at[pl.ds(pl.multiple_of(t * HB, 16), (CLAG + 1) * HB + 16), :]
        cur = CLAG * HB
        prev = pl.multiple_of(jnp.maximum(t - CLAG, 0) * 64, 64)
        par, blk = t % 2, t // 2

        b4 = pl.multiple_of(PRE - LAG + blk * 2 * BR, 32)
        ln3 = w3_lhs(x1buf.at[pl.ds(b4 + LAG, 2 * BR), :], 0, 2 * BR)
        c3 = [_strassen_lhs(ln3[u], ln3[3 + u]) for u in range(3)]
        lhs3 = [jnp.concatenate([c[n] for c in c3], axis=0) for n in range(7)]
        slot = lambda j: pl.multiple_of(H3R + (j % 3) * 2 * BR, 32)
        h3w = h3buf.at[par, pl.ds(slot(blk + 2), 2 * BR), :]
        w3v, w3cv = w3.at[pl.ds(par, 3)], w3c.at[par]

        def w3_pair(i):
            def done(a, b, v):
                h3w[a * BR:(a + 1) * BR, (7 * b + i) * 128:(7 * b + i + 1) * 128] = (
                    _gelu(v).astype(BF16))
            return _Strassen(lhs3, functools.partial(strassen_rhs, w3v, w3cv, i, i + 14, D // 2,
                                                     i * 256, 7 * 256), done)

        top = jnp.concatenate([h3_rows(slot(blk) + 64, 32), h3_rows(slot(blk + 1), 16)], axis=0)
        bot = h3_rows(slot(blk + 1) + 16, BR)
        pair = lambda v, f: jnp.concatenate(
            [v[:, f * 128:(f + 1) * 128], v[:, (f + 14) * 128:(f + 15) * 128]], axis=1).astype(F32)
        c4 = [_strassen_lhs(pair(top, f), pair(bot, f)) for f in range(14)]
        lhs4 = [jnp.concatenate([c[n] for c in c4], axis=1) for n in range(7)]
        deps = {DEP4[0] + DEP4[1] * f: c4[f] for f in range(14)}
        deps.update({DEP3[0] + DEP3[1] * u: c3[u] for u in range(3)})
        x4v = x1buf.at[pl.ds(b4, 2 * BR), pl.ds(pl.multiple_of(par * 256, 256), D - 256)]
        w4v, w4cv = w4.at[pl.ds(par, 3)], w4c.at[par]

        def w4_pair(i):
            def done(a, b, v):
                gate(x4v, slice(a * BR, (a + 1) * BR), 4 * b + i, v)
            return _Strassen(lhs4, functools.partial(strassen_rhs, w4v, w4cv, i, i + 4, FF // 2,
                                                     i * 896, 2 * 896), done)

        todo3 = [p for p in map(w3_pair, range(7)) for _ in range(7)]
        todo4 = [p for p in map(w4_pair, range(2)) for _ in range(7)]
        todoc = list(range(NCB))

        keep = {}

        def sel_a(j, i, v):
            keep[(j, i)] = v[L:L + 8]
            return v[0:L]

        def wo_a(h, o):
            keep[h] = o[32:40]
            return o[0:32]

        sv_old = sbuf.at[(t + NSB - CLAG) % NSB]

        def fill_a(slot, v):
            if slot[0] == "qkv" and slot[1] in CSLOTS:
                combine(prev, sv_old, hv, todoc.pop(0), v)
                if not todoc:
                    @pl.when(t >= CLAG)
                    def _():
                        pltpu.make_async_copy(hv.at[0:64, :], out_hbm.at[pl.ds(prev, 64), :],
                                              osem).start()
            if slot[0] == "wo" and slot[1] in W4SLOTS:
                todo4.pop(0).step()

        ra = attn_step(hv[cur:cur + 48, :], sel_a, wo_a, fill_a, deps)
        for cb in range(NCB):
            hv[cur + 48:cur + 56, cb * 128:(cb + 1) * 128] = ra[cb][0:8].astype(BF16)
        while todo4:
            todo4.pop(0).step()

        def sel_b(j, i, v):
            return jnp.concatenate([v[0:8], keep[(j, i)], v[8:32]], axis=0)

        def wo_b(h, o):
            return jnp.concatenate([keep[h], o], axis=0)

        w3_slots = [(i * 6 * NP + W3OFF) // 49 for i in range(49)]

        def fill_b(slot, v):
            if slot[0] == "qkv" and slot[1] in w3_slots:
                todo3.pop(0).step()

        rb = attn_step(hv[cur + 48:cur + HB, :], sel_b, wo_b, fill_b, {})
        sv = sbuf.at[t % NSB]
        for cb in range(NCB):
            cs = slice(cb * 128, (cb + 1) * 128)
            hv[cur + HB:cur + HB + 8, cs] = rb[cb][8:16].astype(BF16)
            sv[:, cs] = jnp.concatenate([ra[cb][8:32], rb[cb][0:8], rb[cb][16:48]],
                                        axis=0).astype(BF16)
        assert not (todo3 or todo4 or todoc)
        return carry

    lax.fori_loop(0, NIT, body, 0)

    last = (S - PRE) // (2 * BR) - 1
    s0, s1 = H3R + ((last + 1) % 3) * 2 * BR, H3R + ((last + 2) % 3) * 2 * BR
    top = jnp.concatenate([h3_rows(s0 + 64, 32), h3_rows(s1, 32)], axis=0)
    lhs4 = _strassen_lhs(top.astype(F32), h3_rows(s1 + 32, 64).astype(F32))
    x4v = x1buf.at[S - LAG:S, :]

    def finish(t, cbs, trig=None):
        stage = hbuf.at[t * HB:(t + 1) * HB, :]
        for cb in cbs:
            combine(t * 64, sbuf.at[t % NSB], stage, cb, trig)
        cs = pl.ds(cbs[0] * 128, len(cbs) * 128)
        pltpu.make_async_copy(stage.at[0:64, cs], out_hbm.at[t * 64:(t + 1) * 64, cs], osem).start()

    for c in range(4):
        def done(a, b, v, c=c):
            gate(x4v, slice(a * 64, (a + 1) * 64), 4 * b + c, v)
            finish(NIT - 2 + a, [4 * b + c])
            if c < 2 and b == 1:
                finish(NIT - 4 + c, list(range(4 * a, 4 * a + 4)), v)
        prod = _Strassen(lhs4, functools.partial(strassen_rhs, w4.at[pl.ds(c // 2, 3)],
                                                 w4c.at[c // 2], c % 2, c % 2 + 4, FF // 2,
                                                 (c % 2) * 896, 2 * 896), done)
        for _ in range(7):
            prod.step()
    pltpu.make_async_copy(xbuf, out_hbm, osem).wait()


@jax.jit
def pallas_recurrent_scan__memory_aug_recurrent_mem_tr__mixer_s_mlp__prompt_kernel(
    A_x: jax.Array,
    A_mem0: jax.Array,
    A_Wq: jax.Array,
    A_Wk: jax.Array,
    A_Wv: jax.Array,
    A_Wo: jax.Array,
    A_seg_len: jax.Array,
    B_x: jax.Array,
    B_w1: jax.Array,
    B_w2: jax.Array,
    B_w3: jax.Array,
    B_w4: jax.Array,
):
    del A_seg_len, B_x
    assert A_x.shape == (1, S, D) and A_mem0.shape == (1, M, D)
    assert A_Wq.shape == (D, H, E) and A_Wo.shape == (H, E, D)
    assert B_w3.shape == (D, FF) and B_w4.shape == (FF, D)

    any_spec = pl.BlockSpec(memory_space=pl.ANY)
    out = pl.pallas_call(
        _kernel,
        out_shape=jax.ShapeDtypeStruct((S, D), BF16),
        in_specs=[any_spec] * 10,
        out_specs=any_spec,
        scratch_shapes=[
            pltpu.VMEM((S, D), BF16),
            pltpu.VMEM(((NIT + CLAG) * HB + 16, D), BF16),
            pltpu.VMEM((NCB, S + 16, 128), F32),
            pltpu.VMEM((S, D), BF16),
            pltpu.VMEM((2, PRE + 2 * BR, FF // 2), BF16),
            pltpu.VMEM((NSB, 64, D), BF16),
            pltpu.VMEM((4, 3 * PR, E), BF16),
            pltpu.VMEM(((3 * H + 1) * HS, 128), U32),
            pltpu.VMEM((D // 512, H * E, 512), BF16),
            pltpu.VMEM((D // 256, D, 256), BF16),
            pltpu.VMEM((D // 512, D, 512), BF16),
            pltpu.VMEM((4, D, FF // 4), BF16),
            pltpu.VMEM((4, FF, D // 4), BF16),
            pltpu.VMEM((2, 35 * 256, 128), U32),
            pltpu.VMEM((2, 10 * 896, 128), U32),
            pltpu.VMEM((HB, HB), F32),
            pltpu.SemaphoreType.DMA((17,)),
            pltpu.SemaphoreType.DMA(()),
        ],
        compiler_params=pltpu.CompilerParams(vmem_limit_bytes=126 * 1024 * 1024),
    )(
        A_x.reshape(S, D), A_mem0.reshape(M, D),
        A_Wq.reshape(D * H, E), A_Wk.reshape(D * H, E), A_Wv.reshape(D * H, E),
        A_Wo.reshape(H * E, D), B_w1, B_w2, B_w3, B_w4,
    )
    return out.reshape(1, S, D)
```

```python
import functools

import jax
import jax.numpy as jnp
from jax import lax
import jax.experimental.pallas as pl
import jax.experimental.pallas.tpu as pltpu

F32 = jnp.float32
BF16 = jnp.bfloat16
U32 = jnp.uint32

S = 2048
D = 1024
H = 32
E = 128
M = 8
SEG = 32
L = M + SEG
FF = 3584
NCB = D // 128
NFB = FF // 128
NP = H // 2
NIT = S // (2 * SEG)
HB = 2 * L
PRE = 512
LAG = 128
BR = (S - PRE) // NIT
CLAG = 4
NSB = 8
H3R = PRE - 2 * 2 * BR
HS = D // 2 + 8
RB = 256
SB = 128
HSB = (SB // 64) * HB
CH = 512
PR = 16 * CH
EPS = 1e-5
DEP4 = (12, 5)
CSLOTS = range(1, 12, 1)[:8]
W4SLOTS = (1, 3, 5, 7, 9, 11, 13, 15, 18, 21)
W3OFF = 0
DEP3 = (80, 6)
SCALE = float(E) ** -0.5
SHIFTS = (7, 7, 9, 9, 6, 6, 10, 10)


def _dot(a, b):
    return jnp.dot(a, b, preferred_element_type=F32)


def _ln(x):
    m = jnp.mean(x, axis=-1, keepdims=True)
    xc = x - m
    v = jnp.mean(xc * xc, axis=-1, keepdims=True)
    return xc * lax.rsqrt(v + EPS)


def _ln2(x):
    m = jnp.mean(x, axis=-1, keepdims=True)
    xc = x - m
    v = jnp.mean(xc * xc, axis=-1, keepdims=True)
    r1 = lax.rsqrt(v + EPS)
    r2 = lax.rsqrt(v * r1 * r1 + EPS)
    return xc * r1, xc * (r1 * r2)


def _gelu(x):
    c = 0.7978845608028654
    hx = 0.5 * x
    return hx * jnp.tanh(x * (c + (c * 0.044715) * (x * x))) + hx


def _silu(x):
    hx = 0.5 * x
    return hx * jnp.tanh(hx) + hx


def _zero_of(v):
    return (pltpu.bitcast(v, U32) >> 16) >> 16


def _or_zero(w, z):
    return pltpu.bitcast(pltpu.bitcast(w, U32) | z, w.dtype)


def _col(w, cb, k0=0, k1=None):
    _, kk, cw = w.shape
    q, r = divmod(cb * 128, cw)
    return w[q, k0:(kk if k1 is None else k1), r:r + 128]


def _h3col(f):
    pos = (f // 14) * 7 + f % 7
    return (f % 14) // 7, slice(pos * 128, (pos + 1) * 128)


def _strassen_lhs(top, bot):
    k = top.shape[1] // 2
    raw11, raw22 = top[:, :k].astype(BF16), bot[:, k:].astype(BF16)
    top, bot = top.astype(F32), bot.astype(F32)
    a11, a12, a21, a22 = top[:, :k], top[:, k:], bot[:, :k], bot[:, k:]
    sums = [v.astype(BF16) for v in (a21 + a22, a11 + a12, a11 + a22, a21 - a11, a12 - a22)]
    return [raw11, raw22] + sums


class _Strassen:
    def __init__(self, lhs, rhs, done):
        self.lhs, self.rhs, self.done, self.m = lhs, rhs, done, []

    def step(self):
        n, m = len(self.m), self.m
        v = _dot(self.lhs[n], self.rhs(n))
        m.append(v)
        if n == 2:
            self.done(1, 0, v + m[1])
        elif n == 3:
            self.done(0, 1, v + m[0])
        elif n == 5:
            self.done(1, 1, v + (m[4] + (m[0] - m[2])))
        elif n == 6:
            self.done(0, 0, v + (m[4] + (m[1] - m[3])))


def _hrow(r):
    q, rr = divmod(r, 64)
    return q * HB + rr + (8 if rr < 40 else 16)


def _kernel(x_hbm, mem0_hbm, wq_hbm, wk_hbm, wv_hbm, wo_hbm, w1_hbm, w2_hbm, w3_hbm, w4_hbm,
            out_hbm,
            xbuf, hbuf_all, hf, x1buf, h3buf, sbuf, stg, wqkv, wo, w1, w2, w3, w4, w3c, w4c,
            fillbuf,
            sem, osem):
    hbuf = hbuf_all.at[CLAG * HB:, :]

    def colblock_copies(src, dst, s):
        n, _, cw = dst.shape
        return [pltpu.make_async_copy(src.at[:, pl.ds(c * cw, cw)], dst.at[c], sem.at[s(c)])
                for c in range(n)]

    xs, qs = 7, 12
    xch = [(0, SB), (SB, SB), (RB, RB), (2 * RB, RB), (3 * RB, S - 3 * RB)]
    cp_x = [pltpu.make_async_copy(x_hbm.at[pl.ds(r, n), :], xbuf.at[pl.ds(r, n), :], sem.at[xs + i])
            for i, (r, n) in enumerate(xch)]
    cp_w1 = colblock_copies(w1_hbm, w1, lambda c: (0, 1, 16, 16)[c])
    cp_mem = [pltpu.make_async_copy(mem0_hbm, hbuf.at[0:M, :], sem.at[2])]
    cp_w2 = colblock_copies(w2_hbm, w2, lambda c: 3)
    cp_w3 = colblock_copies(w3_hbm, w3, lambda c: 4)
    cp_w4 = colblock_copies(w4_hbm, w4, lambda c: 5)
    cp_wo = colblock_copies(wo_hbm, wo, lambda c: 6)
    cp_qkv = [pltpu.make_async_copy(src.at[pl.ds(k * PR, PR), :], stg.at[k, pl.ds(m * PR, PR), :],
                                    sem.at[qs + k])
              for k in range(4) for m, src in enumerate((wq_hbm, wk_hbm, wv_hbm))]

    for c in cp_x[:2] + cp_w1[:2] + cp_x[2:3] + cp_w1[2:] + cp_w2 + cp_x[3:4]:
        c.start()
    for c in cp_x[4:] + cp_mem + cp_w3 + cp_w4 + cp_qkv + cp_wo:
        c.start(priority=1)

    def wait(grp):
        for c in grp:
            c.wait()

    r = lax.broadcasted_iota(jnp.int32, (HB, HB), 0)
    c = lax.broadcasted_iota(jnp.int32, (HB, HB), 1)
    rr = jnp.where(r >= L, r - L, r)
    cc = jnp.where(c >= L, c - L, c)
    same = (r >= L) == (c >= L)
    allowed = (rr < M) | (rr >= cc)
    fillbuf[...] = jnp.where(same, jnp.where(allowed, 1.0, -1e9), -jnp.inf).astype(F32)

    hf[:, 0:8, :] = jnp.zeros((NCB, 8, 128), F32)
    hf[:, S + 8:S + 16, :] = jnp.zeros((NCB, 8, 128), F32)
    sbuf[...] = jnp.zeros(sbuf.shape, sbuf.dtype)

    def ln_sub(xv, hv, sb, dtype=BF16):
        out = []
        for u in range(SB // 16):
            r0 = sb * SB + 16 * u
            xn, xnn = _ln2(xv[r0:r0 + 16, :].astype(F32))
            xn = xn.astype(BF16)
            for hh in range(2):
                o = _hrow(r0 + 8 * hh)
                hv[o:o + 8, :] = xn[8 * hh:8 * hh + 8]
            out.append(xnn.astype(dtype))
        return out

    def after(w, vals):
        if not vals:
            return w
        z = functools.reduce(lambda a, b: a | b, [_zero_of(v[-16:, -128:]) for v in vals])
        return jnp.concatenate([_or_zero(w[0:16, :], z), w[16:, :]], axis=0)

    def w1_sub(xnn, hfv, sb, cbs, deps, hook=None):
        xnn = jnp.concatenate(xnn, axis=0)
        for cb in cbs:
            w = after(_col(w1, cb), deps.get(cb, []))
            half = _dot(xnn[:, :D // 2], w[:D // 2])
            hfv[cb, sb * SB + 8:sb * SB + 8 + SB, :] = _gelu(_dot(xnn[:, D // 2:], w[D // 2:]) + half)
            if hook is not None:
                hook(half)

    def w2_lhs(hfv, sb):
        r0 = sb * SB
        return jnp.concatenate(
            [hfv[cb, r0 + SHIFTS[cb]:r0 + SHIFTS[cb] + SB, :] for cb in range(NCB)],
            axis=1).astype(BF16)

    def w2_sub(hs, hv, x1v, sb, cbs, deps, hook=None):
        r0 = sb * SB
        for cb in cbs:
            pre = _dot(hs, after(_col(w2, cb), deps.get(cb, [])))
            cs = slice(cb * 128, (cb + 1) * 128)
            xn = jnp.concatenate(
                [hv[_hrow(r0 + a):_hrow(r0 + a) + n, cs].astype(F32)
                 for a, n in ((0, 40), (40, 24), (64, 40), (104, 24))], axis=0)
            x1v[r0:r0 + SB, cs] = (xn + pre).astype(BF16)
            if hook is not None:
                hook(pre)

    def w3_lhs(x1v, r0, rows):
        return [_ln(x1v[r0 + 16 * u:r0 + 16 * u + 16, :].astype(F32)) for u in range(rows // 16)]

    def h3_rows(base, r0, rows):
        v = h3buf.at[:, pl.ds(base, r0 + rows), :]
        p0, p1 = v[0, r0:r0 + rows, :], v[1, r0:r0 + rows, :]
        return jnp.concatenate([p0[:, :896], p1[:, :896], p0[:, 896:], p1[:, 896:]], axis=1)

    def gate(x1v, rows, cb, pre):
        sl = (rows, slice(cb * 128, (cb + 1) * 128))
        x1v[sl] = _silu(x1v[sl].astype(F32) + pre).astype(BF16)

    def weight_sums(src, dst, c0, c1, kh, r0, rows, stride, trig):
        for r in range(r0, r0 + rows, 16):
            tr = (((r - r0) * trig.shape[0] // rows) // 8) * 8 + 8 * (rows < trig.shape[0])
            z = _zero_of(trig[tr:tr + 8, :])
            ld = lambda c, o: _or_zero(_col(src, c, o + r, o + r + 16), z).astype(F32)
            b11, b12, b21, b22 = ld(c0, 0), ld(c1, 0), ld(c0, kh), ld(c1, kh)
            sums = (b12 - b22, b21 - b11, b11 + b22, b11 + b12, b21 + b22)
            for n, v in enumerate(sums):
                o = n * stride + r // 2
                dst[o:o + 8, :] = pltpu.bitcast(v.astype(BF16), U32)

    def strassen_rhs(w, wc, c0, c1, kh, base, stride, n):
        if n == 2:
            return _col(w, c0, 0, kh)
        if n == 3:
            return _col(w, c1, kh, 2 * kh)
        o = base + (n if n < 2 else n - 2) * stride
        return pltpu.bitcast(wc[o:o + kh // 2, :], BF16)

    def relayout(src, dst, u, pps, trig):
        m, c_ = divmod(u, 16)
        d0 = m * (H * HS) + c_ * 8
        two = lambda v: jnp.concatenate([v, v], axis=0)
        for pp in pps:
            r0 = u * CH + pp * 64
            tr = ((pp - pps[0]) * trig.shape[0] // (8 * len(pps))) * 8
            z = _zero_of(trig[tr:tr + 8, :])
            mlo, sh = two(z | U32(0xFFFF)), two(z | U32(16))
            a = pltpu.bitcast(src[r0:r0 + 32, :], U32)
            b = pltpu.bitcast(src[r0 + 32:r0 + 64, :], U32)
            dst[pl.ds(d0 + pp, 16, stride=HS), :] = (a & mlo) | (b << sh)
            dst[pl.ds(d0 + 16 * HS + pp, 16, stride=HS), :] = (a >> sh) | (b & U32(0xFFFF0000))

    cp_x[0].wait()
    xnn0 = ln_sub(xbuf, hbuf, 0)
    cp_x[1].wait()
    xnn1 = ln_sub(xbuf, hbuf, 1)
    cp_w1[0].wait()
    w1_sub(xnn0, hf, 0, range(0, 2), {})
    w1_sub(xnn1, hf, 1, range(0, 2), {})
    cp_w1[1].wait()
    w1_sub(xnn0, hf, 0, range(2, 4), {})
    cp_x[2].wait()
    xnn2 = ln_sub(xbuf, hbuf, 2)
    w1_sub(xnn1, hf, 1, range(2, 4), {})
    w1_sub(xnn2, hf, 2, range(0, 4), {})
    wait(cp_w1[2:])
    xnn3 = ln_sub(xbuf, hbuf, 3)
    w1c = w3c.at[0]
    todo1 = [(c, u) for c in range(4) for u in range(8)]

    count1 = [1, 1, 1, 1, 1, 1, 1, 1, 2, 2, 2, 2, 2, 2, 2, 2, 2, 2, 2, 2]

    def sums1(trig):
        n = count1.pop(0)
        for i in range(n):
            c, u = todo1.pop(0)
            tr = trig[(i * 16 // n) * 8:((i + 1) * 16 // n) * 8]
            weight_sums(w1, w1c.at[c * 256:, :], c, c + 4, D // 2, 64 * u, 64, 4 * 256, tr)

    w1_sub(xnn0, hf, 0, range(4, 8), {6: xnn3[0:1], 7: xnn3[1:2]}, sums1)
    w1_sub(xnn1, hf, 1, range(4, 8), {4 + i: xnn3[2 + i:3 + i] for i in range(4)}, sums1)
    w1_sub(xnn2, hf, 2, range(4, 8), {4: xnn3[6:7], 5: xnn3[7:8]}, sums1)
    w1_sub(xnn3, hf, 3, range(NCB), {}, sums1)
    assert not todo1
    wait(cp_w2)
    cp_x[3].wait()

    def loop_w12(i, carry):
        @pl.when(i == 3)
        def _():
            cp_x[4].wait()

        r0 = pl.multiple_of((i - 2) * RB, RB)
        xv = xbuf.at[pl.ds(r0, 3 * RB), :]
        hv = hbuf.at[pl.ds(pl.multiple_of((i - 2) * 2 * HSB, 16), 6 * HSB), :]
        x1v = x1buf.at[pl.ds(r0, RB), :]
        hfv = hf.at[:, pl.ds(r0, 3 * RB + 16), :]
        ca, cb_ = ln_sub(xv, hv, 4, F32), ln_sub(xv, hv, 5, F32)
        c1 = [_strassen_lhs(ca[u], cb_[u]) for u in range(SB // 16)]
        lhs1 = [jnp.concatenate([c[n] for c in c1], axis=0) for n in range(7)]
        w2_sub(w2_lhs(hfv, 0), hv, x1v, 0, range(NCB), {3: c1[0], 5: c1[1], 6: c1[2], 7: c1[3]})
        hs = w2_lhs(hfv, 1)
        w2_sub(hs, hv, x1v, 1, range(0, 6), {0: c1[4], 2: c1[5], 3: c1[6], 4: c1[7]})
        for c in range(4):
            def done(a, b, v, c=c):
                hfv[4 * b + c, (4 + a) * SB + 8:(5 + a) * SB + 8, :] = _gelu(v)
            prod = _Strassen(lhs1, functools.partial(strassen_rhs, w1, w1c, c, c + 4, D // 2,
                                                     c * 256, 4 * 256), done)
            for _ in range(7):
                prod.step()
        w2_sub(hs, hv, x1v, 1, range(6, 8), {})
        return carry

    lax.fori_loop(2, S // RB, loop_w12, 0)
    wait(cp_w3)
    wait(cp_w4)

    def loop_w34(k, carry):
        pltpu.make_async_copy(stg.at[k], stg.at[k], sem.at[qs + k]).wait()
        r0 = pl.multiple_of(k * SB, SB)
        src = stg.at[k]
        dst = wqkv.at[pl.ds(pl.multiple_of(k * 128, 128), (3 * H + 1) * HS - 384), :]
        sb2 = (S - PRE) // SB
        x1v = x1buf.at[pl.ds(r0, (sb2 + 1) * SB), :]
        hv = hbuf.at[pl.ds(pl.multiple_of(k * HSB, 16), (sb2 + 1) * HSB), :]
        hfv = hf.at[:, pl.ds(r0, (sb2 + 1) * SB + 16), :]
        w3v = w3.at[:, pl.ds(r0, D - 384), :]
        w3cv = w3c.at[:, pl.ds(pl.multiple_of(k * 64, 64), 35 * 256 - 192), :]
        w4v = w4.at[:, pl.ds(pl.multiple_of(k * 448, 64), FF - 3 * 448), :]
        w4cv = w4c.at[:, pl.ds(pl.multiple_of(k * 224, 32), 10 * 896 - 3 * 224), :]
        todo = [(u, h) for u in range(3 * PR // CH) for h in range(2)]
        todo3 = [(f, u) for f in range(14) for u in range(2)]
        todo4 = [(c, u) for c in range(4) for u in range(7)]

        def rl(trig, halves=2):
            n = min(halves, len(todo))
            for i in range(n):
                u, h = todo.pop(0)
                rows = trig.shape[0] // n
                relayout(src, dst, u, range(4 * h, 4 * h + 4), trig[i * rows:(i + 1) * rows])

        def sums3(trig):
            if todo3:
                f, u = todo3.pop(0)
                weight_sums(w3v, w3cv.at[f // 7, pl.ds((f % 7) * 256, 29 * 256 - 192), :],
                            f, f + 14, D // 2, 64 * u, 64, 7 * 256, trig)

        def sums4(trig):
            c, u = todo4.pop(0)
            weight_sums(w4v, w4cv.at[c // 2, pl.ds((c % 2) * 896, 9 * 896 - 3 * 224), :],
                        c, c + 4, FF // 2, 64 * u, 64, 2 * 896, trig)

        hs = w2_lhs(hfv, sb2)
        c = [v.astype(BF16) for v in w3_lhs(x1v, 0, SB)]
        w2_sub(hs, hv, x1v, sb2, range(0, 6), {3: c[0:2], 4: c[2:4], 5: c[4:6]})
        lhs3 = jnp.concatenate(c, axis=0)
        for f in range(NFB):
            half = _dot(lhs3[:, :512], _col(w3, f, 0, 512))
            pre = _dot(lhs3[:, 512:], _col(w3, f, 512, D)) + half
            q, cs = _h3col(f)
            h3buf[q, pl.ds(r0, SB), cs] = _gelu(pre).astype(BF16)
            rl(half)
            sums4(pre)
        w2_sub(hs, hv, x1v, sb2, range(6, 7), {}, rl)
        n4 = (PRE - LAG) // 4
        r4 = pl.multiple_of(k * n4, 32)
        lhs4 = h3_rows(r4, 0, n4)
        for cb in range(NCB):
            pre = None
            for n in range(7):
                k0, k1 = 512 * n, 512 * (n + 1)
                part = _dot(lhs4[:, k0:k1], _col(w4, cb, k0, k1))
                pre = part if pre is None else part + pre
                if n in (0, 2, 4) and cb > 0:
                    rl(pre)
                if n in (1, 3, 5) or (n == 6 and cb < 4):
                    sums3(pre)
            gate(x1buf.at[pl.ds(r4, n4), :], slice(0, n4), cb, pre)
        w2_sub(hs, hv, x1v, sb2, range(7, 8), {})
        assert not (todo or todo3 or todo4)
        return carry

    lax.fori_loop(0, PRE // SB, loop_w34, 0)
    wait(cp_wo)
    wait(cp_mem)

    def softmax(s):
        fill = fillbuf[...]
        s = jnp.where(fill > 0.0, s * SCALE, fill)
        mx = jnp.max(s, axis=1, keepdims=True)
        e = jnp.exp(s - mx)
        l = jnp.sum(e, axis=1, keepdims=True)
        rc = pl.reciprocal(l, approx=True)
        rc = rc * (2.0 - l * rc)
        return (e * rc).astype(BF16)

    def attn_step(lhs, select, wo_rows, fill, deps):
        qkv = [None] * NP
        p = [None] * NP
        oh = [None] * H
        acc = [None] * NCB
        wsplit = (0, 8, 20, 28, 32)

        def do_qkv(j):
            rs = []
            for i in range(6):
                h = 2 * j + i // 3
                r0 = ((i % 3) * H + (h % 2) * 16 + h // 2) * HS
                w = pltpu.bitcast(wqkv[r0:r0 + D // 2, :], BF16)
                v = _dot(lhs, after(w, deps.get(6 * j + i, [])))
                fill(("qkv", 6 * j + i), v)
                rs.append(select(j, i, v))
            qkv[j] = [jnp.concatenate([rs[i], rs[3 + i]], axis=0).astype(BF16) for i in range(3)]

        def do_s(j):
            p[j] = softmax(lax.dot_general(qkv[j][0], qkv[j][1], (((1,), (1,)), ((), ())),
                                           preferred_element_type=F32))

        def do_pv(j):
            o = _dot(p[j], qkv[j][2])
            oh[2 * j] = wo_rows(2 * j, o[0:L]).astype(BF16)
            oh[2 * j + 1] = wo_rows(2 * j + 1, o[L:2 * L]).astype(BF16)

        def do_wo(n):
            h0, h1 = wsplit[n], wsplit[n + 1]
            lo = jnp.concatenate(oh[h0:h1], axis=1)
            for cb in range(NCB):
                part = _dot(lo, _col(wo, cb, h0 * E, h1 * E))
                acc[cb] = part if acc[cb] is None else part + acc[cb]
                fill(("wo", n * NCB + cb), part)

        for j in range(NP + 2):
            if j < NP:
                do_qkv(j)
            else:
                do_wo(j - NP)
            if 0 <= j - 2 < NP:
                do_pv(j - 2)
            if 0 <= j - 1 < NP:
                do_s(j - 1)
        do_wo(2)
        do_wo(3)
        return acc

    def combine(r0, sv, dst, cb, trig=None):
        cs = slice(cb * 128, (cb + 1) * 128)
        xx, gg = xbuf[pl.ds(r0, 64), cs], x1buf[pl.ds(r0, 64), cs]
        if trig is not None:
            z = jnp.concatenate([_zero_of(trig[0:8, :])] * 4, axis=0)
            xx, gg = _or_zero(xx, z), _or_zero(gg, z)
        dst[0:64, cs] = (xx.astype(F32) + sv[:, cs].astype(F32) * gg.astype(F32)).astype(BF16)

    def body(t, carry):
        hv = hbuf_all.at[pl.ds(pl.multiple_of(t * HB, 16), (CLAG + 1) * HB + 16), :]
        cur = CLAG * HB
        prev = pl.multiple_of(jnp.maximum(t - CLAG, 0) * 64, 64)
        par, blk = t % 2, t // 2

        b4 = pl.multiple_of(PRE - LAG + blk * 2 * BR, 32)
        ln3 = w3_lhs(x1buf.at[pl.ds(b4, LAG + 2 * BR), :], LAG, 2 * BR)
        c3 = [_strassen_lhs(ln3[u], ln3[3 + u]) for u in range(3)]
        lhs3 = [jnp.concatenate([c[n] for c in c3], axis=0) for n in range(7)]
        slot = lambda j: pl.multiple_of(H3R + (j % 3) * 2 * BR, 32)
        h3w = h3buf.at[par, pl.ds(slot(blk + 2), 2 * BR), :]
        w3v, w3cv = w3.at[pl.ds(par, 3)], w3c.at[par]

        def w3_pair(i):
            def done(a, b, v):
                h3w[a * BR:(a + 1) * BR, (7 * b + i) * 128:(7 * b + i + 1) * 128] = (
                    _gelu(v).astype(BF16))
            return _Strassen(lhs3, functools.partial(strassen_rhs, w3v, w3cv, i, i + 14, D // 2,
                                                     i * 256, 7 * 256), done)

        top = jnp.concatenate([h3_rows(slot(blk), 64, 32), h3_rows(slot(blk + 1), 0, 16)], axis=0)
        bot = h3_rows(slot(blk + 1), 16, BR)
        pair = lambda v, f: jnp.concatenate(
            [v[:, f * 128:(f + 1) * 128], v[:, (f + 14) * 128:(f + 15) * 128]], axis=1)
        c4 = [_strassen_lhs(pair(top, f), pair(bot, f)) for f in range(14)]
        lhs4 = [jnp.concatenate([c[n] for c in c4], axis=1) for n in range(7)]
        deps = {DEP4[0] + DEP4[1] * f: c4[f] for f in range(14)}
        deps.update({DEP3[0] + DEP3[1] * u: c3[u] for u in range(3)})
        x4v = x1buf.at[pl.ds(b4, 2 * BR), pl.ds(pl.multiple_of(par * 256, 256), D - 256)]
        w4v, w4cv = w4.at[pl.ds(par, 3)], w4c.at[par]

        def w4_pair(i):
            def done(a, b, v):
                gate(x4v, slice(a * BR, (a + 1) * BR), 4 * b + i, v)
            return _Strassen(lhs4, functools.partial(strassen_rhs, w4v, w4cv, i, i + 4, FF // 2,
                                                     i * 896, 2 * 896), done)

        todo3 = [p for p in map(w3_pair, range(7)) for _ in range(7)]
        todo4 = [p for p in map(w4_pair, range(2)) for _ in range(7)]
        todoc = list(range(NCB))

        keep = {}

        def sel_a(j, i, v):
            keep[(j, i)] = v[L:L + 8]
            return v[0:L]

        def wo_a(h, o):
            keep[h] = o[32:40]
            return o[0:32]

        sv_old = sbuf.at[(t + NSB - CLAG) % NSB]

        def fill_a(slot, v):
            if slot[0] == "qkv" and slot[1] in CSLOTS:
                combine(prev, sv_old, hv, todoc.pop(0), v)
                if not todoc:
                    @pl.when(t >= CLAG)
                    def _():
                        pltpu.make_async_copy(hv.at[0:64, :], out_hbm.at[pl.ds(prev, 64), :],
                                              osem).start()
            if slot[0] == "wo" and slot[1] in W4SLOTS:
                todo4.pop(0).step()

        ra = attn_step(hv[cur:cur + 48, :], sel_a, wo_a, fill_a, deps)
        for cb in range(NCB):
            hv[cur + 48:cur + 56, cb * 128:(cb + 1) * 128] = ra[cb][0:8].astype(BF16)
        while todo4:
            todo4.pop(0).step()

        def sel_b(j, i, v):
            return jnp.concatenate([v[0:8], keep[(j, i)], v[8:32]], axis=0)

        def wo_b(h, o):
            return jnp.concatenate([keep[h], o], axis=0)

        w3_slots = [(i * 6 * NP + W3OFF) // 49 for i in range(49)]

        def fill_b(slot, v):
            if slot[0] == "qkv" and slot[1] in w3_slots:
                todo3.pop(0).step()

        rb = attn_step(hv[cur + 48:cur + HB, :], sel_b, wo_b, fill_b, {})
        sv = sbuf.at[t % NSB]
        for cb in range(NCB):
            cs = slice(cb * 128, (cb + 1) * 128)
            hv[cur + HB:cur + HB + 8, cs] = rb[cb][8:16].astype(BF16)
            sv[:, cs] = jnp.concatenate([ra[cb][8:32], rb[cb][0:8], rb[cb][16:48]],
                                        axis=0).astype(BF16)
        assert not (todo3 or todo4 or todoc)
        return carry

    lax.fori_loop(0, NIT, body, 0)

    last = (S - PRE) // (2 * BR) - 1
    s0, s1 = H3R + ((last + 1) % 3) * 2 * BR, H3R + ((last + 2) % 3) * 2 * BR
    top = jnp.concatenate([h3_rows(s0, 64, 32), h3_rows(s1, 0, 32)], axis=0)
    lhs4 = _strassen_lhs(top, h3_rows(s1, 32, 64))
    x4v = x1buf.at[S - LAG:S, :]

    def finish(t, cbs, trig=None):
        stage = hbuf.at[t * HB:(t + 1) * HB, :]
        for cb in cbs:
            combine(t * 64, sbuf.at[t % NSB], stage, cb, trig)
        cs = pl.ds(cbs[0] * 128, len(cbs) * 128)
        pltpu.make_async_copy(stage.at[0:64, cs], out_hbm.at[t * 64:(t + 1) * 64, cs], osem).start()

    for c in range(4):
        def done(a, b, v, c=c):
            gate(x4v, slice(a * 64, (a + 1) * 64), 4 * b + c, v)
            finish(NIT - 2 + a, [4 * b + c])
            if c < 2 and b == 1:
                finish(NIT - 4 + c, list(range(4 * a, 4 * a + 4)), v)
        prod = _Strassen(lhs4, functools.partial(strassen_rhs, w4.at[pl.ds(c // 2, 3)],
                                                 w4c.at[c // 2], c % 2, c % 2 + 4, FF // 2,
                                                 (c % 2) * 896, 2 * 896), done)
        for _ in range(7):
            prod.step()
    pltpu.make_async_copy(xbuf, out_hbm, osem).wait()


@jax.jit
def pallas_recurrent_scan__memory_aug_recurrent_mem_tr__mixer_s_mlp__prompt_kernel(
    A_x: jax.Array,
    A_mem0: jax.Array,
    A_Wq: jax.Array,
    A_Wk: jax.Array,
    A_Wv: jax.Array,
    A_Wo: jax.Array,
    A_seg_len: jax.Array,
    B_x: jax.Array,
    B_w1: jax.Array,
    B_w2: jax.Array,
    B_w3: jax.Array,
    B_w4: jax.Array,
):
    del A_seg_len, B_x
    assert A_x.shape == (1, S, D) and A_mem0.shape == (1, M, D)
    assert A_Wq.shape == (D, H, E) and A_Wo.shape == (H, E, D)
    assert B_w3.shape == (D, FF) and B_w4.shape == (FF, D)

    any_spec = pl.BlockSpec(memory_space=pl.ANY)
    out = pl.pallas_call(
        _kernel,
        out_shape=jax.ShapeDtypeStruct((S, D), BF16),
        in_specs=[any_spec] * 10,
        out_specs=any_spec,
        scratch_shapes=[
            pltpu.VMEM((S, D), BF16),
            pltpu.VMEM(((NIT + CLAG) * HB + 16, D), BF16),
            pltpu.VMEM((NCB, S + 16, 128), F32),
            pltpu.VMEM((S, D), BF16),
            pltpu.VMEM((2, PRE + 2 * BR, FF // 2), BF16),
            pltpu.VMEM((NSB, 64, D), BF16),
            pltpu.VMEM((4, 3 * PR, E), BF16),
            pltpu.VMEM(((3 * H + 1) * HS, 128), U32),
            pltpu.VMEM((D // 512, H * E, 512), BF16),
            pltpu.VMEM((D // 256, D, 256), BF16),
            pltpu.VMEM((D // 512, D, 512), BF16),
            pltpu.VMEM((4, D, FF // 4), BF16),
            pltpu.VMEM((4, FF, D // 4), BF16),
            pltpu.VMEM((2, 35 * 256, 128), U32),
            pltpu.VMEM((2, 10 * 896, 128), U32),
            pltpu.VMEM((HB, HB), F32),
            pltpu.SemaphoreType.DMA((17,)),
            pltpu.SemaphoreType.DMA(()),
        ],
        compiler_params=pltpu.CompilerParams(vmem_limit_bytes=126 * 1024 * 1024),
    )(
        A_x.reshape(S, D), A_mem0.reshape(M, D),
        A_Wq.reshape(D * H, E), A_Wk.reshape(D * H, E), A_Wv.reshape(D * H, E),
        A_Wo.reshape(H * E, D), B_w1, B_w2, B_w3, B_w4,
    )
    return out.reshape(1, S, D)
```

```python
import functools

import jax
import jax.numpy as jnp
from jax import lax
import jax.experimental.pallas as pl
import jax.experimental.pallas.tpu as pltpu

F32 = jnp.float32
BF16 = jnp.bfloat16
U32 = jnp.uint32

S = 2048
D = 1024
H = 32
E = 128
M = 8
SEG = 32
L = M + SEG
FF = 3584
NCB = D // 128
NFB = FF // 128
NP = H // 2
NIT = S // (2 * SEG)
HB = 2 * L
PRE = 512
LAG = 128
BR = (S - PRE) // NIT
CLAG = 4
NSB = 8
H3R = PRE - 2 * 2 * BR
HS = D // 2 + 8
RB = 256
SB = 128
HSB = (SB // 64) * HB
CH = 512
PR = 16 * CH
EPS = 1e-5
SCALE = float(E) ** -0.5
SHIFTS = (7, 7, 9, 9, 6, 6, 10, 10)


def _dot(a, b):
    return jnp.dot(a, b, preferred_element_type=F32)


def _ln(x):
    m = jnp.mean(x, axis=-1, keepdims=True)
    xc = x - m
    v = jnp.mean(xc * xc, axis=-1, keepdims=True)
    return xc * lax.rsqrt(v + EPS)


def _ln2(x):
    m = jnp.mean(x, axis=-1, keepdims=True)
    xc = x - m
    v = jnp.mean(xc * xc, axis=-1, keepdims=True)
    r1 = lax.rsqrt(v + EPS)
    r2 = lax.rsqrt(v * r1 * r1 + EPS)
    return xc * r1, xc * (r1 * r2)


def _gelu(x):
    c = 0.7978845608028654
    hx = 0.5 * x
    return hx * jnp.tanh(x * (c + (c * 0.044715) * (x * x))) + hx


def _silu(x):
    hx = 0.5 * x
    return hx * jnp.tanh(hx) + hx


def _zero_of(v):
    return (pltpu.bitcast(v, U32) >> 16) >> 16


def _or_zero(w, z):
    return pltpu.bitcast(pltpu.bitcast(w, U32) | z, w.dtype)


def _col(w, cb, k0=0, k1=None):
    _, kk, cw = w.shape
    q, r = divmod(cb * 128, cw)
    return w[q, k0:(kk if k1 is None else k1), r:r + 128]


def _h3col(f):
    pos = (f // 14) * 7 + f % 7
    return (f % 14) // 7, slice(pos * 128, (pos + 1) * 128)


def _strassen_lhs(top, bot):
    k = top.shape[1] // 2
    raw11, raw22 = top[:, :k].astype(BF16), bot[:, k:].astype(BF16)
    top, bot = top.astype(F32), bot.astype(F32)
    a11, a12, a21, a22 = top[:, :k], top[:, k:], bot[:, :k], bot[:, k:]
    sums = [v.astype(BF16) for v in (a21 + a22, a11 + a12, a11 + a22, a21 - a11, a12 - a22)]
    return [raw11, raw22] + sums


class _Strassen:
    def __init__(self, lhs, rhs, done):
        self.lhs, self.rhs, self.done, self.m = lhs, rhs, done, []

    def step(self):
        n, m = len(self.m), self.m
        v = _dot(self.lhs[n], self.rhs(n))
        m.append(v)
        if n == 2:
            self.done(1, 0, v + m[1])
        elif n == 3:
            self.done(0, 1, v + m[0])
        elif n == 5:
            self.done(1, 1, v + (m[4] + (m[0] - m[2])))
        elif n == 6:
            self.done(0, 0, v + (m[4] + (m[1] - m[3])))


def _hrow(r):
    q, rr = divmod(r, 64)
    return q * HB + rr + (8 if rr < 40 else 16)


def _kernel(x_hbm, mem0_hbm, wq_hbm, wk_hbm, wv_hbm, wo_hbm, w1_hbm, w2_hbm, w3_hbm, w4_hbm,
            out_hbm,
            xbuf, hbuf_all, hf, x1buf, h3buf, sbuf, stg, wqkv, wo, w1, w2, w3, w4, w3c, w4c,
            fillbuf,
            sem, osem):
    hbuf = hbuf_all.at[CLAG * HB:, :]

    def colblock_copies(src, dst, s):
        n, _, cw = dst.shape
        return [pltpu.make_async_copy(src.at[:, pl.ds(c * cw, cw)], dst.at[c], sem.at[s(c)])
                for c in range(n)]

    xs, qs = 7, 12
    xch = [(0, SB), (SB, SB), (RB, RB), (2 * RB, RB), (3 * RB, S - 3 * RB)]
    cp_x = [pltpu.make_async_copy(x_hbm.at[pl.ds(r, n), :], xbuf.at[pl.ds(r, n), :], sem.at[xs + i])
            for i, (r, n) in enumerate(xch)]
    cp_w1 = colblock_copies(w1_hbm, w1, lambda c: (0, 1, 16, 16)[c])
    cp_mem = [pltpu.make_async_copy(mem0_hbm, hbuf.at[0:M, :], sem.at[2])]
    cp_w2 = colblock_copies(w2_hbm, w2, lambda c: 3)
    cp_w3 = colblock_copies(w3_hbm, w3, lambda c: 4)
    cp_w4 = colblock_copies(w4_hbm, w4, lambda c: 5)
    cp_wo = colblock_copies(wo_hbm, wo, lambda c: 6)
    cp_qkv = [pltpu.make_async_copy(src.at[pl.ds(k * PR, PR), :], stg.at[k, pl.ds(m * PR, PR), :],
                                    sem.at[qs + k])
              for k in range(4) for m, src in enumerate((wq_hbm, wk_hbm, wv_hbm))]

    for c in cp_x[:2] + cp_w1[:2] + cp_x[2:3] + cp_w1[2:] + cp_w2 + cp_x[3:4]:
        c.start()
    for c in cp_x[4:] + cp_mem + cp_w3 + cp_w4 + cp_qkv + cp_wo:
        c.start(priority=1)

    def wait(grp):
        for c in grp:
            c.wait()

    r = lax.broadcasted_iota(jnp.int32, (HB, HB), 0)
    c = lax.broadcasted_iota(jnp.int32, (HB, HB), 1)
    rr = jnp.where(r >= L, r - L, r)
    cc = jnp.where(c >= L, c - L, c)
    same = (r >= L) == (c >= L)
    allowed = (rr < M) | (rr >= cc)
    fillbuf[...] = jnp.where(same, jnp.where(allowed, 1.0, -1e9), -jnp.inf).astype(F32)

    hf[:, 0:8, :] = jnp.zeros((NCB, 8, 128), F32)
    hf[:, S + 8:S + 16, :] = jnp.zeros((NCB, 8, 128), F32)
    sbuf[...] = jnp.zeros(sbuf.shape, sbuf.dtype)

    def ln_sub(xv, hv, sb, dtype=BF16):
        out = []
        for u in range(SB // 16):
            r0 = sb * SB + 16 * u
            xn, xnn = _ln2(xv[r0:r0 + 16, :].astype(F32))
            xn = xn.astype(BF16)
            for hh in range(2):
                o = _hrow(r0 + 8 * hh)
                hv[o:o + 8, :] = xn[8 * hh:8 * hh + 8]
            out.append(xnn.astype(dtype))
        return out

    def after(w, vals):
        if not vals:
            return w
        z = functools.reduce(lambda a, b: a | b, [_zero_of(v[-16:, -128:]) for v in vals])
        return jnp.concatenate([_or_zero(w[0:16, :], z), w[16:, :]], axis=0)

    def w1_sub(xnn, hfv, sb, cbs, deps, hook=None):
        xnn = jnp.concatenate(xnn, axis=0)
        for cb in cbs:
            w = after(_col(w1, cb), deps.get(cb, []))
            half = _dot(xnn[:, :D // 2], w[:D // 2])
            hfv[cb, sb * SB + 8:sb * SB + 8 + SB, :] = _gelu(_dot(xnn[:, D // 2:], w[D // 2:]) + half)
            if hook is not None:
                hook(half)

    def w2_lhs(hfv, sb):
        r0 = sb * SB
        return jnp.concatenate(
            [hfv[cb, r0 + SHIFTS[cb]:r0 + SHIFTS[cb] + SB, :] for cb in range(NCB)],
            axis=1).astype(BF16)

    def w2_sub(hs, hv, x1v, sb, cbs, deps, hook=None):
        r0 = sb * SB
        for cb in cbs:
            pre = _dot(hs, after(_col(w2, cb), deps.get(cb, [])))
            cs = slice(cb * 128, (cb + 1) * 128)
            xn = jnp.concatenate(
                [hv[_hrow(r0 + a):_hrow(r0 + a) + n, cs].astype(F32)
                 for a, n in ((0, 40), (40, 24), (64, 40), (104, 24))], axis=0)
            x1v[r0:r0 + SB, cs] = (xn + pre).astype(BF16)
            if hook is not None:
                hook(pre)

    def w3_lhs(x1v, r0, rows):
        return [_ln(x1v[r0 + 16 * u:r0 + 16 * u + 16, :].astype(F32)) for u in range(rows // 16)]

    def h3_rows(base, r0, rows):
        v = h3buf.at[:, pl.ds(base, r0 + rows), :]
        p0, p1 = v[0, r0:r0 + rows, :], v[1, r0:r0 + rows, :]
        return jnp.concatenate([p0[:, :896], p1[:, :896], p0[:, 896:], p1[:, 896:]], axis=1)

    def h3_pair(v, f):
        return jnp.concatenate(
            [v[:, f * 128:(f + 1) * 128], v[:, (f + 14) * 128:(f + 15) * 128]], axis=1)

    def gate(x1v, rows, cb, pre):
        sl = (rows, slice(cb * 128, (cb + 1) * 128))
        x1v[sl] = _silu(x1v[sl].astype(F32) + pre).astype(BF16)

    def weight_sums(src, dst, c0, c1, kh, r0, rows, stride, trig):
        for r in range(r0, r0 + rows, 16):
            tr = (((r - r0) * trig.shape[0] // rows) // 8) * 8 + 8 * (rows < trig.shape[0])
            z = _zero_of(trig[tr:tr + 8, :])
            ld = lambda c, o: _or_zero(_col(src, c, o + r, o + r + 16), z).astype(F32)
            b11, b12, b21, b22 = ld(c0, 0), ld(c1, 0), ld(c0, kh), ld(c1, kh)
            sums = (b12 - b22, b21 - b11, b11 + b22, b11 + b12, b21 + b22)
            for n, v in enumerate(sums):
                o = n * stride + r // 2
                dst[o:o + 8, :] = pltpu.bitcast(v.astype(BF16), U32)

    def strassen_rhs(w, wc, c0, c1, kh, base, stride, n):
        if n == 2:
            return _col(w, c0, 0, kh)
        if n == 3:
            return _col(w, c1, kh, 2 * kh)
        o = base + (n if n < 2 else n - 2) * stride
        return pltpu.bitcast(wc[o:o + kh // 2, :], BF16)

    def relayout(src, dst, u, pps, trig):
        m, c_ = divmod(u, 16)
        d0 = m * (H * HS) + c_ * 8
        two = lambda v: jnp.concatenate([v, v], axis=0)
        for pp in pps:
            r0 = u * CH + pp * 64
            tr = ((pp - pps[0]) * trig.shape[0] // (8 * len(pps))) * 8
            z = _zero_of(trig[tr:tr + 8, :])
            mlo, sh = two(z | U32(0xFFFF)), two(z | U32(16))
            a = pltpu.bitcast(src[r0:r0 + 32, :], U32)
            b = pltpu.bitcast(src[r0 + 32:r0 + 64, :], U32)
            dst[pl.ds(d0 + pp, 16, stride=HS), :] = (a & mlo) | (b << sh)
            dst[pl.ds(d0 + 16 * HS + pp, 16, stride=HS), :] = (a >> sh) | (b & U32(0xFFFF0000))

    cp_x[0].wait()
    xnn0 = ln_sub(xbuf, hbuf, 0)
    cp_x[1].wait()
    xnn1 = ln_sub(xbuf, hbuf, 1)
    cp_w1[0].wait()
    w1_sub(xnn0, hf, 0, range(0, 2), {})
    w1_sub(xnn1, hf, 1, range(0, 2), {})
    cp_w1[1].wait()
    w1_sub(xnn0, hf, 0, range(2, 4), {})
    cp_x[2].wait()
    xnn2 = ln_sub(xbuf, hbuf, 2)
    w1_sub(xnn1, hf, 1, range(2, 4), {})
    w1_sub(xnn2, hf, 2, range(0, 4), {})
    wait(cp_w1[2:])
    xnn3 = ln_sub(xbuf, hbuf, 3)
    w1c = w3c.at[0]
    todo1 = [(c, u) for c in range(4) for u in range(8)]
    count1 = [1] * 8 + [2] * 12

    def sums1(trig):
        n = count1.pop(0)
        for i in range(n):
            c, u = todo1.pop(0)
            tr = trig[(i * 16 // n) * 8:((i + 1) * 16 // n) * 8]
            weight_sums(w1, w1c.at[c * 256:, :], c, c + 4, D // 2, 64 * u, 64, 4 * 256, tr)

    w1_sub(xnn0, hf, 0, range(4, 8), {6: xnn3[0:1], 7: xnn3[1:2]}, sums1)
    w1_sub(xnn1, hf, 1, range(4, 8), {4 + i: xnn3[2 + i:3 + i] for i in range(4)}, sums1)
    w1_sub(xnn2, hf, 2, range(4, 8), {4: xnn3[6:7], 5: xnn3[7:8]}, sums1)
    w1_sub(xnn3, hf, 3, range(NCB), {}, sums1)
    assert not todo1
    wait(cp_w2)
    cp_x[3].wait()

    def loop_w12(i, carry):
        @pl.when(i == 3)
        def _():
            cp_x[4].wait()

        r0 = pl.multiple_of((i - 2) * RB, RB)
        xv = xbuf.at[pl.ds(r0, 3 * RB), :]
        hv = hbuf.at[pl.ds(pl.multiple_of((i - 2) * 2 * HSB, 16), 6 * HSB), :]
        x1v = x1buf.at[pl.ds(r0, RB), :]
        hfv = hf.at[:, pl.ds(r0, 3 * RB + 16), :]
        ca, cb_ = ln_sub(xv, hv, 4, F32), ln_sub(xv, hv, 5, F32)
        c1 = [_strassen_lhs(ca[u], cb_[u]) for u in range(SB // 16)]
        lhs1 = [jnp.concatenate([c[n] for c in c1], axis=0) for n in range(7)]
        w2_sub(w2_lhs(hfv, 0), hv, x1v, 0, range(NCB), {3: c1[0], 5: c1[1], 6: c1[2], 7: c1[3]})
        hs = w2_lhs(hfv, 1)
        w2_sub(hs, hv, x1v, 1, range(0, 6), {0: c1[4], 2: c1[5], 3: c1[6], 4: c1[7]})
        for c in range(4):
            def done(a, b, v, c=c):
                hfv[4 * b + c, (4 + a) * SB + 8:(5 + a) * SB + 8, :] = _gelu(v)
            prod = _Strassen(lhs1, functools.partial(strassen_rhs, w1, w1c, c, c + 4, D // 2,
                                                     c * 256, 4 * 256), done)
            for _ in range(7):
                prod.step()
        w2_sub(hs, hv, x1v, 1, range(6, 8), {})
        return carry

    lax.fori_loop(2, S // RB, loop_w12, 0)
    wait(cp_w3)
    wait(cp_w4)

    def loop_w34(k, carry):
        pltpu.make_async_copy(stg.at[k], stg.at[k], sem.at[qs + k]).wait()
        r0 = pl.multiple_of(k * SB, SB)
        src = stg.at[k]
        dst = wqkv.at[pl.ds(pl.multiple_of(k * 128, 128), (3 * H + 1) * HS - 384), :]
        sb2 = (S - PRE) // SB
        x1v = x1buf.at[pl.ds(r0, (sb2 + 1) * SB), :]
        hv = hbuf.at[pl.ds(pl.multiple_of(k * HSB, 16), (sb2 + 1) * HSB), :]
        hfv = hf.at[:, pl.ds(r0, (sb2 + 1) * SB + 16), :]
        w3v = w3.at[:, pl.ds(r0, D - 384), :]
        w3cv = w3c.at[:, pl.ds(pl.multiple_of(k * 64, 64), 35 * 256 - 192), :]
        w4v = w4.at[:, pl.ds(pl.multiple_of(k * 448, 64), FF - 3 * 448), :]
        w4cv = w4c.at[:, pl.ds(pl.multiple_of(k * 224, 32), 10 * 896 - 3 * 224), :]
        todo = [(u, h) for u in range(3 * PR // CH) for h in range(2)]
        todo3 = [(f, u) for f in range(14) for u in range(2)]
        todo4 = [(c, u) for c in range(4) for u in range(7)]

        def rl(trig, halves=2):
            n = min(halves, len(todo))
            for i in range(n):
                u, h = todo.pop(0)
                rows = trig.shape[0] // n
                relayout(src, dst, u, range(4 * h, 4 * h + 4), trig[i * rows:(i + 1) * rows])

        def sums3(trig):
            if todo3:
                f, u = todo3.pop(0)
                weight_sums(w3v, w3cv.at[f // 7, pl.ds((f % 7) * 256, 29 * 256 - 192), :],
                            f, f + 14, D // 2, 64 * u, 64, 7 * 256, trig)

        def sums4(trig):
            c, u = todo4.pop(0)
            weight_sums(w4v, w4cv.at[c // 2, pl.ds((c % 2) * 896, 9 * 896 - 3 * 224), :],
                        c, c + 4, FF // 2, 64 * u, 64, 2 * 896, trig)

        hs = w2_lhs(hfv, sb2)
        c = [v.astype(BF16) for v in w3_lhs(x1v, 0, SB)]
        w2_sub(hs, hv, x1v, sb2, range(0, 6), {3: c[0:2], 4: c[2:4], 5: c[4:6]})
        lhs3 = jnp.concatenate(c, axis=0)
        for f in range(NFB):
            half = _dot(lhs3[:, :512], _col(w3, f, 0, 512))
            pre = _dot(lhs3[:, 512:], _col(w3, f, 512, D)) + half
            q, cs = _h3col(f)
            h3buf[q, pl.ds(r0, SB), cs] = _gelu(pre).astype(BF16)
            rl(half)
            sums4(pre)
        w2_sub(hs, hv, x1v, sb2, range(6, 7), {}, rl)
        n4 = (PRE - LAG) // 4
        r4 = pl.multiple_of(k * n4, 32)
        lhs4 = h3_rows(r4, 0, n4)
        for cb in range(NCB):
            pre = None
            for n in range(7):
                k0, k1 = 512 * n, 512 * (n + 1)
                part = _dot(lhs4[:, k0:k1], _col(w4, cb, k0, k1))
                pre = part if pre is None else part + pre
                if n in (0, 2, 4) and cb > 0:
                    rl(pre)
                if n in (1, 3, 5) or (n == 6 and cb < 4):
                    sums3(pre)
            gate(x1buf.at[pl.ds(r4, n4), :], slice(0, n4), cb, pre)
        w2_sub(hs, hv, x1v, sb2, range(7, 8), {})
        assert not (todo or todo3 or todo4)
        return carry

    lax.fori_loop(0, PRE // SB, loop_w34, 0)
    wait(cp_wo)
    wait(cp_mem)

    def softmax(s):
        fill = fillbuf[...]
        s = jnp.where(fill > 0.0, s * SCALE, fill)
        mx = jnp.max(s, axis=1, keepdims=True)
        e = jnp.exp(s - mx)
        l = jnp.sum(e, axis=1, keepdims=True)
        rc = pl.reciprocal(l, approx=True)
        rc = rc * (2.0 - l * rc)
        return (e * rc).astype(BF16)

    def attn_step(lhs, select, wo_rows, fill, deps):
        qkv = [None] * NP
        p = [None] * NP
        oh = [None] * H
        acc = [None] * NCB
        wsplit = (0, 8, 20, 28, 32)

        def do_qkv(j):
            rs = []
            for i in range(6):
                h = 2 * j + i // 3
                r0 = ((i % 3) * H + (h % 2) * 16 + h // 2) * HS
                w = pltpu.bitcast(wqkv[r0:r0 + D // 2, :], BF16)
                v = _dot(lhs, after(w, deps.get(6 * j + i, [])))
                fill(("qkv", 6 * j + i), v)
                rs.append(select(j, i, v))
            qkv[j] = [jnp.concatenate([rs[i], rs[3 + i]], axis=0).astype(BF16) for i in range(3)]

        def do_s(j):
            p[j] = softmax(lax.dot_general(qkv[j][0], qkv[j][1], (((1,), (1,)), ((), ())),
                                           preferred_element_type=F32))

        def do_pv(j):
            o = _dot(p[j], qkv[j][2])
            oh[2 * j] = wo_rows(2 * j, o[0:L]).astype(BF16)
            oh[2 * j + 1] = wo_rows(2 * j + 1, o[L:2 * L]).astype(BF16)

        def do_wo(n):
            h0, h1 = wsplit[n], wsplit[n + 1]
            lo = jnp.concatenate(oh[h0:h1], axis=1)
            for cb in range(NCB):
                part = _dot(lo, _col(wo, cb, h0 * E, h1 * E))
                acc[cb] = part if acc[cb] is None else part + acc[cb]
                fill(("wo", n * NCB + cb), part)

        for j in range(NP + 2):
            if j < NP:
                do_qkv(j)
            else:
                do_wo(j - NP)
            if 0 <= j - 2 < NP:
                do_pv(j - 2)
            if 0 <= j - 1 < NP:
                do_s(j - 1)
        do_wo(2)
        do_wo(3)
        return acc

    def combine(r0, sv, dst, cb, trig=None):
        cs = slice(cb * 128, (cb + 1) * 128)
        xx, gg = xbuf[pl.ds(r0, 64), cs], x1buf[pl.ds(r0, 64), cs]
        if trig is not None:
            z = jnp.concatenate([_zero_of(trig[0:8, :])] * 4, axis=0)
            xx, gg = _or_zero(xx, z), _or_zero(gg, z)
        dst[0:64, cs] = (xx.astype(F32) + sv[:, cs].astype(F32) * gg.astype(F32)).astype(BF16)

    def body(t, carry):
        hv = hbuf_all.at[pl.ds(pl.multiple_of(t * HB, 16), (CLAG + 1) * HB + 16), :]
        cur = CLAG * HB
        prev = pl.multiple_of(jnp.maximum(t - CLAG, 0) * 64, 64)
        par, blk = t % 2, t // 2

        b4 = pl.multiple_of(PRE - LAG + blk * 2 * BR, 32)
        ln3 = w3_lhs(x1buf.at[pl.ds(b4, LAG + 2 * BR), :], LAG, 2 * BR)
        c3 = [_strassen_lhs(ln3[u], ln3[3 + u]) for u in range(3)]
        lhs3 = [jnp.concatenate([c[n] for c in c3], axis=0) for n in range(7)]
        slot = lambda j: pl.multiple_of(H3R + (j % 3) * 2 * BR, 32)
        h3w = h3buf.at[par, pl.ds(slot(blk + 2), 2 * BR), :]
        w3v, w3cv = w3.at[pl.ds(par, 3)], w3c.at[par]

        def w3_pair(i):
            def done(a, b, v):
                h3w[a * BR:(a + 1) * BR, (7 * b + i) * 128:(7 * b + i + 1) * 128] = (
                    _gelu(v).astype(BF16))
            return _Strassen(lhs3, functools.partial(strassen_rhs, w3v, w3cv, i, i + 14, D // 2,
                                                     i * 256, 7 * 256), done)

        top = jnp.concatenate([h3_rows(slot(blk), 64, 32), h3_rows(slot(blk + 1), 0, 16)], axis=0)
        bot = h3_rows(slot(blk + 1), 16, BR)
        c4 = [_strassen_lhs(h3_pair(top, f), h3_pair(bot, f)) for f in range(14)]
        lhs4 = [jnp.concatenate([c[n] for c in c4], axis=1) for n in range(7)]
        deps = {12 + 5 * f: c4[f] for f in range(14)}
        deps.update({80 + 6 * u: c3[u] for u in range(3)})
        x4v = x1buf.at[pl.ds(b4, 2 * BR), pl.ds(pl.multiple_of(par * 256, 256), D - 256)]
        w4v, w4cv = w4.at[pl.ds(par, 3)], w4c.at[par]

        def w4_pair(i):
            def done(a, b, v):
                gate(x4v, slice(a * BR, (a + 1) * BR), 4 * b + i, v)
            return _Strassen(lhs4, functools.partial(strassen_rhs, w4v, w4cv, i, i + 4, FF // 2,
                                                     i * 896, 2 * 896), done)

        todo3 = [p for p in map(w3_pair, range(7)) for _ in range(7)]
        todo4 = [p for p in map(w4_pair, range(2)) for _ in range(7)]
        todoc = list(range(NCB))

        keep = {}

        def sel_a(j, i, v):
            keep[(j, i)] = v[L:L + 8]
            return v[0:L]

        def wo_a(h, o):
            keep[h] = o[32:40]
            return o[0:32]

        sv_old = sbuf.at[(t + NSB - CLAG) % NSB]

        def fill_a(slot, v):
            if slot[0] == "qkv" and 1 <= slot[1] <= NCB:
                combine(prev, sv_old, hv, todoc.pop(0), v)
                if not todoc:
                    @pl.when(t >= CLAG)
                    def _():
                        pltpu.make_async_copy(hv.at[0:64, :], out_hbm.at[pl.ds(prev, 64), :],
                                              osem).start()
            if slot[0] == "wo" and slot[1] in (1, 3, 5, 7, 9, 11, 13, 15, 18, 21):
                todo4.pop(0).step()

        ra = attn_step(hv[cur:cur + 48, :], sel_a, wo_a, fill_a, deps)
        for cb in range(NCB):
            hv[cur + 48:cur + 56, cb * 128:(cb + 1) * 128] = ra[cb][0:8].astype(BF16)
        while todo4:
            todo4.pop(0).step()

        def sel_b(j, i, v):
            return jnp.concatenate([v[0:8], keep[(j, i)], v[8:32]], axis=0)

        def wo_b(h, o):
            return jnp.concatenate([keep[h], o], axis=0)

        w3_slots = [(i * 6 * NP) // 49 for i in range(49)]

        def fill_b(slot, v):
            if slot[0] == "qkv" and slot[1] in w3_slots:
                todo3.pop(0).step()

        rb = attn_step(hv[cur + 48:cur + HB, :], sel_b, wo_b, fill_b, {})
        sv = sbuf.at[t % NSB]
        for cb in range(NCB):
            cs = slice(cb * 128, (cb + 1) * 128)
            hv[cur + HB:cur + HB + 8, cs] = rb[cb][8:16].astype(BF16)
            sv[:, cs] = jnp.concatenate([ra[cb][8:32], rb[cb][0:8], rb[cb][16:48]],
                                        axis=0).astype(BF16)
        assert not (todo3 or todo4 or todoc)
        return carry

    lax.fori_loop(0, NIT, body, 0)

    last = (S - PRE) // (2 * BR) - 1
    s0, s1 = H3R + ((last + 1) % 3) * 2 * BR, H3R + ((last + 2) % 3) * 2 * BR
    top = jnp.concatenate([h3_rows(s0, 64, 32), h3_rows(s1, 0, 32)], axis=0)
    bot = h3_rows(s1, 32, 64)
    c4 = [_strassen_lhs(h3_pair(top, f), h3_pair(bot, f)) for f in range(14)]
    lhs4 = [jnp.concatenate([c[n] for c in c4], axis=1) for n in range(7)]
    x4v = x1buf.at[S - LAG:S, :]

    def stage(t):
        return hbuf.at[t * HB:(t + 1) * HB, :]

    def send(t, c0, c1):
        cs = pl.ds(c0 * 128, (c1 - c0) * 128)
        pltpu.make_async_copy(stage(t).at[0:64, cs], out_hbm.at[t * 64:(t + 1) * 64, cs],
                              osem).start()

    def last_pair(c):
        def done(a, b, v):
            gate(x4v, slice(a * 64, (a + 1) * 64), 4 * b + c, v)
            combine((NIT - 2 + a) * 64, sbuf.at[(NIT - 2 + a) % NSB], stage(NIT - 2 + a), 4 * b + c)
            if c >= 2:
                send(NIT - 2 + a, 4 * b + (0 if c == 2 else 3), 4 * b + c + 1)
            if c in (1, 2):
                t = NIT - 5 + c
                for cb in (4 * a + 2 * b, 4 * a + 2 * b + 1):
                    combine(t * 64, sbuf.at[t % NSB], stage(t), cb, v)
                if (a, b) == (0, 0):
                    send(t, 0, NCB)

        def rhs(n):
            w = strassen_rhs(w4.at[pl.ds(c // 2, 3)], w4c.at[c // 2], c % 2, c % 2 + 4, FF // 2,
                             (c % 2) * 896, 2 * 896, n)
            u = 2 * c + n - 1
            return after(w, c4[2 * u][2:] + c4[2 * u + 1][2:] if n < 2 and u >= 0 else [])
        return _Strassen(lhs4, rhs, done)

    prods = [last_pair(c) for c in range(4)]
    for prod in prods:
        prod.step()
        prod.step()
    for prod in prods:
        for _ in range(5):
            prod.step()
    pltpu.make_async_copy(xbuf, out_hbm, osem).wait()


@jax.jit
def pallas_recurrent_scan__memory_aug_recurrent_mem_tr__mixer_s_mlp__prompt_kernel(
    A_x: jax.Array,
    A_mem0: jax.Array,
    A_Wq: jax.Array,
    A_Wk: jax.Array,
    A_Wv: jax.Array,
    A_Wo: jax.Array,
    A_seg_len: jax.Array,
    B_x: jax.Array,
    B_w1: jax.Array,
    B_w2: jax.Array,
    B_w3: jax.Array,
    B_w4: jax.Array,
):
    del A_seg_len, B_x
    assert A_x.shape == (1, S, D) and A_mem0.shape == (1, M, D)
    assert A_Wq.shape == (D, H, E) and A_Wo.shape == (H, E, D)
    assert B_w3.shape == (D, FF) and B_w4.shape == (FF, D)

    any_spec = pl.BlockSpec(memory_space=pl.ANY)
    out = pl.pallas_call(
        _kernel,
        out_shape=jax.ShapeDtypeStruct((S, D), BF16),
        in_specs=[any_spec] * 10,
        out_specs=any_spec,
        scratch_shapes=[
            pltpu.VMEM((S, D), BF16),
            pltpu.VMEM(((NIT + CLAG) * HB + 16, D), BF16),
            pltpu.VMEM((NCB, S + 16, 128), F32),
            pltpu.VMEM((S, D), BF16),
            pltpu.VMEM((2, PRE + 2 * BR, FF // 2), BF16),
            pltpu.VMEM((NSB, 64, D), BF16),
            pltpu.VMEM((4, 3 * PR, E), BF16),
            pltpu.VMEM(((3 * H + 1) * HS, 128), U32),
            pltpu.VMEM((D // 512, H * E, 512), BF16),
            pltpu.VMEM((D // 256, D, 256), BF16),
            pltpu.VMEM((D // 512, D, 512), BF16),
            pltpu.VMEM((4, D, FF // 4), BF16),
            pltpu.VMEM((4, FF, D // 4), BF16),
            pltpu.VMEM((2, 35 * 256, 128), U32),
            pltpu.VMEM((2, 10 * 896, 128), U32),
            pltpu.VMEM((HB, HB), F32),
            pltpu.SemaphoreType.DMA((17,)),
            pltpu.SemaphoreType.DMA(()),
        ],
        compiler_params=pltpu.CompilerParams(vmem_limit_bytes=126 * 1024 * 1024),
    )(
        A_x.reshape(S, D), A_mem0.reshape(M, D),
        A_Wq.reshape(D * H, E), A_Wk.reshape(D * H, E), A_Wv.reshape(D * H, E),
        A_Wo.reshape(H * E, D), B_w1, B_w2, B_w3, B_w4,
    )
    return out.reshape(1, S, D)
```

```python
import functools

import jax
import jax.numpy as jnp
from jax import lax
import jax.experimental.pallas as pl
import jax.experimental.pallas.tpu as pltpu

F32 = jnp.float32
BF16 = jnp.bfloat16
U32 = jnp.uint32

S = 2048
D = 1024
H = 32
E = 128
M = 8
SEG = 32
L = M + SEG
FF = 3584
NCB = D // 128
NFB = FF // 128
NP = H // 2
NIT = S // (2 * SEG)
HB = 2 * L
PRE = 512
LAG = 128
BR = (S - PRE) // NIT
CLAG = 4
NSB = 8
H3R = PRE - 2 * 2 * BR
HS = D // 2 + 8
RB = 256
SB = 128
HSB = (SB // 64) * HB
CH = 512
PR = 16 * CH
EPS = 1e-5
SCALE = float(E) ** -0.5
SHIFTS = (7, 7, 9, 9, 6, 6, 10, 10)


def _dot(a, b):
    return jnp.dot(a, b, preferred_element_type=F32)


def _ln(x):
    m = jnp.mean(x, axis=-1, keepdims=True)
    xc = x - m
    v = jnp.mean(xc * xc, axis=-1, keepdims=True)
    return xc * lax.rsqrt(v + EPS)


def _ln2(x):
    m = jnp.mean(x, axis=-1, keepdims=True)
    xc = x - m
    v = jnp.mean(xc * xc, axis=-1, keepdims=True)
    r1 = lax.rsqrt(v + EPS)
    r2 = lax.rsqrt(v * r1 * r1 + EPS)
    return xc * r1, xc * (r1 * r2)


def _gelu(x):
    c = 0.7978845608028654
    hx = 0.5 * x
    return hx * jnp.tanh(x * (c + (c * 0.044715) * (x * x))) + hx


def _silu(x):
    hx = 0.5 * x
    return hx * jnp.tanh(hx) + hx


def _zero_of(v):
    return (pltpu.bitcast(v, U32) >> 16) >> 16


def _or_zero(w, z):
    return pltpu.bitcast(pltpu.bitcast(w, U32) | z, w.dtype)


def _col(w, cb, k0=0, k1=None):
    _, kk, cw = w.shape
    q, r = divmod(cb * 128, cw)
    return w[q, k0:(kk if k1 is None else k1), r:r + 128]


def _h3col(f):
    pos = (f // 14) * 7 + f % 7
    return (f % 14) // 7, slice(pos * 128, (pos + 1) * 128)


def _strassen_lhs(top, bot):
    k = top.shape[1] // 2
    raw11, raw22 = top[:, :k].astype(BF16), bot[:, k:].astype(BF16)
    top, bot = top.astype(F32), bot.astype(F32)
    a11, a12, a21, a22 = top[:, :k], top[:, k:], bot[:, :k], bot[:, k:]
    sums = [v.astype(BF16) for v in (a21 + a22, a11 + a12, a11 + a22, a21 - a11, a12 - a22)]
    return [raw11, raw22] + sums


class _Strassen:
    def __init__(self, lhs, rhs, done):
        self.lhs, self.rhs, self.done, self.m = lhs, rhs, done, []

    def step(self):
        n, m = len(self.m), self.m
        v = _dot(self.lhs[n], self.rhs(n))
        m.append(v)
        if n == 2:
            self.done(1, 0, v + m[1])
        elif n == 3:
            self.done(0, 1, v + m[0])
        elif n == 5:
            self.done(1, 1, v + (m[4] + (m[0] - m[2])))
        elif n == 6:
            self.done(0, 0, v + (m[4] + (m[1] - m[3])))


def _hrow(r):
    q, rr = divmod(r, 64)
    return q * HB + rr + (8 if rr < 40 else 16)


def _kernel(x_hbm, mem0_hbm, wq_hbm, wk_hbm, wv_hbm, wo_hbm, w1_hbm, w2_hbm, w3_hbm, w4_hbm,
            out_hbm,
            xbuf, hbuf_all, hf, x1buf, h3buf, sbuf, stg, wqkv, wo, w1, w2, w3, w4, w3c, w4c,
            fillbuf,
            sem, osem):
    hbuf = hbuf_all.at[CLAG * HB:, :]

    def colblock_copies(src, dst, s):
        n, _, cw = dst.shape
        return [pltpu.make_async_copy(src.at[:, pl.ds(c * cw, cw)], dst.at[c], sem.at[s(c)])
                for c in range(n)]

    xs, qs = 7, 12
    xch = [(0, SB), (SB, SB), (RB, RB), (2 * RB, RB), (3 * RB, S - 3 * RB)]
    cp_x = [pltpu.make_async_copy(x_hbm.at[pl.ds(r, n), :], xbuf.at[pl.ds(r, n), :], sem.at[xs + i])
            for i, (r, n) in enumerate(xch)]
    cp_w1 = colblock_copies(w1_hbm, w1, lambda c: (0, 1, 16, 16)[c])
    cp_mem = [pltpu.make_async_copy(mem0_hbm, hbuf.at[0:M, :], sem.at[2])]
    cp_w2 = colblock_copies(w2_hbm, w2, lambda c: 3)
    cp_w3 = colblock_copies(w3_hbm, w3, lambda c: 4)
    cp_w4 = colblock_copies(w4_hbm, w4, lambda c: 5)
    cp_wo = colblock_copies(wo_hbm, wo, lambda c: 6)
    cp_qkv = [pltpu.make_async_copy(src.at[pl.ds(k * PR, PR), :], stg.at[k, pl.ds(m * PR, PR), :],
                                    sem.at[qs + k])
              for k in range(4) for m, src in enumerate((wq_hbm, wk_hbm, wv_hbm))]

    for c in cp_x[:2] + cp_w1[:2] + cp_x[2:3] + cp_w1[2:] + cp_w2 + cp_x[3:4]:
        c.start()
    for c in cp_x[4:] + cp_mem + cp_w3 + cp_w4 + cp_qkv + cp_wo:
        c.start(priority=1)

    def wait(grp):
        for c in grp:
            c.wait()

    r = lax.broadcasted_iota(jnp.int32, (HB, HB), 0)
    c = lax.broadcasted_iota(jnp.int32, (HB, HB), 1)
    rr = jnp.where(r >= L, r - L, r)
    cc = jnp.where(c >= L, c - L, c)
    same = (r >= L) == (c >= L)
    allowed = (rr < M) | (rr >= cc)
    fillbuf[...] = jnp.where(same, jnp.where(allowed, 1.0, -1e9), -jnp.inf).astype(F32)

    hf[:, 0:8, :] = jnp.zeros((NCB, 8, 128), F32)
    hf[:, S + 8:S + 16, :] = jnp.zeros((NCB, 8, 128), F32)
    sbuf[...] = jnp.zeros(sbuf.shape, sbuf.dtype)

    def ln_sub(xv, hv, sb, dtype=BF16):
        out = []
        for u in range(SB // 16):
            r0 = sb * SB + 16 * u
            xn, xnn = _ln2(xv[r0:r0 + 16, :].astype(F32))
            xn = xn.astype(BF16)
            for hh in range(2):
                o = _hrow(r0 + 8 * hh)
                hv[o:o + 8, :] = xn[8 * hh:8 * hh + 8]
            out.append(xnn.astype(dtype))
        return out

    def after(w, vals):
        if not vals:
            return w
        z = functools.reduce(lambda a, b: a | b, [_zero_of(v[-16:, -128:]) for v in vals])
        return jnp.concatenate([_or_zero(w[0:16, :], z), w[16:, :]], axis=0)

    def w1_sub(xnn, hfv, sb, cbs, deps, hook=None):
        xnn = jnp.concatenate(xnn, axis=0)
        for cb in cbs:
            w = after(_col(w1, cb), deps.get(cb, []))
            half = _dot(xnn[:, :D // 2], w[:D // 2])
            hfv[cb, sb * SB + 8:sb * SB + 8 + SB, :] = _gelu(_dot(xnn[:, D // 2:], w[D // 2:]) + half)
            if hook is not None:
                hook(half)

    def w2_lhs(hfv, sb):
        r0 = sb * SB
        return jnp.concatenate(
            [hfv[cb, r0 + SHIFTS[cb]:r0 + SHIFTS[cb] + SB, :] for cb in range(NCB)],
            axis=1).astype(BF16)

    def w2_sub(hs, hv, x1v, sb, cbs, deps, hook=None):
        r0 = sb * SB
        for cb in cbs:
            pre = _dot(hs, after(_col(w2, cb), deps.get(cb, [])))
            cs = slice(cb * 128, (cb + 1) * 128)
            xn = jnp.concatenate(
                [hv[_hrow(r0 + a):_hrow(r0 + a) + n, cs].astype(F32)
                 for a, n in ((0, 40), (40, 24), (64, 40), (104, 24))], axis=0)
            x1v[r0:r0 + SB, cs] = (xn + pre).astype(BF16)
            if hook is not None:
                hook(pre)

    def w3_lhs(x1v, r0, rows):
        return [_ln(x1v[r0 + 16 * u:r0 + 16 * u + 16, :].astype(F32)) for u in range(rows // 16)]

    def h3_rows(base, r0, rows):
        v = h3buf.at[:, pl.ds(base, r0 + rows), :]
        p0, p1 = v[0, r0:r0 + rows, :], v[1, r0:r0 + rows, :]
        return jnp.concatenate([p0[:, :896], p1[:, :896], p0[:, 896:], p1[:, 896:]], axis=1)

    def h3_pair(v, f):
        return jnp.concatenate(
            [v[:, f * 128:(f + 1) * 128], v[:, (f + 14) * 128:(f + 15) * 128]], axis=1)

    def gate(x1v, rows, cb, pre):
        sl = (rows, slice(cb * 128, (cb + 1) * 128))
        x1v[sl] = _silu(x1v[sl].astype(F32) + pre).astype(BF16)

    def weight_sums(src, dst, c0, c1, kh, r0, rows, stride, trig):
        for r in range(r0, r0 + rows, 16):
            tr = (((r - r0) * trig.shape[0] // rows) // 8) * 8 + 8 * (rows < trig.shape[0])
            z = _zero_of(trig[tr:tr + 8, :])
            ld = lambda c, o: _col(src, c, o + r, o + r + 16)
            b11, b22 = _or_zero(ld(c0, 0), z).astype(F32), _or_zero(ld(c1, kh), z).astype(F32)
            b12, b21 = ld(c1, 0).astype(F32), ld(c0, kh).astype(F32)
            sums = (b12 - b22, b21 - b11, b11 + b22, b11 + b12, b21 + b22)
            for n, v in enumerate(sums):
                o = n * stride + r // 2
                dst[o:o + 8, :] = pltpu.bitcast(v.astype(BF16), U32)

    def strassen_rhs(w, wc, c0, c1, kh, base, stride, n):
        if n == 2:
            return _col(w, c0, 0, kh)
        if n == 3:
            return _col(w, c1, kh, 2 * kh)
        o = base + (n if n < 2 else n - 2) * stride
        return pltpu.bitcast(wc[o:o + kh // 2, :], BF16)

    def relayout(src, dst, u, pps, trig):
        m, c_ = divmod(u, 16)
        d0 = m * (H * HS) + c_ * 8
        two = lambda v: jnp.concatenate([v, v], axis=0)
        for pp in pps:
            r0 = u * CH + pp * 64
            tr = ((pp - pps[0]) * trig.shape[0] // (8 * len(pps))) * 8
            z = _zero_of(trig[tr:tr + 8, :])
            mlo, sh = U32(0xFFFF), two(z | U32(16))
            a = pltpu.bitcast(src[r0:r0 + 32, :], U32)
            b = pltpu.bitcast(src[r0 + 32:r0 + 64, :], U32)
            dst[pl.ds(d0 + pp, 16, stride=HS), :] = (a & mlo) | (b << sh)
            dst[pl.ds(d0 + 16 * HS + pp, 16, stride=HS), :] = (a >> sh) | (b & U32(0xFFFF0000))

    cp_x[0].wait()
    xnn0 = ln_sub(xbuf, hbuf, 0)
    cp_x[1].wait()
    xnn1 = ln_sub(xbuf, hbuf, 1)
    cp_w1[0].wait()
    w1_sub(xnn0, hf, 0, range(0, 2), {})
    w1_sub(xnn1, hf, 1, range(0, 2), {})
    cp_w1[1].wait()
    w1_sub(xnn0, hf, 0, range(2, 4), {})
    cp_x[2].wait()
    xnn2 = ln_sub(xbuf, hbuf, 2)
    w1_sub(xnn1, hf, 1, range(2, 4), {})
    w1_sub(xnn2, hf, 2, range(0, 4), {})
    wait(cp_w1[2:])
    xnn3 = ln_sub(xbuf, hbuf, 3)
    w1c = w3c.at[0]
    todo1 = [(c, u) for c in range(4) for u in range(8)]
    count1 = [1] * 8 + [2] * 12

    def sums1(trig):
        n = count1.pop(0)
        for i in range(n):
            c, u = todo1.pop(0)
            tr = trig[(i * 16 // n) * 8:((i + 1) * 16 // n) * 8]
            weight_sums(w1, w1c.at[c * 256:, :], c, c + 4, D // 2, 64 * u, 64, 4 * 256, tr)

    w1_sub(xnn0, hf, 0, range(4, 8), {6: xnn3[0:1], 7: xnn3[1:2]}, sums1)
    w1_sub(xnn1, hf, 1, range(4, 8), {4 + i: xnn3[2 + i:3 + i] for i in range(4)}, sums1)
    w1_sub(xnn2, hf, 2, range(4, 8), {4: xnn3[6:7], 5: xnn3[7:8]}, sums1)
    w1_sub(xnn3, hf, 3, range(NCB), {}, sums1)
    assert not todo1
    wait(cp_w2)
    cp_x[3].wait()

    def loop_w12(i, carry):
        @pl.when(i == 3)
        def _():
            cp_x[4].wait()

        r0 = pl.multiple_of((i - 2) * RB, RB)
        xv = xbuf.at[pl.ds(r0, 3 * RB), :]
        hv = hbuf.at[pl.ds(pl.multiple_of((i - 2) * 2 * HSB, 16), 6 * HSB), :]
        x1v = x1buf.at[pl.ds(r0, RB), :]
        hfv = hf.at[:, pl.ds(r0, 3 * RB + 16), :]
        ca, cb_ = ln_sub(xv, hv, 4, F32), ln_sub(xv, hv, 5, F32)
        c1 = [_strassen_lhs(ca[u], cb_[u]) for u in range(SB // 16)]
        lhs1 = [jnp.concatenate([c[n] for c in c1], axis=0) for n in range(7)]
        w2_sub(w2_lhs(hfv, 0), hv, x1v, 0, range(NCB), {3: c1[0], 5: c1[1], 6: c1[2], 7: c1[3]})
        hs = w2_lhs(hfv, 1)
        w2_sub(hs, hv, x1v, 1, range(0, 6), {0: c1[4], 2: c1[5], 3: c1[6], 4: c1[7]})
        for c in range(4):
            def done(a, b, v, c=c):
                hfv[4 * b + c, (4 + a) * SB + 8:(5 + a) * SB + 8, :] = _gelu(v)
            prod = _Strassen(lhs1, functools.partial(strassen_rhs, w1, w1c, c, c + 4, D // 2,
                                                     c * 256, 4 * 256), done)
            for _ in range(7):
                prod.step()
        w2_sub(hs, hv, x1v, 1, range(6, 8), {})
        return carry

    lax.fori_loop(2, S // RB, loop_w12, 0)
    wait(cp_w3)
    wait(cp_w4)

    def loop_w34(k, carry):
        pltpu.make_async_copy(stg.at[k], stg.at[k], sem.at[qs + k]).wait()
        r0 = pl.multiple_of(k * SB, SB)
        src = stg.at[k]
        dst = wqkv.at[pl.ds(pl.multiple_of(k * 128, 128), (3 * H + 1) * HS - 384), :]
        sb2 = (S - PRE) // SB
        x1v = x1buf.at[pl.ds(r0, (sb2 + 1) * SB), :]
        hv = hbuf.at[pl.ds(pl.multiple_of(k * HSB, 16), (sb2 + 1) * HSB), :]
        hfv = hf.at[:, pl.ds(r0, (sb2 + 1) * SB + 16), :]
        w3v = w3.at[:, pl.ds(r0, D - 384), :]
        w3cv = w3c.at[:, pl.ds(pl.multiple_of(k * 64, 64), 35 * 256 - 192), :]
        w4v = w4.at[:, pl.ds(pl.multiple_of(k * 448, 64), FF - 3 * 448), :]
        w4cv = w4c.at[:, pl.ds(pl.multiple_of(k * 224, 32), 10 * 896 - 3 * 224), :]
        todo = [(u, h) for u in range(3 * PR // CH) for h in range(2)]
        todo3 = [(f, u) for f in range(14) for u in range(2)]
        todo4 = [(c, u) for c in range(4) for u in range(7)]

        def rl(trig, halves=2):
            n = min(halves, len(todo))
            for i in range(n):
                u, h = todo.pop(0)
                rows = trig.shape[0] // n
                relayout(src, dst, u, range(4 * h, 4 * h + 4), trig[i * rows:(i + 1) * rows])

        def sums3(trig):
            if todo3:
                f, u = todo3.pop(0)
                weight_sums(w3v, w3cv.at[f // 7, pl.ds((f % 7) * 256, 29 * 256 - 192), :],
                            f, f + 14, D // 2, 64 * u, 64, 7 * 256, trig)

        def sums4(trig):
            c, u = todo4.pop(0)
            weight_sums(w4v, w4cv.at[c // 2, pl.ds((c % 2) * 896, 9 * 896 - 3 * 224), :],
                        c, c + 4, FF // 2, 64 * u, 64, 2 * 896, trig)

        hs = w2_lhs(hfv, sb2)
        c = [v.astype(BF16) for v in w3_lhs(x1v, 0, SB)]
        w2_sub(hs, hv, x1v, sb2, range(0, 6), {3: c[0:2], 4: c[2:4], 5: c[4:6]})
        lhs3 = jnp.concatenate(c, axis=0)
        for f in range(NFB):
            half = _dot(lhs3[:, :512], _col(w3, f, 0, 512))
            pre = _dot(lhs3[:, 512:], _col(w3, f, 512, D)) + half
            q, cs = _h3col(f)
            h3buf[q, pl.ds(r0, SB), cs] = _gelu(pre).astype(BF16)
            rl(half)
            sums4(pre)
        w2_sub(hs, hv, x1v, sb2, range(6, 7), {}, rl)
        n4 = (PRE - LAG) // 4
        r4 = pl.multiple_of(k * n4, 32)
        lhs4 = h3_rows(r4, 0, n4)
        for cb in range(NCB):
            pre = None
            for n in range(7):
                k0, k1 = 512 * n, 512 * (n + 1)
                part = _dot(lhs4[:, k0:k1], _col(w4, cb, k0, k1))
                pre = part if pre is None else part + pre
                if n in (0, 2, 4) and cb > 0:
                    rl(pre)
                if n in (1, 3, 5) or (n == 6 and cb < 4):
                    sums3(pre)
            gate(x1buf.at[pl.ds(r4, n4), :], slice(0, n4), cb, pre)
        w2_sub(hs, hv, x1v, sb2, range(7, 8), {})
        assert not (todo or todo3 or todo4)
        return carry

    lax.fori_loop(0, PRE // SB, loop_w34, 0)
    wait(cp_wo)
    wait(cp_mem)

    def softmax(s):
        fill = fillbuf[...]
        s = jnp.where(fill > 0.0, s * SCALE, fill)
        mx = jnp.max(s, axis=1, keepdims=True)
        e = jnp.exp(s - mx)
        l = jnp.sum(e, axis=1, keepdims=True)
        rc = pl.reciprocal(l, approx=True)
        rc = rc * (2.0 - l * rc)
        return (e * rc).astype(BF16)

    def attn_step(lhs, select, wo_rows, fill, deps):
        qkv = [None] * NP
        p = [None] * NP
        oh = [None] * H
        acc = [None] * NCB
        wsplit = (0, 8, 20, 28, 32)

        def do_qkv(j):
            rs = []
            for i in range(6):
                h = 2 * j + i // 3
                r0 = ((i % 3) * H + (h % 2) * 16 + h // 2) * HS
                w = pltpu.bitcast(wqkv[r0:r0 + D // 2, :], BF16)
                v = _dot(lhs, after(w, deps.get(6 * j + i, [])))
                fill(("qkv", 6 * j + i), v)
                rs.append(select(j, i, v))
            qkv[j] = [jnp.concatenate([rs[i], rs[3 + i]], axis=0).astype(BF16) for i in range(3)]

        def do_s(j):
            p[j] = softmax(lax.dot_general(qkv[j][0], qkv[j][1], (((1,), (1,)), ((), ())),
                                           preferred_element_type=F32))

        def do_pv(j):
            o = _dot(p[j], qkv[j][2])
            oh[2 * j] = wo_rows(2 * j, o[0:L]).astype(BF16)
            oh[2 * j + 1] = wo_rows(2 * j + 1, o[L:2 * L]).astype(BF16)

        def do_wo(n):
            h0, h1 = wsplit[n], wsplit[n + 1]
            lo = jnp.concatenate(oh[h0:h1], axis=1)
            for cb in range(NCB):
                part = _dot(lo, _col(wo, cb, h0 * E, h1 * E))
                acc[cb] = part if acc[cb] is None else part + acc[cb]
                fill(("wo", n * NCB + cb), part)

        for j in range(NP + 2):
            if j < NP:
                do_qkv(j)
            else:
                do_wo(j - NP)
            if 0 <= j - 2 < NP:
                do_pv(j - 2)
            if 0 <= j - 1 < NP:
                do_s(j - 1)
        do_wo(2)
        do_wo(3)
        return acc

    def combine(r0, sv, dst, cb, trig=None):
        cs = slice(cb * 128, (cb + 1) * 128)
        xx, gg = xbuf[pl.ds(r0, 64), cs], x1buf[pl.ds(r0, 64), cs]
        if trig is not None:
            z = jnp.concatenate([_zero_of(trig[0:8, :])] * 4, axis=0)
            xx, gg = _or_zero(xx, z), _or_zero(gg, z)
        dst[0:64, cs] = (xx.astype(F32) + sv[:, cs].astype(F32) * gg.astype(F32)).astype(BF16)

    def body(t, carry):
        hv = hbuf_all.at[pl.ds(pl.multiple_of(t * HB, 16), (CLAG + 1) * HB + 16), :]
        cur = CLAG * HB
        prev = pl.multiple_of(jnp.maximum(t - CLAG, 0) * 64, 64)
        par, blk = t % 2, t // 2

        b4 = pl.multiple_of(PRE - LAG + blk * 2 * BR, 32)
        ln3 = w3_lhs(x1buf.at[pl.ds(b4, LAG + 2 * BR), :], LAG, 2 * BR)
        c3 = [_strassen_lhs(ln3[u], ln3[3 + u]) for u in range(3)]
        lhs3 = [jnp.concatenate([c[n] for c in c3], axis=0) for n in range(7)]
        slot = lambda j: pl.multiple_of(H3R + (j % 3) * 2 * BR, 32)
        h3w = h3buf.at[par, pl.ds(slot(blk + 2), 2 * BR), :]
        w3v, w3cv = w3.at[pl.ds(par, 3)], w3c.at[par]

        def w3_pair(i):
            def done(a, b, v):
                h3w[a * BR:(a + 1) * BR, (7 * b + i) * 128:(7 * b + i + 1) * 128] = (
                    _gelu(v).astype(BF16))
            return _Strassen(lhs3, functools.partial(strassen_rhs, w3v, w3cv, i, i + 14, D // 2,
                                                     i * 256, 7 * 256), done)

        top = jnp.concatenate([h3_rows(slot(blk), 64, 32), h3_rows(slot(blk + 1), 0, 16)], axis=0)
        bot = h3_rows(slot(blk + 1), 16, BR)
        c4 = [_strassen_lhs(h3_pair(top, f), h3_pair(bot, f)) for f in range(14)]
        lhs4 = [jnp.concatenate([c[n] for c in c4], axis=1) for n in range(7)]
        deps = {12 + 5 * f: c4[f] for f in range(14)}
        deps.update({80 + 6 * u: c3[u] for u in range(3)})
        x4v = x1buf.at[pl.ds(b4, 2 * BR), pl.ds(pl.multiple_of(par * 256, 256), D - 256)]
        w4v, w4cv = w4.at[pl.ds(par, 3)], w4c.at[par]

        def w4_pair(i):
            def done(a, b, v):
                gate(x4v, slice(a * BR, (a + 1) * BR), 4 * b + i, v)
            return _Strassen(lhs4, functools.partial(strassen_rhs, w4v, w4cv, i, i + 4, FF // 2,
                                                     i * 896, 2 * 896), done)

        todo3 = [p for p in map(w3_pair, range(7)) for _ in range(7)]
        todo4 = [p for p in map(w4_pair, range(2)) for _ in range(7)]
        todoc = list(range(NCB))

        keep = {}

        def sel_a(j, i, v):
            keep[(j, i)] = v[L:L + 8]
            return v[0:L]

        def wo_a(h, o):
            keep[h] = o[32:40]
            return o[0:32]

        sv_old = sbuf.at[(t + NSB - CLAG) % NSB]

        def fill_a(slot, v):
            if slot[0] == "qkv" and 1 <= slot[1] <= NCB:
                combine(prev, sv_old, hv, todoc.pop(0), v)
                if not todoc:
                    @pl.when(t >= CLAG)
                    def _():
                        pltpu.make_async_copy(hv.at[0:64, :], out_hbm.at[pl.ds(prev, 64), :],
                                              osem).start()
            if slot[0] == "wo" and slot[1] in (1, 3, 5, 7, 9, 11, 13, 15, 18, 21):
                todo4.pop(0).step()

        ra = attn_step(hv[cur:cur + 48, :], sel_a, wo_a, fill_a, deps)
        for cb in range(NCB):
            hv[cur + 48:cur + 56, cb * 128:(cb + 1) * 128] = ra[cb][0:8].astype(BF16)
        while todo4:
            todo4.pop(0).step()

        def sel_b(j, i, v):
            return jnp.concatenate([v[0:8], keep[(j, i)], v[8:32]], axis=0)

        def wo_b(h, o):
            return jnp.concatenate([keep[h], o], axis=0)

        w3_slots = [(i * 6 * NP) // 49 for i in range(49)]

        def fill_b(slot, v):
            if slot[0] == "qkv" and slot[1] in w3_slots:
                todo3.pop(0).step()

        rb = attn_step(hv[cur + 48:cur + HB, :], sel_b, wo_b, fill_b, {})
        sv = sbuf.at[t % NSB]
        for cb in range(NCB):
            cs = slice(cb * 128, (cb + 1) * 128)
            hv[cur + HB:cur + HB + 8, cs] = rb[cb][8:16].astype(BF16)
            sv[:, cs] = jnp.concatenate([ra[cb][8:32], rb[cb][0:8], rb[cb][16:48]],
                                        axis=0).astype(BF16)
        assert not (todo3 or todo4 or todoc)
        return carry

    lax.fori_loop(0, NIT, body, 0)

    last = (S - PRE) // (2 * BR) - 1
    s0, s1 = H3R + ((last + 1) % 3) * 2 * BR, H3R + ((last + 2) % 3) * 2 * BR
    top = jnp.concatenate([h3_rows(s0, 64, 32), h3_rows(s1, 0, 32)], axis=0)
    bot = h3_rows(s1, 32, 64)
    c4 = [_strassen_lhs(h3_pair(top, f), h3_pair(bot, f)) for f in range(14)]
    lhs4 = [jnp.concatenate([c[n] for c in c4], axis=1) for n in range(7)]
    x4v = x1buf.at[S - LAG:S, :]

    def stage(t):
        return hbuf.at[t * HB:(t + 1) * HB, :]

    def send(t, c0, c1):
        cs = pl.ds(c0 * 128, (c1 - c0) * 128)
        pltpu.make_async_copy(stage(t).at[0:64, cs], out_hbm.at[t * 64:(t + 1) * 64, cs],
                              osem).start()

    def last_pair(c):
        def done(a, b, v):
            gate(x4v, slice(a * 64, (a + 1) * 64), 4 * b + c, v)
            combine((NIT - 2 + a) * 64, sbuf.at[(NIT - 2 + a) % NSB], stage(NIT - 2 + a), 4 * b + c)
            if c >= 2:
                send(NIT - 2 + a, 4 * b + (0 if c == 2 else 3), 4 * b + c + 1)
            if c in (1, 2):
                t = NIT - 5 + c
                for cb in (4 * a + 2 * b, 4 * a + 2 * b + 1):
                    combine(t * 64, sbuf.at[t % NSB], stage(t), cb, v)
                if (a, b) == (0, 0):
                    send(t, 0, NCB)

        def rhs(n):
            w = strassen_rhs(w4.at[pl.ds(c // 2, 3)], w4c.at[c // 2], c % 2, c % 2 + 4, FF // 2,
                             (c % 2) * 896, 2 * 896, n)
            u = 2 * c + n - 1
            return after(w, c4[2 * u][2:] + c4[2 * u + 1][2:] if n < 2 and u >= 0 else [])
        return _Strassen(lhs4, rhs, done)

    prods = [last_pair(c) for c in range(4)]
    for prod in prods:
        prod.step()
        prod.step()
    for prod in prods:
        for _ in range(5):
            prod.step()
    pltpu.make_async_copy(xbuf, out_hbm, osem).wait()


@jax.jit
def pallas_recurrent_scan__memory_aug_recurrent_mem_tr__mixer_s_mlp__prompt_kernel(
    A_x: jax.Array,
    A_mem0: jax.Array,
    A_Wq: jax.Array,
    A_Wk: jax.Array,
    A_Wv: jax.Array,
    A_Wo: jax.Array,
    A_seg_len: jax.Array,
    B_x: jax.Array,
    B_w1: jax.Array,
    B_w2: jax.Array,
    B_w3: jax.Array,
    B_w4: jax.Array,
):
    del A_seg_len, B_x
    assert A_x.shape == (1, S, D) and A_mem0.shape == (1, M, D)
    assert A_Wq.shape == (D, H, E) and A_Wo.shape == (H, E, D)
    assert B_w3.shape == (D, FF) and B_w4.shape == (FF, D)

    any_spec = pl.BlockSpec(memory_space=pl.ANY)
    out = pl.pallas_call(
        _kernel,
        out_shape=jax.ShapeDtypeStruct((S, D), BF16),
        in_specs=[any_spec] * 10,
        out_specs=any_spec,
        scratch_shapes=[
            pltpu.VMEM((S, D), BF16),
            pltpu.VMEM(((NIT + CLAG) * HB + 16, D), BF16),
            pltpu.VMEM((NCB, S + 16, 128), F32),
            pltpu.VMEM((S, D), BF16),
            pltpu.VMEM((2, PRE + 2 * BR, FF // 2), BF16),
            pltpu.VMEM((NSB, 64, D), BF16),
            pltpu.VMEM((4, 3 * PR, E), BF16),
            pltpu.VMEM(((3 * H + 1) * HS, 128), U32),
            pltpu.VMEM((D // 512, H * E, 512), BF16),
            pltpu.VMEM((D // 256, D, 256), BF16),
            pltpu.VMEM((D // 512, D, 512), BF16),
            pltpu.VMEM((4, D, FF // 4), BF16),
            pltpu.VMEM((4, FF, D // 4), BF16),
            pltpu.VMEM((2, 35 * 256, 128), U32),
            pltpu.VMEM((2, 10 * 896, 128), U32),
            pltpu.VMEM((HB, HB), F32),
            pltpu.SemaphoreType.DMA((17,)),
            pltpu.SemaphoreType.DMA(()),
        ],
        compiler_params=pltpu.CompilerParams(vmem_limit_bytes=126 * 1024 * 1024),
    )(
        A_x.reshape(S, D), A_mem0.reshape(M, D),
        A_Wq.reshape(D * H, E), A_Wk.reshape(D * H, E), A_Wv.reshape(D * H, E),
        A_Wo.reshape(H * E, D), B_w1, B_w2, B_w3, B_w4,
    )
    return out.reshape(1, S, D)
```

```python
import functools

import jax
import jax.numpy as jnp
from jax import lax
import jax.experimental.pallas as pl
import jax.experimental.pallas.tpu as pltpu

F32 = jnp.float32
BF16 = jnp.bfloat16
U32 = jnp.uint32

S = 2048
D = 1024
H = 32
E = 128
M = 8
SEG = 32
L = M + SEG
FF = 3584
NCB = D // 128
NFB = FF // 128
NP = H // 2
NIT = S // (2 * SEG)
HB = 2 * L
PRE = 512
LAG = 128
BR = (S - PRE) // NIT
CLAG = 4
NSB = 8
H3R = PRE - 2 * 2 * BR
HS = D // 2 + 8
RB = 256
SB = 128
HSB = (SB // 64) * HB
CH = 512
PR = 16 * CH
EPS = 1e-5
SCALE = float(E) ** -0.5
SHIFTS = (7, 7, 9, 9, 6, 6, 10, 10)


def _dot(a, b):
    return jnp.dot(a, b, preferred_element_type=F32)


def _ln(x):
    m = jnp.mean(x, axis=-1, keepdims=True)
    xc = x - m
    v = jnp.mean(xc * xc, axis=-1, keepdims=True)
    return xc * lax.rsqrt(v + EPS)


def _ln2(x):
    m = jnp.mean(x, axis=-1, keepdims=True)
    xc = x - m
    v = jnp.mean(xc * xc, axis=-1, keepdims=True)
    r1 = lax.rsqrt(v + EPS)
    r2 = lax.rsqrt(v * r1 * r1 + EPS)
    return xc * r1, xc * (r1 * r2)


def _gelu(x):
    c = 0.7978845608028654
    hx = 0.5 * x
    return hx * jnp.tanh(x * (c + (c * 0.044715) * (x * x))) + hx


def _silu(x):
    hx = 0.5 * x
    return hx * jnp.tanh(hx) + hx


def _zero_of(v):
    return (pltpu.bitcast(v, U32) >> 16) >> 16


def _or_zero(w, z):
    return pltpu.bitcast(pltpu.bitcast(w, U32) | z, w.dtype)


def _col(w, cb, k0=0, k1=None):
    _, kk, cw = w.shape
    q, r = divmod(cb * 128, cw)
    return w[q, k0:(kk if k1 is None else k1), r:r + 128]


def _h3col(f):
    pos = (f // 14) * 7 + f % 7
    return (f % 14) // 7, slice(pos * 128, (pos + 1) * 128)


def _strassen_lhs(top, bot):
    k = top.shape[1] // 2
    raw11, raw22 = top[:, :k].astype(BF16), bot[:, k:].astype(BF16)
    top, bot = top.astype(F32), bot.astype(F32)
    a11, a12, a21, a22 = top[:, :k], top[:, k:], bot[:, :k], bot[:, k:]
    sums = [v.astype(BF16) for v in (a21 + a22, a11 + a12, a11 + a22, a21 - a11, a12 - a22)]
    return [raw11, raw22] + sums


class _Strassen:
    def __init__(self, lhs, rhs, done):
        self.lhs, self.rhs, self.done, self.m = lhs, rhs, done, []

    def step(self):
        n, m = len(self.m), self.m
        v = _dot(self.lhs[n], self.rhs(n))
        m.append(v)
        if n == 2:
            self.done(1, 0, v + m[1])
        elif n == 3:
            self.done(0, 1, v + m[0])
        elif n == 5:
            self.done(1, 1, v + (m[4] + (m[0] - m[2])))
        elif n == 6:
            self.done(0, 0, v + (m[4] + (m[1] - m[3])))


def _hrow(r):
    q, rr = divmod(r, 64)
    return q * HB + rr + (8 if rr < 40 else 16)


def _kernel(x_hbm, mem0_hbm, wq_hbm, wk_hbm, wv_hbm, wo_hbm, w1_hbm, w2_hbm, w3_hbm, w4_hbm,
            out_hbm,
            xbuf, hbuf_all, hf, x1buf, h3buf, sbuf, stg, wqkv, wo, w1, w2, w3, w4, w3c, w4c,
            fillbuf,
            sem, osem):
    hbuf = hbuf_all.at[CLAG * HB:, :]

    def colblock_copies(src, dst, s):
        n, _, cw = dst.shape
        return [pltpu.make_async_copy(src.at[:, pl.ds(c * cw, cw)], dst.at[c], sem.at[s(c)])
                for c in range(n)]

    xs, qs = 7, 12
    xch = [(0, SB), (SB, SB), (RB, RB), (2 * RB, RB), (3 * RB, S - 3 * RB)]
    cp_x = [pltpu.make_async_copy(x_hbm.at[pl.ds(r, n), :], xbuf.at[pl.ds(r, n), :], sem.at[xs + i])
            for i, (r, n) in enumerate(xch)]
    cp_w1 = colblock_copies(w1_hbm, w1, lambda c: (0, 1, 16, 16)[c])
    cp_mem = [pltpu.make_async_copy(mem0_hbm, hbuf.at[0:M, :], sem.at[2])]
    cp_w2 = colblock_copies(w2_hbm, w2, lambda c: 3)
    cp_w3 = colblock_copies(w3_hbm, w3, lambda c: 4)
    cp_w4 = colblock_copies(w4_hbm, w4, lambda c: 5)
    cp_wo = colblock_copies(wo_hbm, wo, lambda c: 6)
    cp_qkv = [pltpu.make_async_copy(src.at[pl.ds(k * PR, PR), :], stg.at[k, pl.ds(m * PR, PR), :],
                                    sem.at[qs + 5 * (m // 2) + k])
              for k in range(4) for m, src in enumerate((wq_hbm, wk_hbm, wv_hbm))]

    for c in cp_x[:2] + cp_w1[:2] + cp_x[2:3] + cp_w1[2:] + cp_w2 + cp_x[3:4]:
        c.start()

    def wait(grp):
        for c in grp:
            c.wait()

    r = lax.broadcasted_iota(jnp.int32, (HB, HB), 0)
    c = lax.broadcasted_iota(jnp.int32, (HB, HB), 1)
    rr = jnp.where(r >= L, r - L, r)
    cc = jnp.where(c >= L, c - L, c)
    same = (r >= L) == (c >= L)
    allowed = (rr < M) | (rr >= cc)
    fillbuf[...] = jnp.where(same, jnp.where(allowed, 1.0, -1e9), -jnp.inf).astype(F32)

    hf[:, 0:8, :] = jnp.zeros((NCB, 8, 128), F32)
    hf[:, S + 8:S + 16, :] = jnp.zeros((NCB, 8, 128), F32)
    sbuf[...] = jnp.zeros(sbuf.shape, sbuf.dtype)

    def ln_sub(xv, hv, sb, dtype=BF16):
        out = []
        for u in range(SB // 16):
            r0 = sb * SB + 16 * u
            xn, xnn = _ln2(xv[r0:r0 + 16, :].astype(F32))
            xn = xn.astype(BF16)
            for hh in range(2):
                o = _hrow(r0 + 8 * hh)
                hv[o:o + 8, :] = xn[8 * hh:8 * hh + 8]
            out.append(xnn.astype(dtype))
        return out

    def after(w, vals):
        if not vals:
            return w
        z = functools.reduce(lambda a, b: a | b, [_zero_of(v[-16:, -128:]) for v in vals])
        return jnp.concatenate([_or_zero(w[0:16, :], z), w[16:, :]], axis=0)

    def w1_sub(xnn, hfv, sb, cbs, deps, hook=None):
        xnn = jnp.concatenate(xnn, axis=0)
        for cb in cbs:
            w = after(_col(w1, cb), deps.get(cb, []))
            half = _dot(xnn[:, :D // 2], w[:D // 2])
            pre = _dot(xnn[:, D // 2:], w[D // 2:]) + half
            hfv[cb, sb * SB + 8:sb * SB + 8 + SB, :] = _gelu(pre)
            if hook is not None:
                hook(half)
                hook(pre)

    def w2_lhs(hfv, sb):
        r0 = sb * SB
        return jnp.concatenate(
            [hfv[cb, r0 + SHIFTS[cb]:r0 + SHIFTS[cb] + SB, :] for cb in range(NCB)],
            axis=1).astype(BF16)

    def xn_rows(hv, r0, cs):
        return jnp.concatenate(
            [hv[_hrow(r0 + a):_hrow(r0 + a) + n, cs].astype(F32)
             for a, n in ((0, 40), (40, 24), (64, 40), (104, 24))], axis=0)

    def w2_sub(hs, hv, x1v, sb, cbs, deps, hook=None):
        r0 = sb * SB
        for cb in cbs:
            pre = _dot(hs, after(_col(w2, cb), deps.get(cb, [])))
            cs = slice(cb * 128, (cb + 1) * 128)
            x1v[r0:r0 + SB, cs] = (xn_rows(hv, r0, cs) + pre).astype(BF16)
            if hook is not None:
                hook(pre)

    def w3_lhs(x1v, r0, rows):
        return [_ln(x1v[r0 + 16 * u:r0 + 16 * u + 16, :].astype(F32)) for u in range(rows // 16)]

    def h3_rows(base, r0, rows):
        v = h3buf.at[:, pl.ds(base, r0 + rows), :]
        p0, p1 = v[0, r0:r0 + rows, :], v[1, r0:r0 + rows, :]
        return jnp.concatenate([p0[:, :896], p1[:, :896], p0[:, 896:], p1[:, 896:]], axis=1)

    def h3_pair(v, f):
        return jnp.concatenate(
            [v[:, f * 128:(f + 1) * 128], v[:, (f + 14) * 128:(f + 15) * 128]], axis=1)

    def gate(x1v, rows, cb, pre):
        sl = (rows, slice(cb * 128, (cb + 1) * 128))
        x1v[sl] = _silu(x1v[sl].astype(F32) + pre).astype(BF16)

    def weight_sums(src, put, c0, c1, kh, r0, rows, trig):
        for r in range(r0, r0 + rows, 16):
            tr = (((r - r0) * trig.shape[0] // rows) // 8) * 8 + 8 * (rows < trig.shape[0])
            z = _zero_of(trig[tr:tr + 8, :])
            ld = lambda c, o: _col(src, c, o + r, o + r + 16)
            b11, b22 = _or_zero(ld(c0, 0), z).astype(F32), _or_zero(ld(c1, kh), z).astype(F32)
            b12, b21 = ld(c1, 0).astype(F32), ld(c0, kh).astype(F32)
            sums = (b12 - b22, b21 - b11, b11 + b22, b11 + b12, b21 + b22)
            for n, v in enumerate(sums):
                put(n, r, v.astype(BF16))

    def packed_put(dst, base, stride):
        def put(n, r, v):
            o = base + n * stride + r // 2
            dst[o:o + 8, :] = pltpu.bitcast(v, U32)
        return put

    def packed_get(wc, base, stride, kh):
        return lambda n: pltpu.bitcast(wc[base + n * stride:base + n * stride + kh // 2, :], BF16)

    def strassen_rhs(w, c0, c1, kh, get, n):
        if n == 2:
            return _col(w, c0, 0, kh)
        if n == 3:
            return _col(w, c1, kh, 2 * kh)
        return get(n if n < 2 else n - 2)

    def w2c_at(c, n):
        q, col = divmod(5 * c + n, 14)
        return q, slice(col * 128, (col + 1) * 128)

    def w2_put(c, n, r, v):
        q, cs = w2c_at(c, n)
        h3buf[q, r:r + 16, cs] = v

    def w2_get(c, n):
        q, cs = w2c_at(c, n)
        return h3buf[q, 0:D // 2, cs]

    def relayout(src, dst, u, pps, trig):
        m, c_ = divmod(u, 16)
        d0 = m * (H * HS) + c_ * 8
        two = lambda v: jnp.concatenate([v, v], axis=0)
        for pp in pps:
            r0 = u * CH + pp * 64
            tr = ((pp - pps[0]) * trig.shape[0] // (8 * len(pps))) * 8
            z = _zero_of(trig[tr:tr + 8, :])
            mlo, sh = U32(0xFFFF), two(z | U32(16))
            a = pltpu.bitcast(src[r0:r0 + 32, :], U32)
            b = pltpu.bitcast(src[r0 + 32:r0 + 64, :], U32)
            dst[pl.ds(d0 + pp, 16, stride=HS), :] = (a & mlo) | (b << sh)
            dst[pl.ds(d0 + 16 * HS + pp, 16, stride=HS), :] = (a >> sh) | (b & U32(0xFFFF0000))

    cp_x[0].wait()
    xnn0 = ln_sub(xbuf, hbuf, 0)
    cp_x[1].wait()
    xnn1 = ln_sub(xbuf, hbuf, 1)
    cp_w1[0].wait()
    w1_sub(xnn0, hf, 0, range(0, 2), {})
    w1_sub(xnn1, hf, 1, range(0, 2), {})
    cp_w1[1].wait()
    w1_sub(xnn0, hf, 0, range(2, 4), {})
    cp_x[2].wait()
    xnn2 = ln_sub(xbuf, hbuf, 2)
    w1_sub(xnn1, hf, 1, range(2, 4), {})
    w1_sub(xnn2, hf, 2, range(0, 4), {})
    wait(cp_w1[2:])
    xnn3 = ln_sub(xbuf, hbuf, 3)
    w1c = w3c.at[0]
    put1 = lambda c: packed_put(w1c, c * 256, 4 * 256)
    put2 = lambda c: functools.partial(w2_put, c)
    todo1 = ([(w1, put1, c, u) for c in range(4) for u in range(8)]
             + [(w2, put2, c, u) for c in range(4) for u in range(8)])
    count1 = [2, 0] * 5 + [2, 1, 2, 0] * 4 + [2, 0] + [3, 3, 3, 2] * 2 + [3, 2] * 2

    def sums1(trig):
        n = count1.pop(0)
        for i in range(n):
            w, put, c, u = todo1.pop(0)
            tr = trig[(i * 16 // n) * 8:((i + 1) * 16 // n) * 8]
            weight_sums(w, put(c), c, c + 4, D // 2, 64 * u, 64, tr)

    w1_sub(xnn0, hf, 0, range(4, 8), {6: xnn3[0:1], 7: xnn3[1:2]}, sums1)
    w1_sub(xnn1, hf, 1, range(4, 8), {4 + i: xnn3[2 + i:3 + i] for i in range(4)}, sums1)
    w1_sub(xnn2, hf, 2, range(4, 8), {4: xnn3[6:7], 5: xnn3[7:8]}, sums1)
    w1_sub(xnn3, hf, 3, range(0, 2), {}, sums1)
    assert len(todo1) == 32
    wait(cp_w2)
    for c in cp_x[4:] + cp_mem + cp_w3 + cp_qkv[:2] + cp_w4 + cp_qkv[2:] + cp_wo:
        c.start()
    w1_sub(xnn3, hf, 3, range(2, NCB), {}, sums1)
    assert not todo1
    cp_x[3].wait()

    def loop_w12(i, carry):
        @pl.when(i == 3)
        def _():
            cp_x[4].wait()

        r0 = pl.multiple_of((i - 2) * RB, RB)
        xv = xbuf.at[pl.ds(r0, 3 * RB), :]
        hv = hbuf.at[pl.ds(pl.multiple_of((i - 2) * 2 * HSB, 16), 6 * HSB), :]
        x1v = x1buf.at[pl.ds(r0, RB), :]
        hfv = hf.at[:, pl.ds(r0, 3 * RB + 16), :]
        ca, cb_ = ln_sub(xv, hv, 4, F32), ln_sub(xv, hv, 5, F32)
        c1 = [_strassen_lhs(ca[u], cb_[u]) for u in range(SB // 16)]
        lhs1 = [jnp.concatenate([c[n] for c in c1], axis=0) for n in range(7)]
        shifted = lambda cb, sb: hfv[cb, sb * SB + SHIFTS[cb]:(sb + 1) * SB + SHIFTS[cb], :]
        c2 = [_strassen_lhs(*[jnp.concatenate([shifted(c, sb), shifted(c + 4, sb)], axis=1)
                              for sb in range(2)]) for c in range(4)]
        lhs2 = [jnp.concatenate([c[n] for c in c2], axis=1) for n in range(7)]
        deps = {4 * (n - 2) + c + 4: [c2[c][n]] for n in range(2, 7) for c in range(4)}
        for u, d in enumerate((9, 11, 13, 15, 17, 19, 21, 23)):
            deps[d] = deps.get(d, []) + c1[u]
        count = [0]

        def w2_pair(c):
            def done(a, b, v):
                cs = slice((4 * b + c) * 128, (4 * b + c + 1) * 128)
                x1v[a * SB:(a + 1) * SB, cs] = (xn_rows(hv, a * SB, cs) + v).astype(BF16)

            def rhs(n):
                count[0] += 1
                w = strassen_rhs(w2, c, c + 4, D // 2, functools.partial(w2_get, c), n)
                return after(w, deps.get(count[0] - 1, []))
            return _Strassen(lhs2, rhs, done)

        def w1_pair(c):
            def done(a, b, v):
                hfv[4 * b + c, (4 + a) * SB + 8:(5 + a) * SB + 8, :] = _gelu(v)
            get = packed_get(w1c, c * 256, 4 * 256, D // 2)
            return _Strassen(lhs1, functools.partial(strassen_rhs, w1, c, c + 4, D // 2, get), done)

        p2, p1 = [w2_pair(c) for c in range(4)], [w1_pair(c) for c in range(4)]
        order = [p for _ in range(7) for p in p2]
        for p in order[:-4] + [p for p in p1 for _ in range(7)] + order[-4:]:
            p.step()
        return carry

    lax.fori_loop(2, S // RB, loop_w12, 0)
    wait(cp_w3)

    def loop_w34(k, carry):
        qk, vv = stg.at[k, 0:2 * PR, :], stg.at[k, 2 * PR:3 * PR, :]
        pltpu.make_async_copy(qk, qk, sem.at[qs + k]).wait()
        r0 = pl.multiple_of(k * SB, SB)
        src = stg.at[k]
        dst = wqkv.at[pl.ds(pl.multiple_of(k * 128, 128), (3 * H + 1) * HS - 384), :]
        sb2 = (S - PRE) // SB
        x1v = x1buf.at[pl.ds(r0, (sb2 + 1) * SB), :]
        hv = hbuf.at[pl.ds(pl.multiple_of(k * HSB, 16), (sb2 + 1) * HSB), :]
        hfv = hf.at[:, pl.ds(r0, (sb2 + 1) * SB + 16), :]
        w3v = w3.at[:, pl.ds(r0, D - 384), :]
        w3cv = w3c.at[:, pl.ds(pl.multiple_of(k * 64, 64), 35 * 256 - 192), :]
        w4v = w4.at[:, pl.ds(pl.multiple_of(k * 448, 64), FF - 3 * 448), :]
        w4cv = w4c.at[:, pl.ds(pl.multiple_of(k * 224, 32), 10 * 896 - 3 * 224), :]
        todo = [(u, h) for u in range(3 * PR // CH) for h in range(2)]
        todo3 = [(f, u) for f in range(14) for u in range(2)]
        todo4 = [(c, u) for c in range(4) for u in range(7)]

        def rl(trig, halves=2):
            n = min(halves, len(todo))
            for i in range(n):
                u, h = todo.pop(0)
                rows = trig.shape[0] // n
                relayout(src, dst, u, range(4 * h, 4 * h + 4), trig[i * rows:(i + 1) * rows])

        def sums3(trig):
            f, u = todo3.pop(0)
            weight_sums(w3v, packed_put(w3cv.at[f // 7], (f % 7) * 256, 7 * 256),
                        f, f + 14, D // 2, 64 * u, 64, trig)

        def sums4(trig):
            c, u = todo4.pop(0)
            weight_sums(w4v, packed_put(w4cv.at[c // 2], (c % 2) * 896, 2 * 896),
                        c, c + 4, FF // 2, 64 * u, 64, trig)

        hs = w2_lhs(hfv, sb2)
        c = [v.astype(BF16) for v in w3_lhs(x1v, 0, SB)]
        w2_sub(hs, hv, x1v, sb2, range(0, 6), {3: c[0:2], 4: c[2:4], 5: c[4:6]})
        lhs3 = jnp.concatenate(c, axis=0)
        for f in range(NFB):
            half = _dot(lhs3[:, :512], _col(w3, f, 0, 512))
            pre = _dot(lhs3[:, 512:], _col(w3, f, 512, D)) + half
            q, cs = _h3col(f)
            h3buf[q, pl.ds(r0, SB), cs] = _gelu(pre).astype(BF16)
            rl(half)
            sums3(pre)
        w2_sub(hs, hv, x1v, sb2, range(6, 7), {})

        @pl.when(k == 0)
        def _():
            wait(cp_w4)

        pltpu.make_async_copy(vv, vv, sem.at[qs + 5 + k]).wait()
        n4 = (PRE - LAG) // 4
        r4 = pl.multiple_of(k * n4, 32)
        lhs4 = h3_rows(r4, 0, n4)
        for cb in range(NCB):
            pre = None
            for n in range(7):
                k0, k1 = 512 * n, 512 * (n + 1)
                part = _dot(lhs4[:, k0:k1], _col(w4, cb, k0, k1))
                pre = part if pre is None else part + pre
                if n in (0, 2, 4) and cb > 0:
                    rl(pre)
                if n in (1, 3, 5) or (n == 6 and cb < 4):
                    sums4(pre)
            gate(x1buf.at[pl.ds(r4, n4), :], slice(0, n4), cb, pre)
        w2_sub(hs, hv, x1v, sb2, range(7, 8), {})
        assert not (todo or todo3 or todo4)
        return carry

    lax.fori_loop(0, PRE // SB, loop_w34, 0)
    wait(cp_wo)
    wait(cp_mem)

    def softmax(s):
        fill = fillbuf[...]
        s = jnp.where(fill > 0.0, s * SCALE, fill)
        mx = jnp.max(s, axis=1, keepdims=True)
        e = jnp.exp(s - mx)
        l = jnp.sum(e, axis=1, keepdims=True)
        rc = pl.reciprocal(l, approx=True)
        rc = rc * (2.0 - l * rc)
        return (e * rc).astype(BF16)

    def attn_step(lhs, select, wo_rows, fill, deps):
        qkv = [None] * NP
        p = [None] * NP
        oh = [None] * H
        acc = [None] * NCB
        wsplit = (0, 8, 20, 28, 32)

        def do_qkv(j):
            rs = []
            for i in range(6):
                h = 2 * j + i // 3
                r0 = ((i % 3) * H + (h % 2) * 16 + h // 2) * HS
                w = pltpu.bitcast(wqkv[r0:r0 + D // 2, :], BF16)
                v = _dot(lhs, after(w, deps.get(6 * j + i, [])))
                fill(("qkv", 6 * j + i), v)
                rs.append(select(j, i, v))
            qkv[j] = [jnp.concatenate([rs[i], rs[3 + i]], axis=0).astype(BF16) for i in range(3)]

        def do_s(j):
            p[j] = softmax(lax.dot_general(qkv[j][0], qkv[j][1], (((1,), (1,)), ((), ())),
                                           preferred_element_type=F32))

        def do_pv(j):
            o = _dot(p[j], qkv[j][2])
            oh[2 * j] = wo_rows(2 * j, o[0:L]).astype(BF16)
            oh[2 * j + 1] = wo_rows(2 * j + 1, o[L:2 * L]).astype(BF16)

        def do_wo(n):
            h0, h1 = wsplit[n], wsplit[n + 1]
            lo = jnp.concatenate(oh[h0:h1], axis=1)
            for cb in range(NCB):
                part = _dot(lo, _col(wo, cb, h0 * E, h1 * E))
                acc[cb] = part if acc[cb] is None else part + acc[cb]
                fill(("wo", n * NCB + cb), part)

        for j in range(NP + 2):
            if j < NP:
                do_qkv(j)
            else:
                do_wo(j - NP)
            if 0 <= j - 2 < NP:
                do_pv(j - 2)
            if 0 <= j - 1 < NP:
                do_s(j - 1)
        do_wo(2)
        do_wo(3)
        return acc

    def combine(r0, sv, dst, cb, trig=None):
        cs = slice(cb * 128, (cb + 1) * 128)
        xx, gg = xbuf[pl.ds(r0, 64), cs], x1buf[pl.ds(r0, 64), cs]
        if trig is not None:
            z = jnp.concatenate([_zero_of(trig[0:8, :])] * 4, axis=0)
            xx, gg = _or_zero(xx, z), _or_zero(gg, z)
        dst[0:64, cs] = (xx.astype(F32) + sv[:, cs].astype(F32) * gg.astype(F32)).astype(BF16)

    def body(t, carry):
        hv = hbuf_all.at[pl.ds(pl.multiple_of(t * HB, 16), (CLAG + 1) * HB + 16), :]
        cur = CLAG * HB
        prev = pl.multiple_of(jnp.maximum(t - CLAG, 0) * 64, 64)
        par, blk = t % 2, t // 2

        b4 = pl.multiple_of(PRE - LAG + blk * 2 * BR, 32)
        ln3 = w3_lhs(x1buf.at[pl.ds(b4, LAG + 2 * BR), :], LAG, 2 * BR)
        c3 = [_strassen_lhs(ln3[u], ln3[3 + u]) for u in range(3)]
        lhs3 = [jnp.concatenate([c[n] for c in c3], axis=0) for n in range(7)]
        slot = lambda j: pl.multiple_of(H3R + (j % 3) * 2 * BR, 32)
        h3w = h3buf.at[par, pl.ds(slot(blk + 2), 2 * BR), :]
        w3v, w3cv = w3.at[pl.ds(par, 3)], w3c.at[par]

        def w3_pair(i):
            def done(a, b, v):
                h3w[a * BR:(a + 1) * BR, (7 * b + i) * 128:(7 * b + i + 1) * 128] = (
                    _gelu(v).astype(BF16))
            get = packed_get(w3cv, i * 256, 7 * 256, D // 2)
            return _Strassen(lhs3, functools.partial(strassen_rhs, w3v, i, i + 14, D // 2, get), done)

        top = jnp.concatenate([h3_rows(slot(blk), 64, 32), h3_rows(slot(blk + 1), 0, 16)], axis=0)
        bot = h3_rows(slot(blk + 1), 16, BR)
        c4 = [_strassen_lhs(h3_pair(top, f), h3_pair(bot, f)) for f in range(14)]
        lhs4 = [jnp.concatenate([c[n] for c in c4], axis=1) for n in range(7)]
        deps = {12 + 5 * f: c4[f] for f in range(14)}
        deps.update({80 + 6 * u: c3[u] for u in range(3)})
        x4v = x1buf.at[pl.ds(b4, 2 * BR), pl.ds(pl.multiple_of(par * 256, 256), D - 256)]
        w4v, w4cv = w4.at[pl.ds(par, 3)], w4c.at[par]

        def w4_pair(i):
            def done(a, b, v):
                gate(x4v, slice(a * BR, (a + 1) * BR), 4 * b + i, v)
            get = packed_get(w4cv, i * 896, 2 * 896, FF // 2)
            return _Strassen(lhs4, functools.partial(strassen_rhs, w4v, i, i + 4, FF // 2, get), done)

        todo3 = [p for p in map(w3_pair, range(7)) for _ in range(7)]
        todo4 = [p for p in map(w4_pair, range(2)) for _ in range(7)]
        todoc = list(range(NCB))

        keep = {}

        def sel_a(j, i, v):
            keep[(j, i)] = v[L:L + 8]
            return v[0:L]

        def wo_a(h, o):
            keep[h] = o[32:40]
            return o[0:32]

        sv_old = sbuf.at[(t + NSB - CLAG) % NSB]

        def fill_a(slot, v):
            if slot[0] == "qkv" and 1 <= slot[1] <= NCB:
                combine(prev, sv_old, hv, todoc.pop(0), v)
                if not todoc:
                    @pl.when(t >= CLAG)
                    def _():
                        pltpu.make_async_copy(hv.at[0:64, :], out_hbm.at[pl.ds(prev, 64), :],
                                              osem).start()
            if slot[0] == "wo" and slot[1] in (1, 3, 5, 7, 9, 11, 13, 15, 18, 21):
                todo4.pop(0).step()

        ra = attn_step(hv[cur:cur + 48, :], sel_a, wo_a, fill_a, deps)
        for cb in range(NCB):
            hv[cur + 48:cur + 56, cb * 128:(cb + 1) * 128] = ra[cb][0:8].astype(BF16)
        while todo4:
            todo4.pop(0).step()

        def sel_b(j, i, v):
            return jnp.concatenate([v[0:8], keep[(j, i)], v[8:32]], axis=0)

        def wo_b(h, o):
            return jnp.concatenate([keep[h], o], axis=0)

        w3_slots = [(i * 6 * NP) // 49 for i in range(49)]

        def fill_b(slot, v):
            if slot[0] == "qkv" and slot[1] in w3_slots:
                todo3.pop(0).step()

        rb = attn_step(hv[cur + 48:cur + HB, :], sel_b, wo_b, fill_b, {})
        sv = sbuf.at[t % NSB]
        for cb in range(NCB):
            cs = slice(cb * 128, (cb + 1) * 128)
            hv[cur + HB:cur + HB + 8, cs] = rb[cb][8:16].astype(BF16)
            sv[:, cs] = jnp.concatenate([ra[cb][8:32], rb[cb][0:8], rb[cb][16:48]],
                                        axis=0).astype(BF16)
        assert not (todo3 or todo4 or todoc)
        return carry

    lax.fori_loop(0, NIT, body, 0)

    last = (S - PRE) // (2 * BR) - 1
    s0, s1 = H3R + ((last + 1) % 3) * 2 * BR, H3R + ((last + 2) % 3) * 2 * BR
    top = jnp.concatenate([h3_rows(s0, 64, 32), h3_rows(s1, 0, 32)], axis=0)
    bot = h3_rows(s1, 32, 64)
    c4 = [_strassen_lhs(h3_pair(top, f), h3_pair(bot, f)) for f in range(14)]
    lhs4 = [jnp.concatenate([c[n] for c in c4], axis=1) for n in range(7)]
    x4v = x1buf.at[S - LAG:S, :]

    def stage(t):
        return hbuf.at[t * HB:(t + 1) * HB, :]

    def send(t, c0, c1):
        cs = pl.ds(c0 * 128, (c1 - c0) * 128)
        pltpu.make_async_copy(stage(t).at[0:64, cs], out_hbm.at[t * 64:(t + 1) * 64, cs],
                              osem).start()

    def last_pair(c):
        def done(a, b, v):
            gate(x4v, slice(a * 64, (a + 1) * 64), 4 * b + c, v)
            combine((NIT - 2 + a) * 64, sbuf.at[(NIT - 2 + a) % NSB], stage(NIT - 2 + a), 4 * b + c)
            if c >= 2:
                send(NIT - 2 + a, 4 * b + (0 if c == 2 else 3), 4 * b + c + 1)
            if c in (1, 2):
                t = NIT - 5 + c
                for cb in (4 * a + 2 * b, 4 * a + 2 * b + 1):
                    combine(t * 64, sbuf.at[t % NSB], stage(t), cb, v)
                if (a, b) == (0, 0):
                    send(t, 0, NCB)

        def rhs(n):
            get = packed_get(w4c.at[c // 2], (c % 2) * 896, 2 * 896, FF // 2)
            w = strassen_rhs(w4.at[pl.ds(c // 2, 3)], c % 2, c % 2 + 4, FF // 2, get, n)
            u = 2 * c + n - 1
            return after(w, c4[2 * u][2:] + c4[2 * u + 1][2:] if n < 2 and u >= 0 else [])
        return _Strassen(lhs4, rhs, done)

    prods = [last_pair(c) for c in range(4)]
    for prod in prods:
        prod.step()
        prod.step()
    for prod in prods:
        for _ in range(5):
            prod.step()
    pltpu.make_async_copy(xbuf, out_hbm, osem).wait()


@jax.jit
def pallas_recurrent_scan__memory_aug_recurrent_mem_tr__mixer_s_mlp__prompt_kernel(
    A_x: jax.Array,
    A_mem0: jax.Array,
    A_Wq: jax.Array,
    A_Wk: jax.Array,
    A_Wv: jax.Array,
    A_Wo: jax.Array,
    A_seg_len: jax.Array,
    B_x: jax.Array,
    B_w1: jax.Array,
    B_w2: jax.Array,
    B_w3: jax.Array,
    B_w4: jax.Array,
):
    del A_seg_len, B_x
    assert A_x.shape == (1, S, D) and A_mem0.shape == (1, M, D)
    assert A_Wq.shape == (D, H, E) and A_Wo.shape == (H, E, D)
    assert B_w3.shape == (D, FF) and B_w4.shape == (FF, D)

    any_spec = pl.BlockSpec(memory_space=pl.ANY)
    out = pl.pallas_call(
        _kernel,
        out_shape=jax.ShapeDtypeStruct((S, D), BF16),
        in_specs=[any_spec] * 10,
        out_specs=any_spec,
        scratch_shapes=[
            pltpu.VMEM((S, D), BF16),
            pltpu.VMEM(((NIT + CLAG) * HB + 16, D), BF16),
            pltpu.VMEM((NCB, S + 16, 128), F32),
            pltpu.VMEM((S, D), BF16),
            pltpu.VMEM((2, PRE + 2 * BR, FF // 2), BF16),
            pltpu.VMEM((NSB, 64, D), BF16),
            pltpu.VMEM((4, 3 * PR, E), BF16),
            pltpu.VMEM(((3 * H + 1) * HS, 128), U32),
            pltpu.VMEM((D // 512, H * E, 512), BF16),
            pltpu.VMEM((D // 256, D, 256), BF16),
            pltpu.VMEM((D // 512, D, 512), BF16),
            pltpu.VMEM((4, D, FF // 4), BF16),
            pltpu.VMEM((4, FF, D // 4), BF16),
            pltpu.VMEM((2, 35 * 256, 128), U32),
            pltpu.VMEM((2, 10 * 896, 128), U32),
            pltpu.VMEM((HB, HB), F32),
            pltpu.SemaphoreType.DMA((21,)),
            pltpu.SemaphoreType.DMA(()),
        ],
        compiler_params=pltpu.CompilerParams(vmem_limit_bytes=126 * 1024 * 1024),
    )(
        A_x.reshape(S, D), A_mem0.reshape(M, D),
        A_Wq.reshape(D * H, E), A_Wk.reshape(D * H, E), A_Wv.reshape(D * H, E),
        A_Wo.reshape(H * E, D), B_w1, B_w2, B_w3, B_w4,
    )
    return out.reshape(1, S, D)
```

```python
import functools

import jax
import jax.numpy as jnp
from jax import lax
import jax.experimental.pallas as pl
import jax.experimental.pallas.tpu as pltpu

F32 = jnp.float32
BF16 = jnp.bfloat16
U32 = jnp.uint32

S = 2048
D = 1024
H = 32
E = 128
M = 8
SEG = 32
L = M + SEG
FF = 3584
NCB = D // 128
NFB = FF // 128
NP = H // 2
NIT = S // (2 * SEG)
HB = 2 * L
PRE = 512
LAG = 128
BR = (S - PRE) // NIT
CLAG = 4
NSB = 5
H3R = PRE - 2 * 2 * BR
HS = D // 2 + 8
RB = 256
SB = 128
HSB = (SB // 64) * HB
CH = 512
PR = 16 * CH
EPS = 1e-5
SCALE = float(E) ** -0.5
SHIFTS = (7, 7, 9, 9, 6, 6, 10, 10)


def _dot(a, b):
    return jnp.dot(a, b, preferred_element_type=F32)


def _ln(x):
    m = jnp.mean(x, axis=-1, keepdims=True)
    xc = x - m
    v = jnp.mean(xc * xc, axis=-1, keepdims=True)
    return xc * lax.rsqrt(v + EPS)


def _ln2(x):
    m = jnp.mean(x, axis=-1, keepdims=True)
    xc = x - m
    v = jnp.mean(xc * xc, axis=-1, keepdims=True)
    r1 = lax.rsqrt(v + EPS)
    r2 = lax.rsqrt(v * r1 * r1 + EPS)
    return xc * r1, xc * (r1 * r2)


def _gelu(x):
    c = 0.7978845608028654
    hx = 0.5 * x
    return hx * jnp.tanh(x * (c + (c * 0.044715) * (x * x))) + hx


def _silu(x):
    hx = 0.5 * x
    return hx * jnp.tanh(hx) + hx


def _zero_of(v):
    return (pltpu.bitcast(v, U32) >> 16) >> 16


def _or_zero(w, z):
    return pltpu.bitcast(pltpu.bitcast(w, U32) | z, w.dtype)


def _col(w, cb, k0=0, k1=None):
    _, kk, cw = w.shape
    q, r = divmod(cb * 128, cw)
    return w[q, k0:(kk if k1 is None else k1), r:r + 128]


def _h3col(f):
    pos = (f // 14) * 7 + f % 7
    return (f % 14) // 7, slice(pos * 128, (pos + 1) * 128)


def _strassen_lhs(top, bot):
    k = top.shape[1] // 2
    raw11, raw22 = top[:, :k].astype(BF16), bot[:, k:].astype(BF16)
    top, bot = top.astype(F32), bot.astype(F32)
    a11, a12, a21, a22 = top[:, :k], top[:, k:], bot[:, :k], bot[:, k:]
    sums = [v.astype(BF16) for v in (a21 + a22, a11 + a12, a11 + a22, a21 - a11, a12 - a22)]
    return [raw11, raw22] + sums


class _Strassen:
    def __init__(self, lhs, rhs, done):
        self.lhs, self.rhs, self.done, self.m = lhs, rhs, done, []

    def step(self):
        n, m = len(self.m), self.m
        v = _dot(self.lhs[n], self.rhs(n))
        m.append(v)
        if n == 2:
            self.done(1, 0, v + m[1])
        elif n == 3:
            self.done(0, 1, v + m[0])
        elif n == 5:
            self.done(1, 1, v + (m[4] + (m[0] - m[2])))
        elif n == 6:
            self.done(0, 0, v + (m[4] + (m[1] - m[3])))


def _hrow(r):
    q, rr = divmod(r, 64)
    return q * HB + rr + (8 if rr < 40 else 16)


def _kernel(x_hbm, mem0_hbm, wq_hbm, wk_hbm, wv_hbm, wo_hbm, w1_hbm, w2_hbm, w3_hbm, w4_hbm,
            out_hbm,
            xbuf, hbuf_all, hf, x1buf, h3buf, sbuf, stg, wqkv, wo, w1, w2, w3, w4, w2c, w3c, w4c,
            fillbuf,
            sem, osem):
    hbuf = hbuf_all.at[CLAG * HB:, :]

    def colblock_copies(src, dst, s):
        n, _, cw = dst.shape
        return [pltpu.make_async_copy(src.at[:, pl.ds(c * cw, cw)], dst.at[c], sem.at[s(c)])
                for c in range(n)]

    xs, qs = 7, 12
    xch = [(0, SB), (SB, SB), (RB, RB), (2 * RB, RB), (3 * RB, S - 3 * RB)]
    cp_x = [pltpu.make_async_copy(x_hbm.at[pl.ds(r, n), :], xbuf.at[pl.ds(r, n), :], sem.at[xs + i])
            for i, (r, n) in enumerate(xch)]
    cp_w1 = colblock_copies(w1_hbm, w1, lambda c: (0, 1, 16, 16)[c])
    cp_mem = [pltpu.make_async_copy(mem0_hbm, hbuf.at[0:M, :], sem.at[2])]
    cp_w2 = colblock_copies(w2_hbm, w2, lambda c: 3)
    cp_w3 = colblock_copies(w3_hbm, w3, lambda c: 4)
    cp_w4 = colblock_copies(w4_hbm, w4, lambda c: 5)
    cp_wo = colblock_copies(wo_hbm, wo, lambda c: 6)
    cp_qkv = [pltpu.make_async_copy(src.at[pl.ds(k * PR, PR), :], stg.at[k, pl.ds(m * PR, PR), :],
                                    sem.at[qs + 5 * (m // 2) + k])
              for k in range(4) for m, src in enumerate((wq_hbm, wk_hbm, wv_hbm))]

    for c in cp_x[:2] + cp_w1[:2] + cp_x[2:3] + cp_w1[2:] + cp_w2 + cp_x[3:4]:
        c.start()

    def wait(grp):
        for c in grp:
            c.wait()

    r = lax.broadcasted_iota(jnp.int32, (HB, HB), 0)
    c = lax.broadcasted_iota(jnp.int32, (HB, HB), 1)
    rr = jnp.where(r >= L, r - L, r)
    cc = jnp.where(c >= L, c - L, c)
    same = (r >= L) == (c >= L)
    allowed = (rr < M) | (rr >= cc)
    fillbuf[...] = jnp.where(same, jnp.where(allowed, 1.0, -1e9), -jnp.inf).astype(F32)

    hf[:, 0:8, :] = jnp.zeros((NCB, 8, 128), F32)
    hf[:, S + 8:S + 16, :] = jnp.zeros((NCB, 8, 128), F32)
    sbuf[...] = jnp.zeros(sbuf.shape, sbuf.dtype)

    def ln_sub(xv, hv, sb, dtype=BF16):
        out = []
        for u in range(SB // 16):
            r0 = sb * SB + 16 * u
            xn, xnn = _ln2(xv[r0:r0 + 16, :].astype(F32))
            xn = xn.astype(BF16)
            for hh in range(2):
                o = _hrow(r0 + 8 * hh)
                hv[o:o + 8, :] = xn[8 * hh:8 * hh + 8]
            out.append(xnn.astype(dtype))
        return out

    def after(w, vals):
        if not vals:
            return w
        z = functools.reduce(lambda a, b: a | b, [_zero_of(v[-16:, -128:]) for v in vals])
        return jnp.concatenate([_or_zero(w[0:16, :], z), w[16:, :]], axis=0)

    def w1_sub(xnn, hfv, sb, cbs, deps, hook=None):
        xnn = jnp.concatenate(xnn, axis=0)
        for cb in cbs:
            w = after(_col(w1, cb), deps.get(cb, []))
            half = _dot(xnn[:, :D // 2], w[:D // 2])
            pre = _dot(xnn[:, D // 2:], w[D // 2:]) + half
            hfv[cb, sb * SB + 8:sb * SB + 8 + SB, :] = _gelu(pre)
            if hook is not None:
                hook(half)
                hook(pre)

    def xn_rows(hv, r0, rows, cs):
        return jnp.concatenate(
            [hv[_hrow(r + a):_hrow(r + a) + n, cs].astype(F32)
             for r in range(r0, r0 + rows, 64) for a, n in ((0, 40), (40, 24))], axis=0)

    def w3_lhs(x1v, r0, rows):
        return [_ln(x1v[r0 + 16 * u:r0 + 16 * u + 16, :].astype(F32)) for u in range(rows // 16)]

    def h3_rows(base, r0, rows):
        v = h3buf.at[:, pl.ds(base, r0 + rows), :]
        p0, p1 = v[0, r0:r0 + rows, :], v[1, r0:r0 + rows, :]
        return jnp.concatenate([p0[:, :896], p1[:, :896], p0[:, 896:], p1[:, 896:]], axis=1)

    def h3_pair(v, f):
        return jnp.concatenate(
            [v[:, f * 128:(f + 1) * 128], v[:, (f + 14) * 128:(f + 15) * 128]], axis=1)

    def gate(x1v, rows, cb, pre):
        sl = (rows, slice(cb * 128, (cb + 1) * 128))
        x1v[sl] = _silu(x1v[sl].astype(F32) + pre).astype(BF16)

    def weight_sums(src, put, c0, c1, kh, r0, rows, trig):
        for r in range(r0, r0 + rows, 16):
            tr = (((r - r0) * trig.shape[0] // rows) // 8) * 8 + 8 * (rows < trig.shape[0])
            z = _zero_of(trig[tr:tr + 8, :])
            ld = lambda c, o: _col(src, c, o + r, o + r + 16)
            b11, b22 = _or_zero(ld(c0, 0), z).astype(F32), _or_zero(ld(c1, kh), z).astype(F32)
            b12, b21 = ld(c1, 0).astype(F32), ld(c0, kh).astype(F32)
            sums = (b12 - b22, b21 - b11, b11 + b22, b11 + b12, b21 + b22)
            for n, v in enumerate(sums):
                put(n, r, v.astype(BF16))

    def packed_put(dst, base, stride):
        def put(n, r, v):
            o = base + n * stride + r // 2
            dst[o:o + 8, :] = pltpu.bitcast(v, U32)
        return put

    def packed_get(wc, base, stride, kh):
        return lambda n: pltpu.bitcast(wc[base + n * stride:base + n * stride + kh // 2, :], BF16)

    def strassen_rhs(w, c0, c1, kh, get, n):
        if n == 2:
            return _col(w, c0, 0, kh)
        if n == 3:
            return _col(w, c1, kh, 2 * kh)
        return get(n if n < 2 else n - 2)

    def w1c_at(c, n):
        q, col = divmod(5 * c + n, 14)
        return q, slice(col * 128, (col + 1) * 128)

    def w1_put(c, n, r, v):
        q, cs = w1c_at(c, n)
        h3buf[q, r:r + 16, cs] = v

    def w1_get(c, n):
        q, cs = w1c_at(c, n)
        return h3buf[q, 0:D // 2, cs]

    def w2_put(c, n, r, v):
        w2c[5 * c + n, r:r + 16, :] = v

    def w2_products(hfv, hv, x1v, r0, half, off, deps):
        shifted = lambda cb, r: hfv[cb, r + SHIFTS[cb]:r + SHIFTS[cb] + half, :]
        c2 = [_strassen_lhs(*[jnp.concatenate([shifted(c, r), shifted(c + 4, r)], axis=1)
                              for r in (r0, r0 + half)]) for c in range(4)]
        lhs2 = [jnp.concatenate([c[n] for c in c2], axis=1) for n in range(7)]
        deps = dict(deps)
        for n in range(2, 7):
            for c in range(4):
                d = 4 * n + c - off
                deps[d] = deps.get(d, []) + [c2[c][n]]
        count = [0]

        def pair(c):
            def done(a, b, v):
                cs = slice((4 * b + c) * 128, (4 * b + c + 1) * 128)
                r = r0 + a * half
                x1v[r:r + half, cs] = (xn_rows(hv, r, half, cs) + v).astype(BF16)

            def rhs(n):
                count[0] += 1
                w = strassen_rhs(w2, c, c + 4, D // 2, lambda i: w2c[5 * c + i], n)
                return after(w, deps.get(count[0] - 1, []))
            return _Strassen(lhs2, rhs, done)

        pairs = [pair(c) for c in range(4)]
        return [p for _ in range(7) for p in pairs]

    def relayout(src, dst, u, pps, trig):
        m, c_ = divmod(u, 16)
        d0 = m * (H * HS) + c_ * 8
        two = lambda v: jnp.concatenate([v, v], axis=0)
        for pp in pps:
            r0 = u * CH + pp * 64
            tr = ((pp - pps[0]) * trig.shape[0] // (8 * len(pps))) * 8
            z = _zero_of(trig[tr:tr + 8, :])
            mlo, sh = U32(0xFFFF), two(z | U32(16))
            a = pltpu.bitcast(src[r0:r0 + 32, :], U32)
            b = pltpu.bitcast(src[r0 + 32:r0 + 64, :], U32)
            dst[pl.ds(d0 + pp, 16, stride=HS), :] = (a & mlo) | (b << sh)
            dst[pl.ds(d0 + 16 * HS + pp, 16, stride=HS), :] = (a >> sh) | (b & U32(0xFFFF0000))

    cp_x[0].wait()
    xnn0 = ln_sub(xbuf, hbuf, 0)
    cp_x[1].wait()
    xnn1 = ln_sub(xbuf, hbuf, 1)
    cp_w1[0].wait()
    w1_sub(xnn0, hf, 0, range(0, 2), {})
    w1_sub(xnn1, hf, 1, range(0, 2), {})
    cp_w1[1].wait()
    w1_sub(xnn0, hf, 0, range(2, 4), {})
    cp_x[2].wait()
    xnn2 = ln_sub(xbuf, hbuf, 2)
    w1_sub(xnn1, hf, 1, range(2, 4), {})
    w1_sub(xnn2, hf, 2, range(0, 4), {})
    wait(cp_w1[2:])
    xnn3 = ln_sub(xbuf, hbuf, 3)
    put1 = lambda c: functools.partial(w1_put, c)
    put2 = lambda c: functools.partial(w2_put, c)
    todo1 = ([(w1, put1, c, u) for c in range(4) for u in range(8)]
             + [(w2, put2, c, u) for c in range(4) for u in range(8)])
    count1 = [2, 0] * 13 + [2, 1] * 2 + [4, 3, 3, 3, 4, 3, 3, 3, 3, 3]

    def sums1(trig):
        n = count1.pop(0)
        for i in range(n):
            w, put, c, u = todo1.pop(0)
            tr = trig[(i * 16 // n) * 8:((i + 1) * 16 // n) * 8]
            weight_sums(w, put(c), c, c + 4, D // 2, 64 * u, 64, tr)

    w1_sub(xnn0, hf, 0, range(4, 8), {6: xnn3[0:1], 7: xnn3[1:2]}, sums1)
    w1_sub(xnn1, hf, 1, range(4, 8), {4 + i: xnn3[2 + i:3 + i] for i in range(4)}, sums1)
    w1_sub(xnn2, hf, 2, range(4, 8), {4: xnn3[6:7], 5: xnn3[7:8]}, sums1)
    w1_sub(xnn3, hf, 3, range(0, 3), {}, sums1)
    assert len(todo1) == 32
    wait(cp_w2)
    for c in cp_x[4:] + cp_mem + cp_w3 + cp_qkv[:2] + cp_w4 + cp_qkv[2:] + cp_wo:
        c.start()
    w1_sub(xnn3, hf, 3, range(3, NCB), {}, sums1)
    assert not todo1
    cp_x[3].wait()

    def loop_w12(i, carry):
        @pl.when(i == 3)
        def _():
            cp_x[4].wait()

        r0 = pl.multiple_of((i - 2) * RB, RB)
        xv = xbuf.at[pl.ds(r0, 3 * RB), :]
        hv = hbuf.at[pl.ds(pl.multiple_of((i - 2) * 2 * HSB, 16), 6 * HSB), :]
        x1v = x1buf.at[pl.ds(r0, RB), :]
        hfv = hf.at[:, pl.ds(r0, 3 * RB + 16), :]
        ca, cb_ = ln_sub(xv, hv, 4, F32), ln_sub(xv, hv, 5, F32)
        c1 = [_strassen_lhs(ca[u], cb_[u]) for u in range(SB // 16)]
        lhs1 = [jnp.concatenate([c[n] for c in c1], axis=0) for n in range(7)]
        order = w2_products(hfv, hv, x1v, 0, SB, 4, {9 + 2 * u: c1[u] for u in range(8)})

        def w1_pair(c):
            def done(a, b, v):
                hfv[4 * b + c, (4 + a) * SB + 8:(5 + a) * SB + 8, :] = _gelu(v)
            get = functools.partial(w1_get, c)
            return _Strassen(lhs1, functools.partial(strassen_rhs, w1, c, c + 4, D // 2, get), done)

        p1 = [w1_pair(c) for c in range(4)]
        for p in order[:-4] + [p for p in p1 for _ in range(7)] + order[-4:]:
            p.step()
        return carry

    lax.fori_loop(2, S // RB, loop_w12, 0)
    wait(cp_w3)

    def loop_w34(k, carry):
        qk, vv = stg.at[k, 0:2 * PR, :], stg.at[k, 2 * PR:3 * PR, :]
        pltpu.make_async_copy(qk, qk, sem.at[qs + k]).wait()
        r0 = pl.multiple_of(k * SB, SB)
        src = stg.at[k]
        dst = wqkv.at[pl.ds(pl.multiple_of(k * 128, 128), (3 * H + 1) * HS - 384), :]
        sb2 = (S - PRE) // SB
        x1v = x1buf.at[pl.ds(r0, (sb2 + 1) * SB), :]
        hv = hbuf.at[pl.ds(pl.multiple_of(k * HSB, 16), (sb2 + 1) * HSB), :]
        hfv = hf.at[:, pl.ds(r0, (sb2 + 1) * SB + 16), :]
        w3v = w3.at[:, pl.ds(r0, D - 384), :]
        w3cv = w3c.at[:, pl.ds(pl.multiple_of(k * 64, 64), 35 * 256 - 192), :]
        w4v = w4.at[:, pl.ds(pl.multiple_of(k * 448, 64), FF - 3 * 448), :]
        w4cv = w4c.at[:, pl.ds(pl.multiple_of(k * 224, 32), 10 * 896 - 3 * 224), :]
        todo = [(u, h) for u in range(3 * PR // CH) for h in range(2)]
        todo3 = [(f, u) for f in range(14) for u in range(2)]
        todo4 = [(c, u) for c in range(4) for u in range(7)]

        def rl(trig, halves=2):
            n = min(halves, len(todo))
            for i in range(n):
                u, h = todo.pop(0)
                rows = trig.shape[0] // n
                relayout(src, dst, u, range(4 * h, 4 * h + 4), trig[i * rows:(i + 1) * rows])

        def sums3(trig):
            f, u = todo3.pop(0)
            weight_sums(w3v, packed_put(w3cv.at[f // 7], (f % 7) * 256, 7 * 256),
                        f, f + 14, D // 2, 64 * u, 64, trig)

        def sums4(trig):
            c, u = todo4.pop(0)
            weight_sums(w4v, packed_put(w4cv.at[c // 2], (c % 2) * 896, 2 * 896),
                        c, c + 4, FF // 2, 64 * u, 64, trig)

        c = [v.astype(BF16) for v in w3_lhs(x1v, 0, SB)]
        order = w2_products(hfv, hv, x1v, sb2 * SB, SB // 2, 1, {6 + 2 * u: c[u:u + 1] for u in range(8)})
        for p in order[:22]:
            p.step()
        lhs3 = jnp.concatenate(c, axis=0)
        for f in range(NFB):
            half = _dot(lhs3[:, :512], _col(w3, f, 0, 512))
            pre = _dot(lhs3[:, 512:], _col(w3, f, 512, D)) + half
            q, cs = _h3col(f)
            h3buf[q, pl.ds(r0, SB), cs] = _gelu(pre).astype(BF16)
            rl(half)
            sums3(pre)
        for p in order[22:25]:
            p.step()

        @pl.when(k == 0)
        def _():
            wait(cp_w4)

        pltpu.make_async_copy(vv, vv, sem.at[qs + 5 + k]).wait()
        n4 = (PRE - LAG) // 4
        r4 = pl.multiple_of(k * n4, 32)
        lhs4 = h3_rows(r4, 0, n4)
        for cb in range(NCB):
            pre = None
            for n in range(7):
                k0, k1 = 512 * n, 512 * (n + 1)
                part = _dot(lhs4[:, k0:k1], _col(w4, cb, k0, k1))
                pre = part if pre is None else part + pre
                if n in (0, 2, 4) and cb > 0:
                    rl(pre)
                if n in (1, 3, 5) or (n == 6 and cb < 4):
                    sums4(pre)
            gate(x1buf.at[pl.ds(r4, n4), :], slice(0, n4), cb, pre)
        for p in order[25:]:
            p.step()
        assert not (todo or todo3 or todo4)
        return carry

    lax.fori_loop(0, PRE // SB, loop_w34, 0)
    wait(cp_wo)
    wait(cp_mem)

    def softmax(s):
        fill = fillbuf[...]
        s = jnp.where(fill > 0.0, s * SCALE, fill)
        mx = jnp.max(s, axis=1, keepdims=True)
        e = jnp.exp(s - mx)
        l = jnp.sum(e, axis=1, keepdims=True)
        rc = pl.reciprocal(l, approx=True)
        rc = rc * (2.0 - l * rc)
        return (e * rc).astype(BF16)

    def attn_step(lhs, select, wo_rows, fill, deps):
        qkv = [None] * NP
        p = [None] * NP
        oh = [None] * H
        acc = [None] * NCB
        wsplit = (0, 8, 20, 28, 32)

        def do_qkv(j):
            rs = []
            for i in range(6):
                h = 2 * j + i // 3
                r0 = ((i % 3) * H + (h % 2) * 16 + h // 2) * HS
                w = pltpu.bitcast(wqkv[r0:r0 + D // 2, :], BF16)
                v = _dot(lhs, after(w, deps.get(6 * j + i, [])))
                fill(("qkv", 6 * j + i), v)
                rs.append(select(j, i, v))
            qkv[j] = [jnp.concatenate([rs[i], rs[3 + i]], axis=0).astype(BF16) for i in range(3)]

        def do_s(j):
            p[j] = softmax(lax.dot_general(qkv[j][0], qkv[j][1], (((1,), (1,)), ((), ())),
                                           preferred_element_type=F32))

        def do_pv(j):
            o = _dot(p[j], qkv[j][2])
            oh[2 * j] = wo_rows(2 * j, o[0:L]).astype(BF16)
            oh[2 * j + 1] = wo_rows(2 * j + 1, o[L:2 * L]).astype(BF16)

        def do_wo(n):
            h0, h1 = wsplit[n], wsplit[n + 1]
            lo = jnp.concatenate(oh[h0:h1], axis=1)
            for cb in range(NCB):
                part = _dot(lo, _col(wo, cb, h0 * E, h1 * E))
                acc[cb] = part if acc[cb] is None else part + acc[cb]
                fill(("wo", n * NCB + cb), part)

        for j in range(NP + 2):
            if j < NP:
                do_qkv(j)
            else:
                do_wo(j - NP)
            if 0 <= j - 2 < NP:
                do_pv(j - 2)
            if 0 <= j - 1 < NP:
                do_s(j - 1)
        do_wo(2)
        do_wo(3)
        return acc

    def combine(r0, sv, dst, cb, trig=None):
        cs = slice(cb * 128, (cb + 1) * 128)
        xx, gg = xbuf[pl.ds(r0, 64), cs], x1buf[pl.ds(r0, 64), cs]
        if trig is not None:
            z = jnp.concatenate([_zero_of(trig[0:8, :])] * 4, axis=0)
            xx, gg = _or_zero(xx, z), _or_zero(gg, z)
        dst[0:64, cs] = (xx.astype(F32) + sv[:, cs].astype(F32) * gg.astype(F32)).astype(BF16)

    def body(t, carry):
        hv = hbuf_all.at[pl.ds(pl.multiple_of(t * HB, 16), (CLAG + 1) * HB + 16), :]
        cur = CLAG * HB
        prev = pl.multiple_of(jnp.maximum(t - CLAG, 0) * 64, 64)
        par, blk = t % 2, t // 2

        b4 = pl.multiple_of(PRE - LAG + blk * 2 * BR, 32)
        ln3 = w3_lhs(x1buf.at[pl.ds(b4, LAG + 2 * BR), :], LAG, 2 * BR)
        c3 = [_strassen_lhs(ln3[u], ln3[3 + u]) for u in range(3)]
        lhs3 = [jnp.concatenate([c[n] for c in c3], axis=0) for n in range(7)]
        slot = lambda j: pl.multiple_of(H3R + (j % 3) * 2 * BR, 32)
        h3w = h3buf.at[par, pl.ds(slot(blk + 2), 2 * BR), :]
        w3v, w3cv = w3.at[pl.ds(par, 3)], w3c.at[par]

        def w3_pair(i):
            def done(a, b, v):
                h3w[a * BR:(a + 1) * BR, (7 * b + i) * 128:(7 * b + i + 1) * 128] = (
                    _gelu(v).astype(BF16))
            get = packed_get(w3cv, i * 256, 7 * 256, D // 2)
            return _Strassen(lhs3, functools.partial(strassen_rhs, w3v, i, i + 14, D // 2, get), done)

        top = jnp.concatenate([h3_rows(slot(blk), 64, 32), h3_rows(slot(blk + 1), 0, 16)], axis=0)
        bot = h3_rows(slot(blk + 1), 16, BR)
        c4 = [_strassen_lhs(h3_pair(top, f), h3_pair(bot, f)) for f in range(14)]
        lhs4 = [jnp.concatenate([c[n] for c in c4], axis=1) for n in range(7)]
        deps = {12 + 5 * f: c4[f] for f in range(14)}
        deps.update({80 + 6 * u: c3[u] for u in range(3)})
        x4v = x1buf.at[pl.ds(b4, 2 * BR), pl.ds(pl.multiple_of(par * 256, 256), D - 256)]
        w4v, w4cv = w4.at[pl.ds(par, 3)], w4c.at[par]

        def w4_pair(i):
            def done(a, b, v):
                gate(x4v, slice(a * BR, (a + 1) * BR), 4 * b + i, v)
            get = packed_get(w4cv, i * 896, 2 * 896, FF // 2)
            return _Strassen(lhs4, functools.partial(strassen_rhs, w4v, i, i + 4, FF // 2, get), done)

        todo3 = [p for p in map(w3_pair, range(7)) for _ in range(7)]
        todo4 = [p for p in map(w4_pair, range(2)) for _ in range(7)]
        todoc = list(range(NCB))

        keep = {}

        def sel_a(j, i, v):
            keep[(j, i)] = v[L:L + 8]
            return v[0:L]

        def wo_a(h, o):
            keep[h] = o[32:40]
            return o[0:32]

        sv_old = sbuf.at[(t + NSB - CLAG) % NSB]

        def fill_a(slot, v):
            if slot[0] == "qkv" and 1 <= slot[1] <= NCB:
                combine(prev, sv_old, hv, todoc.pop(0), v)
                if not todoc:
                    @pl.when(t >= CLAG)
                    def _():
                        pltpu.make_async_copy(hv.at[0:64, :], out_hbm.at[pl.ds(prev, 64), :],
                                              osem).start()
            if slot[0] == "wo" and slot[1] in (1, 3, 5, 7, 9, 11, 13, 15, 18, 21):
                todo4.pop(0).step()

        ra = attn_step(hv[cur:cur + 48, :], sel_a, wo_a, fill_a, deps)
        for cb in range(NCB):
            hv[cur + 48:cur + 56, cb * 128:(cb + 1) * 128] = ra[cb][0:8].astype(BF16)
        while todo4:
            todo4.pop(0).step()

        def sel_b(j, i, v):
            return jnp.concatenate([v[0:8], keep[(j, i)], v[8:32]], axis=0)

        def wo_b(h, o):
            return jnp.concatenate([keep[h], o], axis=0)

        w3_slots = [(i * 6 * NP) // 49 for i in range(49)]

        def fill_b(slot, v):
            if slot[0] == "qkv" and slot[1] in w3_slots:
                todo3.pop(0).step()

        rb = attn_step(hv[cur + 48:cur + HB, :], sel_b, wo_b, fill_b, {})
        sv = sbuf.at[t % NSB]
        for cb in range(NCB):
            cs = slice(cb * 128, (cb + 1) * 128)
            hv[cur + HB:cur + HB + 8, cs] = rb[cb][8:16].astype(BF16)
            sv[:, cs] = jnp.concatenate([ra[cb][8:32], rb[cb][0:8], rb[cb][16:48]],
                                        axis=0).astype(BF16)
        assert not (todo3 or todo4 or todoc)
        return carry

    lax.fori_loop(0, NIT, body, 0)

    last = (S - PRE) // (2 * BR) - 1
    s0, s1 = H3R + ((last + 1) % 3) * 2 * BR, H3R + ((last + 2) % 3) * 2 * BR
    top = jnp.concatenate([h3_rows(s0, 64, 32), h3_rows(s1, 0, 32)], axis=0)
    bot = h3_rows(s1, 32, 64)
    c4 = [_strassen_lhs(h3_pair(top, f), h3_pair(bot, f)) for f in range(14)]
    lhs4 = [jnp.concatenate([c[n] for c in c4], axis=1) for n in range(7)]
    x4v = x1buf.at[S - LAG:S, :]

    def stage(t):
        return hbuf.at[t * HB:(t + 1) * HB, :]

    def send(t, c0, c1):
        cs = pl.ds(c0 * 128, (c1 - c0) * 128)
        pltpu.make_async_copy(stage(t).at[0:64, cs], out_hbm.at[t * 64:(t + 1) * 64, cs],
                              osem).start()

    def last_pair(c):
        def done(a, b, v):
            gate(x4v, slice(a * 64, (a + 1) * 64), 4 * b + c, v)
            combine((NIT - 2 + a) * 64, sbuf.at[(NIT - 2 + a) % NSB], stage(NIT - 2 + a), 4 * b + c)
            if c >= 2:
                send(NIT - 2 + a, 4 * b + (0 if c == 2 else 3), 4 * b + c + 1)
            if c in (1, 2):
                t = NIT - 5 + c
                for cb in (4 * a + 2 * b, 4 * a + 2 * b + 1):
                    combine(t * 64, sbuf.at[t % NSB], stage(t), cb, v)
                if (a, b) == (0, 0):
                    send(t, 0, NCB)

        def rhs(n):
            get = packed_get(w4c.at[c // 2], (c % 2) * 896, 2 * 896, FF // 2)
            w = strassen_rhs(w4.at[pl.ds(c // 2, 3)], c % 2, c % 2 + 4, FF // 2, get, n)
            u = 2 * c + n - 1
            return after(w, c4[2 * u][2:] + c4[2 * u + 1][2:] if n < 2 and u >= 0 else [])
        return _Strassen(lhs4, rhs, done)

    prods = [last_pair(c) for c in range(4)]
    for prod in prods:
        prod.step()
        prod.step()
    for prod in prods:
        for _ in range(5):
            prod.step()
    pltpu.make_async_copy(xbuf, out_hbm, osem).wait()


@jax.jit
def pallas_recurrent_scan__memory_aug_recurrent_mem_tr__mixer_s_mlp__prompt_kernel(
    A_x: jax.Array,
    A_mem0: jax.Array,
    A_Wq: jax.Array,
    A_Wk: jax.Array,
    A_Wv: jax.Array,
    A_Wo: jax.Array,
    A_seg_len: jax.Array,
    B_x: jax.Array,
    B_w1: jax.Array,
    B_w2: jax.Array,
    B_w3: jax.Array,
    B_w4: jax.Array,
):
    del A_seg_len, B_x
    assert A_x.shape == (1, S, D) and A_mem0.shape == (1, M, D)
    assert A_Wq.shape == (D, H, E) and A_Wo.shape == (H, E, D)
    assert B_w3.shape == (D, FF) and B_w4.shape == (FF, D)

    any_spec = pl.BlockSpec(memory_space=pl.ANY)
    out = pl.pallas_call(
        _kernel,
        out_shape=jax.ShapeDtypeStruct((S, D), BF16),
        in_specs=[any_spec] * 10,
        out_specs=any_spec,
        scratch_shapes=[
            pltpu.VMEM((S, D), BF16),
            pltpu.VMEM(((NIT + CLAG) * HB + 16, D), BF16),
            pltpu.VMEM((NCB, S + 16, 128), F32),
            pltpu.VMEM((S, D), BF16),
            pltpu.VMEM((2, PRE + 2 * BR, FF // 2), BF16),
            pltpu.VMEM((NSB, 64, D), BF16),
            pltpu.VMEM((4, 3 * PR, E), BF16),
            pltpu.VMEM(((3 * H + 1) * HS, 128), U32),
            pltpu.VMEM((D // 512, H * E, 512), BF16),
            pltpu.VMEM((D // 256, D, 256), BF16),
            pltpu.VMEM((D // 512, D, 512), BF16),
            pltpu.VMEM((4, D, FF // 4), BF16),
            pltpu.VMEM((4, FF, D // 4), BF16),
            pltpu.VMEM((20, D // 2, 128), BF16),
            pltpu.VMEM((2, 35 * 256, 128), U32),
            pltpu.VMEM((2, 10 * 896, 128), U32),
            pltpu.VMEM((HB, HB), F32),
            pltpu.SemaphoreType.DMA((21,)),
            pltpu.SemaphoreType.DMA(()),
        ],
        compiler_params=pltpu.CompilerParams(vmem_limit_bytes=128 * 1024 * 1024),
    )(
        A_x.reshape(S, D), A_mem0.reshape(M, D),
        A_Wq.reshape(D * H, E), A_Wk.reshape(D * H, E), A_Wv.reshape(D * H, E),
        A_Wo.reshape(H * E, D), B_w1, B_w2, B_w3, B_w4,
    )
    return out.reshape(1, S, D)
```
